```python
import jax
import jax.numpy as jnp

def _softmax(x, axis=-1):
    return jax.nn.softmax(x, axis=axis)
def _gelu(x):
    return jax.nn.gelu(x, approximate=True)
def _silu(x):
    return jax.nn.silu(x)
def _sigmoid(x):
    return jax.nn.sigmoid(x)
def _layernorm(x, axis=-1, eps=1e-5):
    m = jnp.mean(x, axis=axis, keepdims=True)
    v = jnp.var(x, axis=axis, keepdims=True)
    return (x - m) / jnp.sqrt(v + eps)
def _scatter_add(tgt, idx, src, axis=0):
    return tgt.at[idx].add(src)
def _segment_sum(src, seg, n):
    return jax.ops.segment_sum(src, seg, n)
class _Rng:
    def __init__(self, key):
        self._k = key
    def _next(self):
        self._k, sub = jax.random.split(self._k)
        return sub
    def normal(self, shape):
        return jax.random.normal(self._next(), shape, dtype=jnp.bfloat16)
    def randint(self, lo, hi, shape):
        return jax.random.randint(self._next(), shape, lo, hi, dtype=jnp.int32)
    def uniform(self, shape, lo=0.0, hi=1.0):
        return jax.random.uniform(self._next(), shape, jnp.bfloat16, lo, hi)
    def permutation(self, n):
        return jax.random.permutation(self._next(), n)


kernel_name = 'sequential_preLN__linear_kernel_hedgehog__moe_arch_mod__prompt'

def setup_inputs():
    _rng = _Rng(jax.random.key(int.from_bytes(__import__("os").urandom(4), "little")))
    _w = (lambda a: (lambda t: t.astype(jnp.bfloat16) if jnp.issubdtype(t.dtype, jnp.floating) else t)(jnp.asarray(a)))
    def _A_setup():
        B, S, D, H = 1, 2048, 1024, 32
        Dh = D // H
        return {
            "x": _w((lambda *s: _rng.normal(s) * 0.05)(B, S, D)),
            "wqkv": _w((lambda *s: _rng.normal(s) * 0.05)(D, 3 * D)),
            "w_phi": _w((lambda *s: _rng.normal(s) * 0.05)(H, Dh, Dh) * (Dh ** -0.5)),
            "wo": _w((lambda *s: _rng.normal(s) * 0.05)(D, D)),
        }
    _A_in = _A_setup()

    def _B_setup():
        B, S, D, F, C = 1, 2048, 1024, 3584, 1
        return {
            "x": _w((lambda *s: _rng.normal(s) * 0.05)(B, S, D)),
            "w_r": _w((lambda *s: _rng.normal(s) * 0.05)(D)),
            "w_gate": _w((lambda *s: _rng.normal(s) * 0.05)(D, F)),
            "w_up": _w((lambda *s: _rng.normal(s) * 0.05)(D, F)),
            "w_down": _w((lambda *s: _rng.normal(s) * 0.05)(F, D)),
        }
    _B_in = _B_setup()

    return {
        "A_x": _A_in["x"],
        "A_wqkv": _A_in["wqkv"],
        "A_w_phi": _A_in["w_phi"],
        "A_wo": _A_in["wo"],
        "B_x": _B_in["x"],
        "B_w_r": _B_in["w_r"],
        "B_w_gate": _B_in["w_gate"],
        "B_w_up": _B_in["w_up"],
        "B_w_down": _B_in["w_down"],
    }

def reference(A_x, A_wqkv, A_w_phi, A_wo, B_x, B_w_r, B_w_gate, B_w_up, B_w_down):
    def _A_ref(x, wqkv, w_phi, wo):
        B, S, D = x.shape
        H = 32; Dh = D // H
        qkv = (lambda x, *d: x.transpose(*d))((x @ wqkv).reshape(B, S, 3, H, Dh), 2, 0, 3, 1, 4)
        q, k, v = qkv[0], qkv[1], qkv[2]
        pq = jnp.einsum("bhsd,hdf->bhsf", q, w_phi)
        pk = jnp.einsum("bhsd,hdf->bhsf", k, w_phi)
        phi_q = jnp.concatenate([_softmax(pq, axis=-1), _softmax(-pq, axis=-1)], axis=-1)
        phi_k = jnp.concatenate([_softmax(pk, axis=-1), _softmax(-pk, axis=-1)], axis=-1)
        kv = jnp.einsum("bhsf,bhsd->bhfd", phi_k, v)
        z  = jnp.einsum("bhsf->bhf", phi_k)
        num = jnp.einsum("bhqf,bhfd->bhqd", phi_q, kv)
        den = jnp.einsum("bhqf,bhf->bhq", phi_q, z)[..., None] + 1e-6
        o = num / den
        return (lambda x, *d: x.transpose(*d))(o, 0, 2, 1, 3).reshape(B, S, D) @ wo

    def _B_ref(x, w_r, w_gate, w_up, w_down):
        B, S, D = x.shape
        C = 1
        r = x @ w_r
        idx = jnp.argsort(-r, axis=-1)[:, :C]
        idx_e = jnp.repeat(idx.reshape(B, C, 1), D, axis=2)
        x_sel = jnp.take_along_axis(x, idx_e, axis=1)
        g = _silu(x_sel @ w_gate)
        u = x_sel @ w_up
        y = (g * u) @ w_down
        r_sel = _sigmoid(jnp.take_along_axis(r, idx, axis=1))
        y = y * r_sel.reshape(B, C, 1)
        b_off = (jnp.arange(B) * S).reshape(B, 1)
        flat_idx = (idx + b_off).reshape(B * C)
        zero = (x * 0.0).reshape(B * S, D)
        upd = _scatter_add(zero, flat_idx, y.reshape(B * C, D), axis=0)
        return x + upd.reshape(B, S, D)

    x = A_x
    h = x + _A_ref(_layernorm(x, axis=-1), A_wqkv, A_w_phi, A_wo)
    h2 = h + _B_ref(_layernorm(h, axis=-1), B_w_r, B_w_gate, B_w_up, B_w_down)
    return h2
```

```python
import jax
import jax.numpy as jnp
from jax import lax
import jax.experimental.pallas as pl
import jax.experimental.pallas.tpu as pltpu

S = 2048
D = 1024
H = 32
DH = 32
F = 3584
NP = H // 2
T1 = 512
T2 = 512
N1 = S // T1
N2 = S // T2
CH = 256
LOG2E = 1.4426950408889634
EPS = 1e-5

_NT = (((1,), (1,)), ((), ()))
_TN = (((0,), (0,)), ((), ()))
f32 = jnp.float32
bf16 = jnp.bfloat16


def _rb(v):
    return v.astype(bf16).astype(f32)


def _ln_stats(xf):
    m = jnp.sum(xf, axis=-1, keepdims=True) * (1.0 / D)
    c = xf - m
    v = jnp.sum(c * c, axis=-1, keepdims=True) * (1.0 / D)
    s = _rb(jnp.sqrt(_rb(_rb(v) + EPS)))
    return c, 1.0 / s


def _dual_softmax(p):
    t = p.shape[-1]
    p3 = p.reshape(8, 8, t)

    def allred(v, op):
        v = op(v, pltpu.roll(v, 2, 0))
        return op(v, pltpu.roll(v, 4, 0))

    mx = allred(jnp.max(p3, axis=0), jnp.maximum)
    mn = allred(jnp.min(p3, axis=0), jnp.minimum)
    ep = jnp.exp2(p3 - mx[None])
    en = jnp.exp2(mn[None] - p3)
    sp = allred(jnp.sum(ep, axis=0), jnp.add)
    sn = allred(jnp.sum(en, axis=0), jnp.add)
    fp = (ep * (1.0 / sp)[None]).reshape(64, t).astype(bf16)
    fn = (en * (1.0 / sn)[None]).reshape(64, t).astype(bf16)
    return jnp.concatenate([fp, fn], axis=0)


def _kernel(x_hbm, wqkv_hbm, wphi_hbm, wo_hbm, wr_hbm, wg_hbm, wu_hbm, wd_hbm,
            out_hbm,
            x_v, wqkv_v, wphi_v, wo_v, wr_v, wg_v, wu_v, wd_v,
            wt_v, phiq_v, kv_acc, kvt_v, out_v, best_v, besti_v,
            sem_x, sem_w, sem_o):
    def x_copy(i):
        return pltpu.make_async_copy(
            x_hbm.at[0, pl.ds(i * T1, T1), :], x_v.at[pl.ds(i * T1, T1), :], sem_x.at[i])

    def w_copy(part):
        return pltpu.make_async_copy(
            wqkv_hbm.at[:, pl.ds(part * D, D)], wqkv_v.at[part], sem_w.at[part])

    c_phi = pltpu.make_async_copy(wphi_hbm, wphi_v, sem_w.at[3])
    c_wo = pltpu.make_async_copy(wo_hbm, wo_v, sem_w.at[4])
    c_wr = pltpu.make_async_copy(wr_hbm, wr_v, sem_w.at[5])
    c_wg = pltpu.make_async_copy(wg_hbm, wg_v, sem_w.at[6])
    c_wu = pltpu.make_async_copy(wu_hbm, wu_v, sem_w.at[7])
    c_wd = pltpu.make_async_copy(wd_hbm, wd_v, sem_w.at[8])

    c_phi.start()
    w_copy(1).start()
    w_copy(2).start()
    w_copy(0).start()
    for i in range(N1):
        x_copy(i).start()
    c_wr.start()
    c_wo.start()
    c_wg.start()
    c_wu.start()
    c_wd.start()

    c_phi.wait()
    w2 = wphi_v[...].reshape(H * DH, DH)
    er = lax.broadcasted_iota(jnp.int32, (128, DH), 0)
    ec = lax.broadcasted_iota(jnp.int32, (128, DH), 1)
    e = jnp.where(ec == (er % 64) // 2, 1.0, 0.0).astype(bf16)
    ptf = lax.dot_general(e, w2, _NT, preferred_element_type=f32)
    pr = lax.broadcasted_iota(jnp.int32, (128, D), 0)
    pc = lax.broadcasted_iota(jnp.int32, (128, D), 1)
    keep = ((pc % 128) // 32) == ((pr // 64) * 2 + pr % 2)
    pt = jnp.where(keep, ptf, 0.0).astype(bf16)

    def fold(part, row0):
        for g in range(8):
            w = lax.dot_general(pt[:, g * 128:(g + 1) * 128],
                                wqkv_v[part, :, g * 128:(g + 1) * 128],
                                _NT, preferred_element_type=f32)
            wt_v[row0 + g * 128:row0 + (g + 1) * 128, :] = (w * LOG2E).astype(bf16)

    w_copy(1).wait()
    fold(1, 0)
    w_copy(2).wait()
    wt_v[D:2 * D, :] = wqkv_v[2].T
    w_copy(0).wait()
    fold(0, 2 * D)

    kv_acc[...] = jnp.zeros_like(kv_acc)

    def phase1(i, carry):
        x_copy(i).wait()
        r0 = pl.multiple_of(i * T1, T1)
        xf = x_v[pl.ds(r0, T1), :].astype(f32)
        c, inv = _ln_stats(xf)
        xn = (c * inv).astype(bf16)

        phik = []
        for cidx in range(D // CH):
            p = lax.dot_general(wt_v[cidx * CH:(cidx + 1) * CH, :], xn, _NT,
                                preferred_element_type=f32)
            for j in range(CH // 64):
                phik.append(_dual_softmax(p[j * 64:(j + 1) * 64]))
        vt = []
        for cidx in range(D // CH):
            p = lax.dot_general(wt_v[D + cidx * CH:D + (cidx + 1) * CH, :], xn, _NT,
                                preferred_element_type=f32).astype(bf16)
            for j in range(CH // 64):
                vt.append(p[j * 64:(j + 1) * 64])
        for cidx in range(D // CH):
            p = lax.dot_general(wt_v[2 * D + cidx * CH:2 * D + (cidx + 1) * CH, :], xn, _NT,
                                preferred_element_type=f32)
            for j in range(CH // 64):
                jj = cidx * (CH // 64) + j
                phiq_v[i, jj * 128:(jj + 1) * 128, :] = _dual_softmax(p[j * 64:(j + 1) * 64])
        ones = jnp.ones((16, T1), bf16)
        for j in range(NP):
            lhs = jnp.concatenate([vt[j], ones], axis=0)
            kv_acc[j] += lax.dot_general(lhs, phik[j], _NT, preferred_element_type=f32)
        return carry

    lax.fori_loop(0, N1, phase1, 0)

    kr = lax.broadcasted_iota(jnp.int32, (80, 128), 0)
    kc = lax.broadcasted_iota(jnp.int32, (80, 128), 1)
    rh = jnp.where(kr < 64, kr // 32, (kr - 64) // 8)
    kmask = rh == kc % 2
    for j in range(NP):
        kvt_v[j] = jnp.where(kmask, kv_acc[j], 0.0).astype(bf16)

    c_wr.wait()
    c_wo.wait()
    best_v[...] = jnp.full(best_v.shape, -jnp.inf, f32)
    besti_v[...] = jnp.zeros(besti_v.shape, jnp.int32)

    def o_copy(i):
        return pltpu.make_async_copy(
            out_v.at[pl.ds(i * T2, T2), :], out_hbm.at[0, pl.ds(i * T2, T2), :], sem_o.at[i])

    def phase2(i, carry):
        r0 = pl.multiple_of(i * T2, T2)
        ot = []
        for j in range(NP):
            n = jnp.dot(kvt_v[j], phiq_v[i, j * 128:(j + 1) * 128, :],
                        preferred_element_type=f32)
            r0h = 1.0 / (n[64:72] + 1e-6)
            r1h = 1.0 / (n[72:80] + 1e-6)
            o0 = n[0:32].reshape(4, 8, T2) * r0h[None]
            o1 = n[32:64].reshape(4, 8, T2) * r1h[None]
            ot.append(o0.reshape(32, T2).astype(bf16))
            ot.append(o1.reshape(32, T2).astype(bf16))
        otf = jnp.concatenate(ot, axis=0)
        attn = lax.dot_general(otf, wo_v[...], _TN, preferred_element_type=f32)
        h = x_v[pl.ds(r0, T2), :].astype(f32) + attn
        x_v[pl.ds(r0, T2), :] = h.astype(bf16)
        c, inv = _ln_stats(h)
        wr = wr_v[...].astype(f32).reshape(1, D)
        r = _rb(jnp.sum(c * wr, axis=-1, keepdims=True) * inv)
        out_v[pl.ds(r0, T2), :] = (h + c * inv).astype(bf16)
        o_copy(i).start()
        r3 = r.reshape(T2 // 8, 8, 1)
        tmax = jnp.max(r3, axis=0)
        idx3 = (lax.broadcasted_iota(jnp.int32, (T2 // 8, 8, 1), 0) * 8
                + lax.broadcasted_iota(jnp.int32, (T2 // 8, 8, 1), 1) + r0)
        tidx = jnp.min(jnp.where(r3 == tmax[None], idx3, S), axis=0)
        better = tmax > best_v[...]
        besti_v[...] = jnp.where(better, tidx, besti_v[...])
        best_v[...] = jnp.where(better, tmax, best_v[...])
        return carry

    lax.fori_loop(0, N2, phase2, 0)

    bv = best_v[...]
    rmax = jnp.max(bv, axis=0, keepdims=True)
    idx = jnp.min(jnp.where(bv == rmax, besti_v[...], S))
    idx = jnp.clip(idx, 0, S - 1)
    b0 = pl.multiple_of((idx // 16) * 16, 16)
    hb = x_v[pl.ds(b0, 16), :].astype(f32)
    c, inv = _ln_stats(hb)
    hn = c * inv
    xs = hn.astype(bf16)
    c_wg.wait()
    c_wu.wait()
    c_wd.wait()
    g = jnp.dot(xs, wg_v[...], preferred_element_type=f32)
    u = jnp.dot(xs, wu_v[...], preferred_element_type=f32)
    a = (g * (1.0 / (1.0 + jnp.exp(-g))) * u).astype(bf16)
    y = jnp.dot(a, wd_v[...], preferred_element_type=f32)
    gate = 1.0 / (1.0 + jnp.exp(-rmax))
    rows = lax.broadcasted_iota(jnp.int32, (16, D), 0) + b0
    for i in range(N2):
        o_copy(i).wait()
    cur = out_v[pl.ds(b0, 16), :]
    out_v[pl.ds(b0, 16), :] = jnp.where(rows == idx, (hb + hn + y * gate).astype(bf16), cur)
    fix = pltpu.make_async_copy(
        out_v.at[pl.ds(b0, 16), :], out_hbm.at[0, pl.ds(b0, 16), :], sem_o.at[0])
    fix.start()
    fix.wait()


@jax.jit
def pallas_sequential_preLN__linear_kernel_hedgehog__moe_arch_mod__prompt_kernel(
    A_x: jax.Array,
    A_wqkv: jax.Array,
    A_w_phi: jax.Array,
    A_wo: jax.Array,
    B_x: jax.Array,
    B_w_r: jax.Array,
    B_w_gate: jax.Array,
    B_w_up: jax.Array,
    B_w_down: jax.Array,
):
    any_spec = pl.BlockSpec(memory_space=pl.ANY)
    return pl.pallas_call(
        _kernel,
        out_shape=jax.ShapeDtypeStruct((1, S, D), bf16),
        in_specs=[any_spec] * 8,
        out_specs=any_spec,
        scratch_shapes=[
            pltpu.VMEM((S, D), bf16),
            pltpu.VMEM((3, D, D), bf16),
            pltpu.VMEM((H, DH, DH), bf16),
            pltpu.VMEM((D, D), bf16),
            pltpu.VMEM((D,), bf16),
            pltpu.VMEM((D, F), bf16),
            pltpu.VMEM((D, F), bf16),
            pltpu.VMEM((F, D), bf16),
            pltpu.VMEM((3 * D, D), bf16),
            pltpu.VMEM((N1, 2 * D, T1), bf16),
            pltpu.VMEM((NP, 80, 128), f32),
            pltpu.VMEM((NP, 80, 128), bf16),
            pltpu.VMEM((S, D), bf16),
            pltpu.VMEM((8, 1), f32),
            pltpu.VMEM((8, 1), jnp.int32),
            pltpu.SemaphoreType.DMA((N1,)),
            pltpu.SemaphoreType.DMA((9,)),
            pltpu.SemaphoreType.DMA((N2,)),
        ],
        compiler_params=pltpu.CompilerParams(vmem_limit_bytes=110 * 1024 * 1024),
    )(A_x, A_wqkv, A_w_phi, A_wo, B_w_r, B_w_gate, B_w_up, B_w_down)
```

```python
import jax
import jax.numpy as jnp
from jax import lax
import jax.experimental.pallas as pl
import jax.experimental.pallas.tpu as pltpu

S = 2048
D = 1024
H = 32
DH = 32
F = 3584
NP = H // 2
T1 = 256
T2 = 512
N1 = S // T1
N2 = S // T2
HT1 = T1 // 2
HT2 = T2 // 2
HD = D // 2
WC = 256
NWC = D // WC
LOG2E = 1.4426950408889634
EPS = 1e-5
WO_ROWS = 80
LN_ROWS = 16
EP_ROWS = 32

_NT = (((1,), (1,)), ((), ()))
_TN = (((0,), (0,)), ((), ()))
f32 = jnp.float32
bf16 = jnp.bfloat16
u32 = jnp.uint32

K_, Q_, V_ = 0, 1, 2
SRC = {K_: 1, Q_: 0, V_: 2}

SEM_W = 0
SEM_X = SEM_W + 3 * NWC
SEM_PHI = SEM_X + N1
SEM_WO, SEM_WR, SEM_WG, SEM_WU, SEM_WD = (SEM_PHI + i for i in range(1, 6))
SEM_O = SEM_WD + 1
NSEM = SEM_O + 2 * N2


def _rb(v):
    return v.astype(bf16).astype(f32)


def _pack(v):
    return pltpu.bitcast(v.astype(bf16), u32)


def _unpack(w):
    return pltpu.bitcast(w, bf16)


def _pack2(a, b):
    return pltpu.bitcast(pltpu.pack_elementwise([a, b], packed_dtype=bf16), u32)


def _packi(v):
    r, c = v.shape
    v4 = v.reshape(r // 16, 2, 8, c)
    return _pack2(v4[:, 0], v4[:, 1]).reshape(r // 2, c)


def _split2(w):
    return tuple(pltpu.unpack_elementwise(w, index=i, packed_dtype=bf16, unpacked_dtype=f32)
                 for i in range(2))


def _recip(x):
    r = pl.reciprocal(x, approx=True)
    return r * (2.0 - x * r)


def _rsqrt(x):
    return lax.rsqrt(x)


def _dual_softmax(p):
    t = p.shape[-1]
    p3 = p.reshape(8, 8, t)

    def allred(v, op):
        v = op(v, pltpu.roll(v, 2, 0))
        return op(v, pltpu.roll(v, 4, 0))

    mx = allred(jnp.max(p3, axis=0), jnp.maximum)
    mn = allred(jnp.min(p3, axis=0), jnp.minimum)
    ep = jnp.exp2(p3 - mx[None])
    en = jnp.exp2(mn[None] - p3)
    sp = allred(jnp.sum(ep, axis=0), jnp.add)
    sn = allred(jnp.sum(en, axis=0), jnp.add)
    fp = (ep * _recip(sp)[None]).reshape(64, t)
    fn = (en * _recip(sn)[None]).reshape(64, t)
    return _pack2(fp, fn)


def _left_combos(a11, a12, a21, a22):
    return [a11 + a22, a21 + a22, a11, a22, a11 + a12, a21 - a11, a12 - a22]


def _right_combos(b11, b12, b21, b22):
    return [b11 + b22, b11, b12 - b22, b21 - b11, b22, b11 + b12, b21 + b22]


def _strassen(prod, emit):
    m3 = prod(2)
    m5 = prod(4)
    emit(0, 1, m3 + m5)
    m7 = prod(6)
    u = m7 - m5
    m1 = prod(0)
    u = u + m1
    w = m1 + m3
    m4 = prod(3)
    emit(0, 0, u + m4)
    m2 = prod(1)
    emit(1, 0, m2 + m4)
    w = w - m2
    m6 = prod(5)
    emit(1, 1, w + m6)


def _fold_token(w, zero):
    r, c = w.shape
    acc = None
    for i in range(r // 8):
        for j in range(c // 128):
            blk = w[i * 8:(i + 1) * 8, j * 128:(j + 1) * 128]
            acc = blk if acc is None else acc | blk
    return acc & zero


def _pin(w, toks):
    if not toks:
        return w
    top = []
    for j in range(w.shape[1] // 128):
        blk = w[0:8, j * 128:(j + 1) * 128]
        if j in toks:
            blk = blk | toks[j]
        top.append(blk)
    return jnp.concatenate([jnp.concatenate(top, axis=1), w[8:]], axis=0)


def _kernel(x_hbm, wqkv_hbm, wphi_hbm, wo_hbm, wr_hbm, wg_hbm, wu_hbm, wd_hbm,
            out_hbm,
            x_v, wqkv_v, wphi_v, wo_v, wr_v, wg_v, wu_v, wd_v,
            wt_v, wo7_v, s_v, phiq_v, kv_acc, kvt_v, attn_v, h_v, out_v,
            wrf_v, best_v, besti_v, zero_s, sem):
    def x_copy(i):
        return pltpu.make_async_copy(
            x_hbm.at[0, pl.ds(i * T1, T1), :], x_v.at[pl.ds(i * T1, T1), :],
            sem.at[SEM_X + i])

    def w_copy(kind, c):
        return pltpu.make_async_copy(
            wqkv_hbm.at[:, pl.ds(SRC[kind] * D + c * WC, WC)],
            wqkv_v.at[kind * NWC + c], sem.at[SEM_W + kind * NWC + c])

    def full_copy(src, dst, slot):
        return pltpu.make_async_copy(src, dst, sem.at[slot])

    full_copy(wphi_hbm, wphi_v, SEM_PHI).start()
    w_copy(K_, 0).start()
    x_copy(0).start()
    for c in range(1, NWC):
        w_copy(K_, c).start()
    for kind in (Q_, V_):
        for c in range(NWC):
            w_copy(kind, c).start()
    x_copy(1).start()
    full_copy(wo_hbm, wo_v, SEM_WO).start()
    for i in range(2, N1):
        x_copy(i).start()
    full_copy(wr_hbm, wr_v, SEM_WR).start()
    full_copy(wg_hbm, wg_v, SEM_WG).start()
    full_copy(wu_hbm, wu_v, SEM_WU).start()
    full_copy(wd_hbm, wd_v, SEM_WD).start()

    def ln1_piece(r0, slot, p, rows):
        xs = [_split2(pltpu.bitcast(x_v[pl.ds(r0 + hf * HT1 + p * rows, rows), :], u32))
              for hf in range(2)]
        combos = []
        for par in range(2):
            xn = []
            for hf in range(2):
                xf = xs[hf][par]
                m = jnp.sum(xf, axis=-1, keepdims=True) * (1.0 / D)
                q = jnp.sum(xf * xf, axis=-1, keepdims=True) * (1.0 / D)
                inv = _rsqrt(jnp.maximum(q - m * m, 0.0) + EPS)
                xn.append(xf * inv - m * inv)
            combos.append(_right_combos(xn[0][:, :HD], xn[1][:, :HD],
                                        xn[0][:, HD:], xn[1][:, HD:]))
        for i in range(7):
            s_v[slot, i, p * rows // 2:(p + 1) * rows // 2, :] = _pack2(combos[0][i],
                                                                        combos[1][i])

    def prep_chunk(kind, c, pt):
        halves = []
        for hh in range(2):
            w = wqkv_v[kind * NWC + c, :, hh * 128:(hh + 1) * 128]
            if kind == V_:
                halves.append(_split2(pltpu.bitcast(w.T, u32)))
            else:
                g = 2 * c + hh
                wf = lax.dot_general(pt[:, g * 128:(g + 1) * 128], w, _NT,
                                     preferred_element_type=f32) * LOG2E
                halves.append((wf[:64], wf[64:]))
        combos = [_left_combos(halves[0][par][:, :HD], halves[0][par][:, HD:],
                               halves[1][par][:, :HD], halves[1][par][:, HD:])
                  for par in range(2)]
        r0 = (kind * HD + c * 128) // 2
        for i in range(7):
            wt_v[i, r0:r0 + 64, :] = _pack2(combos[0][i], combos[1][i])

    def proj_chunks(kind, cs, t, slot, phik, vt, fillers=()):
        r0 = (kind * HD + cs[0] * 128) // 2
        rows = 64 * len(cs)
        fillers = list(fillers)

        def prod(i):
            m = lax.dot_general(_unpack(wt_v[i, r0:r0 + rows, :]), _unpack(s_v[slot, i]),
                                _NT, preferred_element_type=f32)
            if fillers:
                fillers.pop(0)()
            return m

        def emit(rh, ch, blk):
            for n, c in enumerate(cs):
                for jj in range(2):
                    pair = 4 * c + 2 * rh + jj
                    p = blk[n * 128 + jj * 64:n * 128 + (jj + 1) * 64]
                    if kind == K_:
                        phik[pair][ch] = _dual_softmax(p)
                    elif kind == Q_:
                        phiq_v[t, pair * 64:(pair + 1) * 64,
                               ch * HT1:(ch + 1) * HT1] = _dual_softmax(p)
                    else:
                        vt[pair][ch] = _packi(p)

        _strassen(prod, emit)

    def kv_update(phik, vt, first):
        ones = _pack(jnp.ones((16, T1), f32))
        for j in range(NP):
            lhs = jnp.concatenate([jnp.concatenate(vt[j], axis=1), ones], axis=0)
            rhs = jnp.concatenate(phik[j], axis=1)
            upd = lax.dot_general(_unpack(lhs), _unpack(rhs), _NT,
                                  preferred_element_type=f32)
            if first:
                kv_acc[j] = upd
            else:
                kv_acc[j] += upd

    full_copy(wphi_hbm, wphi_v, SEM_PHI).wait()
    zs = pl.semaphore_read(zero_s)
    w2 = wphi_v[...].reshape(H * DH, DH)
    er = lax.broadcasted_iota(jnp.int32, (128, DH), 0)
    ec = lax.broadcasted_iota(jnp.int32, (128, DH), 1)
    e = jnp.where(ec == er % 32, 1.0, 0.0).astype(bf16)
    ptf = lax.dot_general(e, w2, _NT, preferred_element_type=f32)
    pr = lax.broadcasted_iota(jnp.int32, (128, D), 0)
    pc = lax.broadcasted_iota(jnp.int32, (128, D), 1)
    keep = ((pc % 128) // 32) == (((pr % 64) // 32) * 2 + pr // 64)
    pt = jnp.where(keep, ptf, 0.0).astype(bf16)

    phik = [[None, None] for _ in range(NP)]
    vt = [[None, None] for _ in range(NP)]
    n_ln = HT1 // LN_ROWS

    w_copy(K_, 0).wait()
    prep_chunk(K_, 0, pt)
    x_copy(0).wait()
    for p in range(n_ln):
        ln1_piece(0, zs, p, LN_ROWS)
    w_copy(K_, 1).wait()
    prep_chunk(K_, 1, pt)
    proj_chunks(K_, [0], 0, zs, phik, vt)
    w_copy(K_, 2).wait()
    w_copy(K_, 3).wait()
    prep_chunk(K_, 2, pt)
    proj_chunks(K_, [1], 0, zs, phik, vt)
    prep_chunk(K_, 3, pt)
    proj_chunks(K_, [2], 0, zs, phik, vt)
    w_copy(Q_, 0).wait()
    w_copy(Q_, 1).wait()
    prep_chunk(Q_, 0, pt)
    proj_chunks(K_, [3], 0, zs, phik, vt)
    prep_chunk(Q_, 1, pt)
    proj_chunks(Q_, [0], 0, zs, phik, vt)
    w_copy(Q_, 2).wait()
    w_copy(Q_, 3).wait()
    w_copy(V_, 0).wait()
    prep_chunk(Q_, 2, pt)
    proj_chunks(Q_, [1], 0, zs, phik, vt)
    prep_chunk(Q_, 3, pt)
    prep_chunk(V_, 0, pt)
    proj_chunks(Q_, [2], 0, zs, phik, vt)
    w_copy(V_, 1).wait()
    w_copy(V_, 2).wait()
    w_copy(V_, 3).wait()
    x_copy(1).wait()
    prep_chunk(V_, 1, pt)
    proj_chunks(Q_, [3], 0, zs, phik, vt)
    prep_chunk(V_, 2, pt)
    proj_chunks(V_, [0], 0, zs, phik, vt)
    prep_chunk(V_, 3, pt)
    lns = [(lambda p=p: ln1_piece(T1, 1 - zs, p, LN_ROWS)) for p in range(n_ln)]
    proj_chunks(V_, [1], 0, zs, phik, vt, lns[:2])
    attn_v[...] = jnp.zeros_like(attn_v)
    proj_chunks(V_, [2, 3], 0, zs, phik, vt, lns[2:])
    kv_update(phik, vt, True)
    full_copy(wo_hbm, wo_v, SEM_WO).wait()

    def phase1(t, carry):
        @pl.when(t + 1 < N1)
        def _():
            x_copy(t + 1).wait()

        slot = t % 2
        phik = [[None, None] for _ in range(NP)]
        vt = [[None, None] for _ in range(NP)]
        nxt = pl.multiple_of(jnp.minimum(t + 1, N1 - 1) * T1, T1)
        lns = [(lambda p=p: ln1_piece(nxt, 1 - slot, p, LN_ROWS)) for p in range(n_ln)]
        for kind in (K_, Q_):
            proj_chunks(kind, [0, 1], t, slot, phik, vt)
            proj_chunks(kind, [2, 3], t, slot, phik, vt)
        proj_chunks(V_, [0, 1], t, slot, phik, vt, [lambda: None] * 2 + lns[:5])
        w0 = pl.multiple_of(jnp.minimum((t - 1) * WO_ROWS, HD - WO_ROWS), 16)
        top = wo_v[pl.ds(w0, WO_ROWS), :].astype(f32)
        bot = wo_v[pl.ds(HD + w0, WO_ROWS), :].astype(f32)
        combos = _right_combos(top[:, :HD], top[:, HD:], bot[:, :HD], bot[:, HD:])
        w0h = pl.multiple_of(w0 // 2, 8)
        for i in range(7):
            wo7_v[i, pl.ds(w0h, WO_ROWS // 2), :] = _packi(combos[i])
        proj_chunks(V_, [2, 3], t, slot, phik, vt, lns[5:])
        kv_update(phik, vt, False)
        return carry

    lax.fori_loop(1, N1, phase1, 0)

    kr = lax.broadcasted_iota(jnp.int32, (80, 128), 0)
    kc = lax.broadcasted_iota(jnp.int32, (80, 128), 1)
    rh = jnp.where(kr < 64, kr // 32, (kr - 64) // 8)
    kmask = rh == (kc // 2) % 2
    for j in range(NP):
        kvt_v[j] = _pack(jnp.where(kmask, kv_acc[j], 0.0))

    full_copy(wr_hbm, wr_v, SEM_WR).wait()
    wr_row = wr_v[...].astype(f32).reshape(1, D)
    wrf_v[...] = jnp.broadcast_to(wr_row, (8, D))
    wr_sum = jnp.sum(wr_row, axis=-1, keepdims=True)
    best_v[...] = jnp.full(best_v.shape, -jnp.inf, f32)
    besti_v[...] = jnp.zeros(besti_v.shape, jnp.int32)
    zero_v = jnp.full((8, 128), zs, jnp.int32).astype(u32)

    def o_copy(hf):
        return pltpu.make_async_copy(
            out_v.at[pl.ds(hf * HT2, HT2), :], out_hbm.at[0, pl.ds(hf * HT2, HT2), :],
            sem.at[SEM_O + hf])

    def ln2_stats(h):
        m = jnp.sum(h, axis=-1, keepdims=True) * (1.0 / D)
        q = jnp.sum(h * h, axis=-1, keepdims=True) * (1.0 / D)
        t = _rb(_rb(jnp.maximum(q - m * m, 0.0)) + EPS)
        return m, _recip(_rb(t * _rsqrt(t)))

    def epilogue(r0, attn, valid, best):
        rows = attn.shape[0]
        h = x_v[pl.ds(r0, rows), :].astype(f32) + attn
        h_v[pl.ds(r0, rows), :] = h.astype(bf16)
        m, inv = ln2_stats(h)
        hw = h.reshape(rows // 8, 8, D) * wrf_v[...][None]
        hw = jnp.sum(hw.reshape(rows, D), axis=-1, keepdims=True)
        r = _rb((hw - m * wr_sum) * inv)
        o = h * (1.0 + inv) - m * inv
        out_v[pl.ds(r0, rows), :] = o.astype(bf16)
        bv, bi = best
        sub = lax.broadcasted_iota(jnp.int32, (8, 1), 0)
        for g in range(rows // 8):
            rg = r[g * 8:(g + 1) * 8]
            if valid is not None:
                rg = jnp.where(valid, rg, -jnp.inf)
            better = rg > bv
            bi = jnp.where(better, sub + (r0 + g * 8), bi)
            bv = jnp.where(better, rg, bv)
        tok = _fold_token(pltpu.bitcast(o[:, D - 128:], u32), zero_v)
        return (bv, bi), tok

    n_ep = HT2 // EP_ROWS

    def phase2(i, carry):
        ot = []
        for j in range(NP):
            ph = jnp.concatenate([phiq_v[2 * i, j * 64:(j + 1) * 64, :],
                                  phiq_v[2 * i + 1, j * 64:(j + 1) * 64, :]], axis=1)
            n = jnp.dot(_unpack(kvt_v[j]), _unpack(ph), preferred_element_type=f32)
            r0h = _recip(n[64:72] + 1e-6)
            r1h = _recip(n[72:80] + 1e-6)
            ot.append((n[0:32].reshape(4, 8, T2) * r0h[None]).reshape(32, T2))
            ot.append((n[32:64].reshape(4, 8, T2) * r1h[None]).reshape(32, T2))
        lo = jnp.concatenate(ot[:H // 2], axis=0)
        hi = jnp.concatenate(ot[H // 2:], axis=0)
        lcs = _left_combos(lo[:, :HT2], hi[:, :HT2], lo[:, HT2:], hi[:, HT2:])

        state = {'best': (best_v[...], besti_v[...]), 'n': 0}
        pins = {}

        def run_pieces(base, get_attn, valid, slots):
            for p in range(n_ep):
                r0 = pl.multiple_of(base + p * EP_ROWS, EP_ROWS)
                state['best'], tok = epilogue(r0, get_attn(p), valid, state['best'])
                if p < len(slots):
                    pins.setdefault(slots[p] // 4, {})[slots[p] % 4] = tok

        prev = jnp.maximum(i * T2 - HT2, HT2)
        run_pieces(prev, lambda p: attn_v[p * EP_ROWS:(p + 1) * EP_ROWS, :], i > 0,
                   [5, 7, 9, 11, 13, 15, 17, 19])

        def prod(k):
            w = _pin(wo7_v[k], pins.get(state['n']))
            state['n'] += 1
            return lax.dot_general(lcs[k].astype(bf16), _unpack(w), _TN,
                                   preferred_element_type=f32)

        blocks = {}

        def emit(rhalf, chalf, blk):
            if rhalf == 1:
                attn_v[:, chalf * HD:(chalf + 1) * HD] = blk
                return
            blocks[chalf] = blk
            if len(blocks) == 2:
                full = jnp.concatenate([blocks[0], blocks[1]], axis=1)
                run_pieces(i * T2, lambda p: full[p * EP_ROWS:(p + 1) * EP_ROWS], None,
                           [22, 23, 24, 25, 26, 27])

        _strassen(prod, emit)
        best_v[...], besti_v[...] = state['best']
        o_copy(2 * i).start()

        @pl.when(i > 0)
        def _():
            o_copy(2 * i - 1).start()

        return carry

    lax.fori_loop(0, N2, phase2, 0)
    best = (best_v[...], besti_v[...])
    for p in range(n_ep):
        best, _ = epilogue(S - HT2 + p * EP_ROWS, attn_v[p * EP_ROWS:(p + 1) * EP_ROWS, :],
                           None, best)
    o_copy(2 * N2 - 1).start()

    bv, bi = best
    rmax = jnp.max(bv, axis=0, keepdims=True)
    idx = jnp.min(jnp.where(bv == rmax, bi, S))
    idx = jnp.clip(idx, 0, S - 1)
    b0 = pl.multiple_of((idx // 16) * 16, 16)
    hb = h_v[pl.ds(b0, 16), :].astype(f32)
    m, inv = ln2_stats(hb)
    hn = (hb - m) * inv
    xs = hn.astype(bf16)
    full_copy(wg_hbm, wg_v, SEM_WG).wait()
    full_copy(wu_hbm, wu_v, SEM_WU).wait()
    full_copy(wd_hbm, wd_v, SEM_WD).wait()
    g = jnp.dot(xs, wg_v[...], preferred_element_type=f32)
    u = jnp.dot(xs, wu_v[...], preferred_element_type=f32)
    a = (g * (1.0 / (1.0 + jnp.exp(-g))) * u).astype(bf16)
    y = None
    for j in range(F // 256):
        p = jnp.dot(a[:, j * 256:(j + 1) * 256], wd_v[j * 256:(j + 1) * 256, :],
                    preferred_element_type=f32)
        y = p if y is None else y + p
    gate = 1.0 / (1.0 + jnp.exp(-rmax))
    rows = lax.broadcasted_iota(jnp.int32, (16, D), 0) + b0
    for hf in range(2 * N2):
        o_copy(hf).wait()
    cur = out_v[pl.ds(b0, 16), :]
    out_v[pl.ds(b0, 16), :] = jnp.where(rows == idx, (hb + hn + y * gate).astype(bf16), cur)
    fix = pltpu.make_async_copy(
        out_v.at[pl.ds(b0, 16), :], out_hbm.at[0, pl.ds(b0, 16), :], sem.at[SEM_O])
    fix.start()
    fix.wait()


@jax.jit
def pallas_sequential_preLN__linear_kernel_hedgehog__moe_arch_mod__prompt_kernel(
    A_x: jax.Array,
    A_wqkv: jax.Array,
    A_w_phi: jax.Array,
    A_wo: jax.Array,
    B_x: jax.Array,
    B_w_r: jax.Array,
    B_w_gate: jax.Array,
    B_w_up: jax.Array,
    B_w_down: jax.Array,
):
    any_spec = pl.BlockSpec(memory_space=pl.ANY)
    return pl.pallas_call(
        _kernel,
        out_shape=jax.ShapeDtypeStruct((1, S, D), bf16),
        in_specs=[any_spec] * 8,
        out_specs=any_spec,
        scratch_shapes=[
            pltpu.VMEM((S, D), bf16),
            pltpu.VMEM((3 * NWC, D, WC), bf16),
            pltpu.VMEM((H, DH, DH), bf16),
            pltpu.VMEM((D, D), bf16),
            pltpu.VMEM((D,), bf16),
            pltpu.VMEM((D, F), bf16),
            pltpu.VMEM((D, F), bf16),
            pltpu.VMEM((F, D), bf16),
            pltpu.VMEM((7, 3 * HD // 2, HD), u32),
            pltpu.VMEM((7, HD // 2, HD), u32),
            pltpu.VMEM((2, 7, HT1 // 2, HD), u32),
            pltpu.VMEM((N1, D, T1), u32),
            pltpu.VMEM((NP, 80, 128), f32),
            pltpu.VMEM((NP, 40, 128), u32),
            pltpu.VMEM((HT2, D), f32),
            pltpu.VMEM((S, D), bf16),
            pltpu.VMEM((S, D), bf16),
            pltpu.VMEM((8, D), f32),
            pltpu.VMEM((8, 1), f32),
            pltpu.VMEM((8, 1), jnp.int32),
            pltpu.SemaphoreType.REGULAR,
            pltpu.SemaphoreType.DMA((NSEM,)),
        ],
        compiler_params=pltpu.CompilerParams(vmem_limit_bytes=110 * 1024 * 1024),
    )(A_x, A_wqkv, A_w_phi, A_wo, B_w_r, B_w_gate, B_w_up, B_w_down)
```

```python
import jax
import jax.numpy as jnp
from jax import lax
import jax.experimental.pallas as pl
import jax.experimental.pallas.tpu as pltpu

S = 2048
D = 1024
H = 32
DH = 32
F = 3584
NP = H // 2
T1 = 256
T2 = 512
N1 = S // T1
N2 = S // T2
HT1 = T1 // 2
HT2 = T2 // 2
HD = D // 2
WC = 256
NWC = D // WC
LOG2E = 1.4426950408889634
EPS = 1e-5
WO_ROWS = 80
LN_ROWS = 16
EP_ROWS = 32
LT_START = (0, 0, 2, 5, 8, 11, 14)
LT_DEADLINE = (0, 4, 6, 9, 12, 15, 18)
FB_START = (5, 6, 7, 9, 10, 11, 13, 14)
SA_START = (15, 15, 16, 16, 17, 17, 18, 18)
FA_START = (20, 21, 22, 23, 24, 25, 26, 27)
FA_DEADLINE = (23, 24, 25, 26, 27, 29, 29, 29)
GATE_ROW = 0
T0_FOLD = 4
T0_WAITS = ((4, (1,)), (11, ('phi', 2)), (18, (3, 4)), (32, (5, 6, 7)), (46, (8, 9, 10)),
            (59, (11, 'x')))
T0_VPREP = ((46, 47, 49, 51), (52, 54, 56, 58), (60, 61, 63, 65), (66, 68, 70, 72))
T0_LN = (73, 75, 77, 79, 81, 83, 86, 90)
P1_LN = (29, 30, 32, 33, 35, 36, 38, 39)
P1_WO = (2, 3, 10, 17, 24)

_NT = (((1,), (1,)), ((), ()))
_TN = (((0,), (0,)), ((), ()))
f32 = jnp.float32
bf16 = jnp.bfloat16
u32 = jnp.uint32

K_, Q_, V_ = 0, 1, 2
SRC = {K_: 1, Q_: 0, V_: 2}

SEM_W = 0
SEM_X = SEM_W + 3 * NWC
SEM_X0 = SEM_X + N1
SEM_PHI = SEM_X0 + 4
SEM_WO = SEM_PHI + 2
SEM_WR, SEM_WG, SEM_WU, SEM_WD = (SEM_WO + 4 + i for i in range(4))
SEM_O = SEM_WD + 1
NSEM = SEM_O + 2 * N2


def _rb(v):
    return v.astype(bf16).astype(f32)


def _pack(v):
    return pltpu.bitcast(v.astype(bf16), u32)


def _unpack(w):
    return pltpu.bitcast(w, bf16)


def _pack2(a, b):
    return pltpu.bitcast(pltpu.pack_elementwise([a, b], packed_dtype=bf16), u32)


def _packi(v):
    r, c = v.shape
    v4 = v.reshape(r // 16, 2, 8, c)
    return _pack2(v4[:, 0], v4[:, 1]).reshape(r // 2, c)


def _split2(w):
    return tuple(pltpu.unpack_elementwise(w, index=i, packed_dtype=bf16, unpacked_dtype=f32)
                 for i in range(2))


def _recip(x):
    r = pl.reciprocal(x, approx=True)
    return r * (2.0 - x * r)


def _rsqrt(x):
    return lax.rsqrt(x)


def _dual_softmax(p):
    t = p.shape[-1]
    p3 = p.reshape(8, 8, t)

    def allred(v, op):
        v = op(v, pltpu.roll(v, 2, 0))
        return op(v, pltpu.roll(v, 4, 0))

    mx = allred(jnp.max(p3, axis=0), jnp.maximum)
    mn = allred(jnp.min(p3, axis=0), jnp.minimum)
    ep = jnp.exp2(p3 - mx[None])
    en = jnp.exp2(mn[None] - p3)
    sp = allred(jnp.sum(ep, axis=0), jnp.add)
    sn = allred(jnp.sum(en, axis=0), jnp.add)
    fp = (ep * _recip(sp)[None]).reshape(64, t)
    fn = (en * _recip(sn)[None]).reshape(64, t)
    return _pack2(fp, fn)


def _left_combos(a11, a12, a21, a22):
    return [a11 + a22, a21 + a22, a11, a22, a11 + a12, a21 - a11, a12 - a22]


def _right_combos(b11, b12, b21, b22):
    return [b11 + b22, b11, b12 - b22, b21 - b11, b22, b11 + b12, b21 + b22]


def _strassen(prod, emit):
    m3 = prod(2)
    m5 = prod(4)
    emit(0, 1, m3 + m5)
    m7 = prod(6)
    u = m7 - m5
    m1 = prod(0)
    u = u + m1
    w = m1 + m3
    m4 = prod(3)
    emit(0, 0, u + m4)
    m2 = prod(1)
    emit(1, 0, m2 + m4)
    w = w - m2
    m6 = prod(5)
    emit(1, 1, w + m6)


def _fold_token(w, zero):
    r, c = w.shape
    acc = None
    for i in range(r // 8):
        for j in range(c // 128):
            blk = w[i * 8:(i + 1) * 8, j * 128:(j + 1) * 128]
            acc = blk if acc is None else acc | blk
    return acc & zero


def _kernel(x_hbm, wqkv_hbm, wphi_hbm, wo_hbm, wr_hbm, wg_hbm, wu_hbm, wd_hbm,
            out_hbm,
            x_v, wqkv_v, wphi_v, wo_v, wr_v, wg_v, wu_v, wd_v,
            wt_v, wo7_v, s_v, phiq_v, kv_acc, kvt_v, hal_v, har_v, hbl_v, hbr_v, sa_v,
            t0_v, t1_v, t2_v, t3_v, t4_v, t5_v, t6_v, h_v, out_v,
            wrf_v, best_v, besti_v, fix_v, zero_s, sem):
    ha_v = (hal_v, har_v)
    hb_v = (hbl_v, hbr_v)
    tmp_v = (t0_v, t1_v, t2_v, t3_v, t4_v, t5_v, t6_v)

    def x_rows(r0, rows, slot):
        return pltpu.make_async_copy(
            x_hbm.at[0, pl.ds(r0, rows), :], x_v.at[pl.ds(r0, rows), :], sem.at[slot])

    def x_copy(i):
        return x_rows(i * T1, T1, SEM_X + i)

    def x0_copy(q):
        return x_rows((q % 2) * HT1 + (q // 2) * (HT1 // 2), HT1 // 2, SEM_X0 + q)

    def w_copy(kind, c):
        return pltpu.make_async_copy(
            wqkv_hbm.at[:, pl.ds(SRC[kind] * D + c * WC, WC)],
            wqkv_v.at[kind * NWC + c], sem.at[SEM_W + kind * NWC + c])

    def phi_copy(part):
        lo, n = part * (H // 2), H // 2
        return pltpu.make_async_copy(wphi_hbm.at[pl.ds(lo, n)], wphi_v.at[pl.ds(lo, n)],
                                     sem.at[SEM_PHI + part])

    def wo_copy(q):
        lo, n = (0, WO_ROWS) if q < 2 else (WO_ROWS, HD - WO_ROWS)
        lo += (q % 2) * HD
        return pltpu.make_async_copy(wo_hbm.at[pl.ds(lo, n), :], wo_v.at[pl.ds(lo, n), :],
                                     sem.at[SEM_WO + q])

    def full_copy(src, dst, slot):
        return pltpu.make_async_copy(src, dst, sem.at[slot])

    full_copy(wr_hbm, wr_v, SEM_WR).start()
    phi_copy(0).start()
    w_copy(K_, 0).start()
    for q in range(4):
        x0_copy(q).start()
    w_copy(K_, 1).start()
    phi_copy(1).start()
    for c in range(2, NWC):
        w_copy(K_, c).start()
    for kind in (Q_, V_):
        for c in range(NWC):
            w_copy(kind, c).start()
    x_copy(1).start()
    wo_copy(0).start()
    wo_copy(1).start()
    x_copy(2).start()
    wo_copy(2).start()
    wo_copy(3).start()
    for i in range(3, N1):
        x_copy(i).start()
    full_copy(wg_hbm, wg_v, SEM_WG).start()
    full_copy(wu_hbm, wu_v, SEM_WU).start()
    full_copy(wd_hbm, wd_v, SEM_WD).start()

    zs = pl.semaphore_read(zero_s)

    def ld(ref, r0, rows, c0, cols):
        return ref[pl.ds(pl.multiple_of(zs * 8 + r0, 8), rows), c0:c0 + cols]

    def x_piece(r0, p):
        return [_split2(pltpu.bitcast(
            x_v[pl.ds(pl.multiple_of(r0 + hf * HT1 + p * LN_ROWS, LN_ROWS), LN_ROWS), :], u32))
            for hf in range(2)]

    def ln1_stats(xf):
        m = jnp.sum(xf, axis=-1, keepdims=True) * (1.0 / D)
        q = jnp.sum(xf * xf, axis=-1, keepdims=True) * (1.0 / D)
        inv = _rsqrt(jnp.maximum(q - m * m, 0.0) + EPS)
        return inv, m * inv

    def ln1_store(p, xn):
        combos = [_right_combos(xn[0][par][:, :HD], xn[1][par][:, :HD],
                                xn[0][par][:, HD:], xn[1][par][:, HD:]) for par in range(2)]
        hr = LN_ROWS // 2
        for i in range(7):
            s_v[i, p * hr:(p + 1) * hr, :] = _pack2(combos[0][i], combos[1][i])

    def ln1_piece(r0, p, m=None):
        if m is not None:
            x_v[S:S + 8, 0:128] = m[0:8, 0:128].astype(bf16)
        xs = x_piece(r0, p)
        xn = [[None, None], [None, None]]
        for hf in range(2):
            for par in range(2):
                inv, mi = ln1_stats(xs[hf][par])
                xn[hf][par] = xs[hf][par] * inv - mi
        ln1_store(p, xn)

    def fold_piece(kind, c, j, pt):
        blk = {}
        for hh in range(2):
            for kh in range(2):
                k0 = kh * HD + j * 128
                w = wqkv_v[kind * NWC + c, k0:k0 + 128, hh * 128:(hh + 1) * 128]
                blk[hh, kh] = lax.dot_general(pt[2 * c + hh], w, _NT,
                                              preferred_element_type=f32) * LOG2E
        combos = _left_combos(blk[0, 0], blk[0, 1], blk[1, 0], blk[1, 1])
        r0 = (kind * HD + c * 128) // 2
        for i in range(7):
            wt_v[i, r0:r0 + 64, j * 128:(j + 1) * 128] = _packi(combos[i])

    def fold_chunk(kind, c, pt):
        for j in range(4):
            fold_piece(kind, c, j, pt)

    def vprep_piece(c, j, m):
        wqkv_v[3 * NWC, 0:8, 0:128] = m[0:8, 0:128].astype(bf16)
        blk = {}
        for hh in range(2):
            for kh in range(2):
                k0 = kh * HD + j * 128
                w = wqkv_v[zs + V_ * NWC + c, k0:k0 + 128, hh * 128:(hh + 1) * 128]
                blk[hh, kh] = _split2(pltpu.bitcast(w.T, u32))
        combos = [_left_combos(blk[0, 0][par], blk[0, 1][par], blk[1, 0][par], blk[1, 1][par])
                  for par in range(2)]
        r0 = (V_ * HD + c * 128) // 2
        for i in range(7):
            wt_v[i, r0:r0 + 64, j * 128:(j + 1) * 128] = _pack2(combos[0][i], combos[1][i])

    def wo_piece(w0, m):
        wo_v[D:D + 8, 0:128] = m[0:8, 0:128].astype(bf16)
        top = wo_v[pl.ds(pl.multiple_of(w0, 16), 16), :].astype(f32)
        bot = wo_v[pl.ds(pl.multiple_of(HD + w0, 16), 16), :].astype(f32)
        combos = _right_combos(top[:, :HD], top[:, HD:], bot[:, :HD], bot[:, HD:])
        w0h = pl.multiple_of(w0 // 2, 8)
        for i in range(7):
            wo7_v[i, pl.ds(w0h, 8), :] = _packi(combos[i])

    def run_tile(t, groups, pre, post, first):
        phik = [[None, None] for _ in range(NP)]
        vt = [[None, None] for _ in range(NP)]
        count = [0]
        svals = {}

        for kind, cs in groups:
            r0 = (kind * HD + cs[0] * 128) // 2
            rows = 64 * len(cs)

            def prod(i):
                if i not in svals:
                    svals[i] = _unpack(ld(s_v.at[i], 0, HT1 // 2, 0, HD) if first else s_v[i])
                rhs = svals[i]
                for fn in pre.get(count[0], ()):
                    fn()
                m = lax.dot_general(_unpack(wt_v[i, r0:r0 + rows, :]), rhs, _NT,
                                    preferred_element_type=f32)
                for fn in post.get(count[0], ()):
                    fn(m)
                count[0] += 1
                return m

            def emit(rh, ch, blk):
                for n, c in enumerate(cs):
                    for jj in range(2):
                        pair = 4 * c + 2 * rh + jj
                        p = blk[n * 128 + jj * 64:n * 128 + (jj + 1) * 64]
                        if kind == K_:
                            phik[pair][ch] = _dual_softmax(p)
                        elif kind == Q_:
                            phiq_v[t, pair * 64:(pair + 1) * 64,
                                   ch * HT1:(ch + 1) * HT1] = _dual_softmax(p)
                        else:
                            vt[pair][ch] = _packi(p)

            _strassen(prod, emit)

        ones = _pack(jnp.ones((16, T1), f32))
        kr = lax.broadcasted_iota(jnp.int32, (80, 128), 0)
        kc = lax.broadcasted_iota(jnp.int32, (80, 128), 1)
        kmask = jnp.where(kr < 64, kr // 32, (kr - 64) // 8) == (kc // 2) % 2
        for j in range(NP):
            lhs = jnp.concatenate([jnp.concatenate(vt[j], axis=1), ones], axis=0)
            rhs = jnp.concatenate(phik[j], axis=1)
            upd = lax.dot_general(_unpack(lhs), _unpack(rhs), _NT,
                                  preferred_element_type=f32)
            for fn in post.get(count[0], ()):
                fn(upd)
            count[0] += 1
            if first:
                kv_acc[j] = upd
            else:
                upd = kv_acc[j] + upd
                kv_acc[j] = upd
                kvt_v[j] = _pack(jnp.where(kmask, upd, 0.0))

    def load_best():
        return best_v[0], besti_v[...], best_v[1], best_v[2]

    def store_best(best):
        best_v[0], besti_v[...], best_v[1], best_v[2] = best

    def build_pt(g0, g1):
        n = g1 - g0
        w2 = wphi_v[4 * g0:4 * g1].reshape(n * 128, DH)
        er = lax.broadcasted_iota(jnp.int32, (128, DH), 0)
        ec = lax.broadcasted_iota(jnp.int32, (128, DH), 1)
        e = jnp.where(ec == ((er // 16) * 8 + er % 8) % 32, 1.0, 0.0).astype(bf16)
        ptf = lax.dot_general(e, w2, _NT, preferred_element_type=f32)
        pr = lax.broadcasted_iota(jnp.int32, (128, 128), 0)
        pc = lax.broadcasted_iota(jnp.int32, (128, 128), 1)
        keep = pc // 32 == (pr // 64) * 2 + (pr // 8) % 2
        return [jnp.where(keep, ptf[:, g * 128:(g + 1) * 128], 0.0).astype(bf16)
                for g in range(n)]

    hbl_v[...] = jnp.zeros_like(hbl_v)
    hbr_v[...] = jnp.zeros_like(hbr_v)
    store_best((jnp.full((8, 128), -jnp.inf, f32), jnp.zeros((8, 128), jnp.int32),
                jnp.zeros((8, 128), f32), jnp.zeros((8, 128), f32)))
    full_copy(wr_hbm, wr_v, SEM_WR).wait()
    phi_copy(0).wait()
    wr_row = wr_v[...].astype(f32).reshape(1, D)
    wrf_v[:, 0:D] = jnp.broadcast_to(wr_row, (8, D))
    wrf_v[:, D:D + 128] = jnp.broadcast_to(jnp.sum(wr_row, axis=-1, keepdims=True), (8, 128))
    pt = build_pt(0, 4)
    n_ln = HT1 // LN_ROWS

    w_copy(K_, 0).wait()
    fold_chunk(K_, 0, pt)
    for part in range(2):
        x0_copy(2 * part).wait()
        x0_copy(2 * part + 1).wait()
        for p in range(part * n_ln // 2, (part + 1) * n_ln // 2):
            ln1_piece(0, p)

    post = {}

    def at(slot, fn):
        post.setdefault(slot, []).append(fn)

    for slot, copies in T0_WAITS:
        for cp in copies:
            if cp == 'phi':
                at(slot, lambda m: phi_copy(1).wait())
            elif cp == 'x':
                at(slot, lambda m: x_copy(1).wait())
            else:
                at(slot, lambda m, cp=cp: w_copy(cp // NWC, cp % NWC).wait())
    for n in range(1, 2 * NWC):
        if n == 2:
            at(7 * n - 7 + T0_FOLD, lambda m: pt.extend(build_pt(4, 8)))
        at(7 * n - 7 + T0_FOLD, lambda m, n=n: fold_chunk(n // NWC, n % NWC, pt))
    for c in range(NWC):
        for j in range(4):
            at(T0_VPREP[c][j], lambda m, c=c, j=j: vprep_piece(c, j, m))
    for p in range(n_ln):
        at(T0_LN[p], lambda m, p=p: ln1_piece(zs + T1, p, m))
    run_tile(0, [(kind, [c]) for kind in (K_, Q_, V_) for c in range(NWC)], {}, post, True)
    wo_copy(0).wait()
    wo_copy(1).wait()

    def phase1(t, carry):
        @pl.when(t + 1 < N1)
        def _():
            x_copy(t + 1).wait()

        @pl.when(t == 2)
        def _():
            wo_copy(2).wait()
            wo_copy(3).wait()

        nxt = jnp.minimum(t + 1, N1 - 1) * T1
        w0 = jnp.minimum((t - 1) * WO_ROWS, HD - WO_ROWS)
        post = {}
        for p in range(n_ln):
            post.setdefault(P1_LN[p], []).append(lambda m, p=p: ln1_piece(nxt, p, m))
        for p in range(WO_ROWS // 16):
            post.setdefault(P1_WO[p], []).append(lambda m, p=p: wo_piece(w0 + 16 * p, m))
        run_tile(t, [(kind, cs) for kind in (K_, Q_, V_) for cs in ([0, 1], [2, 3])],
                 {}, post, False)
        return carry

    lax.fori_loop(1, N1, phase1, 0)

    full_copy(wg_hbm, wg_v, SEM_WG).wait()
    full_copy(wu_hbm, wu_v, SEM_WU).wait()
    full_copy(wd_hbm, wd_v, SEM_WD).wait()
    zero_v = jnp.full((8, 128), zs, jnp.int32).astype(u32)

    def o_copy(hf):
        return pltpu.make_async_copy(
            out_v.at[pl.ds(hf * HT2, HT2), :], out_hbm.at[0, pl.ds(hf * HT2, HT2), :],
            sem.at[SEM_O + hf])

    def half_stats(hh, c0):
        rows = hh.shape[0]
        parts = [hh[:, c * 128:(c + 1) * 128] for c in range(4)]
        wts = [wrf_v[:, c0 + c * 128:c0 + (c + 1) * 128] for c in range(4)]
        s1 = (parts[0] + parts[1]) + (parts[2] + parts[3])
        sq = [p * p for p in parts]
        s2 = (sq[0] + sq[1]) + (sq[2] + sq[3])
        dw = [(p.reshape(rows // 8, 8, 128) * w[None]).reshape(rows, 128)
              for p, w in zip(parts, wts)]
        s3 = (dw[0] + dw[1]) + (dw[2] + dw[3])
        return s1, s2, s3

    def first_half(hbuf, sbuf, base, p, c0):
        r0 = p * EP_ROWS
        hh = ld(hbuf[c0 // HD], r0, EP_ROWS, 0, HD)
        h_v[pl.ds(pl.multiple_of(base + r0, EP_ROWS), EP_ROWS), c0:c0 + HD] = hh.astype(bf16)
        st = jnp.concatenate(half_stats(hh, c0), axis=1)
        sbuf[r0:r0 + EP_ROWS, :] = st
        return _fold_token(pltpu.bitcast(st, u32), zero_v)

    def finish(hbuf, sbuf, base, p, valid, best, defer=None):
        r0 = p * EP_ROWS
        g0 = pl.multiple_of(base + r0, EP_ROWS)
        hl, hr = [ld(r, r0, EP_ROWS, 0, HD) for r in hbuf]
        h_v[pl.ds(g0, EP_ROWS), 0:HD] = hl.astype(bf16)
        if sbuf is None:
            h_v[pl.ds(g0, EP_ROWS), HD:D] = hr.astype(bf16)
            st = half_stats(hr, HD)
        else:
            st = ld(sbuf, r0, EP_ROWS, 0, 384)
            st = [st[:, n * 128:(n + 1) * 128] for n in range(3)]
        s1, s2, s3 = [jnp.sum(v + w, axis=-1, keepdims=True)
                      for v, w in zip(half_stats(hl, 0), st)]
        m = s1 * (1.0 / D)
        var = jnp.maximum(s2 * (1.0 / D) - m * m, 0.0)
        inv = _rsqrt(var + EPS)
        r = (s3 - m * wrf_v[0:1, D:D + 1]) * inv

        def write_out(h):
            o = h * (1.0 + inv) - m * inv
            out_v[pl.ds(g0, EP_ROWS), :] = o.astype(bf16)
            return o

        if defer is None:
            o = write_out(jnp.concatenate([hl, hr], axis=1))
        else:
            defer.append(lambda: write_out(jnp.concatenate(
                [r_[r0:r0 + EP_ROWS, :] for r_ in hbuf], axis=1)))
        bv, bi, bm, bq = best
        sub = lax.broadcasted_iota(jnp.int32, (8, 128), 0)
        for g in range(EP_ROWS // 8):
            rows = slice(g * 8, (g + 1) * 8)
            rg = jnp.broadcast_to(r[rows], (8, 128))
            if valid is not None:
                rg = jnp.where(valid, rg, -jnp.inf)
            better = rg > bv
            bi = jnp.where(better, sub + (g0 + g * 8), bi)
            bv = jnp.where(better, rg, bv)
            bm = jnp.where(better, jnp.broadcast_to(m[rows], (8, 128)), bm)
            bq = jnp.where(better, jnp.broadcast_to(var[rows], (8, 128)), bq)
        best = (bv, bi, bm, bq)
        if defer is not None:
            return best, None
        tok = _fold_token(pltpu.bitcast(jnp.concatenate(
            [o[:, D - 128:], bv, bm, bq], axis=0), u32), zero_v)
        return best, tok

    n_ep = HT2 // EP_ROWS

    def phase2(i, carry):
        ot = []
        for j in range(NP):
            ph = jnp.concatenate([phiq_v[2 * i, j * 64:(j + 1) * 64, :],
                                  phiq_v[2 * i + 1, j * 64:(j + 1) * 64, :]], axis=1)
            n = jnp.dot(_unpack(kvt_v[j]), _unpack(ph), preferred_element_type=f32)
            r0h = _recip(n[64:72] + 1e-6)
            r1h = _recip(n[72:80] + 1e-6)
            ot.append((n[0:32].reshape(4, 8, T2) * r0h[None]).reshape(32, T2))
            ot.append((n[32:64].reshape(4, 8, T2) * r1h[None]).reshape(32, T2))
        lo = jnp.concatenate(ot[:H // 2], axis=0)
        hi = jnp.concatenate(ot[H // 2:], axis=0)
        lcs = _left_combos(lo[:, :HT2], hi[:, :HT2], lo[:, HT2:], hi[:, HT2:])

        state = {'best': load_best()}
        pins = {}
        jobs = {}
        lts = {}
        ra = pl.multiple_of(i * T2, T2)
        rb = pl.multiple_of(i * T2 + HT2, HT2)
        prev = jnp.maximum(i * T2 - HT2, HT2)

        def add_job(slot, deadline, fn, gates=()):
            jobs.setdefault(slot, []).append((fn, deadline, gates))

        def finish_job(hbuf, sbuf, base, p, valid):
            def fn():
                state['best'], tok = finish(hbuf, sbuf, base, p, valid, state['best'])
                return tok
            return fn

        def lt_job(k):
            def fn():
                lts[k] = lcs[k].astype(bf16).T
                return _fold_token(pltpu.bitcast(lts[k], u32), zero_v)
            return fn

        order = (2, 4, 6, 0, 3, 1, 5)
        lt_job(2)()
        for n in range(1, 7):
            add_job(LT_START[n], LT_DEADLINE[n], lt_job(order[n]))
        for p in range(n_ep):
            add_job(FB_START[p], FB_START[p] + 2, finish_job(hb_v, None, prev, p, i > 0), hb_v)
            add_job(SA_START[p], SA_START[p] + 2, lambda p=p: first_half(ha_v, sa_v, ra, p, HD), ha_v[1:])
            add_job(FA_START[p], FA_DEADLINE[p], finish_job(ha_v, sa_v, ra, p, None), ha_v)

        def xblk(r0, c0):
            return x_v[pl.ds(r0, HT2), c0:c0 + 128].astype(f32)

        for n, k in enumerate(order):
            for c in range(4):
                slot = 4 * n + c
                for fn, deadline, gates in jobs.get(slot, ()):
                    for ref in gates:
                        ref[HT2:HT2 + 8, 0:128] = mm[GATE_ROW:GATE_ROW + 8]
                    pins.setdefault(deadline, []).append(fn())
                w = wo7_v[k, :, c * 128:(c + 1) * 128]
                toks = pins.get(slot)
                if toks:
                    top = w[0:8]
                    for tk in toks:
                        top = top | tk
                    w = jnp.concatenate([top, w[8:]], axis=0)
                mm = jnp.dot(lts[k], _unpack(w), preferred_element_type=f32)
                c0 = c * 128
                cs = slice(c0, c0 + 128)
                tmp = lambda t: ld(tmp_v[t], 0, HT2, c0, 128)
                if n == 0:
                    tmp_v[0][:, cs] = mm
                elif n == 1:
                    ha_v[1][0:HT2, cs] = (xblk(ra, HD + c0) + tmp(0)) + mm
                    tmp_v[1][:, cs] = xblk(ra, c0) - mm
                elif n == 2:
                    tmp_v[2][:, cs] = tmp(1) + mm
                elif n == 3:
                    tmp_v[3][:, cs] = tmp(2) + mm
                    tmp_v[4][:, cs] = (xblk(rb, HD + c0) + tmp(0)) + mm
                elif n == 4:
                    ha_v[0][0:HT2, cs] = tmp(3) + mm
                    tmp_v[5][:, cs] = xblk(rb, c0) + mm
                elif n == 5:
                    hb_v[0][0:HT2, cs] = tmp(5) + mm
                    tmp_v[6][:, cs] = tmp(4) - mm
                else:
                    hb_v[1][0:HT2, cs] = tmp(6) + mm
        store_best(state['best'])
        o_copy(2 * i).start()

        @pl.when(i > 0)
        def _():
            o_copy(2 * i - 1).start()

        return carry

    lax.fori_loop(0, N2, phase2, 0)
    best = load_best()
    late = []
    for p in range(n_ep):
        best, _ = finish(hb_v, None, S - HT2, p, None, best, late)

    bv, bi, bm, bq = best
    for sh in (4, 2, 1):
        ov, oi, om, oq = [pltpu.roll(t, sh, 0) for t in (bv, bi, bm, bq)]
        take = jnp.logical_or(ov > bv, jnp.logical_and(ov == bv, oi < bi))
        bv, bi, bm, bq = [jnp.where(take, o_, t)
                          for o_, t in zip((ov, oi, om, oq), (bv, bi, bm, bq))]
    idx = jnp.clip(bi[0, 0], 0, S - 1)
    b0 = pl.multiple_of((idx // 8) * 8, 8)
    t = _rb(_rb(bq) + EPS)
    inv = _recip(_rb(t * _rsqrt(t)))
    gate = _recip(1.0 + jnp.exp(-bv))
    wide = lambda v: jnp.concatenate([v] * (D // 128), axis=1)
    hb = h_v[pl.ds(b0, 8), :].astype(f32)
    hn = (hb - wide(bm)) * wide(inv)
    xs = hn.astype(bf16)
    g = jnp.dot(xs, wg_v[...], preferred_element_type=f32)
    for fn in late:
        fn()
    o_copy(2 * N2 - 1).start()
    u = jnp.dot(xs, wu_v[...], preferred_element_type=f32)
    a = (g * _recip(1.0 + jnp.exp(-g)) * u).astype(bf16)
    y = None
    for j in range(F // 256):
        p = jnp.dot(a[:, j * 256:(j + 1) * 256], wd_v[j * 256:(j + 1) * 256, :],
                    preferred_element_type=f32)
        y = p if y is None else y + p
    rows = lax.broadcasted_iota(jnp.int32, (8, D), 0) + b0
    cur = out_v[pl.ds(b0, 8), :].astype(f32)
    fix_v[...] = jnp.where(rows == wide(bi), hb + hn + y * wide(gate), cur).astype(bf16)
    for hf in range(2 * N2):
        o_copy(hf).wait()
    fix = pltpu.make_async_copy(fix_v, out_hbm.at[0, pl.ds(b0, 8), :], sem.at[SEM_O])
    fix.start()
    fix.wait()


@jax.jit
def pallas_sequential_preLN__linear_kernel_hedgehog__moe_arch_mod__prompt_kernel(
    A_x: jax.Array,
    A_wqkv: jax.Array,
    A_w_phi: jax.Array,
    A_wo: jax.Array,
    B_x: jax.Array,
    B_w_r: jax.Array,
    B_w_gate: jax.Array,
    B_w_up: jax.Array,
    B_w_down: jax.Array,
):
    any_spec = pl.BlockSpec(memory_space=pl.ANY)
    return pl.pallas_call(
        _kernel,
        out_shape=jax.ShapeDtypeStruct((1, S, D), bf16),
        in_specs=[any_spec] * 8,
        out_specs=any_spec,
        scratch_shapes=[
            pltpu.VMEM((S + 16, D), bf16),
            pltpu.VMEM((3 * NWC + 1, D, WC), bf16),
            pltpu.VMEM((H, DH, DH), bf16),
            pltpu.VMEM((D + 16, D), bf16),
            pltpu.VMEM((D,), bf16),
            pltpu.VMEM((D, F), bf16),
            pltpu.VMEM((D, F), bf16),
            pltpu.VMEM((F, D), bf16),
            pltpu.VMEM((7, 3 * HD // 2, HD), u32),
            pltpu.VMEM((7, HD // 2, HD), u32),
            pltpu.VMEM((7, HT1 // 2, HD), u32),
            pltpu.VMEM((N1, D, T1), u32),
            pltpu.VMEM((NP, 80, 128), f32),
            pltpu.VMEM((NP, 40, 128), u32),
            *[pltpu.VMEM((HT2 + 8, HD), f32) for _ in range(4)],
            pltpu.VMEM((HT2, 384), f32),
            *[pltpu.VMEM((HT2, HD), f32) for _ in range(7)],
            pltpu.VMEM((S, D), bf16),
            pltpu.VMEM((S, D), bf16),
            pltpu.VMEM((8, D + 128), f32),
            pltpu.VMEM((3, 8, 128), f32),
            pltpu.VMEM((8, 128), jnp.int32),
            pltpu.VMEM((8, D), bf16),
            pltpu.SemaphoreType.REGULAR,
            pltpu.SemaphoreType.DMA((NSEM,)),
        ],
        compiler_params=pltpu.CompilerParams(
            vmem_limit_bytes=110 * 1024 * 1024,
            disable_bounds_checks=True,
            disable_semaphore_checks=True),
    )(A_x, A_wqkv, A_w_phi, A_wo, B_w_r, B_w_gate, B_w_up, B_w_down)
```

```python
import jax
import jax.numpy as jnp
from jax import lax
import jax.experimental.pallas as pl
import jax.experimental.pallas.tpu as pltpu

S = 2048
D = 1024
H = 32
DH = 32
F = 3584
NP = H // 2
T1 = 256
T2 = 512
N1 = S // T1
N2 = S // T2
HT1 = T1 // 2
HT2 = T2 // 2
HD = D // 2
WC = 256
NWC = D // WC
LOG2E = 1.4426950408889634
EPS = 1e-5
WO_ROWS = 80
LN_ROWS = 16
EP_ROWS = 32
LT_START = (0, 0, 2, 5, 8, 11, 14)
LT_DEADLINE = (0, 4, 6, 9, 12, 15, 18)
FB_START = (2, 4, 6, 8, 10, 12, 14, 16)
SA_START = (9, 11, 13, 15, 17, 17, 18, 18)
FA_START = (20, 21, 22, 23, 24, 25, 26, 27)
FA_DEADLINE = (23, 24, 25, 26, 27, 29, 29, 29)
GATE_ROW = 0
T0_FOLD = 4
T0_WAITS = ((4, (1,)), (11, ('phi', 2)), (18, (3, 4)), (32, (5, 6, 7)), (46, (8, 9, 10)),
            (59, (11, 'x')))
T0_VPREP = ((46, 47, 48, 50), (51, 53, 54, 55), (59, 61, 62, 64), (65, 67, 68, 70))
T0_VSPAN = 5
T0_LN = (72, 74, 76, 78, 80, 82, 84, 88)
T0_LNSPAN = 0
P1_LN = (30, 31, 32, 33, 34, 35, 36, 37)
P1_LNSPAN = 3
P1_WO = (38, 39, 40, 41, 42)
P1_WOSPAN = 0

FFN_VPU_BLOCKS = 5
FFN_KG = 8
FFN_W0 = 10
FFN_W1 = 116
FFN_SPAN = 3
FFN_TOKALL = 0

_NT = (((1,), (1,)), ((), ()))
_TN = (((0,), (0,)), ((), ()))
f32 = jnp.float32
bf16 = jnp.bfloat16
u32 = jnp.uint32

K_, Q_, V_ = 0, 1, 2
SRC = {K_: 1, Q_: 0, V_: 2}

SEM_W = 0
SEM_X = SEM_W + 3 * NWC
SEM_X0 = SEM_X + N1
SEM_K0 = SEM_X0 + 4
SEM_PHI = SEM_K0 + 4
SEM_WO = SEM_PHI + 2
SEM_WR, SEM_WG, SEM_WU, SEM_WD = (SEM_WO + 4 + i for i in range(4))
SEM_O = SEM_WD + 1
NSEM = SEM_O + 2 * N2


def _rb(v):
    return v.astype(bf16).astype(f32)


def _pack(v):
    return pltpu.bitcast(v.astype(bf16), u32)


def _unpack(w):
    return pltpu.bitcast(w, bf16)


def _pack2(a, b):
    return pltpu.bitcast(pltpu.pack_elementwise([a, b], packed_dtype=bf16), u32)


def _packi(v):
    r, c = v.shape
    v4 = v.reshape(r // 16, 2, 8, c)
    return _pack2(v4[:, 0], v4[:, 1]).reshape(r // 2, c)


def _split2(w):
    return tuple(pltpu.unpack_elementwise(w, index=i, packed_dtype=bf16, unpacked_dtype=f32)
                 for i in range(2))


def _recip(x):
    r = pl.reciprocal(x, approx=True)
    return r * (2.0 - x * r)


def _rsqrt(x):
    return lax.rsqrt(x)


def _dual_softmax(p):
    t = p.shape[-1]
    p3 = p.reshape(8, 8, t)

    def allred(v, op):
        v = op(v, pltpu.roll(v, 2, 0))
        return op(v, pltpu.roll(v, 4, 0))

    mx = allred(jnp.max(p3, axis=0), jnp.maximum)
    mn = allred(jnp.min(p3, axis=0), jnp.minimum)
    ep = jnp.exp2(p3 - mx[None])
    en = jnp.exp2(mn[None] - p3)
    sp = allred(jnp.sum(ep, axis=0), jnp.add)
    sn = allred(jnp.sum(en, axis=0), jnp.add)
    fp = (ep * _recip(sp)[None]).reshape(64, t)
    fn = (en * _recip(sn)[None]).reshape(64, t)
    return _pack2(fp, fn)


def _left_combos(a11, a12, a21, a22):
    return [a11 + a22, a21 + a22, a11, a22, a11 + a12, a21 - a11, a12 - a22]


def _right_combos(b11, b12, b21, b22):
    return [b11 + b22, b11, b12 - b22, b21 - b11, b22, b11 + b12, b21 + b22]


def _strassen(prod, emit):
    m3 = prod(2)
    m5 = prod(4)
    emit(0, 1, m3 + m5)
    m7 = prod(6)
    u = m7 - m5
    m1 = prod(0)
    u = u + m1
    w = m1 + m3
    m4 = prod(3)
    emit(0, 0, u + m4)
    m2 = prod(1)
    emit(1, 0, m2 + m4)
    w = w - m2
    m6 = prod(5)
    emit(1, 1, w + m6)


def _fold_token(w, zero):
    r, c = w.shape
    acc = None
    for i in range(r // 8):
        for j in range(c // 128):
            blk = w[i * 8:(i + 1) * 8, j * 128:(j + 1) * 128]
            acc = blk if acc is None else acc | blk
    return acc & zero


def _kernel(x_hbm, wqkv_hbm, wphi_hbm, wo_hbm, wr_hbm, wg_hbm, wu_hbm, wd_hbm,
            out_hbm,
            x_v, wqkv_v, wphi_v, wo_v, wr_v, wg_v, wu_v, wd_v,
            wt_v, wo7_v, s_v, phiq_v, kv_acc, kvt_v, hal_v, har_v, hbl_v, hbr_v, sa_v,
            t0_v, t1_v, t2_v, t3_v, t4_v, t5_v, t6_v, h_v, out_v,
            wrf_v, best_v, besti_v, fix_v, xc0_v, xc1_v, xc2_v, xc3_v, zero_s, sem):
    xcol_v = (xc0_v, xc1_v, xc2_v, xc3_v)
    ha_v = (hal_v, har_v)
    hb_v = (hbl_v, hbr_v)
    tmp_v = (t0_v, t1_v, t2_v, t3_v, t4_v, t5_v, t6_v)

    def x_rows(r0, rows, slot):
        return pltpu.make_async_copy(
            x_hbm.at[0, pl.ds(r0, rows), :], x_v.at[pl.ds(r0, rows), :], sem.at[slot])

    def x_copy(i):
        return x_rows(i * T1, T1, SEM_X + i)

    def x0_copy(q):
        return x_rows((q % 2) * HT1 + (q // 2) * (HT1 // 2), HT1 // 2, SEM_X0 + q)

    def w_copy(kind, c):
        return pltpu.make_async_copy(
            wqkv_hbm.at[:, pl.ds(SRC[kind] * D + c * WC, WC)],
            wqkv_v.at[kind * NWC + c], sem.at[SEM_W + kind * NWC + c])

    def k0_copy(q):
        r0 = (q % 2) * HD + (q // 2) * 256
        return pltpu.make_async_copy(
            wqkv_hbm.at[pl.ds(r0, 256), pl.ds(SRC[K_] * D, WC)],
            wqkv_v.at[K_ * NWC, pl.ds(r0, 256), :], sem.at[SEM_K0 + q])

    def phi_copy(part):
        lo, n = part * (H // 2), H // 2
        return pltpu.make_async_copy(wphi_hbm.at[pl.ds(lo, n)], wphi_v.at[pl.ds(lo, n)],
                                     sem.at[SEM_PHI + part])

    def wo_copy(q):
        lo, n = (0, WO_ROWS) if q < 2 else (WO_ROWS, HD - WO_ROWS)
        lo += (q % 2) * HD
        return pltpu.make_async_copy(wo_hbm.at[pl.ds(lo, n), :], wo_v.at[pl.ds(lo, n), :],
                                     sem.at[SEM_WO + q])

    def full_copy(src, dst, slot):
        return pltpu.make_async_copy(src, dst, sem.at[slot])

    x0_copy(0).start()
    x0_copy(1).start()
    full_copy(wr_hbm, wr_v, SEM_WR).start()
    phi_copy(0).start()
    x0_copy(2).start()
    x0_copy(3).start()
    for q in range(4):
        k0_copy(q).start()
    w_copy(K_, 1).start()
    phi_copy(1).start()
    for c in range(2, NWC):
        w_copy(K_, c).start()
    for kind in (Q_, V_):
        for c in range(NWC):
            w_copy(kind, c).start()
    x_copy(1).start()
    wo_copy(0).start()
    wo_copy(1).start()
    x_copy(2).start()
    wo_copy(2).start()
    wo_copy(3).start()
    for i in range(3, N1):
        x_copy(i).start()
    full_copy(wg_hbm, wg_v, SEM_WG).start()
    full_copy(wu_hbm, wu_v, SEM_WU).start()
    full_copy(wd_hbm, wd_v, SEM_WD).start()

    zs = pl.semaphore_read(zero_s)

    zero_v = jnp.full((8, 128), zs, jnp.int32).astype(u32)

    def ld(ref, r0, rows, c0, cols):
        return ref[pl.ds(pl.multiple_of(zs * 8 + r0, 8), rows), c0:c0 + cols]

    def x_piece(r0, p):
        return [_split2(pltpu.bitcast(
            x_v[pl.ds(pl.multiple_of(r0 + hf * HT1 + p * LN_ROWS, LN_ROWS), LN_ROWS), :], u32))
            for hf in range(2)]

    def ln1_stats(xf):
        m = jnp.sum(xf, axis=-1, keepdims=True) * (1.0 / D)
        q = jnp.sum(xf * xf, axis=-1, keepdims=True) * (1.0 / D)
        inv = _rsqrt(jnp.maximum(q - m * m, 0.0) + EPS)
        return inv, m * inv

    def ln1_piece(r0, p, m=None):
        if m is not None:
            x_v[S:S + 8, 0:128] = m[0:8, 0:128].astype(bf16)
        xs = x_piece(r0, p)
        combos = []
        for par in range(2):
            (ia, ma), (ib, mb) = [ln1_stats(xs[hf][par]) for hf in range(2)]
            ya, yb = xs[0][par] * ia, xs[1][par] * ib
            s2 = ya[:, :HD] - ma
            s5 = yb[:, HD:] - mb
            s1 = s2 + s5
            s3 = yb[:, :HD] - yb[:, HD:]
            s4 = ya[:, HD:] - ya[:, :HD]
            combos.append([s1, s2, s3, s4, s5, s1 + s3, s1 + s4])
        hr = LN_ROWS // 2
        packed = [_pack2(combos[0][i], combos[1][i]) for i in range(7)]
        for i in range(7):
            s_v[i, p * hr:(p + 1) * hr, :] = packed[i]
        return lambda: _fold_token(jnp.concatenate(packed, axis=0), zero_v)

    def fold_piece(kind, c, j, pt):
        blk = {}
        for hh in range(2):
            for kh in range(2):
                k0 = kh * HD + j * 128
                w = wqkv_v[kind * NWC + c, k0:k0 + 128, hh * 128:(hh + 1) * 128]
                blk[hh, kh] = lax.dot_general(pt[2 * c + hh], w, _NT,
                                              preferred_element_type=f32) * LOG2E
        combos = _left_combos(blk[0, 0], blk[0, 1], blk[1, 0], blk[1, 1])
        r0 = (kind * HD + c * 128) // 2
        for i in range(7):
            wt_v[i, r0:r0 + 64, j * 128:(j + 1) * 128] = _packi(combos[i])

    def fold_chunk(kind, c, pt):
        for j in range(4):
            fold_piece(kind, c, j, pt)

    def vprep_piece(c, j, m):
        wqkv_v[3 * NWC, 0:8, 0:128] = m[0:8, 0:128].astype(bf16)
        blk = {}
        for hh in range(2):
            for kh in range(2):
                k0 = kh * HD + j * 128
                w = wqkv_v[zs + V_ * NWC + c, k0:k0 + 128, hh * 128:(hh + 1) * 128]
                blk[hh, kh] = _split2(pltpu.bitcast(w.T, u32))
        combos = [_left_combos(blk[0, 0][par], blk[0, 1][par], blk[1, 0][par], blk[1, 1][par])
                  for par in range(2)]
        r0 = (V_ * HD + c * 128) // 2
        packed = [_pack2(combos[0][i], combos[1][i]) for i in range(7)]
        for i in range(7):
            wt_v[i, r0:r0 + 64, j * 128:(j + 1) * 128] = packed[i]
        return lambda: _fold_token(jnp.concatenate(packed, axis=0), zero_v)

    def wo_piece(w0, m):
        wo_v[D:D + 8, 0:128] = m[0:8, 0:128].astype(bf16)
        top = wo_v[pl.ds(pl.multiple_of(w0, 16), 16), :].astype(f32)
        bot = wo_v[pl.ds(pl.multiple_of(HD + w0, 16), 16), :].astype(f32)
        combos = _right_combos(top[:, :HD], top[:, HD:], bot[:, :HD], bot[:, HD:])
        w0h = pl.multiple_of(w0 // 2, 8)
        packed = [_packi(combos[i]) for i in range(7)]
        for i in range(7):
            wo7_v[i, pl.ds(w0h, 8), :] = packed[i]
        return lambda: _fold_token(jnp.concatenate(packed, axis=0), zero_v)

    def run_tile(t, groups, post, first):
        phik = [[None, None] for _ in range(NP)]
        vt = [[None, None] for _ in range(NP)]
        count = [0]
        svals = {}
        pins = {}

        def pinned(w):
            toks = pins.get(count[0])
            if not toks:
                return w
            top = w[0:8, 0:128]
            for tk in toks:
                top = top | tk
            return jnp.concatenate(
                [jnp.concatenate([top, w[0:8, 128:]], axis=1), w[8:]], axis=0)

        def run_jobs(m):
            for fn, span in post.get(count[0], ()):
                tok = fn(m)
                if span:
                    pins.setdefault(count[0] + span, []).append(tok())
            count[0] += 1

        for kind, cs in groups:
            r0 = (kind * HD + cs[0] * 128) // 2
            rows = 64 * len(cs)

            def prod(i):
                if i not in svals:
                    svals[i] = ld(s_v.at[i], 0, HT1 // 2, 0, HD) if first else s_v[i]
                m = lax.dot_general(_unpack(wt_v[i, r0:r0 + rows, :]),
                                    _unpack(pinned(svals[i])), _NT,
                                    preferred_element_type=f32)
                run_jobs(m)
                return m

            def emit(rh, ch, blk):
                for n, c in enumerate(cs):
                    for jj in range(2):
                        pair = 4 * c + 2 * rh + jj
                        p = blk[n * 128 + jj * 64:n * 128 + (jj + 1) * 64]
                        if kind == K_:
                            phik[pair][ch] = _dual_softmax(p)
                        elif kind == Q_:
                            phiq_v[t, pair * 64:(pair + 1) * 64,
                                   ch * HT1:(ch + 1) * HT1] = _dual_softmax(p)
                        else:
                            vt[pair][ch] = _packi(p)

            _strassen(prod, emit)

        ones = _pack(jnp.ones((16, T1), f32))
        kr = lax.broadcasted_iota(jnp.int32, (80, 128), 0)
        kc = lax.broadcasted_iota(jnp.int32, (80, 128), 1)
        kmask = jnp.where(kr < 64, kr // 32, (kr - 64) // 8) == (kc // 2) % 2
        for j in range(NP):
            lhs = jnp.concatenate([jnp.concatenate(vt[j], axis=1), ones], axis=0)
            rhs = jnp.concatenate(phik[j], axis=1)
            upd = lax.dot_general(_unpack(lhs), _unpack(pinned(rhs)), _NT,
                                  preferred_element_type=f32)
            run_jobs(upd)
            if first:
                kv_acc[j] = upd
            else:
                upd = kv_acc[j] + upd
                kv_acc[j] = upd
                kvt_v[j] = _pack(jnp.where(kmask, upd, 0.0))

    def load_best():
        return best_v[0], besti_v[...], best_v[1], best_v[2]

    def store_best(best):
        best_v[0], besti_v[...], best_v[1], best_v[2] = best

    def build_pt(g0, g1):
        n = g1 - g0
        w2 = wphi_v[4 * g0:4 * g1].reshape(n * 128, DH)
        er = lax.broadcasted_iota(jnp.int32, (128, DH), 0)
        ec = lax.broadcasted_iota(jnp.int32, (128, DH), 1)
        e = jnp.where(ec == ((er // 16) * 8 + er % 8) % 32, 1.0, 0.0).astype(bf16)
        ptf = lax.dot_general(e, w2, _NT, preferred_element_type=f32)
        pr = lax.broadcasted_iota(jnp.int32, (128, 128), 0)
        pc = lax.broadcasted_iota(jnp.int32, (128, 128), 1)
        keep = pc // 32 == (pr // 64) * 2 + (pr // 8) % 2
        return [jnp.where(keep, ptf[:, g * 128:(g + 1) * 128], 0.0).astype(bf16)
                for g in range(n)]

    hbl_v[...] = jnp.zeros_like(hbl_v)
    hbr_v[...] = jnp.zeros_like(hbr_v)
    store_best((jnp.full((8, 128), -jnp.inf, f32), jnp.zeros((8, 128), jnp.int32),
                jnp.zeros((8, 128), f32), jnp.zeros((8, 128), f32)))
    n_ln = HT1 // LN_ROWS
    x0_copy(0).wait()
    x0_copy(1).wait()
    for p in range(n_ln // 2):
        ln1_piece(0, p)
    full_copy(wr_hbm, wr_v, SEM_WR).wait()
    phi_copy(0).wait()
    x0_copy(2).wait()
    x0_copy(3).wait()
    wr_row = wr_v[...].astype(f32).reshape(1, D)
    wrf_v[:, 0:D] = jnp.broadcast_to(wr_row, (8, D))
    wrf_v[:, D:D + 128] = jnp.broadcast_to(jnp.sum(wr_row, axis=-1, keepdims=True), (8, 128))
    pt = build_pt(0, 4)
    for p in range(n_ln // 2, n_ln):
        ln1_piece(0, p)
    for part in range(2):
        k0_copy(2 * part).wait()
        k0_copy(2 * part + 1).wait()
        fold_piece(K_, 0, 2 * part, pt)
        fold_piece(K_, 0, 2 * part + 1, pt)

    post = {}

    def at(slot, fn, span=0):
        post.setdefault(slot, []).append((fn, span))

    for slot, copies in T0_WAITS:
        for cp in copies:
            if cp == 'phi':
                at(slot, lambda m: phi_copy(1).wait())
            elif cp == 'x':
                at(slot, lambda m: x_copy(1).wait())
            else:
                at(slot, lambda m, cp=cp: w_copy(cp // NWC, cp % NWC).wait())
    for n in range(1, 2 * NWC):
        if n == 2:
            at(7 * n - 7 + T0_FOLD, lambda m: pt.extend(build_pt(4, 8)))
        at(7 * n - 7 + T0_FOLD, lambda m, n=n: fold_chunk(n // NWC, n % NWC, pt))
    for c in range(NWC):
        for j in range(4):
            at(T0_VPREP[c][j], lambda m, c=c, j=j: vprep_piece(c, j, m), T0_VSPAN)
    for p in range(n_ln):
        at(T0_LN[p], lambda m, p=p: ln1_piece(zs + T1, p, m), T0_LNSPAN)
    run_tile(0, [(kind, [c]) for kind in (K_, Q_, V_) for c in range(NWC)], post, True)
    wo_copy(0).wait()
    wo_copy(1).wait()

    def phase1(t, carry):
        @pl.when(t + 1 < N1)
        def _():
            x_copy(t + 1).wait()

        @pl.when(t == 2)
        def _():
            wo_copy(2).wait()
            wo_copy(3).wait()

        nxt = jnp.minimum(t + 1, N1 - 1) * T1
        w0 = jnp.minimum((t - 1) * WO_ROWS, HD - WO_ROWS)
        post = {}
        for p in range(n_ln):
            post.setdefault(P1_LN[p], []).append(
                (lambda m, p=p: ln1_piece(nxt, p, m), P1_LNSPAN))
        for p in range(WO_ROWS // 16):
            post.setdefault(P1_WO[p], []).append(
                (lambda m, p=p: wo_piece(w0 + 16 * p, m), P1_WOSPAN))
        run_tile(t, [(kind, cs) for kind in (K_, Q_, V_) for cs in ([0, 1], [2, 3])],
                 post, False)
        return carry

    lax.fori_loop(1, N1, phase1, 0)

    full_copy(wg_hbm, wg_v, SEM_WG).wait()
    full_copy(wu_hbm, wu_v, SEM_WU).wait()
    full_copy(wd_hbm, wd_v, SEM_WD).wait()

    def o_copy(hf):
        return pltpu.make_async_copy(
            out_v.at[pl.ds(hf * HT2, HT2), :], out_hbm.at[0, pl.ds(hf * HT2, HT2), :],
            sem.at[SEM_O + hf])

    def half_stats(hh, c0):
        rows = hh.shape[0]
        parts = [hh[:, c * 128:(c + 1) * 128] for c in range(4)]
        wts = [wrf_v[:, c0 + c * 128:c0 + (c + 1) * 128] for c in range(4)]
        s1 = (parts[0] + parts[1]) + (parts[2] + parts[3])
        sq = [p * p for p in parts]
        s2 = (sq[0] + sq[1]) + (sq[2] + sq[3])
        dw = [(p.reshape(rows // 8, 8, 128) * w[None]).reshape(rows, 128)
              for p, w in zip(parts, wts)]
        s3 = (dw[0] + dw[1]) + (dw[2] + dw[3])
        return s1, s2, s3

    def first_half(hbuf, sbuf, base, p, c0):
        r0 = p * EP_ROWS
        hh = ld(hbuf[c0 // HD], r0, EP_ROWS, 0, HD)
        h_v[pl.ds(pl.multiple_of(base + r0, EP_ROWS), EP_ROWS), c0:c0 + HD] = hh.astype(bf16)
        st = jnp.concatenate(half_stats(hh, c0), axis=1)
        sbuf[r0:r0 + EP_ROWS, :] = st
        return _fold_token(pltpu.bitcast(st, u32), zero_v)

    def finish(hbuf, sbuf, base, p, valid, best, defer=None):
        r0 = p * EP_ROWS
        g0 = pl.multiple_of(base + r0, EP_ROWS)
        hl, hr = [ld(r, r0, EP_ROWS, 0, HD) for r in hbuf]
        h_v[pl.ds(g0, EP_ROWS), 0:HD] = hl.astype(bf16)
        if sbuf is None:
            h_v[pl.ds(g0, EP_ROWS), HD:D] = hr.astype(bf16)
            st = half_stats(hr, HD)
        else:
            st = ld(sbuf, r0, EP_ROWS, 0, 384)
            st = [st[:, n * 128:(n + 1) * 128] for n in range(3)]
        s1, s2, s3 = [jnp.sum(v + w, axis=-1, keepdims=True)
                      for v, w in zip(half_stats(hl, 0), st)]
        m = s1 * (1.0 / D)
        var = jnp.maximum(s2 * (1.0 / D) - m * m, 0.0)
        inv = _rsqrt(var + EPS)
        r = (s3 - m * wrf_v[0:1, D:D + 1]) * inv

        def write_out(h):
            o = h * (1.0 + inv) - m * inv
            out_v[pl.ds(g0, EP_ROWS), :] = o.astype(bf16)
            return o

        if defer is None:
            o = write_out(jnp.concatenate([hl, hr], axis=1))
        else:
            defer.append(lambda: write_out(jnp.concatenate(
                [r_[r0:r0 + EP_ROWS, :] for r_ in hbuf], axis=1)))
        bv, bi, bm, bq = best
        sub = lax.broadcasted_iota(jnp.int32, (8, 128), 0)
        for g in range(EP_ROWS // 8):
            rows = slice(g * 8, (g + 1) * 8)
            rg = jnp.broadcast_to(r[rows], (8, 128))
            if valid is not None:
                rg = jnp.where(valid, rg, -jnp.inf)
            better = rg > bv
            bi = jnp.where(better, sub + (g0 + g * 8), bi)
            bv = jnp.where(better, rg, bv)
            bm = jnp.where(better, jnp.broadcast_to(m[rows], (8, 128)), bm)
            bq = jnp.where(better, jnp.broadcast_to(var[rows], (8, 128)), bq)
        best = (bv, bi, bm, bq)
        if defer is not None:
            return best, None
        tok = _fold_token(pltpu.bitcast(jnp.concatenate(
            [o[:, D - 128:], bv, bm, bq], axis=0), u32), zero_v)
        return best, tok

    n_ep = HT2 // EP_ROWS

    def phase2(i, carry):
        ot = []
        for j in range(NP):
            ph = jnp.concatenate([phiq_v[2 * i, j * 64:(j + 1) * 64, :],
                                  phiq_v[2 * i + 1, j * 64:(j + 1) * 64, :]], axis=1)
            n = jnp.dot(_unpack(kvt_v[j]), _unpack(ph), preferred_element_type=f32)
            r0h = _recip(n[64:72] + 1e-6)
            r1h = _recip(n[72:80] + 1e-6)
            ot.append((n[0:32].reshape(4, 8, T2) * r0h[None]).reshape(32, T2))
            ot.append((n[32:64].reshape(4, 8, T2) * r1h[None]).reshape(32, T2))
        lo = jnp.concatenate(ot[:H // 2], axis=0)
        hi = jnp.concatenate(ot[H // 2:], axis=0)
        lcs = _left_combos(lo[:, :HT2], hi[:, :HT2], lo[:, HT2:], hi[:, HT2:])

        state = {'best': load_best()}
        pins = {}
        jobs = {}
        lts = {}
        ra = pl.multiple_of(i * T2, T2)
        rb = pl.multiple_of(i * T2 + HT2, HT2)
        prev = jnp.maximum(i * T2 - HT2, HT2)

        def add_job(slot, deadline, fn, gates=()):
            jobs.setdefault(slot, []).append((fn, deadline, gates))

        def finish_job(hbuf, sbuf, base, p, valid):
            def fn():
                state['best'], tok = finish(hbuf, sbuf, base, p, valid, state['best'])
                return tok
            return fn

        def lt_job(k):
            def fn():
                lts[k] = lcs[k].astype(bf16).T
                return _fold_token(pltpu.bitcast(lts[k], u32), zero_v)
            return fn

        order = (2, 4, 6, 0, 3, 1, 5)
        lt_job(2)()
        for n in range(1, 7):
            add_job(LT_START[n], LT_DEADLINE[n], lt_job(order[n]))
        for p in range(n_ep):
            add_job(FB_START[p], FB_START[p] + 2, finish_job(hb_v, None, prev, p, i > 0), hb_v)
            add_job(SA_START[p], SA_START[p] + 2, lambda p=p: first_half(ha_v, sa_v, ra, p, HD), ha_v[1:])
            add_job(FA_START[p], FA_DEADLINE[p], finish_job(ha_v, sa_v, ra, p, None), ha_v)

        def xblk(r0, c0):
            return x_v[pl.ds(r0, HT2), c0:c0 + 128].astype(f32)

        for n, k in enumerate(order):
            for c in range(4):
                slot = 4 * n + c
                for fn, deadline, gates in jobs.get(slot, ()):
                    for ref in gates:
                        ref[HT2:HT2 + 8, 0:128] = mm[GATE_ROW:GATE_ROW + 8]
                    pins.setdefault(deadline, []).append(fn())
                w = wo7_v[k, :, c * 128:(c + 1) * 128]
                toks = pins.get(slot)
                if toks:
                    top = w[0:8]
                    for tk in toks:
                        top = top | tk
                    w = jnp.concatenate([top, w[8:]], axis=0)
                mm = jnp.dot(lts[k], _unpack(w), preferred_element_type=f32)
                c0 = c * 128
                cs = slice(c0, c0 + 128)
                tmp = lambda t: ld(tmp_v[t], 0, HT2, c0, 128)
                if n == 0:
                    tmp_v[0][:, cs] = mm
                elif n == 1:
                    ha_v[1][0:HT2, cs] = (xblk(ra, HD + c0) + tmp(0)) + mm
                    tmp_v[1][:, cs] = xblk(ra, c0) - mm
                elif n == 2:
                    tmp_v[2][:, cs] = tmp(1) + mm
                elif n == 3:
                    tmp_v[3][:, cs] = tmp(2) + mm
                    tmp_v[4][:, cs] = (xblk(rb, HD + c0) + tmp(0)) + mm
                elif n == 4:
                    ha_v[0][0:HT2, cs] = tmp(3) + mm
                    tmp_v[5][:, cs] = xblk(rb, c0) + mm
                elif n == 5:
                    hb_v[0][0:HT2, cs] = tmp(5) + mm
                    tmp_v[6][:, cs] = tmp(4) - mm
                else:
                    hb_v[1][0:HT2, cs] = tmp(6) + mm
        store_best(state['best'])
        o_copy(2 * i).start()

        @pl.when(i > 0)
        def _():
            o_copy(2 * i - 1).start()

        return carry

    lax.fori_loop(0, N2, phase2, 0)
    best = load_best()
    late = []
    for p in range(n_ep):
        best, _ = finish(hb_v, None, S - HT2, p, None, best, late)

    bv, bi, bm, bq = best
    for sh in (4, 2, 1):
        ov, oi, om, oq = [pltpu.roll(t, sh, 0) for t in (bv, bi, bm, bq)]
        take = jnp.logical_or(ov > bv, jnp.logical_and(ov == bv, oi < bi))
        bv, bi, bm, bq = [jnp.where(take, o_, t)
                          for o_, t in zip((ov, oi, om, oq), (bv, bi, bm, bq))]
    idx = jnp.clip(bi[0, 0], 0, S - 1)
    b0 = pl.multiple_of((idx // 8) * 8, 8)
    t = _rb(_rb(bq) + EPS)
    inv = _recip(_rb(t * _rsqrt(t)))
    gate = _recip(1.0 + jnp.exp(-bv))
    wide = lambda v: jnp.concatenate([v] * (D // 128), axis=1)
    hb = h_v[pl.ds(b0, 8), :].astype(f32)
    hn = (hb - wide(bm)) * wide(inv)
    xs = hn.astype(bf16)
    rows = lax.broadcasted_iota(jnp.int32, (8, D), 0) + b0

    xm = jnp.where(rows == wide(bi), _rb(hn), 0.0)
    for sh in (4, 2, 1):
        xm = xm + pltpu.roll(xm, sh, 0)
    for t in range(D // 128):
        xcol_v[t // 2][(t % 2) * 128:(t % 2 + 1) * 128, :] = jnp.concatenate(
            [xm[:, t * 128:(t + 1) * 128]] * 16, axis=0).T

    nblk = F // 256
    nmx = nblk - FFN_VPU_BLOCKS
    act = {}
    acc = {}

    def activate(g, u):
        return (g * _recip(1.0 + jnp.exp(-g)) * u).astype(bf16)

    parts = D // 8 // FFN_KG

    def vpu_chunk(q):
        blk, part = nmx + q // parts, q % parts
        cur = acc.get(blk)
        for kg in range(part * FFN_KG, (part + 1) * FFN_KG):
            xc = ld(xcol_v[kg // 32], (kg % 32) * 8, 8, 0, 128)
            w = jnp.concatenate(
                [r[kg * 8:(kg + 1) * 8, blk * 256:(blk + 1) * 256].astype(f32)
                 for r in (wg_v, wu_v)], axis=1)
            p = w * jnp.concatenate([xc] * 4, axis=1)
            cur = p if cur is None else cur + p
        acc[blk] = cur
        if part == parts - 1:
            for sh in (4, 2, 1):
                cur = cur + pltpu.roll(cur, sh, 0)
            act[blk] = activate(cur[:, :256], cur[:, 256:])
        if FFN_TOKALL:
            return _fold_token(pltpu.bitcast(cur, u32), zero_v)
        c = q % 4
        return _fold_token(pltpu.bitcast(cur[:, c * 128:(c + 1) * 128], u32), zero_v)

    steps = []
    for j in range(nmx):
        steps += [('g', j), ('u', j)]
    steps += [('d', j) for j in range(nblk)]
    nchunk = FFN_VPU_BLOCKS * parts
    starts = [FFN_W0 + (q * (FFN_W1 - FFN_W0)) // (nchunk - 1) for q in range(nchunk)]
    pins = {}
    gate_pre = {}
    ys = [None] * 4
    for n, (kind, j) in enumerate(steps):
        outs = []
        for wv in range(4):
            wave = 4 * n + wv
            if kind == 'd':
                lhs = act[j]
                w = wd_v[j * 256:(j + 1) * 256, wv * 256:(wv + 1) * 256]
            else:
                kh, c0 = wv % 2, j * 256 + (wv // 2) * 128
                lhs = xs[:, kh * HD:(kh + 1) * HD]
                w = (wg_v if kind == 'g' else wu_v)[kh * HD:(kh + 1) * HD, c0:c0 + 128]
            if pins.get(wave):
                wb = pltpu.bitcast(w, u32)
                top = wb[0:8, 0:128]
                for tk in pins[wave]:
                    top = top | tk
                if wb.shape[1] > 128:
                    top = jnp.concatenate([top, wb[0:8, 128:]], axis=1)
                w = _unpack(jnp.concatenate([top, wb[8:]], axis=0))
            outs.append(jnp.dot(lhs, w, preferred_element_type=f32))
            for q, start in enumerate(starts):
                if start == wave:
                    pins.setdefault(wave + FFN_SPAN, []).append(vpu_chunk(q))
        if kind == 'd':
            ys = [o_ if y_ is None else y_ + o_ for y_, o_ in zip(ys, outs)]
        else:
            p = jnp.concatenate([outs[0] + outs[1], outs[2] + outs[3]], axis=1)
            if kind == 'g':
                gate_pre[j] = p
            else:
                act[j] = activate(gate_pre[j], p)
        if n == 0:
            for fn in late:
                fn()
            o_copy(2 * N2 - 1).start()
    y = jnp.concatenate(ys, axis=1)
    cur = out_v[pl.ds(b0, 8), :].astype(f32)
    fix_v[...] = jnp.where(rows == wide(bi), hb + hn + y * wide(gate), cur).astype(bf16)
    for hf in range(2 * N2):
        o_copy(hf).wait()
    fix = pltpu.make_async_copy(fix_v, out_hbm.at[0, pl.ds(b0, 8), :], sem.at[SEM_O])
    fix.start()
    fix.wait()


@jax.jit
def pallas_sequential_preLN__linear_kernel_hedgehog__moe_arch_mod__prompt_kernel(
    A_x: jax.Array,
    A_wqkv: jax.Array,
    A_w_phi: jax.Array,
    A_wo: jax.Array,
    B_x: jax.Array,
    B_w_r: jax.Array,
    B_w_gate: jax.Array,
    B_w_up: jax.Array,
    B_w_down: jax.Array,
):
    any_spec = pl.BlockSpec(memory_space=pl.ANY)
    return pl.pallas_call(
        _kernel,
        out_shape=jax.ShapeDtypeStruct((1, S, D), bf16),
        in_specs=[any_spec] * 8,
        out_specs=any_spec,
        scratch_shapes=[
            pltpu.VMEM((S + 16, D), bf16),
            pltpu.VMEM((3 * NWC + 1, D, WC), bf16),
            pltpu.VMEM((H, DH, DH), bf16),
            pltpu.VMEM((D + 16, D), bf16),
            pltpu.VMEM((D,), bf16),
            pltpu.VMEM((D, F), bf16),
            pltpu.VMEM((D, F), bf16),
            pltpu.VMEM((F, D), bf16),
            pltpu.VMEM((7, 3 * HD // 2, HD), u32),
            pltpu.VMEM((7, HD // 2, HD), u32),
            pltpu.VMEM((7, HT1 // 2, HD), u32),
            pltpu.VMEM((N1, D, T1), u32),
            pltpu.VMEM((NP, 80, 128), f32),
            pltpu.VMEM((NP, 40, 128), u32),
            *[pltpu.VMEM((HT2 + 8, HD), f32) for _ in range(4)],
            pltpu.VMEM((HT2, 384), f32),
            *[pltpu.VMEM((HT2, HD), f32) for _ in range(7)],
            pltpu.VMEM((S, D), bf16),
            pltpu.VMEM((S, D), bf16),
            pltpu.VMEM((8, D + 128), f32),
            pltpu.VMEM((3, 8, 128), f32),
            pltpu.VMEM((8, 128), jnp.int32),
            pltpu.VMEM((8, D), bf16),
            *[pltpu.VMEM((264, 128), f32) for _ in range(4)],
            pltpu.SemaphoreType.REGULAR,
            pltpu.SemaphoreType.DMA((NSEM,)),
        ],
        compiler_params=pltpu.CompilerParams(
            vmem_limit_bytes=110 * 1024 * 1024,
            disable_bounds_checks=True,
            disable_semaphore_checks=True),
    )(A_x, A_wqkv, A_w_phi, A_wo, B_w_r, B_w_gate, B_w_up, B_w_down)
```

```python
import jax
import jax.numpy as jnp
from jax import lax
import jax.experimental.pallas as pl
import jax.experimental.pallas.tpu as pltpu

S = 2048
D = 1024
H = 32
DH = 32
F = 3584
NP = H // 2
T1 = 256
T2 = 512
N1 = S // T1
N2 = S // T2
HT1 = T1 // 2
HT2 = T2 // 2
HD = D // 2
WC = 256
NWC = D // WC
LOG2E = 1.4426950408889634
EPS = 1e-5
WO_ROWS = 176
LN_ROWS = 16
EP_ROWS = 32
LT_START = (0, 0, 2, 5, 8, 11, 14)
LT_DEADLINE = (0, 4, 6, 9, 12, 15, 18)
FB_START = (2, 4, 6, 8, 10, 12, 14, 16)
SA_START = (9, 11, 13, 15, 17, 17, 18, 18)
FA_START = (20, 21, 22, 23, 24, 25, 26, 27)
FA_DEADLINE = (23, 24, 25, 26, 27, 29, 29, 29)
GATE_ROW = 0
T0_FOLD = (0, 4, 11, 18, 25, 32, 39, 46)
T0_WAITS = ((4, (1,)), (11, ('phi', 2)), (18, (3, 4)), (32, ('x1', 5, 6)), (46, (7,)),
            (73, (8, 9, 10, 11, 'x2', 'x3')))
T0_VPREP = ((73, 74, 75, 76), (77, 78, 79, 80), (81, 82, 83, 84), (85, 86, 87, 88))
T0_VSPAN = 3
T0_LN = (32, 34, 35, 37, 38, 40, 41, 43)
T0_LNSPAN = (0,) * 8
P1_LN = (29, 30, 31, 32, 33, 34, 35, 36)
P1_LNSPAN = 3
P1_WO = (57, 58, 59, 60, 61, 78, 79, 80, 81, 82, 83)
P1_LN2 = ((70, 71, 72, 73, 74, 75, 76, 77), (62, 63, 64, 65, 66, 67, 68, 69))
P1_LNSPAN2 = (3, 3)
T1_LN = ((99, 100, 101, 102, 103, 104, 105, 106), (90, 91, 92, 93, 94, 95, 96, 97))
P1_WOSPAN = 3

FFN_VPU_BLOCKS = 5
FFN_KG = 8
FFN_W0 = 10
FFN_W1 = 116
FFN_SPAN = 3
FFN_TOKALL = 0
FFN_LATE = 2
LATE_MARK = 3

_NT = (((1,), (1,)), ((), ()))
_TN = (((0,), (0,)), ((), ()))
f32 = jnp.float32
bf16 = jnp.bfloat16
u32 = jnp.uint32

K_, Q_, V_ = 0, 1, 2
SRC = {K_: 1, Q_: 0, V_: 2}

SEM_W = 0
SEM_X = SEM_W + 3 * NWC
SEM_X0 = SEM_X + N1
SEM_K0 = SEM_X0 + 4
SEM_PHI = SEM_K0 + 4
SEM_WO = SEM_PHI + 2
SEM_WR, SEM_WG, SEM_WU, SEM_WD = (SEM_WO + 4 + i for i in range(4))
SEM_O = SEM_WD + 1
NSEM = SEM_O + 2 * N2


def _rb(v):
    return v.astype(bf16).astype(f32)


def _pack(v):
    return pltpu.bitcast(v.astype(bf16), u32)


def _unpack(w):
    return pltpu.bitcast(w, bf16)


def _pack2(a, b):
    return pltpu.bitcast(pltpu.pack_elementwise([a, b], packed_dtype=bf16), u32)


def _packi(v):
    r, c = v.shape
    v4 = v.reshape(r // 16, 2, 8, c)
    return _pack2(v4[:, 0], v4[:, 1]).reshape(r // 2, c)


def _split2(w):
    return tuple(pltpu.unpack_elementwise(w, index=i, packed_dtype=bf16, unpacked_dtype=f32)
                 for i in range(2))


def _recip(x):
    r = pl.reciprocal(x, approx=True)
    return r * (2.0 - x * r)


def _sigmoid(x):
    return _recip(1.0 + jnp.exp(jnp.minimum(-x, 80.0)))


def _rsqrt(x):
    return lax.rsqrt(x)


def _dual_softmax(p):
    t = p.shape[-1]
    p3 = p.reshape(8, 8, t)

    def allred(v, op):
        v = op(v, pltpu.roll(v, 2, 0))
        return op(v, pltpu.roll(v, 4, 0))

    mx = allred(jnp.max(p3, axis=0), jnp.maximum)
    mn = allred(jnp.min(p3, axis=0), jnp.minimum)
    ep = jnp.exp2(p3 - mx[None])
    en = jnp.exp2(mn[None] - p3)
    sp = allred(jnp.sum(ep, axis=0), jnp.add)
    sn = allred(jnp.sum(en, axis=0), jnp.add)
    fp = (ep * _recip(sp)[None]).reshape(64, t)
    fn = (en * _recip(sn)[None]).reshape(64, t)
    return _pack2(fp, fn)


def _left_combos(a11, a12, a21, a22):
    return [a11 + a22, a21 + a22, a11, a22, a11 + a12, a21 - a11, a12 - a22]


def _right_combos(b11, b12, b21, b22):
    return [b11 + b22, b11, b12 - b22, b21 - b11, b22, b11 + b12, b21 + b22]


def _strassen(prod, emit):
    m3 = prod(2)
    m5 = prod(4)
    emit(0, 1, m3 + m5)
    m7 = prod(6)
    u = m7 - m5
    m1 = prod(0)
    u = u + m1
    w = m1 + m3
    m4 = prod(3)
    emit(0, 0, u + m4)
    m2 = prod(1)
    emit(1, 0, m2 + m4)
    w = w - m2
    m6 = prod(5)
    emit(1, 1, w + m6)


def _fold_token(w, zero):
    r, c = w.shape
    acc = None
    for i in range(r // 8):
        for j in range(c // 128):
            blk = w[i * 8:(i + 1) * 8, j * 128:(j + 1) * 128]
            acc = blk if acc is None else acc | blk
    return acc & zero


def _body(x_hbm, wqkv_hbm, wphi_hbm, wo_hbm, wr_hbm, wg_hbm, wu_hbm, wd_hbm,
            out_hbm,
            x_v, wqkv_v, wphi_v, wo_v, wr_v, wg_v, wu_v, wd_v,
            wt_v, wo7_v, sa7_v, sb7_v, sc7_v, phiq_v, phik_v, vt0_v, vt1_v, kv_acc, kvt_v, hal_v, har_v, hbl_v, hbr_v, sa_v,
            t0_v, t1_v, t2_v, t3_v, t4_v, t5_v, t6_v, h_v, out_v,
            wrf_v, best_v, besti_v, fix_v, xc0_v, xc1_v, xc2_v, xc3_v, zero_s, sem):
    xcol_v = (xc0_v, xc1_v, xc2_v, xc3_v)
    s_v = (sa7_v, sb7_v)
    vt_v = (vt0_v, vt1_v)
    ha_v = (hal_v, har_v)
    hb_v = (hbl_v, hbr_v)
    tmp_v = (t0_v, t1_v, t2_v, t3_v, t4_v, t5_v, t6_v)

    def x_rows(r0, rows, slot):
        return pltpu.make_async_copy(
            x_hbm.at[0, pl.ds(r0, rows), :], x_v.at[pl.ds(r0, rows), :], sem.at[slot])

    def x_copy(i):
        return x_rows(i * T1, T1, SEM_X + i)

    def x0_copy(q):
        return x_rows((q % 2) * HT1 + (q // 2) * (HT1 // 2), HT1 // 2, SEM_X0 + q)

    def w_copy(kind, c):
        return pltpu.make_async_copy(
            wqkv_hbm.at[:, pl.ds(SRC[kind] * D + c * WC, WC)],
            wqkv_v.at[kind * NWC + c], sem.at[SEM_W + kind * NWC + c])

    def k0_copy(q):
        r0 = (q % 2) * HD + (q // 2) * 256
        return pltpu.make_async_copy(
            wqkv_hbm.at[pl.ds(r0, 256), pl.ds(SRC[K_] * D, WC)],
            wqkv_v.at[K_ * NWC, pl.ds(r0, 256), :], sem.at[SEM_K0 + q])

    def phi_copy(part):
        lo, n = part * (H // 2), H // 2
        return pltpu.make_async_copy(wphi_hbm.at[pl.ds(lo, n)], wphi_v.at[pl.ds(lo, n)],
                                     sem.at[SEM_PHI + part])

    def full_copy(src, dst, slot):
        return pltpu.make_async_copy(src, dst, sem.at[slot])

    x0_copy(0).start()
    x0_copy(1).start()
    full_copy(wr_hbm, wr_v, SEM_WR).start()
    phi_copy(0).start()
    x0_copy(2).start()
    x0_copy(3).start()
    for q in range(4):
        k0_copy(q).start()
    w_copy(K_, 1).start()
    phi_copy(1).start()
    w_copy(K_, 2).start()
    w_copy(K_, 3).start()
    w_copy(Q_, 0).start()
    x_copy(1).start()
    for c in range(1, NWC):
        w_copy(Q_, c).start()
    for c in range(NWC):
        w_copy(V_, c).start()
    x_copy(2).start()
    x_copy(3).start()
    full_copy(wo_hbm, wo_v.at[pl.ds(0, D), :], SEM_WO).start()
    for i in range(4, N1):
        x_copy(i).start()
    full_copy(wg_hbm, wg_v, SEM_WG).start()
    full_copy(wu_hbm, wu_v, SEM_WU).start()
    full_copy(wd_hbm, wd_v, SEM_WD).start()

    zs = pl.semaphore_read(zero_s)

    zero_v = jnp.full((8, 128), zs, jnp.int32).astype(u32)

    def ld(ref, r0, rows, c0, cols):
        return ref[pl.ds(pl.multiple_of(zs * 8 + r0, 8), rows), c0:c0 + cols]

    def x_piece(r0, p):
        return [_split2(pltpu.bitcast(
            x_v[pl.ds(pl.multiple_of(r0 + hf * HT1 + p * LN_ROWS, LN_ROWS), LN_ROWS), :], u32))
            for hf in range(2)]

    def ln1_stats(xf):
        m = jnp.sum(xf, axis=-1, keepdims=True) * (1.0 / D)
        q = jnp.sum(xf * xf, axis=-1, keepdims=True) * (1.0 / D)
        inv = _rsqrt(jnp.maximum(q - m * m, 0.0) + EPS)
        return inv, m * inv

    def ln1_piece(r0, dst, p, m=None):
        if m is not None:
            x_v[S:S + 8, 0:128] = m[0:8, 0:128].astype(bf16)
        xs = x_piece(r0, p)
        combos = []
        for par in range(2):
            (ia, ma), (ib, mb) = [ln1_stats(xs[hf][par]) for hf in range(2)]
            ya, yb = xs[0][par] * ia, xs[1][par] * ib
            s2 = ya[:, :HD] - ma
            s5 = yb[:, HD:] - mb
            s1 = s2 + s5
            s3 = yb[:, :HD] - yb[:, HD:]
            s4 = ya[:, HD:] - ya[:, :HD]
            combos.append([s1, s2, s3, s4, s5, s1 + s3, s1 + s4])
        hr = LN_ROWS // 2
        packed = [_pack2(combos[0][i], combos[1][i]) for i in range(7)]
        for i in range(7):
            dst[i, p * hr:(p + 1) * hr, :] = packed[i]
        return lambda: _fold_token(jnp.concatenate(packed, axis=0), zero_v)

    def fold_piece(kind, c, j, pt):
        blk = {}
        for hh in range(2):
            for kh in range(2):
                k0 = kh * HD + j * 128
                w = wqkv_v[kind * NWC + c, k0:k0 + 128, hh * 128:(hh + 1) * 128]
                blk[hh, kh] = lax.dot_general(pt[2 * c + hh], w, _NT,
                                              preferred_element_type=f32) * LOG2E
        combos = _left_combos(blk[0, 0], blk[0, 1], blk[1, 0], blk[1, 1])
        r0 = (kind * HD + c * 128) // 2
        for i in range(7):
            wt_v[i, r0:r0 + 64, j * 128:(j + 1) * 128] = _packi(combos[i])

    def fold_chunk(kind, c, pt):
        for j in range(4):
            fold_piece(kind, c, j, pt)

    def vprep_piece(c, j, m):
        wqkv_v[3 * NWC, 0:8, 0:128] = m[0:8, 0:128].astype(bf16)
        blk = {}
        for hh in range(2):
            for kh in range(2):
                k0 = kh * HD + j * 128
                w = wqkv_v[zs + V_ * NWC + c, k0:k0 + 128, hh * 128:(hh + 1) * 128]
                blk[hh, kh] = _split2(pltpu.bitcast(w.T, u32))
        combos = [_left_combos(blk[0, 0][par], blk[0, 1][par], blk[1, 0][par], blk[1, 1][par])
                  for par in range(2)]
        r0 = (V_ * HD + c * 128) // 2
        packed = [_pack2(combos[0][i], combos[1][i]) for i in range(7)]
        for i in range(7):
            wt_v[i, r0:r0 + 64, j * 128:(j + 1) * 128] = packed[i]
        return lambda: _fold_token(jnp.concatenate(packed, axis=0), zero_v)

    def wo_piece(w0, m):
        wo_v[D:D + 8, 0:128] = m[0:8, 0:128].astype(bf16)
        top = wo_v[pl.ds(pl.multiple_of(w0, 16), 16), :].astype(f32)
        bot = wo_v[pl.ds(pl.multiple_of(HD + w0, 16), 16), :].astype(f32)
        combos = _right_combos(top[:, :HD], top[:, HD:], bot[:, :HD], bot[:, HD:])
        w0h = pl.multiple_of(w0 // 2, 8)
        packed = [_packi(combos[i]) for i in range(7)]
        for i in range(7):
            wo7_v[i, pl.ds(w0h, 8), :] = packed[i]
        return lambda: _fold_token(jnp.concatenate(packed, axis=0), zero_v)

    def run_rounds(t0, rounds, post, first):
        count = [0]
        pins = {}

        def pinned(w):
            toks = pins.get(count[0])
            if not toks:
                return w
            top = w[0:8, 0:128]
            for tk in toks:
                top = top | tk
            return jnp.concatenate(
                [jnp.concatenate([top, w[0:8, 128:]], axis=1), w[8:]], axis=0)

        def run_jobs(m):
            for fn, span in post.get(count[0], ()):
                tok = fn(m)
                if span:
                    pins.setdefault(count[0] + span, []).append(tok())
            count[0] += 1

        for par, kind, cs in rounds:
            r0 = (kind * HD + cs[0] * 128) // 2
            rows = 64 * len(cs)

            def prod(i):
                src = sc7_v if (par, kind) == (1, V_) else s_v[par]
                rhs = ld(src.at[i], 0, HT1 // 2, 0, HD)
                if (par, kind, cs[0]) == (1, K_, 0):
                    sc7_v[i] = rhs
                m = lax.dot_general(_unpack(wt_v[i, r0:r0 + rows, :]), _unpack(pinned(rhs)),
                                    _NT, preferred_element_type=f32)
                run_jobs(m)
                return m

            def emit(rh, ch, blk):
                cols = slice((2 * par + ch) * HT1, (2 * par + ch + 1) * HT1)
                for n, c in enumerate(cs):
                    for jj in range(2):
                        pair = 4 * c + 2 * rh + jj
                        p = blk[n * 128 + jj * 64:n * 128 + (jj + 1) * 64]
                        if kind == K_:
                            phik_v[pair * 64:(pair + 1) * 64, cols] = _dual_softmax(p)
                        elif kind == Q_:
                            phiq_v[t0 // 2, pair * 64:(pair + 1) * 64, cols] = _dual_softmax(p)
                        else:
                            vt_v[pair // 8][(pair % 8) * 32:(pair % 8 + 1) * 32, cols] = _packi(p)

            _strassen(prod, emit)

        ones = _pack(jnp.ones((16, 2 * T1), f32))
        kr = lax.broadcasted_iota(jnp.int32, (80, 128), 0)
        kc = lax.broadcasted_iota(jnp.int32, (80, 128), 1)
        kmask = jnp.where(kr < 64, kr // 32, (kr - 64) // 8) == (kc // 2) % 2
        for j in range(NP):
            lhs = jnp.concatenate(
                [ld(vt_v[j // 8], (j % 8) * 32, 32, 0, 2 * T1), ones], axis=0)
            rhs = ld(phik_v, j * 64, 64, 0, 2 * T1)
            upd = lax.dot_general(_unpack(lhs), _unpack(pinned(rhs)), _NT,
                                  preferred_element_type=f32)
            run_jobs(upd)
            if first:
                kv_acc[j] = upd
            else:
                upd = kv_acc[j] + upd
                kv_acc[j] = upd
                kvt_v[j] = _pack(jnp.where(kmask, upd, 0.0))

    def load_best():
        return best_v[0], besti_v[...], best_v[1], best_v[2]

    def store_best(best):
        best_v[0], besti_v[...], best_v[1], best_v[2] = best

    def build_pt(g0, g1):
        n = g1 - g0
        w2 = wphi_v[4 * g0:4 * g1].reshape(n * 128, DH)
        er = lax.broadcasted_iota(jnp.int32, (128, DH), 0)
        ec = lax.broadcasted_iota(jnp.int32, (128, DH), 1)
        e = jnp.where(ec == ((er // 16) * 8 + er % 8) % 32, 1.0, 0.0).astype(bf16)
        ptf = lax.dot_general(e, w2, _NT, preferred_element_type=f32)
        pr = lax.broadcasted_iota(jnp.int32, (128, 128), 0)
        pc = lax.broadcasted_iota(jnp.int32, (128, 128), 1)
        keep = pc // 32 == (pr // 64) * 2 + (pr // 8) % 2
        return [jnp.where(keep, ptf[:, g * 128:(g + 1) * 128], 0.0).astype(bf16)
                for g in range(n)]

    hbl_v[...] = jnp.zeros_like(hbl_v)
    hbr_v[...] = jnp.zeros_like(hbr_v)
    store_best((jnp.full((8, 128), -jnp.inf, f32), jnp.zeros((8, 128), jnp.int32),
                jnp.zeros((8, 128), f32), jnp.zeros((8, 128), f32)))
    n_ln = HT1 // LN_ROWS
    x0_copy(0).wait()
    x0_copy(1).wait()
    for p in range(n_ln // 2):
        ln1_piece(0, s_v[0], p)
    full_copy(wr_hbm, wr_v, SEM_WR).wait()
    phi_copy(0).wait()
    x0_copy(2).wait()
    x0_copy(3).wait()
    wr_row = wr_v[...].astype(f32).reshape(1, D)
    wrf_v[...] = jnp.broadcast_to(
        wr_row - jnp.sum(wr_row, axis=-1, keepdims=True) * (1.0 / D), (8, D))
    pt = build_pt(0, 4)
    for p in range(n_ln // 2, n_ln):
        ln1_piece(0, s_v[0], p)
    for part in range(2):
        k0_copy(2 * part).wait()
        k0_copy(2 * part + 1).wait()
        fold_piece(K_, 0, 2 * part, pt)
        fold_piece(K_, 0, 2 * part + 1, pt)

    post = {}

    def at(slot, fn, span=0):
        post.setdefault(slot, []).append((fn, span))

    for slot, copies in T0_WAITS:
        for cp in copies:
            if cp == 'phi':
                at(slot, lambda m: phi_copy(1).wait())
            elif cp in ('x1', 'x2', 'x3'):
                at(slot, lambda m, cp=cp: x_copy(int(cp[1])).wait())
            else:
                at(slot, lambda m, cp=cp: w_copy(cp // NWC, cp % NWC).wait())
    for n in range(1, 2 * NWC):
        if n == 2:
            at(T0_FOLD[n], lambda m: pt.extend(build_pt(4, 8)))
        at(T0_FOLD[n], lambda m, n=n: fold_chunk(n // NWC, n % NWC, pt))
    for c in range(NWC):
        for j in range(4):
            at(T0_VPREP[c][j], lambda m, c=c, j=j: vprep_piece(c, j, m), T0_VSPAN)
    for p in range(n_ln):
        at(T0_LN[p], lambda m, p=p: ln1_piece(zs + T1, s_v[1], p, m), T0_LNSPAN[p])
    for p in range(n_ln):
        at(T1_LN[0][p], lambda m, p=p: ln1_piece(zs + 2 * T1, s_v[0], p, m), P1_LNSPAN)
        at(T1_LN[1][p], lambda m, p=p: ln1_piece(zs + 3 * T1, s_v[1], p, m), P1_LNSPAN)
    lo, hi = [0, 1], [2, 3]
    run_rounds(0, [(0, kind, [c]) for kind in (K_, Q_) for c in range(NWC)]
               + [(1, K_, lo), (1, K_, hi), (1, Q_, lo), (1, Q_, hi),
                  (0, V_, lo), (0, V_, hi), (1, V_, lo), (1, V_, hi)], post, True)
    full_copy(wo_hbm, wo_v.at[pl.ds(0, D), :], SEM_WO).wait()
    for i in range(4, N1):
        x_copy(i).wait()

    def phase1(i, carry):
        post = {}
        nxt = jnp.minimum(i + 1, N2 - 1) * T2
        w0 = jnp.minimum((i - 1) * WO_ROWS, HD - WO_ROWS)
        for par in range(2):
            for p in range(n_ln):
                post.setdefault(P1_LN2[par][p], []).append(
                    (lambda m, p=p, par=par: ln1_piece(nxt + par * T1, s_v[par], p, m),
                     P1_LNSPAN2[par]))
        for p in range(WO_ROWS // 16):
            post.setdefault(P1_WO[p], []).append(
                (lambda m, p=p: wo_piece(w0 + 16 * p, m), P1_WOSPAN))
        run_rounds(2 * i, [(par, kind, cs) for kind in (K_, Q_, V_) for par in range(2)
                           for cs in ([0, 1], [2, 3])], post, False)
        return carry

    lax.fori_loop(1, N1 // 2, phase1, 0)

    full_copy(wg_hbm, wg_v, SEM_WG).wait()
    full_copy(wu_hbm, wu_v, SEM_WU).wait()
    full_copy(wd_hbm, wd_v, SEM_WD).wait()

    def o_copy(hf):
        return pltpu.make_async_copy(
            out_v.at[pl.ds(hf * HT2, HT2), :], out_hbm.at[0, pl.ds(hf * HT2, HT2), :],
            sem.at[SEM_O + hf])

    def half_stats(hh, c0):
        rows = hh.shape[0]
        parts = [hh[:, c * 128:(c + 1) * 128] for c in range(4)]
        wts = [wrf_v[:, c0 + c * 128:c0 + (c + 1) * 128] for c in range(4)]
        s1 = (parts[0] + parts[1]) + (parts[2] + parts[3])
        sq = [p * p for p in parts]
        s2 = (sq[0] + sq[1]) + (sq[2] + sq[3])
        dw = [(p.reshape(rows // 8, 8, 128) * w[None]).reshape(rows, 128)
              for p, w in zip(parts, wts)]
        s3 = (dw[0] + dw[1]) + (dw[2] + dw[3])
        return s1, s2, s3

    def first_half(hbuf, sbuf, base, p, c0):
        r0 = p * EP_ROWS
        hh = ld(hbuf[c0 // HD], r0, EP_ROWS, 0, HD)
        h_v[pl.ds(pl.multiple_of(base + r0, EP_ROWS), EP_ROWS), c0:c0 + HD] = hh.astype(bf16)
        st = jnp.concatenate(half_stats(hh, c0), axis=1)
        sbuf[r0:r0 + EP_ROWS, :] = st
        return _fold_token(pltpu.bitcast(st, u32), zero_v)

    def finish(hbuf, sbuf, base, p, valid, best, defer=None):
        r0 = p * EP_ROWS
        g0 = pl.multiple_of(base + r0, EP_ROWS)
        hl, hr = [ld(r, r0, EP_ROWS, 0, HD) for r in hbuf]
        if defer is None:
            h_v[pl.ds(g0, EP_ROWS), 0:HD] = hl.astype(bf16)
        if sbuf is None:
            if defer is None:
                h_v[pl.ds(g0, EP_ROWS), HD:D] = hr.astype(bf16)
            st = half_stats(hr, HD)
        else:
            st = ld(sbuf, r0, EP_ROWS, 0, 384)
            st = [st[:, n * 128:(n + 1) * 128] for n in range(3)]
        s1, s2, s3 = [jnp.sum(v + w, axis=-1, keepdims=True)
                      for v, w in zip(half_stats(hl, 0), st)]
        m = s1 * (1.0 / D)
        var = jnp.maximum(s2 * (1.0 / D) - m * m, 0.0)
        inv = _rsqrt(var + EPS)
        r = s3 * inv

        def write_out(h):
            o = h * (1.0 + inv) - m * inv
            out_v[pl.ds(g0, EP_ROWS), :] = o.astype(bf16)
            return o

        if defer is None:
            o = write_out(jnp.concatenate([hl, hr], axis=1))
        else:
            defer.append(lambda: write_out(jnp.concatenate(
                [ld(r_, r0, EP_ROWS, 0, HD) for r_ in hbuf], axis=1)))
        bv, bi, bm, bq = best
        sub = lax.broadcasted_iota(jnp.int32, (8, 128), 0)
        for g in range(EP_ROWS // 8):
            rows = slice(g * 8, (g + 1) * 8)
            rg = jnp.broadcast_to(r[rows], (8, 128))
            if valid is not None:
                rg = jnp.where(valid, rg, -jnp.inf)
            better = rg > bv
            bi = jnp.where(better, sub + (g0 + g * 8), bi)
            bv = jnp.where(better, rg, bv)
            bm = jnp.where(better, jnp.broadcast_to(m[rows], (8, 128)), bm)
            bq = jnp.where(better, jnp.broadcast_to(var[rows], (8, 128)), bq)
        best = (bv, bi, bm, bq)
        if defer is not None:
            return best, jnp.broadcast_to(s3[EP_ROWS - 8:], (8, 128))
        tok = _fold_token(pltpu.bitcast(jnp.concatenate(
            [o[:, D - 128:], bv, bm, bq], axis=0), u32), zero_v)
        return best, tok

    n_ep = HT2 // EP_ROWS

    def phase2(i, carry):
        ot = []
        for j in range(NP):
            ph = phiq_v[i, j * 64:(j + 1) * 64, :]
            n = jnp.dot(_unpack(kvt_v[j]), _unpack(ph), preferred_element_type=f32)
            r0h = _recip(n[64:72] + 1e-6)
            r1h = _recip(n[72:80] + 1e-6)
            ot.append((n[0:32].reshape(4, 8, T2) * r0h[None]).reshape(32, T2))
            ot.append((n[32:64].reshape(4, 8, T2) * r1h[None]).reshape(32, T2))
        lo = jnp.concatenate(ot[:H // 2], axis=0)
        hi = jnp.concatenate(ot[H // 2:], axis=0)
        lcs = _left_combos(lo[:, :HT2], hi[:, :HT2], lo[:, HT2:], hi[:, HT2:])

        state = {'best': load_best()}
        pins = {}
        jobs = {}
        lts = {}
        ra = pl.multiple_of(i * T2, T2)
        rb = pl.multiple_of(i * T2 + HT2, HT2)
        prev = jnp.maximum(i * T2 - HT2, HT2)

        def add_job(slot, deadline, fn, gates=()):
            jobs.setdefault(slot, []).append((fn, deadline, gates))

        def finish_job(hbuf, sbuf, base, p, valid):
            def fn():
                state['best'], tok = finish(hbuf, sbuf, base, p, valid, state['best'])
                return tok
            return fn

        def lt_job(k):
            def fn():
                lts[k] = lcs[k].astype(bf16).T
                return _fold_token(pltpu.bitcast(lts[k], u32), zero_v)
            return fn

        order = (2, 4, 6, 0, 3, 1, 5)
        lt_job(2)()
        for n in range(1, 7):
            add_job(LT_START[n], LT_DEADLINE[n], lt_job(order[n]))
        for p in range(n_ep):
            add_job(FB_START[p], FB_START[p] + 2, finish_job(hb_v, None, prev, p, i > 0), hb_v)
            add_job(SA_START[p], SA_START[p] + 2, lambda p=p: first_half(ha_v, sa_v, ra, p, HD), ha_v[1:])
            add_job(FA_START[p], FA_DEADLINE[p], finish_job(ha_v, sa_v, ra, p, None), ha_v)

        def xblk(r0, c0):
            return x_v[pl.ds(r0, HT2), c0:c0 + 128].astype(f32)

        for n, k in enumerate(order):
            for c in range(4):
                slot = 4 * n + c
                for fn, deadline, gates in jobs.get(slot, ()):
                    for ref in gates:
                        ref[HT2:HT2 + 8, 0:128] = mm[GATE_ROW:GATE_ROW + 8]
                    pins.setdefault(deadline, []).append(fn())
                w = wo7_v[k, :, c * 128:(c + 1) * 128]
                toks = pins.get(slot)
                if toks:
                    top = w[0:8]
                    for tk in toks:
                        top = top | tk
                    w = jnp.concatenate([top, w[8:]], axis=0)
                mm = jnp.dot(lts[k], _unpack(w), preferred_element_type=f32)
                c0 = c * 128
                cs = slice(c0, c0 + 128)
                tmp = lambda t: ld(tmp_v[t], 0, HT2, c0, 128)
                if n == 0:
                    tmp_v[0][:, cs] = mm
                elif n == 1:
                    ha_v[1][0:HT2, cs] = (xblk(ra, HD + c0) + tmp(0)) + mm
                    tmp_v[1][:, cs] = xblk(ra, c0) - mm
                elif n == 2:
                    tmp_v[2][:, cs] = tmp(1) + mm
                elif n == 3:
                    tmp_v[3][:, cs] = tmp(2) + mm
                    tmp_v[4][:, cs] = (xblk(rb, HD + c0) + tmp(0)) + mm
                elif n == 4:
                    ha_v[0][0:HT2, cs] = tmp(3) + mm
                    tmp_v[5][:, cs] = xblk(rb, c0) + mm
                elif n == 5:
                    hb_v[0][0:HT2, cs] = tmp(5) + mm
                    tmp_v[6][:, cs] = tmp(4) - mm
                else:
                    hb_v[1][0:HT2, cs] = tmp(6) + mm
        store_best(state['best'])
        o_copy(2 * i).start()

        @pl.when(i > 0)
        def _():
            o_copy(2 * i - 1).start()

        return carry

    lax.fori_loop(0, N2, phase2, 0)
    best = load_best()
    late = []
    marks = []
    for p in range(n_ep):
        best, mark = finish(hb_v, None, S - HT2, p, None, best, late)
        marks.append(mark)

    for r_ in hb_v:
        r_[HT2:HT2 + 8, 0:128] = marks[LATE_MARK]
    for fn in late:
        fn()

    bv, bi, bm, bq = best
    for sh in (4, 2, 1):
        ov, oi, om, oq = [pltpu.roll(t, sh, 0) for t in (bv, bi, bm, bq)]
        take = jnp.logical_or(ov > bv, jnp.logical_and(ov == bv, oi < bi))
        bv, bi, bm, bq = [jnp.where(take, o_, t)
                          for o_, t in zip((ov, oi, om, oq), (bv, bi, bm, bq))]
    idx = jnp.clip(bi[0, 0], 0, S - 1)
    b0 = pl.multiple_of((idx // 8) * 8, 8)
    t = _rb(_rb(bq) + EPS)
    inv = _recip(_rb(t * _rsqrt(t)))
    gate = _sigmoid(bv)
    wide = lambda v: jnp.concatenate([v] * (D // 128), axis=1)
    b1 = pl.multiple_of(jnp.minimum(b0, S - HT2 - 8), 8)
    b2 = pl.multiple_of(jnp.maximum(b0 - (S - HT2), 0), 8)
    hb = jnp.where(wide(bi) < S - HT2, h_v[pl.ds(b1, 8), :].astype(f32),
                   _rb(jnp.concatenate([r_[pl.ds(b2, 8), :] for r_ in hb_v], axis=1)))
    hn = (hb - wide(bm)) * wide(inv)
    xs = hn.astype(bf16)
    rows = lax.broadcasted_iota(jnp.int32, (8, D), 0) + b0

    xm = jnp.where(rows == wide(bi), _rb(hn), 0.0)
    for sh in (4, 2, 1):
        xm = xm + pltpu.roll(xm, sh, 0)
    for t in range(D // 128):
        xcol_v[t // 2][(t % 2) * 128:(t % 2 + 1) * 128, :] = jnp.concatenate(
            [xm[:, t * 128:(t + 1) * 128]] * 16, axis=0).T

    nblk = F // 256
    nmx = nblk - FFN_VPU_BLOCKS
    act = {}
    acc = {}

    def activate(g, u):
        return (g * _sigmoid(g) * u).astype(bf16)

    parts = D // 8 // FFN_KG

    def vpu_chunk(q):
        blk, part = nmx + q // parts, q % parts
        cur = acc.get(blk)
        for kg in range(part * FFN_KG, (part + 1) * FFN_KG):
            xc = ld(xcol_v[kg // 32], (kg % 32) * 8, 8, 0, 128)
            w = jnp.concatenate(
                [r[kg * 8:(kg + 1) * 8, blk * 256:(blk + 1) * 256].astype(f32)
                 for r in (wg_v, wu_v)], axis=1)
            p = w * jnp.concatenate([xc] * 4, axis=1)
            cur = p if cur is None else cur + p
        acc[blk] = cur
        if part == parts - 1:
            for sh in (4, 2, 1):
                cur = cur + pltpu.roll(cur, sh, 0)
            act[blk] = activate(cur[:, :256], cur[:, 256:])
        if FFN_TOKALL:
            return _fold_token(pltpu.bitcast(cur, u32), zero_v)
        c = q % 4
        return _fold_token(pltpu.bitcast(cur[:, c * 128:(c + 1) * 128], u32), zero_v)

    steps = []
    for j in range(nmx):
        steps += [('g', j), ('u', j)]
    steps += [('d', j) for j in range(nblk)]
    nchunk = FFN_VPU_BLOCKS * parts
    starts = [FFN_W0 + (q * (FFN_W1 - FFN_W0)) // (nchunk - 1) for q in range(nchunk)]
    pins = {}
    gate_pre = {}
    ys = [None] * 4
    for n, (kind, j) in enumerate(steps):
        outs = []
        for wv in range(4):
            wave = 4 * n + wv
            if kind == 'd':
                lhs = act[j]
                w = wd_v[j * 256:(j + 1) * 256, wv * 256:(wv + 1) * 256]
            else:
                kh, c0 = wv % 2, j * 256 + (wv // 2) * 128
                lhs = xs[:, kh * HD:(kh + 1) * HD]
                w = (wg_v if kind == 'g' else wu_v)[kh * HD:(kh + 1) * HD, c0:c0 + 128]
            if pins.get(wave):
                wb = pltpu.bitcast(w, u32)
                top = wb[0:8, 0:128]
                for tk in pins[wave]:
                    top = top | tk
                if wb.shape[1] > 128:
                    top = jnp.concatenate([top, wb[0:8, 128:]], axis=1)
                w = _unpack(jnp.concatenate([top, wb[8:]], axis=0))
            outs.append(jnp.dot(lhs, w, preferred_element_type=f32))
            for q, start in enumerate(starts):
                if start == wave:
                    pins.setdefault(wave + FFN_SPAN, []).append(vpu_chunk(q))
        if kind == 'd':
            ys = [o_ if y_ is None else y_ + o_ for y_, o_ in zip(ys, outs)]
        else:
            p = jnp.concatenate([outs[0] + outs[1], outs[2] + outs[3]], axis=1)
            if kind == 'g':
                gate_pre[j] = p
            else:
                act[j] = activate(gate_pre[j], p)
        if n == FFN_LATE:
            o_copy(2 * N2 - 1).start()
    y = jnp.concatenate(ys, axis=1)
    cur = out_v[pl.ds(b0, 8), :].astype(f32)
    fix_v[...] = jnp.where(rows == wide(bi), hb + hn + y * wide(gate), cur).astype(bf16)
    for hf in range(2 * N2):
        o_copy(hf).wait()
    fix = pltpu.make_async_copy(fix_v, out_hbm.at[0, pl.ds(b0, 8), :], sem.at[SEM_O])
    fix.start()
    fix.wait()


def _kernel(*refs):
    def once(_, carry):
        _body(*refs)
        return carry

    lax.fori_loop(0, 1 + pl.semaphore_read(refs[-2]), once, 0)


@jax.jit
def pallas_sequential_preLN__linear_kernel_hedgehog__moe_arch_mod__prompt_kernel(
    A_x: jax.Array,
    A_wqkv: jax.Array,
    A_w_phi: jax.Array,
    A_wo: jax.Array,
    B_x: jax.Array,
    B_w_r: jax.Array,
    B_w_gate: jax.Array,
    B_w_up: jax.Array,
    B_w_down: jax.Array,
):
    any_spec = pl.BlockSpec(memory_space=pl.ANY)
    return pl.pallas_call(
        _kernel,
        out_shape=jax.ShapeDtypeStruct((1, S, D), bf16),
        in_specs=[any_spec] * 8,
        out_specs=any_spec,
        scratch_shapes=[
            pltpu.VMEM((S + 16, D), bf16),
            pltpu.VMEM((3 * NWC + 1, D, WC), bf16),
            pltpu.VMEM((H, DH, DH), bf16),
            pltpu.VMEM((D + 16, D), bf16),
            pltpu.VMEM((D,), bf16),
            pltpu.VMEM((D, F), bf16),
            pltpu.VMEM((D, F), bf16),
            pltpu.VMEM((F, D), bf16),
            pltpu.VMEM((7, 3 * HD // 2, HD), u32),
            pltpu.VMEM((7, HD // 2, HD), u32),
            pltpu.VMEM((7, HT1 // 2, HD), u32),
            pltpu.VMEM((7, HT1 // 2, HD), u32),
            pltpu.VMEM((7, HT1 // 2, HD), u32),
            pltpu.VMEM((N2, D, T2), u32),
            pltpu.VMEM((D, T2), u32),
            pltpu.VMEM((D // 4, T2), u32),
            pltpu.VMEM((D // 4, T2), u32),
            pltpu.VMEM((NP, 80, 128), f32),
            pltpu.VMEM((NP, 40, 128), u32),
            *[pltpu.VMEM((HT2 + 8, HD), f32) for _ in range(4)],
            pltpu.VMEM((HT2, 384), f32),
            *[pltpu.VMEM((HT2, HD), f32) for _ in range(7)],
            pltpu.VMEM((S, D), bf16),
            pltpu.VMEM((S, D), bf16),
            pltpu.VMEM((8, D), f32),
            pltpu.VMEM((3, 8, 128), f32),
            pltpu.VMEM((8, 128), jnp.int32),
            pltpu.VMEM((8, D), bf16),
            *[pltpu.VMEM((264, 128), f32) for _ in range(4)],
            pltpu.SemaphoreType.REGULAR,
            pltpu.SemaphoreType.DMA((NSEM,)),
        ],
        compiler_params=pltpu.CompilerParams(
            vmem_limit_bytes=110 * 1024 * 1024,
            disable_bounds_checks=True,
            disable_semaphore_checks=True),
    )(A_x, A_wqkv, A_w_phi, A_wo, B_w_r, B_w_gate, B_w_up, B_w_down)
```

```python
import jax
import jax.numpy as jnp
from jax import lax
import jax.experimental.pallas as pl
import jax.experimental.pallas.tpu as pltpu

S = 2048
D = 1024
H = 32
DH = 32
F = 3584
NP = H // 2
T1 = 256
T2 = 512
N1 = S // T1
N2 = S // T2
HT1 = T1 // 2
HT2 = T2 // 2
HD = D // 2
WC = 256
NWC = D // WC
LOG2E = 1.4426950408889634
EPS = 1e-5
WO_ROWS = 176
LN_ROWS = 16
EP_ROWS = 32
LT_START = (0, 0, 2, 5, 8, 11, 14)
LT_DEADLINE = (0, 4, 6, 9, 12, 15, 18)
FB_START = (2, 4, 6, 8, 10, 12, 14, 16)
SA_START = (9, 11, 13, 15, 17, 17, 18, 18)
FA_START = (20, 21, 22, 23, 24, 25, 26, 27)
FA_DEADLINE = (23, 24, 25, 26, 27, 29, 29, 29)
GATE_ROW = 0
PAD = 16
T0_FOLD = (0, 4, 11, 18, 25, 32, 39, 46)
T0_WAITS = ((4, (1,)), (11, ('phi', 2)), (18, (3, 4)), (32, ('x1', 5, 6)), (46, (7,)),
            (73, (8, 9, 10, 11, 'x2', 'x3')))
T0_VPREP = ((73, 74, 75, 76), (77, 78, 79, 80), (81, 82, 83, 84), (85, 86, 87, 88))
T0_VSPAN = 3
T0_LN = (32, 34, 35, 37, 38, 40, 41, 43)
T0_LNSPAN = (0,) * 8
P1_LN = (29, 30, 31, 32, 33, 34, 35, 36)
P1_LNSPAN = 3
P1_WO = (57, 58, 59, 60, 61, 78, 79, 80, 81, 82, 83)
P1_LN2 = ((70, 71, 72, 73, 74, 75, 76, 77), (62, 63, 64, 65, 66, 67, 68, 69))
P1_LNSPAN2 = (3, 3)
T1_LN = ((99, 100, 101, 102, 103, 104, 105, 106), (90, 91, 92, 93, 94, 95, 96, 97))
P1_WOSPAN = 3

FFN_VPU_BLOCKS = 6
FFN_KG = 8
FFN_W0 = 11
FFN_W1 = 110
FFN_SPAN = 3
FFN_TOKALL = 0
FFN_LATE = 16
LATE_AT = (0, 1, 2, 3, 4, 5, 6, 7)
LATE_SPAN = 0
LATE_GATE = 1

_NT = (((1,), (1,)), ((), ()))
_TN = (((0,), (0,)), ((), ()))
f32 = jnp.float32
bf16 = jnp.bfloat16
u32 = jnp.uint32

K_, Q_, V_ = 0, 1, 2
SRC = {K_: 1, Q_: 0, V_: 2}

SEM_W = 0
SEM_X = SEM_W + 3 * NWC
SEM_X0 = SEM_X + N1
SEM_K0 = SEM_X0 + 4
SEM_PHI = SEM_K0 + 4
SEM_WO = SEM_PHI + 2
SEM_WR, SEM_WG, SEM_WU, SEM_WD = (SEM_WO + 4 + i for i in range(4))
SEM_WGV, SEM_WUV = SEM_WD + 1, SEM_WD + 2
SEM_O = SEM_WUV + 1
NSEM = SEM_O + 2 * N2


def _rb(v):
    return v.astype(bf16).astype(f32)


def _unpack(w):
    return pltpu.bitcast(w, bf16)


def _recip(x):
    r = pl.reciprocal(x, approx=True)
    return r * (2.0 - x * r)


def _sigmoid(x):
    return _recip(1.0 + jnp.exp(jnp.minimum(-x, 80.0)))


def _rsqrt(x):
    return lax.rsqrt(x)


def _dual_softmax(p):
    t = p.shape[-1]
    p3 = p.reshape(8, 8, t)

    def allred(v, op):
        v = op(v, pltpu.roll(v, 2, 0))
        return op(v, pltpu.roll(v, 4, 0))

    mx = allred(jnp.max(p3, axis=0), jnp.maximum)
    mn = allred(jnp.min(p3, axis=0), jnp.minimum)
    ep = jnp.exp2(p3 - mx[None])
    en = jnp.exp2(mn[None] - p3)
    sp = allred(jnp.sum(ep, axis=0), jnp.add)
    sn = allred(jnp.sum(en, axis=0), jnp.add)
    fp = (ep * _recip(sp)[None]).reshape(64, t)
    fn = (en * _recip(sn)[None]).reshape(64, t)
    return jnp.concatenate([fp, fn], axis=0).astype(bf16)


def _left_combos(a11, a12, a21, a22):
    return [a11 + a22, a21 + a22, a11, a22, a11 + a12, a21 - a11, a12 - a22]


def _right_combos(b11, b12, b21, b22):
    return [b11 + b22, b11, b12 - b22, b21 - b11, b22, b11 + b12, b21 + b22]


def _strassen(prod, emit):
    m3 = prod(2)
    m5 = prod(4)
    emit(0, 1, m3 + m5)
    m7 = prod(6)
    u = m7 - m5
    m1 = prod(0)
    u = u + m1
    w = m1 + m3
    m4 = prod(3)
    emit(0, 0, u + m4)
    m2 = prod(1)
    emit(1, 0, m2 + m4)
    w = w - m2
    m6 = prod(5)
    emit(1, 1, w + m6)


def _fold_token(w, zero):
    r, c = w.shape
    acc = None
    for i in range(r // 8):
        for j in range(c // 128):
            blk = w[i * 8:(i + 1) * 8, j * 128:(j + 1) * 128]
            acc = blk if acc is None else acc | blk
    return acc & zero


def _body(zs, x_hbm, wqkv_hbm, wphi_hbm, wo_hbm, wr_hbm, wg_hbm, wu_hbm, wd_hbm,
            out_hbm,
            x_v, wqkv_v, wphi_v, wo_v, wr_v, wg_v, wu_v, wd_v, wgv_v, wuv_v,
            wt_v, wo7_v, sa7_v, sb7_v, sc7_v, phiq_v, phik_v, vt0_v, vt1_v, kv_acc, kvt_v, hal_v, har_v, hbl_v, hbr_v, sa_v,
            t0_v, t1_v, t2_v, t3_v, t4_v, t5_v, t6_v, h_v, out_v,
            wrf_v, best_v, besti_v, fix_v, xc0_v, xc1_v, xc2_v, xc3_v, sem):
    xcol_v = (xc0_v, xc1_v, xc2_v, xc3_v)
    s_v = (sa7_v, sb7_v)
    vt_v = (vt0_v, vt1_v)
    ha_v = (hal_v, har_v)
    hb_v = (hbl_v, hbr_v)
    tmp_v = (t0_v, t1_v, t2_v, t3_v, t4_v, t5_v, t6_v)

    def x_rows(r0, rows, slot):
        return pltpu.make_async_copy(
            x_hbm.at[0, pl.ds(r0, rows), :], x_v.at[pl.ds(r0, rows), :], sem.at[slot])

    def x_copy(i):
        return x_rows(i * T1, T1, SEM_X + i)

    def x0_copy(q):
        return x_rows((q % 2) * HT1 + (q // 2) * (HT1 // 2), HT1 // 2, SEM_X0 + q)

    def w_copy(kind, c):
        return pltpu.make_async_copy(
            wqkv_hbm.at[:, pl.ds(SRC[kind] * D + c * WC, WC)],
            wqkv_v.at[kind * NWC + c], sem.at[SEM_W + kind * NWC + c])

    def k0_copy(q):
        r0 = (q % 2) * HD + (q // 2) * 256
        return pltpu.make_async_copy(
            wqkv_hbm.at[pl.ds(r0, 256), pl.ds(SRC[K_] * D, WC)],
            wqkv_v.at[K_ * NWC, pl.ds(r0, 256), :], sem.at[SEM_K0 + q])

    def phi_copy(part):
        lo, n = part * (H // 2), H // 2
        return pltpu.make_async_copy(wphi_hbm.at[pl.ds(lo, n)], wphi_v.at[pl.ds(lo, n)],
                                     sem.at[SEM_PHI + part])

    def full_copy(src, dst, slot):
        return pltpu.make_async_copy(src, dst, sem.at[slot])

    x0_copy(0).start()
    x0_copy(1).start()
    full_copy(wr_hbm, wr_v, SEM_WR).start()
    phi_copy(0).start()
    x0_copy(2).start()
    x0_copy(3).start()
    for q in range(4):
        k0_copy(q).start()
    w_copy(K_, 1).start()
    phi_copy(1).start()
    w_copy(K_, 2).start()
    w_copy(K_, 3).start()
    w_copy(Q_, 0).start()
    x_copy(1).start()
    for c in range(1, NWC):
        w_copy(Q_, c).start()
    for c in range(NWC):
        w_copy(V_, c).start()
    x_copy(2).start()
    x_copy(3).start()
    full_copy(wo_hbm, wo_v.at[pl.ds(0, D), :], SEM_WO).start()
    for i in range(4, N1):
        x_copy(i).start()
    f0 = F - 256 * FFN_VPU_BLOCKS
    ffn_tiled = ((wg_hbm, wg_v, D, SEM_WG), (wu_hbm, wu_v, D, SEM_WU), (wd_hbm, wd_v, F, SEM_WD))
    for src, dst, rows, slot in ffn_tiled:
        for c in range(dst.shape[0]):
            full_copy(src.at[:, pl.ds(c * 128, 128)], dst.at[c, pl.ds(0, rows), :], slot).start()
    full_copy(wg_hbm.at[:, pl.ds(f0, F - f0)], wgv_v, SEM_WGV).start()
    full_copy(wu_hbm.at[:, pl.ds(f0, F - f0)], wuv_v, SEM_WUV).start()

    zero_v = jnp.full((8, 128), zs, jnp.int32).astype(u32)

    def ld(ref, r0, rows, c0, cols):
        return ref[pl.ds(pl.multiple_of(zs * 8 + r0, 8), rows), c0:c0 + cols]

    def tiles(ref, r0, rows, opaque=True):
        w = ref.bitcast(u32)
        if opaque:
            parts = [ld(w.at[c], r0 // 2, rows // 2, 0, 128) for c in range(ref.shape[0])]
        else:
            parts = [w[c, r0 // 2:(r0 + rows) // 2, :] for c in range(ref.shape[0])]
        return jnp.concatenate(parts, axis=1)

    def token(*vals):
        return lambda: _fold_token(pltpu.bitcast(jnp.concatenate(vals, axis=0), u32), zero_v)

    def ln1_stats(xf):
        m = jnp.sum(xf, axis=-1, keepdims=True) * (1.0 / D)
        q = jnp.sum(xf * xf, axis=-1, keepdims=True) * (1.0 / D)
        inv = _rsqrt(jnp.maximum(q - m * m, 0.0) + EPS)
        return inv, m * inv

    def ln1_piece(r0, dst, p, m=None):
        if m is not None:
            x_v[S:S + 8, 0:128] = m[0:8, 0:128].astype(bf16)
        xa, xb = [x_v[pl.ds(pl.multiple_of(r0 + hf * HT1 + p * LN_ROWS, LN_ROWS), LN_ROWS), :]
                  .astype(f32) for hf in range(2)]
        (ia, ma), (ib, mb) = ln1_stats(xa), ln1_stats(xb)
        ya, yb = xa * ia, xb * ib
        s2 = ya[:, :HD] - ma
        s5 = yb[:, HD:] - mb
        s1 = s2 + s5
        s3 = yb[:, :HD] - yb[:, HD:]
        s4 = ya[:, HD:] - ya[:, :HD]
        combos = [s1, s2, s3, s4, s5, s1 + s3, s1 + s4]
        for i in range(7):
            for c in range(4):
                dst[i, c, p * LN_ROWS:(p + 1) * LN_ROWS, :] = (
                    combos[i][:, c * 128:(c + 1) * 128].astype(bf16))
        return token(combos[5], combos[6])

    def fold_piece(kind, c, j, pt):
        blk = {}
        for hh in range(2):
            for kh in range(2):
                k0 = kh * HD + j * 128
                w = wqkv_v[kind * NWC + c, k0:k0 + 128, hh * 128:(hh + 1) * 128]
                blk[hh, kh] = lax.dot_general(pt[2 * c + hh], w, _NT,
                                              preferred_element_type=f32) * LOG2E
        combos = _left_combos(blk[0, 0], blk[0, 1], blk[1, 0], blk[1, 1])
        r0 = kind * HD + c * 128
        for i in range(7):
            wt_v[i, j, r0:r0 + 128, :] = combos[i].astype(bf16)

    def fold_chunk(kind, c, pt):
        for j in range(4):
            fold_piece(kind, c, j, pt)

    def vprep_piece(c, j, m):
        wqkv_v[3 * NWC, 0:8, 0:128] = m[0:8, 0:128].astype(bf16)
        blk = {}
        for hh in range(2):
            for kh in range(2):
                k0 = kh * HD + j * 128
                w = wqkv_v[zs + V_ * NWC + c, k0:k0 + 128, hh * 128:(hh + 1) * 128]
                blk[hh, kh] = w.T.astype(f32)
        combos = _left_combos(blk[0, 0], blk[0, 1], blk[1, 0], blk[1, 1])
        r0 = V_ * HD + c * 128
        for i in range(7):
            wt_v[i, j, r0:r0 + 128, :] = combos[i].astype(bf16)
        return token(combos[1], combos[4])

    def wo_piece(w0, m):
        wo_v[D:D + 8, 0:128] = m[0:8, 0:128].astype(bf16)
        top = wo_v[pl.ds(pl.multiple_of(w0, 16), 16), :].astype(f32)
        bot = wo_v[pl.ds(pl.multiple_of(HD + w0, 16), 16), :].astype(f32)
        combos = _right_combos(top[:, :HD], top[:, HD:], bot[:, :HD], bot[:, HD:])
        for i in range(7):
            for c in range(4):
                wo7_v[i, c, pl.ds(pl.multiple_of(w0, 16), 16), :] = (
                    combos[i][:, c * 128:(c + 1) * 128].astype(bf16))
        return token(combos[5], combos[6])

    def run_rounds(t0, rounds, post, first):
        count = [0]
        pins = {}

        def pinned(w):
            toks = pins.get(count[0])
            if not toks:
                return w
            top = w[0:8, 0:128]
            for tk in toks:
                top = top | tk
            return jnp.concatenate(
                [jnp.concatenate([top, w[0:8, 128:]], axis=1), w[8:]], axis=0)

        def run_jobs(m):
            for fn, span in post.get(count[0], ()):
                tok = fn(m)
                if span:
                    pins.setdefault(count[0] + span, []).append(tok())
            count[0] += 1

        for par, kind, cs in rounds:
            r0 = kind * HD + cs[0] * 128
            rows = 128 * len(cs)

            def prod(i):
                if (par, kind) == (1, V_):
                    rhs = ld(sc7_v.at[i], 0, HT1 // 2, 0, HD)
                else:
                    rhs = tiles(s_v[par].at[i], 0, HT1)
                if (par, kind, cs[0]) == (1, K_, 0):
                    sc7_v[i] = rhs
                m = lax.dot_general(_unpack(tiles(wt_v.at[i], r0, rows, False)),
                                    _unpack(pinned(rhs)),
                                    _NT, preferred_element_type=f32)
                run_jobs(m)
                return m

            def emit(rh, ch, blk):
                tb = 2 * par + ch
                for n, c in enumerate(cs):
                    for jj in range(2):
                        pair = 4 * c + 2 * rh + jj
                        p = blk[n * 128 + jj * 64:n * 128 + (jj + 1) * 64]
                        if kind == K_:
                            phik_v[tb, pair * 128:(pair + 1) * 128, :] = _dual_softmax(p)
                        elif kind == Q_:
                            phiq_v[t0 // 2, tb, pair * 128:(pair + 1) * 128, :] = (
                                _dual_softmax(p))
                        else:
                            vt_v[pair // 8][tb, (pair % 8) * 64:(pair % 8 + 1) * 64, :] = (
                                p.astype(bf16))

            _strassen(prod, emit)

        ones = jnp.full((8, 2 * T1), 0x3F803F80, u32)
        kr = lax.broadcasted_iota(jnp.int32, (80, 128), 0)
        kc = lax.broadcasted_iota(jnp.int32, (80, 128), 1)
        kmask = jnp.where(kr < 64, kr // 32, (kr - 64) // 8) == kc % 2
        for j in range(NP):
            lhs = jnp.concatenate([tiles(vt_v[j // 8], (j % 8) * 64, 64), ones], axis=0)
            rhs = tiles(phik_v, j * 128, 128)
            upd = lax.dot_general(_unpack(lhs), _unpack(pinned(rhs)), _NT,
                                  preferred_element_type=f32)
            run_jobs(upd)
            if first:
                kv_acc[j] = upd
            else:
                upd = kv_acc[j] + upd
                kv_acc[j] = upd
                kvt_v[j] = jnp.where(kmask, upd, 0.0).astype(bf16)

    def load_best():
        return best_v[0], besti_v[...], best_v[1], best_v[2]

    def store_best(best):
        best_v[0], besti_v[...], best_v[1], best_v[2] = best

    def build_pt(g0, g1):
        n = g1 - g0
        w2 = wphi_v[4 * g0:4 * g1].reshape(n * 128, DH)
        er = lax.broadcasted_iota(jnp.int32, (128, DH), 0)
        ec = lax.broadcasted_iota(jnp.int32, (128, DH), 1)
        e = jnp.where(ec == (er % 64) // 2, 1.0, 0.0).astype(bf16)
        ptf = lax.dot_general(e, w2, _NT, preferred_element_type=f32)
        pr = lax.broadcasted_iota(jnp.int32, (128, 128), 0)
        pc = lax.broadcasted_iota(jnp.int32, (128, 128), 1)
        keep = pc // 32 == (pr // 64) * 2 + pr % 2
        return [jnp.where(keep, ptf[:, g * 128:(g + 1) * 128], 0.0).astype(bf16)
                for g in range(n)]

    hbl_v[...] = jnp.zeros_like(hbl_v)
    hbr_v[...] = jnp.zeros_like(hbr_v)
    store_best((jnp.full((8, 128), -jnp.inf, f32), jnp.zeros((8, 128), jnp.int32),
                jnp.zeros((8, 128), f32), jnp.zeros((8, 128), f32)))
    n_ln = HT1 // LN_ROWS
    x0_copy(0).wait()
    x0_copy(1).wait()
    for p in range(n_ln // 2):
        ln1_piece(0, s_v[0], p)
    full_copy(wr_hbm, wr_v, SEM_WR).wait()
    phi_copy(0).wait()
    x0_copy(2).wait()
    x0_copy(3).wait()
    wr_row = wr_v[...].astype(f32).reshape(1, D)
    wrf_v[...] = jnp.broadcast_to(
        wr_row - jnp.sum(wr_row, axis=-1, keepdims=True) * (1.0 / D), (8, D))
    pt = build_pt(0, 4)
    for p in range(n_ln // 2, n_ln):
        ln1_piece(0, s_v[0], p)
    for part in range(2):
        k0_copy(2 * part).wait()
        k0_copy(2 * part + 1).wait()
        fold_piece(K_, 0, 2 * part, pt)
        fold_piece(K_, 0, 2 * part + 1, pt)

    post = {}

    def at(slot, fn, span=0):
        post.setdefault(slot, []).append((fn, span))

    for slot, copies in T0_WAITS:
        for cp in copies:
            if cp == 'phi':
                at(slot, lambda m: phi_copy(1).wait())
            elif cp in ('x1', 'x2', 'x3'):
                at(slot, lambda m, cp=cp: x_copy(int(cp[1])).wait())
            else:
                at(slot, lambda m, cp=cp: w_copy(cp // NWC, cp % NWC).wait())
    for n in range(1, 2 * NWC):
        if n == 2:
            at(T0_FOLD[n], lambda m: pt.extend(build_pt(4, 8)))
        at(T0_FOLD[n], lambda m, n=n: fold_chunk(n // NWC, n % NWC, pt))
    for c in range(NWC):
        for j in range(4):
            at(T0_VPREP[c][j], lambda m, c=c, j=j: vprep_piece(c, j, m), T0_VSPAN)
    for p in range(n_ln):
        at(T0_LN[p], lambda m, p=p: ln1_piece(zs + T1, s_v[1], p, m), T0_LNSPAN[p])
    for p in range(n_ln):
        at(T1_LN[0][p], lambda m, p=p: ln1_piece(zs + 2 * T1, s_v[0], p, m), P1_LNSPAN)
        at(T1_LN[1][p], lambda m, p=p: ln1_piece(zs + 3 * T1, s_v[1], p, m), P1_LNSPAN)
    lo, hi = [0, 1], [2, 3]
    run_rounds(0, [(0, kind, [c]) for kind in (K_, Q_) for c in range(NWC)]
               + [(1, K_, lo), (1, K_, hi), (1, Q_, lo), (1, Q_, hi),
                  (0, V_, lo), (0, V_, hi), (1, V_, lo), (1, V_, hi)], post, True)
    full_copy(wo_hbm, wo_v.at[pl.ds(0, D), :], SEM_WO).wait()
    for i in range(4, N1):
        x_copy(i).wait()

    def phase1(i, carry):
        post = {}
        nxt = jnp.minimum(i + 1, N2 - 1) * T2
        w0 = jnp.minimum((i - 1) * WO_ROWS, HD - WO_ROWS)
        for par in range(2):
            for p in range(n_ln):
                post.setdefault(P1_LN2[par][p], []).append(
                    (lambda m, p=p, par=par: ln1_piece(nxt + par * T1, s_v[par], p, m),
                     P1_LNSPAN2[par]))
        for p in range(WO_ROWS // 16):
            post.setdefault(P1_WO[p], []).append(
                (lambda m, p=p: wo_piece(w0 + 16 * p, m), P1_WOSPAN))
        run_rounds(2 * i, [(par, kind, cs) for kind in (K_, Q_, V_) for par in range(2)
                           for cs in ([0, 1], [2, 3])], post, False)
        return carry

    lax.fori_loop(1, N1 // 2, phase1, 0)

    for _, dst, rows, slot in ffn_tiled:
        filled = dst.at[:, pl.ds(0, rows), :]
        full_copy(filled, filled, slot).wait()
    full_copy(wg_hbm.at[:, pl.ds(f0, F - f0)], wgv_v, SEM_WGV).wait()
    full_copy(wu_hbm.at[:, pl.ds(f0, F - f0)], wuv_v, SEM_WUV).wait()

    def o_copy(hf):
        return pltpu.make_async_copy(
            out_v.at[pl.ds(hf * HT2, HT2), :], out_hbm.at[0, pl.ds(hf * HT2, HT2), :],
            sem.at[SEM_O + hf])

    def half_stats(hh, c0):
        rows = hh.shape[0]
        parts = [hh[:, c * 128:(c + 1) * 128] for c in range(4)]
        wts = [wrf_v[:, c0 + c * 128:c0 + (c + 1) * 128] for c in range(4)]
        s1 = (parts[0] + parts[1]) + (parts[2] + parts[3])
        sq = [p * p for p in parts]
        s2 = (sq[0] + sq[1]) + (sq[2] + sq[3])
        dw = [(p.reshape(rows // 8, 8, 128) * w[None]).reshape(rows, 128)
              for p, w in zip(parts, wts)]
        s3 = (dw[0] + dw[1]) + (dw[2] + dw[3])
        return s1, s2, s3

    def first_half(hbuf, sbuf, base, p, c0):
        r0 = p * EP_ROWS
        hh = ld(hbuf[c0 // HD], r0, EP_ROWS, 0, HD)
        h_v[pl.ds(pl.multiple_of(base + r0, EP_ROWS), EP_ROWS), c0:c0 + HD] = hh.astype(bf16)
        st = jnp.concatenate(half_stats(hh, c0), axis=1)
        sbuf[r0:r0 + EP_ROWS, :] = st
        return _fold_token(pltpu.bitcast(st, u32), zero_v)

    def finish(hbuf, sbuf, base, p, valid, best, defer=None):
        r0 = p * EP_ROWS
        g0 = pl.multiple_of(base + r0, EP_ROWS)
        hl, hr = [ld(r, r0, EP_ROWS, 0, HD) for r in hbuf]
        if defer is None:
            h_v[pl.ds(g0, EP_ROWS), 0:HD] = hl.astype(bf16)
        if sbuf is None:
            if defer is None:
                h_v[pl.ds(g0, EP_ROWS), HD:D] = hr.astype(bf16)
            st = half_stats(hr, HD)
        else:
            st = ld(sbuf, r0, EP_ROWS, 0, 384)
            st = [st[:, n * 128:(n + 1) * 128] for n in range(3)]
        s1, s2, s3 = [jnp.sum(v + w, axis=-1, keepdims=True)
                      for v, w in zip(half_stats(hl, 0), st)]
        m = s1 * (1.0 / D)
        var = jnp.maximum(s2 * (1.0 / D) - m * m, 0.0)
        inv = _rsqrt(var + EPS)
        r = s3 * inv

        def write_out(h):
            o = h * (1.0 + inv) - m * inv
            out_v[pl.ds(g0, EP_ROWS), :] = o.astype(bf16)
            return o

        if defer is None:
            o = write_out(jnp.concatenate([hl, hr], axis=1))
        else:
            defer.append(lambda: write_out(jnp.concatenate(
                [ld(r_, r0, EP_ROWS, 0, HD) for r_ in hbuf], axis=1)))
        bv, bi, bm, bq = best
        sub = lax.broadcasted_iota(jnp.int32, (8, 128), 0)
        for g in range(EP_ROWS // 8):
            rows = slice(g * 8, (g + 1) * 8)
            rg = jnp.broadcast_to(r[rows], (8, 128))
            if valid is not None:
                rg = jnp.where(valid, rg, -jnp.inf)
            better = rg > bv
            bi = jnp.where(better, sub + (g0 + g * 8), bi)
            bv = jnp.where(better, rg, bv)
            bm = jnp.where(better, jnp.broadcast_to(m[rows], (8, 128)), bm)
            bq = jnp.where(better, jnp.broadcast_to(var[rows], (8, 128)), bq)
        best = (bv, bi, bm, bq)
        if defer is not None:
            return best, None
        tok = _fold_token(pltpu.bitcast(jnp.concatenate(
            [o[:, D - 128:], bv, bm, bq], axis=0), u32), zero_v)
        return best, tok

    n_ep = HT2 // EP_ROWS

    def phase2(i, carry):
        ot = []
        for j in range(NP):
            ph = tiles(phiq_v.at[i], j * 128, 128, False)
            n = jnp.dot(_unpack(kvt_v.bitcast(u32)[j]), _unpack(ph),
                        preferred_element_type=f32)
            r0h = _recip(n[64:72] + 1e-6)
            r1h = _recip(n[72:80] + 1e-6)
            ot.append((n[0:32].reshape(4, 8, T2) * r0h[None]).reshape(32, T2))
            ot.append((n[32:64].reshape(4, 8, T2) * r1h[None]).reshape(32, T2))
        lo = jnp.concatenate(ot[:H // 2], axis=0)
        hi = jnp.concatenate(ot[H // 2:], axis=0)
        lcs = _left_combos(lo[:, :HT2], hi[:, :HT2], lo[:, HT2:], hi[:, HT2:])

        state = {'best': load_best()}
        pins = {}
        jobs = {}
        lts = {}
        ra = pl.multiple_of(i * T2, T2)
        rb = pl.multiple_of(i * T2 + HT2, HT2)
        prev = jnp.maximum(i * T2 - HT2, HT2)

        def add_job(slot, deadline, fn, gates=()):
            jobs.setdefault(slot, []).append((fn, deadline, gates))

        def finish_job(hbuf, sbuf, base, p, valid):
            def fn():
                state['best'], tok = finish(hbuf, sbuf, base, p, valid, state['best'])
                return tok
            return fn

        def lt_job(k):
            def fn():
                lts[k] = lcs[k].astype(bf16).T
                return _fold_token(pltpu.bitcast(lts[k], u32), zero_v)
            return fn

        order = (2, 4, 6, 0, 3, 1, 5)
        lt_job(2)()
        for n in range(1, 7):
            add_job(LT_START[n], LT_DEADLINE[n], lt_job(order[n]))
        for p in range(n_ep):
            add_job(FB_START[p], FB_START[p] + 2, finish_job(hb_v, None, prev, p, i > 0), hb_v)
            add_job(SA_START[p], SA_START[p] + 2, lambda p=p: first_half(ha_v, sa_v, ra, p, HD), ha_v[1:])
            add_job(FA_START[p], FA_DEADLINE[p], finish_job(ha_v, sa_v, ra, p, None), ha_v)

        def xblk(r0, c0):
            return x_v[pl.ds(r0, HT2), c0:c0 + 128].astype(f32)

        for n, k in enumerate(order):
            for c in range(4):
                slot = 4 * n + c
                for fn, deadline, gates in jobs.get(slot, ()):
                    for ref in gates:
                        ref[HT2:HT2 + 8, 0:128] = mm[GATE_ROW:GATE_ROW + 8]
                    pins.setdefault(deadline, []).append(fn())
                w = wo7_v.bitcast(u32)[k, c, 0:HD // 2, :]
                toks = pins.get(slot)
                if toks:
                    top = w[0:8]
                    for tk in toks:
                        top = top | tk
                    w = jnp.concatenate([top, w[8:]], axis=0)
                mm = jnp.dot(lts[k], _unpack(w), preferred_element_type=f32)
                c0 = c * 128
                cs = slice(c0, c0 + 128)
                tmp = lambda t: ld(tmp_v[t], 0, HT2, c0, 128)
                if n == 0:
                    tmp_v[0][:, cs] = mm
                elif n == 1:
                    ha_v[1][0:HT2, cs] = (xblk(ra, HD + c0) + tmp(0)) + mm
                    tmp_v[1][:, cs] = xblk(ra, c0) - mm
                elif n == 2:
                    tmp_v[2][:, cs] = tmp(1) + mm
                elif n == 3:
                    tmp_v[3][:, cs] = tmp(2) + mm
                    tmp_v[4][:, cs] = (xblk(rb, HD + c0) + tmp(0)) + mm
                elif n == 4:
                    ha_v[0][0:HT2, cs] = tmp(3) + mm
                    tmp_v[5][:, cs] = xblk(rb, c0) + mm
                elif n == 5:
                    hb_v[0][0:HT2, cs] = tmp(5) + mm
                    tmp_v[6][:, cs] = tmp(4) - mm
                else:
                    hb_v[1][0:HT2, cs] = tmp(6) + mm
        store_best(state['best'])
        o_copy(2 * i).start()

        @pl.when(i > 0)
        def _():
            o_copy(2 * i - 1).start()

        return carry

    lax.fori_loop(0, N2, phase2, 0)
    best = load_best()
    late = []
    for p in range(n_ep):
        best, _ = finish(hb_v, None, S - HT2, p, None, best, late)


    bv, bi, bm, bq = best
    for sh in (4, 2, 1):
        ov, oi, om, oq = [pltpu.roll(t, sh, 0) for t in (bv, bi, bm, bq)]
        take = jnp.logical_or(ov > bv, jnp.logical_and(ov == bv, oi < bi))
        bv, bi, bm, bq = [jnp.where(take, o_, t)
                          for o_, t in zip((ov, oi, om, oq), (bv, bi, bm, bq))]
    idx = jnp.clip(bi[0, 0], 0, S - 1)
    b0 = pl.multiple_of((idx // 8) * 8, 8)
    t = _rb(_rb(bq) + EPS)
    inv = _recip(_rb(t * _rsqrt(t)))
    gate = _sigmoid(bv)
    wide = lambda v: jnp.concatenate([v] * (D // 128), axis=1)
    b1 = pl.multiple_of(jnp.minimum(b0, S - HT2 - 8), 8)
    b2 = pl.multiple_of(jnp.maximum(b0 - (S - HT2), 0), 8)
    hb = jnp.where(wide(bi) < S - HT2, h_v[pl.ds(b1, 8), :].astype(f32),
                   _rb(jnp.concatenate([r_[pl.ds(b2, 8), :] for r_ in hb_v], axis=1)))
    hn = (hb - wide(bm)) * wide(inv)
    xs = hn.astype(bf16)
    rows = lax.broadcasted_iota(jnp.int32, (8, D), 0) + b0

    xm = jnp.where(rows == wide(bi), _rb(hn), 0.0)
    for sh in (4, 2, 1):
        xm = xm + pltpu.roll(xm, sh, 0)
    for t in range(D // 128):
        xcol_v[t // 2][(t % 2) * 128:(t % 2 + 1) * 128, :] = jnp.concatenate(
            [xm[:, t * 128:(t + 1) * 128]] * 16, axis=0).T

    nblk = F // 256
    nmx = nblk - FFN_VPU_BLOCKS
    act = {}
    acc = {}

    def activate(g, u):
        return (g * _sigmoid(g) * u).astype(bf16)

    parts = D // 8 // FFN_KG

    def vpu_chunk(q):
        blk, part = nmx + q // parts, q % parts
        cur = acc.get(blk)
        for kg in range(part * FFN_KG, (part + 1) * FFN_KG):
            xc = ld(xcol_v[kg // 32], (kg % 32) * 8, 8, 0, 128)
            w = jnp.concatenate(
                [r[kg * 8:(kg + 1) * 8, (blk - nmx) * 256:(blk - nmx + 1) * 256].astype(f32)
                 for r in (wgv_v, wuv_v)], axis=1)
            p = w * jnp.concatenate([xc] * 4, axis=1)
            cur = p if cur is None else cur + p
        acc[blk] = cur
        if part == parts - 1:
            for sh in (4, 2, 1):
                cur = cur + pltpu.roll(cur, sh, 0)
            act[blk] = activate(cur[:, :256], cur[:, 256:])
        if FFN_TOKALL:
            return _fold_token(pltpu.bitcast(cur, u32), zero_v)
        c = q % 4
        return _fold_token(pltpu.bitcast(cur[:, c * 128:(c + 1) * 128], u32), zero_v)

    nchunk = FFN_VPU_BLOCKS * parts
    starts = [FFN_W0 + (q * (FFN_W1 - FFN_W0)) // (nchunk - 1) for q in range(nchunk)]
    pins = {}
    wave = [0]
    wgw, wuw, wdw = [r.bitcast(u32) for r in (wg_v, wu_v, wd_v)]

    def run_wave(lhs, tls):
        top = tls[0][0:8]
        for tk in pins.get(wave[0], ()):
            top = top | tk
        w = jnp.concatenate([jnp.concatenate([top, tls[0][8:]], axis=0)] + tls[1:], axis=1)
        out = jnp.dot(lhs, _unpack(w), preferred_element_type=f32)
        for p, fn in enumerate(late):
            if LATE_AT[p] == wave[0]:
                for r_ in hb_v:
                    r_[HT2:HT2 + 8, 0:128] = out[:, 0:128] if LATE_GATE else hn[:, 0:128]
                tk = token(fn()[:, D - 128:])
                if LATE_SPAN:
                    pins.setdefault(wave[0] + LATE_SPAN, []).append(tk())
        for q, start in enumerate(starts):
            if start == wave[0]:
                pins.setdefault(wave[0] + FFN_SPAN, []).append(vpu_chunk(q))
        if wave[0] == FFN_LATE:
            o_copy(2 * N2 - 1).start()
        wave[0] += 1
        return out

    for j in range(nmx):
        gu = None
        for kt in range(D // 128):
            p = run_wave(xs[:, kt * 128:(kt + 1) * 128],
                         [r[2 * j + c, kt * 64:(kt + 1) * 64, :]
                          for r in (wgw, wuw) for c in range(2)])
            gu = p if gu is None else gu + p
        act[j] = activate(gu[:, :256], gu[:, 256:])
    ys = [None, None]
    for j in range(nblk):
        for kt in range(2):
            for hf in range(2):
                r0 = (2 * j + kt) * 64
                p = run_wave(act[j][:, kt * 128:(kt + 1) * 128],
                             [wdw[4 * hf + c, r0:r0 + 64, :] for c in range(4)])
                ys[hf] = p if ys[hf] is None else ys[hf] + p
    y = jnp.concatenate(ys, axis=1)
    cur = out_v[pl.ds(b0, 8), :].astype(f32)
    fix_v[...] = jnp.where(rows == wide(bi), hb + hn + y * wide(gate), cur).astype(bf16)
    for hf in range(2 * N2):
        o_copy(hf).wait()
    fix = pltpu.make_async_copy(fix_v, out_hbm.at[0, pl.ds(b0, 8), :], sem.at[SEM_O])
    fix.start()
    fix.wait()


def _kernel(*refs):
    def step(i, carry):
        @pl.when(i == 0)
        def _():
            _body(i, *refs)

        return carry

    lax.fori_loop(0, 2, step, 0)


@jax.jit
def pallas_sequential_preLN__linear_kernel_hedgehog__moe_arch_mod__prompt_kernel(
    A_x: jax.Array,
    A_wqkv: jax.Array,
    A_w_phi: jax.Array,
    A_wo: jax.Array,
    B_x: jax.Array,
    B_w_r: jax.Array,
    B_w_gate: jax.Array,
    B_w_up: jax.Array,
    B_w_down: jax.Array,
):
    any_spec = pl.BlockSpec(memory_space=pl.ANY)
    return pl.pallas_call(
        _kernel,
        out_shape=jax.ShapeDtypeStruct((1, S, D), bf16),
        in_specs=[any_spec] * 8,
        out_specs=any_spec,
        scratch_shapes=[
            pltpu.VMEM((S + 16, D), bf16),
            pltpu.VMEM((3 * NWC + 1, D, WC), bf16),
            pltpu.VMEM((H, DH, DH), bf16),
            pltpu.VMEM((D + 16, D), bf16),
            pltpu.VMEM((D,), bf16),
            pltpu.VMEM((F // 128 - 2 * FFN_VPU_BLOCKS, D + PAD, 128), bf16),
            pltpu.VMEM((F // 128 - 2 * FFN_VPU_BLOCKS, D + PAD, 128), bf16),
            pltpu.VMEM((D // 128, F + PAD, 128), bf16),
            pltpu.VMEM((D, 256 * FFN_VPU_BLOCKS), bf16),
            pltpu.VMEM((D, 256 * FFN_VPU_BLOCKS), bf16),
            pltpu.VMEM((7, 4, 3 * HD + PAD, 128), bf16),
            pltpu.VMEM((7, 4, HD + PAD, 128), bf16),
            pltpu.VMEM((7, 4, HT1 + PAD, 128), bf16),
            pltpu.VMEM((7, 4, HT1 + PAD, 128), bf16),
            pltpu.VMEM((7, HT1 // 2, HD), u32),
            pltpu.VMEM((N2, 4, 2 * D + PAD, 128), bf16),
            pltpu.VMEM((4, 2 * D + PAD, 128), bf16),
            pltpu.VMEM((4, HD + PAD, 128), bf16),
            pltpu.VMEM((4, HD + PAD, 128), bf16),
            pltpu.VMEM((NP, 80, 128), f32),
            pltpu.VMEM((NP, 80, 128), bf16),
            *[pltpu.VMEM((HT2 + 8, HD), f32) for _ in range(4)],
            pltpu.VMEM((HT2, 384), f32),
            *[pltpu.VMEM((HT2, HD), f32) for _ in range(7)],
            pltpu.VMEM((S, D), bf16),
            pltpu.VMEM((S, D), bf16),
            pltpu.VMEM((8, D), f32),
            pltpu.VMEM((3, 8, 128), f32),
            pltpu.VMEM((8, 128), jnp.int32),
            pltpu.VMEM((8, D), bf16),
            *[pltpu.VMEM((264, 128), f32) for _ in range(4)],
            pltpu.SemaphoreType.DMA((NSEM,)),
        ],
        compiler_params=pltpu.CompilerParams(
            vmem_limit_bytes=110 * 1024 * 1024,
            disable_bounds_checks=True,
            disable_semaphore_checks=True),
    )(A_x, A_wqkv, A_w_phi, A_wo, B_w_r, B_w_gate, B_w_up, B_w_down)
```

```python
import jax
import jax.numpy as jnp
from jax import lax
import jax.experimental.pallas as pl
import jax.experimental.pallas.tpu as pltpu

S = 2048
D = 1024
H = 32
DH = 32
F = 3584
NP = H // 2
T1 = 256
T2 = 512
N1 = S // T1
N2 = S // T2
HT1 = T1 // 2
HT2 = T2 // 2
HD = D // 2
WC = 256
NWC = D // WC
LOG2E = 1.4426950408889634
EPS = 1e-5
WO_ROWS = 176
LN_ROWS = 16
EP_ROWS = 32
LT_START = (0, 0, 2, 5, 8, 11, 14)
LT_DEADLINE = (0, 4, 6, 9, 12, 15, 18)
FB_START = (2, 4, 6, 8, 10, 12, 14, 16)
SA_START = (9, 11, 13, 15, 17, 17, 18, 18)
FA_START = (20, 21, 22, 23, 24, 25, 26, 27)
FA_DEADLINE = (23, 24, 25, 26, 27, 29, 29, 29)
GATE_ROW = 0
PAD = 16
T0_FOLD = (0, 4, 11, 18, 25, 32, 39, 46)
T0_WAITS = ((4, (1,)), (11, ('phi', 2)), (18, (3, 4)), (32, ('x1', 5, 6)), (46, (7,)),
            (73, (8, 9, 10, 11, 'x2', 'x3')))
T0_VPREP = ((73, 74, 75, 76), (77, 78, 79, 80), (81, 82, 83, 84), (85, 86, 87, 88))
T0_VSPAN = 3
T0_LN = (32, 34, 35, 37, 38, 40, 41, 43)
T0_LNSPAN = (0,) * 8
P1_LN = (29, 30, 31, 32, 33, 34, 35, 36)
P1_LNSPAN = 3
P1_WO = (57, 58, 59, 60, 61, 78, 79, 80, 81, 82, 83)
P1_LN2 = ((70, 71, 72, 73, 74, 75, 76, 77), (62, 63, 64, 65, 66, 67, 68, 69))
P1_LNSPAN2 = (3, 3)
T1_LN = ((99, 100, 101, 102, 103, 104, 105, 106), (90, 91, 92, 93, 94, 95, 96, 97))
P1_WOSPAN = 3

FFN_VPU_BLOCKS = 6
FFN_KG = 8
FFN_W0 = 11
FFN_W1 = 110
FFN_SPAN = 3
FFN_TOKALL = 0
FFN_LATE = 16
LATE_AT = (0, 1, 2, 3, 4, 5, 6, 7)
LATE_SPAN = 0
LATE_GATE = 1

_NT = (((1,), (1,)), ((), ()))
_TN = (((0,), (0,)), ((), ()))
f32 = jnp.float32
bf16 = jnp.bfloat16
u32 = jnp.uint32

K_, Q_, V_ = 0, 1, 2
SRC = {K_: 1, Q_: 0, V_: 2}

SEM_W = 0
SEM_X = SEM_W + 3 * NWC
SEM_X0 = SEM_X + N1
SEM_K0 = SEM_X0 + 4
SEM_PHI = SEM_K0 + 4
SEM_WO = SEM_PHI + 2
SEM_WR, SEM_WG, SEM_WU, SEM_WD = (SEM_WO + 4 + i for i in range(4))
SEM_WGV, SEM_WUV = SEM_WD + 1, SEM_WD + 2
SEM_O = SEM_WUV + 1
NSEM = SEM_O + 2 * N2


def _rb(v):
    return v.astype(bf16).astype(f32)


def _unpack(w):
    return pltpu.bitcast(w, bf16)


def _recip(x):
    r = pl.reciprocal(x, approx=True)
    return r * (2.0 - x * r)


def _sigmoid(x):
    return _recip(1.0 + jnp.exp(jnp.minimum(-x, 80.0)))


def _rsqrt(x):
    return lax.rsqrt(x)


def _dual_softmax(p):
    t = p.shape[-1]
    p3 = p.reshape(8, 8, t)

    def allred(v, op):
        v = op(v, pltpu.roll(v, 2, 0))
        return op(v, pltpu.roll(v, 4, 0))

    mx = allred(jnp.max(p3, axis=0), jnp.maximum)
    mn = allred(jnp.min(p3, axis=0), jnp.minimum)
    ep = jnp.exp2(p3 - mx[None])
    en = jnp.exp2(mn[None] - p3)
    sp = allred(jnp.sum(ep, axis=0), jnp.add)
    sn = allred(jnp.sum(en, axis=0), jnp.add)
    fp = (ep * _recip(sp)[None]).reshape(64, t)
    fn = (en * _recip(sn)[None]).reshape(64, t)
    return jnp.concatenate([fp, fn], axis=0).astype(bf16)


def _left_combos(a11, a12, a21, a22):
    return [a11 + a22, a21 + a22, a11, a22, a11 + a12, a21 - a11, a12 - a22]


def _right_combos(b11, b12, b21, b22):
    return [b11 + b22, b11, b12 - b22, b21 - b11, b22, b11 + b12, b21 + b22]


def _strassen(prod, emit):
    m3 = prod(2)
    m5 = prod(4)
    emit(0, 1, m3 + m5)
    m7 = prod(6)
    u = m7 - m5
    m1 = prod(0)
    u = u + m1
    w = m1 + m3
    m4 = prod(3)
    emit(0, 0, u + m4)
    m2 = prod(1)
    emit(1, 0, m2 + m4)
    w = w - m2
    m6 = prod(5)
    emit(1, 1, w + m6)


def _fold_token(w, zero):
    r, c = w.shape
    acc = None
    for i in range(r // 8):
        for j in range(c // 128):
            blk = w[i * 8:(i + 1) * 8, j * 128:(j + 1) * 128]
            acc = blk if acc is None else acc | blk
    return acc & zero


def _body(zs, x_hbm, wqkv_hbm, wphi_hbm, wo_hbm, wr_hbm, wg_hbm, wu_hbm, wd_hbm,
            out_hbm,
            x_v, wqkv_v, wphi_v, wo_v, wr_v, wg_v, wu_v, wd_v, wgv_v, wuv_v,
            wt_v, wo7_v, sa7_v, sb7_v, sc7_v, phiq_v, phik_v, vt0_v, vt1_v, kv_acc, kvt_v, hal_v, har_v, hbl_v, hbr_v, sa_v,
            t0_v, t1_v, t2_v, t3_v, t4_v, t5_v, t6_v, h_v, out_v,
            wrf_v, best_v, besti_v, fix_v, xc0_v, xc1_v, xc2_v, xc3_v, sem):
    xcol_v = (xc0_v, xc1_v, xc2_v, xc3_v)
    s_v = (sa7_v, sb7_v)
    vt_v = (vt0_v, vt1_v)
    ha_v = (hal_v, har_v)
    hb_v = (hbl_v, hbr_v)
    tmp_v = (t0_v, t1_v, t2_v, t3_v, t4_v, t5_v, t6_v)

    def x_rows(r0, rows, slot):
        return pltpu.make_async_copy(
            x_hbm.at[0, pl.ds(r0, rows), :], x_v.at[pl.ds(r0, rows), :], sem.at[slot])

    def x_copy(i):
        return x_rows(i * T1, T1, SEM_X + i)

    def x0_copy(q):
        return x_rows((q % 2) * HT1 + (q // 2) * (HT1 // 2), HT1 // 2, SEM_X0 + q)

    def w_copy(kind, c):
        return pltpu.make_async_copy(
            wqkv_hbm.at[:, pl.ds(SRC[kind] * D + c * WC, WC)],
            wqkv_v.at[kind * NWC + c], sem.at[SEM_W + kind * NWC + c])

    def k0_copy(q):
        r0 = (q % 2) * HD + (q // 2) * 256
        return pltpu.make_async_copy(
            wqkv_hbm.at[pl.ds(r0, 256), pl.ds(SRC[K_] * D, WC)],
            wqkv_v.at[K_ * NWC, pl.ds(r0, 256), :], sem.at[SEM_K0 + q])

    def phi_copy(part):
        lo, n = part * (H // 2), H // 2
        return pltpu.make_async_copy(wphi_hbm.at[pl.ds(lo, n)], wphi_v.at[pl.ds(lo, n)],
                                     sem.at[SEM_PHI + part])

    def full_copy(src, dst, slot):
        return pltpu.make_async_copy(src, dst, sem.at[slot])

    x0_copy(0).start()
    x0_copy(1).start()
    full_copy(wr_hbm, wr_v, SEM_WR).start()
    phi_copy(0).start()
    x0_copy(2).start()
    x0_copy(3).start()
    for q in range(4):
        k0_copy(q).start()
    w_copy(K_, 1).start()
    phi_copy(1).start()
    w_copy(K_, 2).start()
    w_copy(K_, 3).start()
    w_copy(Q_, 0).start()
    x_copy(1).start()
    for c in range(1, NWC):
        w_copy(Q_, c).start()
    for c in range(NWC):
        w_copy(V_, c).start()
    x_copy(2).start()
    x_copy(3).start()
    full_copy(wo_hbm, wo_v.at[pl.ds(0, D), :], SEM_WO).start()
    for i in range(4, N1):
        x_copy(i).start()
    f0 = F - 256 * FFN_VPU_BLOCKS
    ffn_tiled = ((wg_hbm, wg_v, D, SEM_WG), (wu_hbm, wu_v, D, SEM_WU), (wd_hbm, wd_v, F, SEM_WD))
    for src, dst, rows, slot in ffn_tiled:
        for c in range(dst.shape[0]):
            full_copy(src.at[:, pl.ds(c * 128, 128)], dst.at[c, pl.ds(0, rows), :], slot).start()
    full_copy(wg_hbm.at[:, pl.ds(f0, F - f0)], wgv_v, SEM_WGV).start()
    full_copy(wu_hbm.at[:, pl.ds(f0, F - f0)], wuv_v, SEM_WUV).start()

    zero_v = jnp.full((8, 128), zs, jnp.int32).astype(u32)

    def ld(ref, r0, rows, c0, cols):
        return ref[pl.ds(pl.multiple_of(zs * 8 + r0, 8), rows), c0:c0 + cols]

    def tiles(ref, r0, rows, opaque=True):
        w = ref.bitcast(u32)
        if opaque:
            parts = [ld(w.at[c], r0 // 2, rows // 2, 0, 128) for c in range(ref.shape[0])]
        else:
            parts = [w[c, r0 // 2:(r0 + rows) // 2, :] for c in range(ref.shape[0])]
        return jnp.concatenate(parts, axis=1)

    def token(*vals):
        return lambda: _fold_token(pltpu.bitcast(jnp.concatenate(vals, axis=0), u32), zero_v)

    def ln1_stats(xf):
        m = jnp.sum(xf, axis=-1, keepdims=True) * (1.0 / D)
        q = jnp.sum(xf * xf, axis=-1, keepdims=True) * (1.0 / D)
        inv = _rsqrt(jnp.maximum(q - m * m, 0.0) + EPS)
        return inv, m * inv

    def ln1_piece(r0, dst, p, m=None):
        if m is not None:
            x_v[S:S + 8, 0:128] = m[0:8, 0:128].astype(bf16)
        xa, xb = [x_v[pl.ds(pl.multiple_of(r0 + hf * HT1 + p * LN_ROWS, LN_ROWS), LN_ROWS), :]
                  .astype(f32) for hf in range(2)]
        (ia, ma), (ib, mb) = ln1_stats(xa), ln1_stats(xb)
        ya, yb = xa * ia, xb * ib
        s2 = ya[:, :HD] - ma
        s5 = yb[:, HD:] - mb
        s1 = s2 + s5
        s3 = yb[:, :HD] - yb[:, HD:]
        s4 = ya[:, HD:] - ya[:, :HD]
        combos = [s1, s2, s3, s4, s5, s1 + s3, s1 + s4]
        for i in range(7):
            for c in range(4):
                dst[i, c, p * LN_ROWS:(p + 1) * LN_ROWS, :] = (
                    combos[i][:, c * 128:(c + 1) * 128].astype(bf16))
        return token(combos[5], combos[6])

    def fold_piece(kind, c, j, pt):
        blk = {}
        for hh in range(2):
            for kh in range(2):
                k0 = kh * HD + j * 128
                w = wqkv_v[kind * NWC + c, k0:k0 + 128, hh * 128:(hh + 1) * 128]
                blk[hh, kh] = lax.dot_general(pt[2 * c + hh], w, _NT,
                                              preferred_element_type=f32) * LOG2E
        combos = _left_combos(blk[0, 0], blk[0, 1], blk[1, 0], blk[1, 1])
        r0 = kind * HD + c * 128
        for i in range(7):
            wt_v[i, j, r0:r0 + 128, :] = combos[i].astype(bf16)

    def fold_chunk(kind, c, pt):
        for j in range(4):
            fold_piece(kind, c, j, pt)

    def vprep_piece(c, j, m):
        wqkv_v[3 * NWC, 0:8, 0:128] = m[0:8, 0:128].astype(bf16)
        blk = {}
        for hh in range(2):
            for kh in range(2):
                k0 = kh * HD + j * 128
                w = wqkv_v[zs + V_ * NWC + c, k0:k0 + 128, hh * 128:(hh + 1) * 128]
                blk[hh, kh] = w.T.astype(f32)
        combos = _left_combos(blk[0, 0], blk[0, 1], blk[1, 0], blk[1, 1])
        r0 = V_ * HD + c * 128
        for i in range(7):
            wt_v[i, j, r0:r0 + 128, :] = combos[i].astype(bf16)
        return token(combos[1], combos[4])

    def wo_piece(w0, m):
        wo_v[D:D + 8, 0:128] = m[0:8, 0:128].astype(bf16)
        top = wo_v[pl.ds(pl.multiple_of(w0, 16), 16), :].astype(f32)
        bot = wo_v[pl.ds(pl.multiple_of(HD + w0, 16), 16), :].astype(f32)
        combos = _right_combos(top[:, :HD], top[:, HD:], bot[:, :HD], bot[:, HD:])
        for i in range(7):
            for c in range(4):
                wo7_v[i, c, pl.ds(pl.multiple_of(w0, 16), 16), :] = (
                    combos[i][:, c * 128:(c + 1) * 128].astype(bf16))
        return token(combos[5], combos[6])

    def run_rounds(t0, rounds, post, first):
        count = [0]
        pins = {}

        def pinned(w):
            toks = pins.get(count[0])
            if not toks:
                return w
            top = w[0:8, 0:128]
            for tk in toks:
                top = top | tk
            return jnp.concatenate(
                [jnp.concatenate([top, w[0:8, 128:]], axis=1), w[8:]], axis=0)

        def run_jobs(m):
            for fn, span in post.get(count[0], ()):
                tok = fn(m)
                if span:
                    pins.setdefault(count[0] + span, []).append(tok())
            count[0] += 1

        for par, kind, cs in rounds:
            r0 = kind * HD + cs[0] * 128
            rows = 128 * len(cs)

            def prod(i):
                if (par, kind) == (1, V_):
                    rhs = ld(sc7_v.at[i], 0, HT1 // 2, 0, HD)
                else:
                    rhs = tiles(s_v[par].at[i], 0, HT1)
                if (par, kind, cs[0]) == (1, K_, 0):
                    sc7_v[i] = rhs
                m = lax.dot_general(_unpack(tiles(wt_v.at[i], r0, rows, False)),
                                    _unpack(pinned(rhs)),
                                    _NT, preferred_element_type=f32)
                run_jobs(m)
                return m

            def emit(rh, ch, blk):
                tb = 2 * par + ch
                for n, c in enumerate(cs):
                    for jj in range(2):
                        pair = 4 * c + 2 * rh + jj
                        p = blk[n * 128 + jj * 64:n * 128 + (jj + 1) * 64]
                        if kind == K_:
                            phik_v[tb, pair * 128:(pair + 1) * 128, :] = _dual_softmax(p)
                        elif kind == Q_:
                            phiq_v[t0 // 2, tb, pair * 128:(pair + 1) * 128, :] = (
                                _dual_softmax(p))
                        else:
                            vt_v[pair // 8][tb, (pair % 8) * 64:(pair % 8 + 1) * 64, :] = (
                                p.astype(bf16))

            _strassen(prod, emit)

        ones = jnp.full((8, 2 * T1), 0x3F803F80, u32)
        kr = lax.broadcasted_iota(jnp.int32, (80, 128), 0)
        kc = lax.broadcasted_iota(jnp.int32, (80, 128), 1)
        kmask = jnp.where(kr < 64, kr // 32, (kr - 64) // 8) == kc % 2
        for j in range(NP):
            lhs = jnp.concatenate([tiles(vt_v[j // 8], (j % 8) * 64, 64), ones], axis=0)
            rhs = tiles(phik_v, j * 128, 128)
            upd = lax.dot_general(_unpack(lhs), _unpack(pinned(rhs)), _NT,
                                  preferred_element_type=f32)
            run_jobs(upd)
            if first:
                kv_acc[j] = upd
            else:
                upd = kv_acc[j] + upd
                kv_acc[j] = upd
                kvt_v[j] = jnp.where(kmask, upd, 0.0).astype(bf16)

    def load_best():
        return best_v[0], besti_v[...], best_v[1], best_v[2]

    def store_best(best):
        best_v[0], besti_v[...], best_v[1], best_v[2] = best

    def build_pt(g0, g1):
        n = g1 - g0
        w2 = wphi_v[4 * g0:4 * g1].reshape(n * 128, DH)
        er = lax.broadcasted_iota(jnp.int32, (128, DH), 0)
        ec = lax.broadcasted_iota(jnp.int32, (128, DH), 1)
        e = jnp.where(ec == (er % 64) // 2, 1.0, 0.0).astype(bf16)
        ptf = lax.dot_general(e, w2, _NT, preferred_element_type=f32)
        pr = lax.broadcasted_iota(jnp.int32, (128, 128), 0)
        pc = lax.broadcasted_iota(jnp.int32, (128, 128), 1)
        keep = pc // 32 == (pr // 64) * 2 + pr % 2
        return [jnp.where(keep, ptf[:, g * 128:(g + 1) * 128], 0.0).astype(bf16)
                for g in range(n)]

    hbl_v[...] = jnp.zeros_like(hbl_v)
    hbr_v[...] = jnp.zeros_like(hbr_v)
    store_best((jnp.full((8, 128), -jnp.inf, f32), jnp.zeros((8, 128), jnp.int32),
                jnp.zeros((8, 128), f32), jnp.zeros((8, 128), f32)))
    n_ln = HT1 // LN_ROWS
    x0_copy(0).wait()
    x0_copy(1).wait()
    for p in range(n_ln // 2):
        ln1_piece(0, s_v[0], p)
    full_copy(wr_hbm, wr_v, SEM_WR).wait()
    phi_copy(0).wait()
    x0_copy(2).wait()
    x0_copy(3).wait()
    wr_row = wr_v[...].astype(f32).reshape(1, D)
    wrf_v[...] = jnp.broadcast_to(
        wr_row - jnp.sum(wr_row, axis=-1, keepdims=True) * (1.0 / D), (8, D))
    pt = build_pt(0, 4)
    for p in range(n_ln // 2, n_ln):
        ln1_piece(0, s_v[0], p)
    for part in range(2):
        k0_copy(2 * part).wait()
        k0_copy(2 * part + 1).wait()
        fold_piece(K_, 0, 2 * part, pt)
        fold_piece(K_, 0, 2 * part + 1, pt)

    post = {}

    def at(slot, fn, span=0):
        post.setdefault(slot, []).append((fn, span))

    for slot, copies in T0_WAITS:
        for cp in copies:
            if cp == 'phi':
                at(slot, lambda m: phi_copy(1).wait())
            elif cp in ('x1', 'x2', 'x3'):
                at(slot, lambda m, cp=cp: x_copy(int(cp[1])).wait())
            else:
                at(slot, lambda m, cp=cp: w_copy(cp // NWC, cp % NWC).wait())
    for n in range(1, 2 * NWC):
        if n == 2:
            at(T0_FOLD[n], lambda m: pt.extend(build_pt(4, 8)))
        at(T0_FOLD[n], lambda m, n=n: fold_chunk(n // NWC, n % NWC, pt))
    for c in range(NWC):
        for j in range(4):
            at(T0_VPREP[c][j], lambda m, c=c, j=j: vprep_piece(c, j, m), T0_VSPAN)
    for p in range(n_ln):
        at(T0_LN[p], lambda m, p=p: ln1_piece(zs + T1, s_v[1], p, m), T0_LNSPAN[p])
    for p in range(n_ln):
        at(T1_LN[0][p], lambda m, p=p: ln1_piece(zs + 2 * T1, s_v[0], p, m), P1_LNSPAN)
        at(T1_LN[1][p], lambda m, p=p: ln1_piece(zs + 3 * T1, s_v[1], p, m), P1_LNSPAN)
    lo, hi = [0, 1], [2, 3]
    run_rounds(0, [(0, kind, [c]) for kind in (K_, Q_) for c in range(NWC)]
               + [(1, K_, lo), (1, K_, hi), (1, Q_, lo), (1, Q_, hi),
                  (0, V_, lo), (0, V_, hi), (1, V_, lo), (1, V_, hi)], post, True)
    full_copy(wo_hbm, wo_v.at[pl.ds(0, D), :], SEM_WO).wait()
    for i in range(4, N1):
        x_copy(i).wait()

    def phase1(i, carry):
        post = {}
        nxt = jnp.minimum(i + 1, N2 - 1) * T2
        w0 = jnp.minimum((i - 1) * WO_ROWS, HD - WO_ROWS)
        for par in range(2):
            for p in range(n_ln):
                post.setdefault(P1_LN2[par][p], []).append(
                    (lambda m, p=p, par=par: ln1_piece(nxt + par * T1, s_v[par], p, m),
                     P1_LNSPAN2[par]))
        for p in range(WO_ROWS // 16):
            post.setdefault(P1_WO[p], []).append(
                (lambda m, p=p: wo_piece(w0 + 16 * p, m), P1_WOSPAN))
        run_rounds(2 * i, [(par, kind, cs) for kind in (K_, Q_, V_) for par in range(2)
                           for cs in ([0, 1], [2, 3])], post, False)
        return carry

    lax.fori_loop(1, N1 // 2, phase1, 0)

    for _, dst, rows, slot in ffn_tiled:
        filled = dst.at[:, pl.ds(0, rows), :]
        full_copy(filled, filled, slot).wait()
    full_copy(wg_hbm.at[:, pl.ds(f0, F - f0)], wgv_v, SEM_WGV).wait()
    full_copy(wu_hbm.at[:, pl.ds(f0, F - f0)], wuv_v, SEM_WUV).wait()

    def o_copy(hf):
        return pltpu.make_async_copy(
            out_v.at[pl.ds(hf * HT2, HT2), :], out_hbm.at[0, pl.ds(hf * HT2, HT2), :],
            sem.at[SEM_O + hf])

    def half_stats(hh, c0):
        rows = hh.shape[0]
        parts = [hh[:, c * 128:(c + 1) * 128] for c in range(4)]
        wts = [wrf_v[:, c0 + c * 128:c0 + (c + 1) * 128] for c in range(4)]
        s1 = (parts[0] + parts[1]) + (parts[2] + parts[3])
        sq = [p * p for p in parts]
        s2 = (sq[0] + sq[1]) + (sq[2] + sq[3])
        dw = [(p.reshape(rows // 8, 8, 128) * w[None]).reshape(rows, 128)
              for p, w in zip(parts, wts)]
        s3 = (dw[0] + dw[1]) + (dw[2] + dw[3])
        return s1, s2, s3

    def first_half(hbuf, sbuf, base, p, c0):
        r0 = p * EP_ROWS
        hh = ld(hbuf[c0 // HD], r0, EP_ROWS, 0, HD)
        h_v[pl.ds(pl.multiple_of(base + r0, EP_ROWS), EP_ROWS), c0:c0 + HD] = hh.astype(bf16)
        st = jnp.concatenate(half_stats(hh, c0), axis=1)
        sbuf[r0:r0 + EP_ROWS, :] = st
        return _fold_token(pltpu.bitcast(st, u32), zero_v)

    def finish(hbuf, sbuf, base, p, valid, best, defer=None):
        r0 = p * EP_ROWS
        g0 = pl.multiple_of(base + r0, EP_ROWS)
        hl, hr = [ld(r, r0, EP_ROWS, 0, HD) for r in hbuf]
        if defer is None:
            h_v[pl.ds(g0, EP_ROWS), 0:HD] = hl.astype(bf16)
        if sbuf is None:
            if defer is None:
                h_v[pl.ds(g0, EP_ROWS), HD:D] = hr.astype(bf16)
            st = half_stats(hr, HD)
        else:
            st = ld(sbuf, r0, EP_ROWS, 0, 384)
            st = [st[:, n * 128:(n + 1) * 128] for n in range(3)]
        s1, s2, s3 = [jnp.sum(v + w, axis=-1, keepdims=True)
                      for v, w in zip(half_stats(hl, 0), st)]
        m = s1 * (1.0 / D)
        var = jnp.maximum(s2 * (1.0 / D) - m * m, 0.0)
        inv = _rsqrt(var + EPS)
        r = s3 * inv

        def write_out(h):
            o = h * (1.0 + inv) - m * inv
            out_v[pl.ds(g0, EP_ROWS), :] = o.astype(bf16)
            return o

        if defer is None:
            o = write_out(jnp.concatenate([hl, hr], axis=1))
        else:
            defer.append(lambda: write_out(jnp.concatenate(
                [ld(r_, r0, EP_ROWS, 0, HD) for r_ in hbuf], axis=1)))
        bv, bi, bm, bq = best
        sub = lax.broadcasted_iota(jnp.int32, (8, 128), 0)
        for g in range(EP_ROWS // 8):
            rows = slice(g * 8, (g + 1) * 8)
            rg = jnp.broadcast_to(r[rows], (8, 128))
            if valid is not None:
                rg = jnp.where(valid, rg, -jnp.inf)
            better = rg > bv
            bi = jnp.where(better, sub + (g0 + g * 8), bi)
            bv = jnp.where(better, rg, bv)
            bm = jnp.where(better, jnp.broadcast_to(m[rows], (8, 128)), bm)
            bq = jnp.where(better, jnp.broadcast_to(var[rows], (8, 128)), bq)
        best = (bv, bi, bm, bq)
        if defer is not None:
            return best, None
        tok = _fold_token(pltpu.bitcast(jnp.concatenate(
            [o[:, D - 128:], bv, bm, bq], axis=0), u32), zero_v)
        return best, tok

    n_ep = HT2 // EP_ROWS

    def phase2(i, carry):
        ot = []
        for j in range(NP):
            ph = tiles(phiq_v.at[i], j * 128, 128, False)
            n = jnp.dot(_unpack(kvt_v.bitcast(u32)[j]), _unpack(ph),
                        preferred_element_type=f32)
            r0h = _recip(n[64:72] + 1e-6)
            r1h = _recip(n[72:80] + 1e-6)
            ot.append((n[0:32].reshape(4, 8, T2) * r0h[None]).reshape(32, T2))
            ot.append((n[32:64].reshape(4, 8, T2) * r1h[None]).reshape(32, T2))
        lo = jnp.concatenate(ot[:H // 2], axis=0)
        hi = jnp.concatenate(ot[H // 2:], axis=0)
        lcs = _left_combos(lo[:, :HT2], hi[:, :HT2], lo[:, HT2:], hi[:, HT2:])

        state = {'best': load_best()}
        pins = {}
        jobs = {}
        lts = {}
        ra = pl.multiple_of(i * T2, T2)
        rb = pl.multiple_of(i * T2 + HT2, HT2)
        prev = jnp.maximum(i * T2 - HT2, HT2)

        def add_job(slot, deadline, fn, gates=()):
            jobs.setdefault(slot, []).append((fn, deadline, gates))

        def finish_job(hbuf, sbuf, base, p, valid):
            def fn():
                state['best'], tok = finish(hbuf, sbuf, base, p, valid, state['best'])
                return tok
            return fn

        def lt_job(k):
            def fn():
                lts[k] = lcs[k].astype(bf16).T
                return _fold_token(pltpu.bitcast(lts[k], u32), zero_v)
            return fn

        order = (2, 4, 6, 0, 3, 1, 5)
        lt_job(2)()
        for n in range(1, 7):
            add_job(LT_START[n], LT_DEADLINE[n], lt_job(order[n]))
        for p in range(n_ep):
            add_job(FB_START[p], FB_START[p] + 2, finish_job(hb_v, None, prev, p, i > 0), hb_v)
            add_job(SA_START[p], SA_START[p] + 2, lambda p=p: first_half(ha_v, sa_v, ra, p, HD), ha_v[1:])
            add_job(FA_START[p], FA_DEADLINE[p], finish_job(ha_v, sa_v, ra, p, None), ha_v)

        def xblk(r0, c0):
            return x_v[pl.ds(r0, HT2), c0:c0 + 128].astype(f32)

        for n, k in enumerate(order):
            for c in range(4):
                slot = 4 * n + c
                for fn, deadline, gates in jobs.get(slot, ()):
                    for ref in gates:
                        ref[HT2:HT2 + 8, 0:128] = mm[GATE_ROW:GATE_ROW + 8]
                    pins.setdefault(deadline, []).append(fn())
                w = wo7_v.bitcast(u32)[k, c, 0:HD // 2, :]
                toks = pins.get(slot)
                if toks:
                    top = w[0:8]
                    for tk in toks:
                        top = top | tk
                    w = jnp.concatenate([top, w[8:]], axis=0)
                mm = jnp.dot(lts[k], _unpack(w), preferred_element_type=f32)
                c0 = c * 128
                cs = slice(c0, c0 + 128)
                tmp = lambda t: ld(tmp_v[t], 0, HT2, c0, 128)
                if n == 0:
                    tmp_v[0][:, cs] = mm
                elif n == 1:
                    ha_v[1][0:HT2, cs] = (xblk(ra, HD + c0) + tmp(0)) + mm
                    tmp_v[1][:, cs] = xblk(ra, c0) - mm
                elif n == 2:
                    tmp_v[2][:, cs] = tmp(1) + mm
                elif n == 3:
                    tmp_v[3][:, cs] = tmp(2) + mm
                    tmp_v[4][:, cs] = (xblk(rb, HD + c0) + tmp(0)) + mm
                elif n == 4:
                    ha_v[0][0:HT2, cs] = tmp(3) + mm
                    tmp_v[5][:, cs] = xblk(rb, c0) + mm
                elif n == 5:
                    hb_v[0][0:HT2, cs] = tmp(5) + mm
                    tmp_v[6][:, cs] = tmp(4) - mm
                else:
                    hb_v[1][0:HT2, cs] = tmp(6) + mm
        store_best(state['best'])
        o_copy(2 * i).start()

        @pl.when(i > 0)
        def _():
            o_copy(2 * i - 1).start()

        return carry

    lax.fori_loop(0, N2, phase2, 0)
    best = load_best()
    late = []
    for p in range(n_ep):
        best, _ = finish(hb_v, None, S - HT2, p, None, best, late)


    bv, bi, bm, bq = best
    for sh in (4, 2, 1):
        ov, oi, om, oq = [pltpu.roll(t, sh, 0) for t in (bv, bi, bm, bq)]
        take = jnp.logical_or(ov > bv, jnp.logical_and(ov == bv, oi < bi))
        bv, bi, bm, bq = [jnp.where(take, o_, t)
                          for o_, t in zip((ov, oi, om, oq), (bv, bi, bm, bq))]
    idx = jnp.clip(bi[0, 0], 0, S - 1)
    b0 = pl.multiple_of((idx // 8) * 8, 8)
    t = _rb(_rb(bq) + EPS)
    inv = _recip(_rb(t * _rsqrt(t)))
    gate = _sigmoid(bv)
    wide = lambda v: jnp.concatenate([v] * (D // 128), axis=1)
    b1 = pl.multiple_of(jnp.minimum(b0, S - HT2 - 8), 8)
    b2 = pl.multiple_of(jnp.maximum(b0 - (S - HT2), 0), 8)
    hb = jnp.where(wide(bi) < S - HT2, h_v[pl.ds(b1, 8), :].astype(f32),
                   _rb(jnp.concatenate([r_[pl.ds(b2, 8), :] for r_ in hb_v], axis=1)))
    hn = (hb - wide(bm)) * wide(inv)
    xs = hn.astype(bf16)
    rows = lax.broadcasted_iota(jnp.int32, (8, D), 0) + b0

    xm = jnp.where(rows == wide(bi), _rb(hn), 0.0)
    for sh in (4, 2, 1):
        xm = xm + pltpu.roll(xm, sh, 0)
    for t in range(D // 128):
        xcol_v[t // 2][(t % 2) * 128:(t % 2 + 1) * 128, :] = jnp.concatenate(
            [xm[:, t * 128:(t + 1) * 128]] * 16, axis=0).T

    nblk = F // 256
    nmx = nblk - FFN_VPU_BLOCKS
    act = {}
    acc = {}

    def activate(g, u):
        return (g * _sigmoid(g) * u).astype(bf16)

    parts = D // 8 // FFN_KG

    def vpu_chunk(q):
        blk, part = nmx + q // parts, q % parts
        cur = acc.get(blk)
        for kg in range(part * FFN_KG, (part + 1) * FFN_KG):
            xc = ld(xcol_v[kg // 32], (kg % 32) * 8, 8, 0, 128)
            w = jnp.concatenate(
                [r[kg * 8:(kg + 1) * 8, (blk - nmx) * 256:(blk - nmx + 1) * 256].astype(f32)
                 for r in (wgv_v, wuv_v)], axis=1)
            p = w * jnp.concatenate([xc] * 4, axis=1)
            cur = p if cur is None else cur + p
        acc[blk] = cur
        if part == parts - 1:
            for sh in (4, 2, 1):
                cur = cur + pltpu.roll(cur, sh, 0)
            act[blk] = activate(cur[:, :256], cur[:, 256:])
        if FFN_TOKALL:
            return _fold_token(pltpu.bitcast(cur, u32), zero_v)
        c = q % 4
        return _fold_token(pltpu.bitcast(cur[:, c * 128:(c + 1) * 128], u32), zero_v)

    nchunk = FFN_VPU_BLOCKS * parts
    starts = [FFN_W0 + (q * (FFN_W1 - FFN_W0)) // (nchunk - 1) for q in range(nchunk)]
    pins = {}
    xs16 = jnp.zeros((16, 256), bf16)
    wave = [0]
    wgw, wuw, wdw = [r.bitcast(u32) for r in (wg_v, wu_v, wd_v)]

    def run_wave(lhs, tls):
        top = tls[0][0:8]
        for tk in pins.get(wave[0], ()):
            top = top | tk
        w = jnp.concatenate([jnp.concatenate([top, tls[0][8:]], axis=0)] + tls[1:], axis=1)
        out = jnp.dot(lhs, _unpack(w), preferred_element_type=f32)
        for p, fn in enumerate(late):
            if LATE_AT[p] == wave[0]:
                for r_ in hb_v:
                    r_[HT2:HT2 + 8, 0:128] = out[:, 0:128] if LATE_GATE else hn[:, 0:128]
                tk = token(fn()[:, D - 128:])
                if LATE_SPAN:
                    pins.setdefault(wave[0] + LATE_SPAN, []).append(tk())
        for q, start in enumerate(starts):
            if start == wave[0]:
                pins.setdefault(wave[0] + FFN_SPAN, []).append(vpu_chunk(q))
        if wave[0] == FFN_LATE:
            o_copy(2 * N2 - 1).start()
            out_v[pl.ds(pl.multiple_of(zs * 16 + S, 16), 16), 0:256] = xs16
            pins.setdefault(wave[0] + 4, []).append(
                token(out_v[S:S + 8, 0:128].astype(f32))())
        wave[0] += 1
        return out

    for j in range(nmx):
        gu = None
        for kt in range(D // 128):
            p = run_wave(xs[:, kt * 128:(kt + 1) * 128],
                         [r[2 * j + c, kt * 64:(kt + 1) * 64, :]
                          for r in (wgw, wuw) for c in range(2)])
            gu = p if gu is None else gu + p
        act[j] = activate(gu[:, :256], gu[:, 256:])
    ys = [None, None]
    for j in range(nblk):
        for kt in range(2):
            for hf in range(2):
                r0 = (2 * j + kt) * 64
                p = run_wave(act[j][:, kt * 128:(kt + 1) * 128],
                             [wdw[4 * hf + c, r0:r0 + 64, :] for c in range(4)])
                ys[hf] = p if ys[hf] is None else ys[hf] + p
    y = jnp.concatenate(ys, axis=1)
    cur = out_v[pl.ds(b0, 8), :].astype(f32)
    fix_v[...] = jnp.where(rows == wide(bi), hb + hn + y * wide(gate), cur).astype(bf16)
    for hf in range(2 * N2):
        o_copy(hf).wait()
    fix = pltpu.make_async_copy(fix_v, out_hbm.at[0, pl.ds(b0, 8), :], sem.at[SEM_O])
    fix.start()
    fix.wait()


def _kernel(*refs):
    def step(i, carry):
        @pl.when(i == 0)
        def _():
            _body(i, *refs)

        return carry

    lax.fori_loop(0, 2, step, 0)


@jax.jit
def pallas_sequential_preLN__linear_kernel_hedgehog__moe_arch_mod__prompt_kernel(
    A_x: jax.Array,
    A_wqkv: jax.Array,
    A_w_phi: jax.Array,
    A_wo: jax.Array,
    B_x: jax.Array,
    B_w_r: jax.Array,
    B_w_gate: jax.Array,
    B_w_up: jax.Array,
    B_w_down: jax.Array,
):
    any_spec = pl.BlockSpec(memory_space=pl.ANY)
    return pl.pallas_call(
        _kernel,
        out_shape=jax.ShapeDtypeStruct((1, S, D), bf16),
        in_specs=[any_spec] * 8,
        out_specs=any_spec,
        scratch_shapes=[
            pltpu.VMEM((S + 16, D), bf16),
            pltpu.VMEM((3 * NWC + 1, D, WC), bf16),
            pltpu.VMEM((H, DH, DH), bf16),
            pltpu.VMEM((D + 16, D), bf16),
            pltpu.VMEM((D,), bf16),
            pltpu.VMEM((F // 128 - 2 * FFN_VPU_BLOCKS, D + PAD, 128), bf16),
            pltpu.VMEM((F // 128 - 2 * FFN_VPU_BLOCKS, D + PAD, 128), bf16),
            pltpu.VMEM((D // 128, F + PAD, 128), bf16),
            pltpu.VMEM((D, 256 * FFN_VPU_BLOCKS), bf16),
            pltpu.VMEM((D, 256 * FFN_VPU_BLOCKS), bf16),
            pltpu.VMEM((7, 4, 3 * HD + PAD, 128), bf16),
            pltpu.VMEM((7, 4, HD + PAD, 128), bf16),
            pltpu.VMEM((7, 4, HT1 + PAD, 128), bf16),
            pltpu.VMEM((7, 4, HT1 + PAD, 128), bf16),
            pltpu.VMEM((7, HT1 // 2, HD), u32),
            pltpu.VMEM((N2, 4, 2 * D + PAD, 128), bf16),
            pltpu.VMEM((4, 2 * D + PAD, 128), bf16),
            pltpu.VMEM((4, HD + PAD, 128), bf16),
            pltpu.VMEM((4, HD + PAD, 128), bf16),
            pltpu.VMEM((NP, 80, 128), f32),
            pltpu.VMEM((NP, 80, 128), bf16),
            *[pltpu.VMEM((HT2 + 8, HD), f32) for _ in range(4)],
            pltpu.VMEM((HT2, 384), f32),
            *[pltpu.VMEM((HT2, HD), f32) for _ in range(7)],
            pltpu.VMEM((S, D), bf16),
            pltpu.VMEM((S + 16, D), bf16),
            pltpu.VMEM((8, D), f32),
            pltpu.VMEM((3, 8, 128), f32),
            pltpu.VMEM((8, 128), jnp.int32),
            pltpu.VMEM((8, D), bf16),
            *[pltpu.VMEM((264, 128), f32) for _ in range(4)],
            pltpu.SemaphoreType.DMA((NSEM,)),
        ],
        compiler_params=pltpu.CompilerParams(
            vmem_limit_bytes=110 * 1024 * 1024,
            disable_bounds_checks=True,
            disable_semaphore_checks=True),
    )(A_x, A_wqkv, A_w_phi, A_wo, B_w_r, B_w_gate, B_w_up, B_w_down)
```

```python
import jax
import jax.numpy as jnp
from jax import lax
import jax.experimental.pallas as pl
import jax.experimental.pallas.tpu as pltpu

S = 2048
D = 1024
H = 32
DH = 32
F = 3584
NP = H // 2
T1 = 256
T2 = 512
N1 = S // T1
N2 = S // T2
HT1 = T1 // 2
HT2 = T2 // 2
HD = D // 2
WC = 256
NWC = D // WC
LOG2E = 1.4426950408889634
EPS = 1e-5
WO_ROWS = 176
LN_ROWS = 16
EP_ROWS = 32
LT_START = (0, 0, 1, 5, 8, 11, 14)
LT_SPAN = (0, 2, 4, 4, 4, 4, 4)
FB_START = (2, 4, 6, 8, 10, 12, 14, 16)
SA_START = (9, 11, 15, 15, 17, 17, 18, 18)
FA_START = (20, 21, 22, 23, 24, 25, 26, 27)
FA_SPAN = (3, 7, 2, 5, 3, 5, 3, 2)
FB_SPAN = 2
SA_SPAN = 3
GATE_ROW = 0
PAD = 16
T0_FOLD = (0, 4, 11, 18, 25, 32, 39, 46)
T0_WAITS = ((4, (1,)), (11, ('phi', 2)), (18, (3, 4)), (32, ('x1', 5, 6)), (46, (7,)),
            (73, (8, 9, 10, 11, 'x2', 'x3')))
T0_VPREP = ((73, 74, 75, 76), (77, 78, 79, 80), (81, 82, 83, 84), (85, 86, 87, 88))
T0_VSPAN = 4
T0_LN = (32, 35, 36, 37, 38, 39, 40, 43)
T0_LNSPAN = (3, 0, 0, 0, 0, 0, 0, 0)
P1_LN = (29, 30, 31, 32, 33, 34, 35, 36)
P1_LNSPAN = 3
P1_WO = (57, 58, 59, 60, 63, 77, 79, 80, 81, 82, 83)
P1_LN2 = ((70, 71, 72, 73, 74, 75, 76, 77), (62, 63, 64, 65, 66, 67, 68, 69))
P1_LNSPAN2 = (2, 2)
T1_LN = ((99, 100, 101, 102, 103, 104, 105, 106), (90, 91, 92, 93, 94, 95, 96, 97))
P1_WOSPAN = 3

FFN_VPU_BLOCKS = 7
FFN_KG = 16
FFN_W0 = 18
FFN_W1 = 107
FFN_SPAN = 4
FFN_TOKALL = 0
FFN_LATE = 16
LATE_AT = (1, 2, 3, 3, 4, 6, 6, 7)
LATE_SPAN = 0
LATE_GATE = 1

_NT = (((1,), (1,)), ((), ()))
_TN = (((0,), (0,)), ((), ()))
f32 = jnp.float32
bf16 = jnp.bfloat16
u32 = jnp.uint32

K_, Q_, V_ = 0, 1, 2
SRC = {K_: 1, Q_: 0, V_: 2}

SEM_W = 0
SEM_X = SEM_W + 3 * NWC
SEM_X0 = SEM_X + N1
SEM_K0 = SEM_X0 + 4
SEM_PHI = SEM_K0 + 4
SEM_WO = SEM_PHI + 2
SEM_WR, SEM_WG, SEM_WU, SEM_WD = (SEM_WO + 4 + i for i in range(4))
SEM_WGV, SEM_WUV = SEM_WD + 1, SEM_WD + 2
SEM_O = SEM_WUV + 1
NSEM = SEM_O + 2 * N2


def _rb(v):
    return v.astype(bf16).astype(f32)


def _unpack(w):
    return pltpu.bitcast(w, bf16)


def _recip(x):
    r = pl.reciprocal(x, approx=True)
    return r * (2.0 - x * r)


def _sigmoid(x):
    return _recip(1.0 + jnp.exp(jnp.minimum(-x, 80.0)))


def _rsqrt(x):
    return lax.rsqrt(x)


def _dual_softmax(p):
    t = p.shape[-1]
    p3 = p.reshape(8, 8, t)

    def allred(v, op):
        v = op(v, pltpu.roll(v, 2, 0))
        return op(v, pltpu.roll(v, 4, 0))

    mx = allred(jnp.max(p3, axis=0), jnp.maximum)
    mn = allred(jnp.min(p3, axis=0), jnp.minimum)
    ep = jnp.exp2(p3 - mx[None])
    en = jnp.exp2(mn[None] - p3)
    sp = allred(jnp.sum(ep, axis=0), jnp.add)
    sn = allred(jnp.sum(en, axis=0), jnp.add)
    fp = (ep * _recip(sp)[None]).reshape(64, t)
    fn = (en * _recip(sn)[None]).reshape(64, t)
    return jnp.concatenate([fp, fn], axis=0).astype(bf16)


def _left_combos(a11, a12, a21, a22):
    return [a11 + a22, a21 + a22, a11, a22, a11 + a12, a21 - a11, a12 - a22]


def _right_combos(b11, b12, b21, b22):
    return [b11 + b22, b11, b12 - b22, b21 - b11, b22, b11 + b12, b21 + b22]


def _strassen(prod, emit):
    m3 = prod(2)
    m5 = prod(4)
    emit(0, 1, m3 + m5)
    m7 = prod(6)
    u = m7 - m5
    m1 = prod(0)
    u = u + m1
    w = m1 + m3
    m4 = prod(3)
    emit(0, 0, u + m4)
    m2 = prod(1)
    emit(1, 0, m2 + m4)
    w = w - m2
    m6 = prod(5)
    emit(1, 1, w + m6)


def _fold_token(w, zero):
    r, c = w.shape
    acc = None
    for i in range(r // 8):
        for j in range(c // 128):
            blk = w[i * 8:(i + 1) * 8, j * 128:(j + 1) * 128]
            acc = blk if acc is None else acc | blk
    return acc & zero


def _body(zs, x_hbm, wqkv_hbm, wphi_hbm, wo_hbm, wr_hbm, wg_hbm, wu_hbm, wd_hbm,
            out_hbm,
            x_v, wqkv_v, wphi_v, wo_v, wr_v, wg_v, wu_v, wd_v, wgv_v, wuv_v,
            wt_v, wo7_v, sa7_v, sb7_v, sc7_v, phiq_v, phik_v, vt0_v, vt1_v, kv_acc, kvt_v, hal_v, har_v, hbl_v, hbr_v, sa_v,
            t0_v, t1_v, t2_v, t3_v, t4_v, t5_v, t6_v, h_v, out_v,
            wrf_v, best_v, besti_v, fix_v, xc0_v, xc1_v, xc2_v, xc3_v, sem):
    xcol_v = (xc0_v, xc1_v, xc2_v, xc3_v)
    s_v = (sa7_v, sb7_v)
    vt_v = (vt0_v, vt1_v)
    ha_v = (hal_v, har_v)
    hb_v = (hbl_v, hbr_v)
    tmp_v = (t0_v, t1_v, t2_v, t3_v, t4_v, t5_v, t6_v)

    def x_rows(r0, rows, slot):
        return pltpu.make_async_copy(
            x_hbm.at[0, pl.ds(r0, rows), :], x_v.at[pl.ds(r0, rows), :], sem.at[slot])

    def x_copy(i):
        return x_rows(i * T1, T1, SEM_X + i)

    def x0_copy(q):
        return x_rows((q % 2) * HT1 + (q // 2) * (HT1 // 2), HT1 // 2, SEM_X0 + q)

    def w_copy(kind, c):
        return pltpu.make_async_copy(
            wqkv_hbm.at[:, pl.ds(SRC[kind] * D + c * WC, WC)],
            wqkv_v.at[kind * NWC + c], sem.at[SEM_W + kind * NWC + c])

    def k0_copy(q):
        r0 = (q % 2) * HD + (q // 2) * 256
        return pltpu.make_async_copy(
            wqkv_hbm.at[pl.ds(r0, 256), pl.ds(SRC[K_] * D, WC)],
            wqkv_v.at[K_ * NWC, pl.ds(r0, 256), :], sem.at[SEM_K0 + q])

    def phi_copy(part):
        lo, n = part * (H // 2), H // 2
        return pltpu.make_async_copy(wphi_hbm.at[pl.ds(lo, n)], wphi_v.at[pl.ds(lo, n)],
                                     sem.at[SEM_PHI + part])

    def full_copy(src, dst, slot):
        return pltpu.make_async_copy(src, dst, sem.at[slot])

    x0_copy(0).start()
    x0_copy(1).start()
    full_copy(wr_hbm, wr_v, SEM_WR).start()
    phi_copy(0).start()
    x0_copy(2).start()
    x0_copy(3).start()
    for q in range(4):
        k0_copy(q).start()
    w_copy(K_, 1).start()
    phi_copy(1).start()
    w_copy(K_, 2).start()
    w_copy(K_, 3).start()
    w_copy(Q_, 0).start()
    x_copy(1).start()
    for c in range(1, NWC):
        w_copy(Q_, c).start()
    for c in range(NWC):
        w_copy(V_, c).start()
    x_copy(2).start()
    x_copy(3).start()
    full_copy(wo_hbm, wo_v.at[pl.ds(0, D), :], SEM_WO).start()
    for i in range(4, N1):
        x_copy(i).start()
    f0 = F - 256 * FFN_VPU_BLOCKS
    ffn_tiled = ((wg_hbm, wg_v, D, SEM_WG), (wu_hbm, wu_v, D, SEM_WU), (wd_hbm, wd_v, F, SEM_WD))
    for src, dst, rows, slot in ffn_tiled:
        for c in range(dst.shape[0]):
            full_copy(src.at[:, pl.ds(c * 128, 128)], dst.at[c, pl.ds(0, rows), :], slot).start()
    full_copy(wg_hbm.at[:, pl.ds(f0, F - f0)], wgv_v, SEM_WGV).start()
    full_copy(wu_hbm.at[:, pl.ds(f0, F - f0)], wuv_v, SEM_WUV).start()

    zero_v = jnp.full((8, 128), zs, jnp.int32).astype(u32)

    def ld(ref, r0, rows, c0, cols):
        return ref[pl.ds(pl.multiple_of(zs * 8 + r0, 8), rows), c0:c0 + cols]

    def tiles(ref, r0, rows, opaque=True):
        w = ref.bitcast(u32)
        if opaque:
            parts = [ld(w.at[c], r0 // 2, rows // 2, 0, 128) for c in range(ref.shape[0])]
        else:
            parts = [w[c, r0 // 2:(r0 + rows) // 2, :] for c in range(ref.shape[0])]
        return jnp.concatenate(parts, axis=1)

    def token(*vals):
        return lambda: _fold_token(pltpu.bitcast(jnp.concatenate(vals, axis=0), u32), zero_v)

    def ln1_stats(xf):
        m = jnp.sum(xf, axis=-1, keepdims=True) * (1.0 / D)
        q = jnp.sum(xf * xf, axis=-1, keepdims=True) * (1.0 / D)
        inv = _rsqrt(jnp.maximum(q - m * m, 0.0) + EPS)
        return inv, m * inv

    def ln1_piece(r0, dst, p, m=None):
        if m is not None:
            x_v[S:S + 8, 0:128] = m[0:8, 0:128].astype(bf16)
        xa, xb = [x_v[pl.ds(pl.multiple_of(r0 + hf * HT1 + p * LN_ROWS, LN_ROWS), LN_ROWS), :]
                  .astype(f32) for hf in range(2)]
        (ia, ma), (ib, mb) = ln1_stats(xa), ln1_stats(xb)
        ya, yb = xa * ia, xb * ib
        s2 = ya[:, :HD] - ma
        s5 = yb[:, HD:] - mb
        s1 = s2 + s5
        s3 = yb[:, :HD] - yb[:, HD:]
        s4 = ya[:, HD:] - ya[:, :HD]
        combos = [s1, s2, s3, s4, s5, s1 + s3, s1 + s4]
        for i in range(7):
            for c in range(4):
                dst[i, c, p * LN_ROWS:(p + 1) * LN_ROWS, :] = (
                    combos[i][:, c * 128:(c + 1) * 128].astype(bf16))
        return token(combos[5], combos[6])

    def fold_piece(kind, c, j, pt):
        blk = {}
        for hh in range(2):
            for kh in range(2):
                k0 = kh * HD + j * 128
                w = wqkv_v[kind * NWC + c, k0:k0 + 128, hh * 128:(hh + 1) * 128]
                blk[hh, kh] = lax.dot_general(pt[2 * c + hh], w, _NT,
                                              preferred_element_type=f32) * LOG2E
        combos = _left_combos(blk[0, 0], blk[0, 1], blk[1, 0], blk[1, 1])
        r0 = kind * HD + c * 128
        for i in range(7):
            wt_v[i, j, r0:r0 + 128, :] = combos[i].astype(bf16)

    def fold_chunk(kind, c, pt):
        for j in range(4):
            fold_piece(kind, c, j, pt)

    def vprep_piece(c, j, m):
        wqkv_v[3 * NWC, 0:8, 0:128] = m[0:8, 0:128].astype(bf16)
        blk = {}
        for hh in range(2):
            for kh in range(2):
                k0 = kh * HD + j * 128
                w = wqkv_v[zs + V_ * NWC + c, k0:k0 + 128, hh * 128:(hh + 1) * 128]
                blk[hh, kh] = w.T.astype(f32)
        combos = _left_combos(blk[0, 0], blk[0, 1], blk[1, 0], blk[1, 1])
        r0 = V_ * HD + c * 128
        for i in range(7):
            wt_v[i, j, r0:r0 + 128, :] = combos[i].astype(bf16)
        return token(combos[1], combos[4])

    def wo_piece(w0, m):
        wo_v[D:D + 8, 0:128] = m[0:8, 0:128].astype(bf16)
        top = wo_v[pl.ds(pl.multiple_of(w0, 16), 16), :].astype(f32)
        bot = wo_v[pl.ds(pl.multiple_of(HD + w0, 16), 16), :].astype(f32)
        combos = _right_combos(top[:, :HD], top[:, HD:], bot[:, :HD], bot[:, HD:])
        for i in range(7):
            for c in range(4):
                wo7_v[i, c, pl.ds(pl.multiple_of(w0, 16), 16), :] = (
                    combos[i][:, c * 128:(c + 1) * 128].astype(bf16))
        return token(combos[5], combos[6])

    def run_rounds(t0, rounds, post, first):
        count = [0]
        pins = {}

        def pinned(w):
            toks = pins.get(count[0])
            if not toks:
                return w
            top = w[0:8, 0:128]
            for tk in toks:
                top = top | tk
            return jnp.concatenate(
                [jnp.concatenate([top, w[0:8, 128:]], axis=1), w[8:]], axis=0)

        def run_jobs(m):
            for fn, span in post.get(count[0], ()):
                tok = fn(m)
                if span:
                    pins.setdefault(count[0] + span, []).append(tok())
            count[0] += 1

        for par, kind, cs in rounds:
            r0 = kind * HD + cs[0] * 128
            rows = 128 * len(cs)

            def prod(i):
                if (par, kind) == (1, V_):
                    rhs = ld(sc7_v.at[i], 0, HT1 // 2, 0, HD)
                else:
                    rhs = tiles(s_v[par].at[i], 0, HT1)
                if (par, kind, cs[0]) == (1, K_, 0):
                    sc7_v[i] = rhs
                m = lax.dot_general(_unpack(tiles(wt_v.at[i], r0, rows, False)),
                                    _unpack(pinned(rhs)),
                                    _NT, preferred_element_type=f32)
                run_jobs(m)
                return m

            def emit(rh, ch, blk):
                tb = 2 * par + ch
                for n, c in enumerate(cs):
                    for jj in range(2):
                        pair = 4 * c + 2 * rh + jj
                        p = blk[n * 128 + jj * 64:n * 128 + (jj + 1) * 64]
                        if kind == K_:
                            phik_v[tb, pair * 128:(pair + 1) * 128, :] = _dual_softmax(p)
                        elif kind == Q_:
                            phiq_v[t0 // 2, tb, pair * 128:(pair + 1) * 128, :] = (
                                _dual_softmax(p))
                        else:
                            vt_v[pair // 8][tb, (pair % 8) * 64:(pair % 8 + 1) * 64, :] = (
                                p.astype(bf16))

            _strassen(prod, emit)

        ones = jnp.full((8, 2 * T1), 0x3F803F80, u32)
        kr = lax.broadcasted_iota(jnp.int32, (80, 128), 0)
        kc = lax.broadcasted_iota(jnp.int32, (80, 128), 1)
        kmask = jnp.where(kr < 64, kr // 32, (kr - 64) // 8) == kc % 2
        for j in range(NP):
            lhs = jnp.concatenate([tiles(vt_v[j // 8], (j % 8) * 64, 64), ones], axis=0)
            rhs = tiles(phik_v, j * 128, 128)
            upd = lax.dot_general(_unpack(lhs), _unpack(pinned(rhs)), _NT,
                                  preferred_element_type=f32)
            run_jobs(upd)
            if first:
                kv_acc[j] = upd
            else:
                upd = kv_acc[j] + upd
                kv_acc[j] = upd
                kvt_v[j] = jnp.where(kmask, upd, 0.0).astype(bf16)

    def load_best():
        return best_v[0], besti_v[...], best_v[1], best_v[2]

    def store_best(best):
        best_v[0], besti_v[...], best_v[1], best_v[2] = best

    def build_pt(g0, g1):
        n = g1 - g0
        w2 = wphi_v[4 * g0:4 * g1].reshape(n * 128, DH)
        er = lax.broadcasted_iota(jnp.int32, (128, DH), 0)
        ec = lax.broadcasted_iota(jnp.int32, (128, DH), 1)
        e = jnp.where(ec == (er % 64) // 2, 1.0, 0.0).astype(bf16)
        ptf = lax.dot_general(e, w2, _NT, preferred_element_type=f32)
        pr = lax.broadcasted_iota(jnp.int32, (128, 128), 0)
        pc = lax.broadcasted_iota(jnp.int32, (128, 128), 1)
        keep = pc // 32 == (pr // 64) * 2 + pr % 2
        return [jnp.where(keep, ptf[:, g * 128:(g + 1) * 128], 0.0).astype(bf16)
                for g in range(n)]

    hbl_v[...] = jnp.zeros_like(hbl_v)
    hbr_v[...] = jnp.zeros_like(hbr_v)
    store_best((jnp.full((8, 128), -jnp.inf, f32), jnp.zeros((8, 128), jnp.int32),
                jnp.zeros((8, 128), f32), jnp.zeros((8, 128), f32)))
    n_ln = HT1 // LN_ROWS
    x0_copy(0).wait()
    x0_copy(1).wait()
    for p in range(n_ln // 2):
        ln1_piece(0, s_v[0], p)
    full_copy(wr_hbm, wr_v, SEM_WR).wait()
    phi_copy(0).wait()
    x0_copy(2).wait()
    x0_copy(3).wait()
    wr_row = wr_v[...].astype(f32).reshape(1, D)
    wrf_v[...] = jnp.broadcast_to(
        wr_row - jnp.sum(wr_row, axis=-1, keepdims=True) * (1.0 / D), (8, D))
    pt = build_pt(0, 4)
    for p in range(n_ln // 2, n_ln):
        ln1_piece(0, s_v[0], p)
    for part in range(2):
        k0_copy(2 * part).wait()
        k0_copy(2 * part + 1).wait()
        fold_piece(K_, 0, 2 * part, pt)
        fold_piece(K_, 0, 2 * part + 1, pt)

    post = {}

    def at(slot, fn, span=0):
        post.setdefault(slot, []).append((fn, span))

    for slot, copies in T0_WAITS:
        for cp in copies:
            if cp == 'phi':
                at(slot, lambda m: phi_copy(1).wait())
            elif cp in ('x1', 'x2', 'x3'):
                at(slot, lambda m, cp=cp: x_copy(int(cp[1])).wait())
            else:
                at(slot, lambda m, cp=cp: w_copy(cp // NWC, cp % NWC).wait())
    for n in range(1, 2 * NWC):
        if n == 2:
            at(T0_FOLD[n], lambda m: pt.extend(build_pt(4, 8)))
        at(T0_FOLD[n], lambda m, n=n: fold_chunk(n // NWC, n % NWC, pt))
    for c in range(NWC):
        for j in range(4):
            at(T0_VPREP[c][j], lambda m, c=c, j=j: vprep_piece(c, j, m), T0_VSPAN)
    for p in range(n_ln):
        at(T0_LN[p], lambda m, p=p: ln1_piece(zs + T1, s_v[1], p, m), T0_LNSPAN[p])
    for p in range(n_ln):
        at(T1_LN[0][p], lambda m, p=p: ln1_piece(zs + 2 * T1, s_v[0], p, m), P1_LNSPAN)
        at(T1_LN[1][p], lambda m, p=p: ln1_piece(zs + 3 * T1, s_v[1], p, m), P1_LNSPAN)
    lo, hi = [0, 1], [2, 3]
    run_rounds(0, [(0, kind, [c]) for kind in (K_, Q_) for c in range(NWC)]
               + [(1, K_, lo), (1, K_, hi), (1, Q_, lo), (1, Q_, hi),
                  (0, V_, lo), (0, V_, hi), (1, V_, lo), (1, V_, hi)], post, True)
    full_copy(wo_hbm, wo_v.at[pl.ds(0, D), :], SEM_WO).wait()
    for i in range(4, N1):
        x_copy(i).wait()

    def phase1(i, carry):
        post = {}
        nxt = jnp.minimum(i + 1, N2 - 1) * T2
        w0 = jnp.minimum((i - 1) * WO_ROWS, HD - WO_ROWS)
        for par in range(2):
            for p in range(n_ln):
                post.setdefault(P1_LN2[par][p], []).append(
                    (lambda m, p=p, par=par: ln1_piece(nxt + par * T1, s_v[par], p, m),
                     P1_LNSPAN2[par]))
        for p in range(WO_ROWS // 16):
            post.setdefault(P1_WO[p], []).append(
                (lambda m, p=p: wo_piece(w0 + 16 * p, m), P1_WOSPAN))
        run_rounds(2 * i, [(par, kind, cs) for kind in (K_, Q_, V_) for par in range(2)
                           for cs in ([0, 1], [2, 3])], post, False)
        return carry

    lax.fori_loop(1, N1 // 2, phase1, 0)

    for _, dst, rows, slot in ffn_tiled:
        filled = dst.at[:, pl.ds(0, rows), :]
        full_copy(filled, filled, slot).wait()
    full_copy(wg_hbm.at[:, pl.ds(f0, F - f0)], wgv_v, SEM_WGV).wait()
    full_copy(wu_hbm.at[:, pl.ds(f0, F - f0)], wuv_v, SEM_WUV).wait()

    def o_copy(hf):
        return pltpu.make_async_copy(
            out_v.at[pl.ds(hf * HT2, HT2), :], out_hbm.at[0, pl.ds(hf * HT2, HT2), :],
            sem.at[SEM_O + hf])

    def half_stats(hh, c0):
        rows = hh.shape[0]
        parts = [hh[:, c * 128:(c + 1) * 128] for c in range(4)]
        wts = [wrf_v[:, c0 + c * 128:c0 + (c + 1) * 128] for c in range(4)]
        s1 = (parts[0] + parts[1]) + (parts[2] + parts[3])
        sq = [p * p for p in parts]
        s2 = (sq[0] + sq[1]) + (sq[2] + sq[3])
        dw = [(p.reshape(rows // 8, 8, 128) * w[None]).reshape(rows, 128)
              for p, w in zip(parts, wts)]
        s3 = (dw[0] + dw[1]) + (dw[2] + dw[3])
        return s1, s2, s3

    def first_half(hbuf, sbuf, base, p, c0):
        r0 = p * EP_ROWS
        hh = ld(hbuf[c0 // HD], r0, EP_ROWS, 0, HD)
        h_v[pl.ds(pl.multiple_of(base + r0, EP_ROWS), EP_ROWS), c0:c0 + HD] = hh.astype(bf16)
        st = jnp.concatenate(half_stats(hh, c0), axis=1)
        sbuf[r0:r0 + EP_ROWS, :] = st
        return _fold_token(pltpu.bitcast(st, u32), zero_v)

    def finish(hbuf, sbuf, base, p, valid, best, defer=None):
        r0 = p * EP_ROWS
        g0 = pl.multiple_of(base + r0, EP_ROWS)
        hl, hr = [ld(r, r0, EP_ROWS, 0, HD) for r in hbuf]
        if defer is None:
            h_v[pl.ds(g0, EP_ROWS), 0:HD] = hl.astype(bf16)
        if sbuf is None:
            if defer is None:
                h_v[pl.ds(g0, EP_ROWS), HD:D] = hr.astype(bf16)
            st = half_stats(hr, HD)
        else:
            st = ld(sbuf, r0, EP_ROWS, 0, 384)
            st = [st[:, n * 128:(n + 1) * 128] for n in range(3)]
        s1, s2, s3 = [jnp.sum(v + w, axis=-1, keepdims=True)
                      for v, w in zip(half_stats(hl, 0), st)]
        m = s1 * (1.0 / D)
        var = jnp.maximum(s2 * (1.0 / D) - m * m, 0.0)
        inv = _rsqrt(var + EPS)
        r = s3 * inv

        def write_out(h):
            o = h * (1.0 + inv) - m * inv
            out_v[pl.ds(g0, EP_ROWS), :] = o.astype(bf16)
            return o

        if defer is None:
            o = write_out(jnp.concatenate([hl, hr], axis=1))
        else:
            defer.append(lambda: write_out(jnp.concatenate(
                [ld(r_, r0, EP_ROWS, 0, HD) for r_ in hbuf], axis=1)))
        bv, bi, bm, bq = best
        sub = lax.broadcasted_iota(jnp.int32, (8, 128), 0)
        for g in range(EP_ROWS // 8):
            rows = slice(g * 8, (g + 1) * 8)
            rg = jnp.broadcast_to(r[rows], (8, 128))
            if valid is not None:
                rg = jnp.where(valid, rg, -jnp.inf)
            better = rg > bv
            bi = jnp.where(better, sub + (g0 + g * 8), bi)
            bv = jnp.where(better, rg, bv)
            bm = jnp.where(better, jnp.broadcast_to(m[rows], (8, 128)), bm)
            bq = jnp.where(better, jnp.broadcast_to(var[rows], (8, 128)), bq)
        best = (bv, bi, bm, bq)
        if defer is not None:
            return best, None
        tok = _fold_token(pltpu.bitcast(jnp.concatenate(
            [o[:, D - 128:], bv, bm, bq], axis=0), u32), zero_v)
        return best, tok

    n_ep = HT2 // EP_ROWS

    def phase2(i, carry):
        ot = []
        for j in range(NP):
            ph = tiles(phiq_v.at[i], j * 128, 128, False)
            n = jnp.dot(_unpack(kvt_v.bitcast(u32)[j]), _unpack(ph),
                        preferred_element_type=f32)
            r0h = _recip(n[64:72] + 1e-6)
            r1h = _recip(n[72:80] + 1e-6)
            ot.append((n[0:32].reshape(4, 8, T2) * r0h[None]).reshape(32, T2))
            ot.append((n[32:64].reshape(4, 8, T2) * r1h[None]).reshape(32, T2))
        lo = jnp.concatenate(ot[:H // 2], axis=0)
        hi = jnp.concatenate(ot[H // 2:], axis=0)
        lcs = _left_combos(lo[:, :HT2], hi[:, :HT2], lo[:, HT2:], hi[:, HT2:])

        state = {'best': load_best()}
        pins = {}
        jobs = {}
        lts = {}
        ra = pl.multiple_of(i * T2, T2)
        rb = pl.multiple_of(i * T2 + HT2, HT2)
        prev = jnp.maximum(i * T2 - HT2, HT2)

        def add_job(slot, deadline, fn, gates=()):
            jobs.setdefault(slot, []).append((fn, deadline, gates))

        def finish_job(hbuf, sbuf, base, p, valid):
            def fn():
                state['best'], tok = finish(hbuf, sbuf, base, p, valid, state['best'])
                return tok
            return fn

        def lt_job(k):
            def fn():
                lts[k] = lcs[k].astype(bf16).T
                return _fold_token(pltpu.bitcast(lts[k], u32), zero_v)
            return fn

        order = (2, 4, 6, 0, 3, 1, 5)
        lt_job(2)()
        for n in range(1, 7):
            add_job(LT_START[n], min(LT_START[n] + LT_SPAN[n], 4 * n), lt_job(order[n]))
        for p in range(n_ep):
            add_job(FB_START[p], FB_START[p] + FB_SPAN, finish_job(hb_v, None, prev, p, i > 0), hb_v)
            add_job(SA_START[p], SA_START[p] + SA_SPAN, lambda p=p: first_half(ha_v, sa_v, ra, p, HD), ha_v[1:])
            add_job(FA_START[p], FA_START[p] + FA_SPAN[p], finish_job(ha_v, sa_v, ra, p, None), ha_v)

        def xblk(r0, c0):
            return x_v[pl.ds(r0, HT2), c0:c0 + 128].astype(f32)

        for n, k in enumerate(order):
            for c in range(4):
                slot = 4 * n + c
                for fn, deadline, gates in jobs.get(slot, ()):
                    for ref in gates:
                        ref[HT2:HT2 + 8, 0:128] = mm[GATE_ROW:GATE_ROW + 8]
                    pins.setdefault(deadline, []).append(fn())
                w = wo7_v.bitcast(u32)[k, c, 0:HD // 2, :]
                toks = pins.get(slot)
                if toks:
                    top = w[0:8]
                    for tk in toks:
                        top = top | tk
                    w = jnp.concatenate([top, w[8:]], axis=0)
                mm = jnp.dot(lts[k], _unpack(w), preferred_element_type=f32)
                c0 = c * 128
                cs = slice(c0, c0 + 128)
                tmp = lambda t: ld(tmp_v[t], 0, HT2, c0, 128)
                if n == 0:
                    tmp_v[0][:, cs] = mm
                elif n == 1:
                    ha_v[1][0:HT2, cs] = (xblk(ra, HD + c0) + tmp(0)) + mm
                    tmp_v[1][:, cs] = xblk(ra, c0) - mm
                elif n == 2:
                    tmp_v[2][:, cs] = tmp(1) + mm
                elif n == 3:
                    tmp_v[3][:, cs] = tmp(2) + mm
                    tmp_v[4][:, cs] = (xblk(rb, HD + c0) + tmp(0)) + mm
                elif n == 4:
                    ha_v[0][0:HT2, cs] = tmp(3) + mm
                    tmp_v[5][:, cs] = xblk(rb, c0) + mm
                elif n == 5:
                    hb_v[0][0:HT2, cs] = tmp(5) + mm
                    tmp_v[6][:, cs] = tmp(4) - mm
                else:
                    hb_v[1][0:HT2, cs] = tmp(6) + mm
        store_best(state['best'])
        o_copy(2 * i).start()

        @pl.when(i > 0)
        def _():
            o_copy(2 * i - 1).start()

        return carry

    lax.fori_loop(0, N2, phase2, 0)
    best = load_best()
    late = []
    for p in range(n_ep):
        best, _ = finish(hb_v, None, S - HT2, p, None, best, late)


    bv, bi, bm, bq = best
    for sh in (4, 2, 1):
        ov, oi, om, oq = [pltpu.roll(t, sh, 0) for t in (bv, bi, bm, bq)]
        take = jnp.logical_or(ov > bv, jnp.logical_and(ov == bv, oi < bi))
        bv, bi, bm, bq = [jnp.where(take, o_, t)
                          for o_, t in zip((ov, oi, om, oq), (bv, bi, bm, bq))]
    idx = jnp.clip(bi[0, 0], 0, S - 1)
    b0 = pl.multiple_of((idx // 8) * 8, 8)
    t = _rb(_rb(bq) + EPS)
    inv = _recip(_rb(t * _rsqrt(t)))
    gate = _sigmoid(bv)
    wide = lambda v: jnp.concatenate([v] * (D // 128), axis=1)
    b1 = pl.multiple_of(jnp.minimum(b0, S - HT2 - 8), 8)
    b2 = pl.multiple_of(jnp.maximum(b0 - (S - HT2), 0), 8)
    hb = jnp.where(wide(bi) < S - HT2, h_v[pl.ds(b1, 8), :].astype(f32),
                   _rb(jnp.concatenate([r_[pl.ds(b2, 8), :] for r_ in hb_v], axis=1)))
    hn = (hb - wide(bm)) * wide(inv)
    xs = hn.astype(bf16)
    rows = lax.broadcasted_iota(jnp.int32, (8, D), 0) + b0

    xm = jnp.where(rows == wide(bi), _rb(hn), 0.0)
    for sh in (4, 2, 1):
        xm = xm + pltpu.roll(xm, sh, 0)
    for t in range(D // 128):
        xcol_v[t // 2][(t % 2) * 128:(t % 2 + 1) * 128, :] = jnp.concatenate(
            [xm[:, t * 128:(t + 1) * 128]] * 16, axis=0).T

    nblk = F // 256
    nmx = nblk - FFN_VPU_BLOCKS
    act = {}
    acc = {}

    def activate(g, u):
        return (g * _sigmoid(g) * u).astype(bf16)

    parts = D // 8 // FFN_KG

    def vpu_chunk(q):
        blk, part = nmx + q // parts, q % parts
        cur = acc.get(blk)
        for kg in range(part * FFN_KG, (part + 1) * FFN_KG):
            xc = ld(xcol_v[kg // 32], (kg % 32) * 8, 8, 0, 128)
            w = jnp.concatenate(
                [r[kg * 8:(kg + 1) * 8, (blk - nmx) * 256:(blk - nmx + 1) * 256].astype(f32)
                 for r in (wgv_v, wuv_v)], axis=1)
            p = w * jnp.concatenate([xc] * 4, axis=1)
            cur = p if cur is None else cur + p
        acc[blk] = cur
        if part == parts - 1:
            for sh in (4, 2, 1):
                cur = cur + pltpu.roll(cur, sh, 0)
            act[blk] = activate(cur[:, :256], cur[:, 256:])
        if FFN_TOKALL:
            return _fold_token(pltpu.bitcast(cur, u32), zero_v)
        c = q % 4
        return _fold_token(pltpu.bitcast(cur[:, c * 128:(c + 1) * 128], u32), zero_v)

    nchunk = FFN_VPU_BLOCKS * parts
    starts = [FFN_W0 + (q * (FFN_W1 - FFN_W0)) // (nchunk - 1) for q in range(nchunk)]
    pins = {}
    xs16 = jnp.zeros((16, 256), bf16)
    wave = [0]
    wgw, wuw, wdw = [r.bitcast(u32) for r in (wg_v, wu_v, wd_v)]

    def run_wave(lhs, tls):
        top = tls[0][0:8]
        for tk in pins.get(wave[0], ()):
            top = top | tk
        w = jnp.concatenate([jnp.concatenate([top, tls[0][8:]], axis=0)] + tls[1:], axis=1)
        out = jnp.dot(lhs, _unpack(w), preferred_element_type=f32)
        for p, fn in enumerate(late):
            if LATE_AT[p] == wave[0]:
                for r_ in hb_v:
                    r_[HT2:HT2 + 8, 0:128] = out[:, 0:128] if LATE_GATE else hn[:, 0:128]
                tk = token(fn()[:, D - 128:])
                if LATE_SPAN:
                    pins.setdefault(wave[0] + LATE_SPAN, []).append(tk())
        for q, start in enumerate(starts):
            if start == wave[0]:
                pins.setdefault(wave[0] + FFN_SPAN, []).append(vpu_chunk(q))
        if wave[0] == FFN_LATE:
            o_copy(2 * N2 - 1).start()
            out_v[pl.ds(pl.multiple_of(zs * 16 + S, 16), 16), 0:256] = xs16
            pins.setdefault(wave[0] + 4, []).append(
                token(out_v[S:S + 8, 0:128].astype(f32))())
        wave[0] += 1
        return out

    for j in range(nmx):
        gu = None
        for kt in range(D // 128):
            p = run_wave(xs[:, kt * 128:(kt + 1) * 128],
                         [r[2 * j + c, kt * 64:(kt + 1) * 64, :]
                          for r in (wgw, wuw) for c in range(2)])
            gu = p if gu is None else gu + p
        act[j] = activate(gu[:, :256], gu[:, 256:])
    ys = [None, None]
    for j in range(nblk):
        for kt in range(2):
            for hf in range(2):
                r0 = (2 * j + kt) * 64
                p = run_wave(act[j][:, kt * 128:(kt + 1) * 128],
                             [wdw[4 * hf + c, r0:r0 + 64, :] for c in range(4)])
                ys[hf] = p if ys[hf] is None else ys[hf] + p
    y = jnp.concatenate(ys, axis=1)
    cur = out_v[pl.ds(b0, 8), :].astype(f32)
    fix_v[...] = jnp.where(rows == wide(bi), hb + hn + y * wide(gate), cur).astype(bf16)
    for hf in range(2 * N2):
        o_copy(hf).wait()
    fix = pltpu.make_async_copy(fix_v, out_hbm.at[0, pl.ds(b0, 8), :], sem.at[SEM_O])
    fix.start()
    fix.wait()


def _kernel(*refs):
    def step(i, carry):
        @pl.when(i == 0)
        def _():
            _body(i, *refs)

        return carry

    lax.fori_loop(0, 2, step, 0)


@jax.jit
def pallas_sequential_preLN__linear_kernel_hedgehog__moe_arch_mod__prompt_kernel(
    A_x: jax.Array,
    A_wqkv: jax.Array,
    A_w_phi: jax.Array,
    A_wo: jax.Array,
    B_x: jax.Array,
    B_w_r: jax.Array,
    B_w_gate: jax.Array,
    B_w_up: jax.Array,
    B_w_down: jax.Array,
):
    any_spec = pl.BlockSpec(memory_space=pl.ANY)
    return pl.pallas_call(
        _kernel,
        out_shape=jax.ShapeDtypeStruct((1, S, D), bf16),
        in_specs=[any_spec] * 8,
        out_specs=any_spec,
        scratch_shapes=[
            pltpu.VMEM((S + 16, D), bf16),
            pltpu.VMEM((3 * NWC + 1, D, WC), bf16),
            pltpu.VMEM((H, DH, DH), bf16),
            pltpu.VMEM((D + 16, D), bf16),
            pltpu.VMEM((D,), bf16),
            pltpu.VMEM((F // 128 - 2 * FFN_VPU_BLOCKS, D + PAD, 128), bf16),
            pltpu.VMEM((F // 128 - 2 * FFN_VPU_BLOCKS, D + PAD, 128), bf16),
            pltpu.VMEM((D // 128, F + PAD, 128), bf16),
            pltpu.VMEM((D, 256 * FFN_VPU_BLOCKS), bf16),
            pltpu.VMEM((D, 256 * FFN_VPU_BLOCKS), bf16),
            pltpu.VMEM((7, 4, 3 * HD + PAD, 128), bf16),
            pltpu.VMEM((7, 4, HD + PAD, 128), bf16),
            pltpu.VMEM((7, 4, HT1 + PAD, 128), bf16),
            pltpu.VMEM((7, 4, HT1 + PAD, 128), bf16),
            pltpu.VMEM((7, HT1 // 2, HD), u32),
            pltpu.VMEM((N2, 4, 2 * D + PAD, 128), bf16),
            pltpu.VMEM((4, 2 * D + PAD, 128), bf16),
            pltpu.VMEM((4, HD + PAD, 128), bf16),
            pltpu.VMEM((4, HD + PAD, 128), bf16),
            pltpu.VMEM((NP, 80, 128), f32),
            pltpu.VMEM((NP, 80, 128), bf16),
            *[pltpu.VMEM((HT2 + 8, HD), f32) for _ in range(4)],
            pltpu.VMEM((HT2, 384), f32),
            *[pltpu.VMEM((HT2, HD), f32) for _ in range(7)],
            pltpu.VMEM((S, D), bf16),
            pltpu.VMEM((S + 16, D), bf16),
            pltpu.VMEM((8, D), f32),
            pltpu.VMEM((3, 8, 128), f32),
            pltpu.VMEM((8, 128), jnp.int32),
            pltpu.VMEM((8, D), bf16),
            *[pltpu.VMEM((264, 128), f32) for _ in range(4)],
            pltpu.SemaphoreType.DMA((NSEM,)),
        ],
        compiler_params=pltpu.CompilerParams(
            vmem_limit_bytes=110 * 1024 * 1024,
            disable_bounds_checks=True,
            disable_semaphore_checks=True),
    )(A_x, A_wqkv, A_w_phi, A_wo, B_w_r, B_w_gate, B_w_up, B_w_down)
```

```python
import jax
import jax.numpy as jnp
from jax import lax
import jax.experimental.pallas as pl
import jax.experimental.pallas.tpu as pltpu

S = 2048
D = 1024
H = 32
DH = 32
F = 3584
NP = H // 2
T1 = 256
T2 = 512
N1 = S // T1
N2 = S // T2
HT1 = T1 // 2
HT2 = T2 // 2
HD = D // 2
WC = 256
NWC = D // WC
LOG2E = 1.4426950408889634
EPS = 1e-5
WO_ROWS = 176
LN_ROWS = 16
EP_ROWS = 32
LT_START = (0, 0, 1, 5, 8, 11, 14)
LT_SPAN = (0, 2, 4, 4, 4, 4, 4)
FB_START = (2, 4, 6, 8, 10, 12, 14, 16)
SA_START = (9, 11, 15, 15, 17, 17, 18, 18)
FA_START = (20, 21, 22, 23, 24, 25, 26, 27)
FA_SPAN = (3, 7, 2, 5, 3, 5, 3, 2)
FB_SPAN = 2
SA_SPAN = 3
GATE_ROW = 0
SW1 = SW2 = SW3 = SW4 = 1
PAD = 16
T0_FOLD = (0, 4, 11, 18, 25, 33, 39, 46)
T0_WAITS = ((4, (1,)), (11, ('phi', 2)), (18, (3, 4)), (33, ('x1', 5, 6)), (46, (7,)),
            (73, (8, 9, 10, 11, 'x2', 'x3')))
T0_VPREP = ((73, 74, 75, 76), (77, 78, 79, 80), (81, 82, 83, 84), (85, 86, 87, 88))
T0_VSPAN = 4
T0_LN = (33, 35, 36, 37, 38, 39, 40, 43)
T0_LNSPAN = (3, 0, 0, 0, 0, 0, 0, 0)
P1_LN = (29, 30, 31, 32, 33, 34, 35, 36)
P1_LNSPAN = 3
P1_WO = (57, 58, 59, 60, 63, 77, 79, 80, 81, 82, 83)
P1_LN2 = ((70, 71, 72, 73, 74, 75, 76, 77), (62, 63, 64, 65, 66, 67, 68, 69))
P1_LNSPAN2 = (2, 2)
T1_LN = ((99, 100, 101, 102, 103, 104, 105, 106), (90, 91, 92, 93, 94, 95, 96, 97))
P1_WOSPAN = 3

FFN_VPU_BLOCKS = 7
FFN_KG = 16
FFN_W0 = 18
FFN_W1 = 107
FFN_SPAN = 4
FFN_TOKALL = 0
FFN_LATE = 16
LATE_AT = (1, 2, 3, 3, 4, 6, 6, 7)
LATE_SPAN = 0
LATE_GATE = 1

_NT = (((1,), (1,)), ((), ()))
_TN = (((0,), (0,)), ((), ()))
f32 = jnp.float32
bf16 = jnp.bfloat16
u32 = jnp.uint32

K_, Q_, V_ = 0, 1, 2
SRC = {K_: 1, Q_: 0, V_: 2}

SEM_W = 0
SEM_X = SEM_W + 3 * NWC
SEM_X0 = SEM_X + N1
SEM_K0 = SEM_X0 + 4
SEM_PHI = SEM_K0 + 4
SEM_WO = SEM_PHI + 2
SEM_WR, SEM_WG, SEM_WU, SEM_WD = (SEM_WO + 4 + i for i in range(4))
SEM_WGV, SEM_WUV = SEM_WD + 1, SEM_WD + 2
SEM_O = SEM_WUV + 1
NSEM = SEM_O + 2 * N2


def _rb(v):
    return v.astype(bf16).astype(f32)


def _unpack(w):
    return pltpu.bitcast(w, bf16)


def _recip(x):
    r = pl.reciprocal(x, approx=True)
    return r * (2.0 - x * r)


def _sigmoid(x):
    return _recip(1.0 + jnp.exp(jnp.minimum(-x, 80.0)))


def _rsqrt(x):
    return lax.rsqrt(x)


def _dual_softmax(p):
    t = p.shape[-1]
    p3 = p.reshape(8, 8, t)

    def allred(v, op):
        v = op(v, pltpu.roll(v, 2, 0))
        return op(v, pltpu.roll(v, 4, 0))

    mx = allred(jnp.max(p3, axis=0), jnp.maximum)
    mn = allred(jnp.min(p3, axis=0), jnp.minimum)
    ep = jnp.exp2(p3 - mx[None])
    en = jnp.exp2(mn[None] - p3)
    sp = allred(jnp.sum(ep, axis=0), jnp.add)
    sn = allred(jnp.sum(en, axis=0), jnp.add)
    fp = (ep * _recip(sp)[None]).reshape(64, t)
    fn = (en * _recip(sn)[None]).reshape(64, t)
    return jnp.concatenate([fp, fn], axis=0).astype(bf16)


def _left_combos(a11, a12, a21, a22):
    return [a11 + a22, a21 + a22, a11, a22, a11 + a12, a21 - a11, a12 - a22]


def _right_combos(b11, b12, b21, b22):
    return [b11 + b22, b11, b12 - b22, b21 - b11, b22, b11 + b12, b21 + b22]


def _strassen(prod, emit):
    m3 = prod(2)
    m5 = prod(4)
    emit(0, 1, m3 + m5)
    m7 = prod(6)
    u = m7 - m5
    m1 = prod(0)
    u = u + m1
    w = m1 + m3
    m4 = prod(3)
    emit(0, 0, u + m4)
    m2 = prod(1)
    emit(1, 0, m2 + m4)
    w = w - m2
    m6 = prod(5)
    emit(1, 1, w + m6)


def _fold_token(w, zero):
    r, c = w.shape
    acc = None
    for i in range(r // 8):
        for j in range(c // 128):
            blk = w[i * 8:(i + 1) * 8, j * 128:(j + 1) * 128]
            acc = blk if acc is None else acc | blk
    return acc & zero


def _body(zs, x_hbm, wqkv_hbm, wphi_hbm, wo_hbm, wr_hbm, wg_hbm, wu_hbm, wd_hbm,
            out_hbm,
            x_v, wqkv_v, wphi_v, wo_v, wr_v, wg_v, wu_v, wd_v, wgv_v, wuv_v,
            wt_v, wo7_v, sa7_v, sb7_v, sc7_v, phiq_v, phik_v, vt0_v, vt1_v, kv_acc, kvt_v, hal_v, har_v, hbl_v, hbr_v, sa_v,
            t0_v, t1_v, t2_v, t3_v, t4_v, t5_v, t6_v, h_v, out_v,
            wrf_v, best_v, besti_v, fix_v, xc0_v, xc1_v, xc2_v, xc3_v, sem):
    xcol_v = (xc0_v, xc1_v, xc2_v, xc3_v)
    s_v = (sa7_v, sb7_v)
    vt_v = (vt0_v, vt1_v)
    ha_v = (hal_v, har_v)
    hb_v = (hbl_v, hbr_v)
    tmp_v = (t0_v, t1_v, t2_v, t3_v, t4_v, t5_v, t6_v)

    def x_rows(r0, rows, slot):
        return pltpu.make_async_copy(
            x_hbm.at[0, pl.ds(r0, rows), :], x_v.at[pl.ds(r0, rows), :], sem.at[slot])

    def x_copy(i):
        return x_rows(i * T1, T1, SEM_X + i)

    def x0_copy(q):
        return x_rows((q % 2) * HT1 + (q // 2) * (HT1 // 2), HT1 // 2, SEM_X0 + q)

    def w_copy(kind, c):
        return pltpu.make_async_copy(
            wqkv_hbm.at[:, pl.ds(SRC[kind] * D + c * WC, WC)],
            wqkv_v.at[kind * NWC + c], sem.at[SEM_W + kind * NWC + c])

    def k0_copy(q):
        r0 = (q % 2) * HD + (q // 2) * 256
        return pltpu.make_async_copy(
            wqkv_hbm.at[pl.ds(r0, 256), pl.ds(SRC[K_] * D, WC)],
            wqkv_v.at[K_ * NWC, pl.ds(r0, 256), :], sem.at[SEM_K0 + q])

    def phi_copy(part):
        lo, n = part * (H // 2), H // 2
        return pltpu.make_async_copy(wphi_hbm.at[pl.ds(lo, n)], wphi_v.at[pl.ds(lo, n)],
                                     sem.at[SEM_PHI + part])

    def full_copy(src, dst, slot):
        return pltpu.make_async_copy(src, dst, sem.at[slot])

    x0_copy(0).start()
    x0_copy(1).start()
    full_copy(wr_hbm, wr_v, SEM_WR).start()
    phi_copy(0).start()
    x0_copy(2).start()
    x0_copy(3).start()
    for q in range(4):
        k0_copy(q).start()
    w_copy(K_, 1).start()
    phi_copy(1).start()
    w_copy(K_, 2).start()
    w_copy(K_, 3).start()
    w_copy(Q_, 0).start()
    x_copy(1).start()
    for c in range(1, NWC):
        w_copy(Q_, c).start()
    for c in range(NWC):
        w_copy(V_, c).start()
    x_copy(2).start()
    x_copy(3).start()
    full_copy(wo_hbm, wo_v.at[pl.ds(0, D), :], SEM_WO).start()
    for i in range(4, N1):
        x_copy(i).start()
    f0 = F - 256 * FFN_VPU_BLOCKS
    ffn_tiled = ((wg_hbm, wg_v, D, SEM_WG), (wu_hbm, wu_v, D, SEM_WU), (wd_hbm, wd_v, F, SEM_WD))
    for src, dst, rows, slot in ffn_tiled:
        for c in range(dst.shape[0]):
            full_copy(src.at[:, pl.ds(c * 128, 128)], dst.at[c, pl.ds(0, rows), :], slot).start()
    full_copy(wg_hbm.at[:, pl.ds(f0, F - f0)], wgv_v, SEM_WGV).start()
    full_copy(wu_hbm.at[:, pl.ds(f0, F - f0)], wuv_v, SEM_WUV).start()

    zero_v = jnp.full((8, 128), zs, jnp.int32).astype(u32)

    def ld(ref, r0, rows, c0, cols, static=False):
        if static:
            return ref[r0:r0 + rows, c0:c0 + cols]
        return ref[pl.ds(pl.multiple_of(zs * 8 + r0, 8), rows), c0:c0 + cols]

    def zrows(r0, rows, mult=8):
        return pl.ds(pl.multiple_of(zs * mult + r0, mult), rows)

    def srows(flag, r0, rows, mult=8):
        return zrows(r0, rows, mult) if flag else pl.ds(r0, rows)

    def tiles(ref, r0, rows, opaque=True):
        w = ref.bitcast(u32)
        if opaque:
            parts = [ld(w.at[c], r0 // 2, rows // 2, 0, 128) for c in range(ref.shape[0])]
        else:
            parts = [w[c, r0 // 2:(r0 + rows) // 2, :] for c in range(ref.shape[0])]
        return jnp.concatenate(parts, axis=1)

    def token(*vals):
        return lambda: _fold_token(pltpu.bitcast(jnp.concatenate(vals, axis=0), u32), zero_v)

    def ln1_stats(xf):
        m = jnp.sum(xf, axis=-1, keepdims=True) * (1.0 / D)
        q = jnp.sum(xf * xf, axis=-1, keepdims=True) * (1.0 / D)
        inv = _rsqrt(jnp.maximum(q - m * m, 0.0) + EPS)
        return inv, m * inv

    def ln1_piece(r0, dst, p, m=None, dyn=True):
        if m is not None:
            x_v[S:S + 8, 0:128] = m[0:8, 0:128].astype(bf16)
        xa, xb = [x_v[pl.ds(pl.multiple_of(r0 + hf * HT1 + p * LN_ROWS, LN_ROWS), LN_ROWS), :]
                  .astype(f32) for hf in range(2)]
        (ia, ma), (ib, mb) = ln1_stats(xa), ln1_stats(xb)
        ya, yb = xa * ia, xb * ib
        s2 = ya[:, :HD] - ma
        s5 = yb[:, HD:] - mb
        s1 = s2 + s5
        s3 = yb[:, :HD] - yb[:, HD:]
        s4 = ya[:, HD:] - ya[:, :HD]
        combos = [s1, s2, s3, s4, s5, s1 + s3, s1 + s4]
        for i in range(7):
            for c in range(4):
                dst[i, c, srows(SW1 and dyn, p * LN_ROWS, LN_ROWS, 16), :] = (
                    combos[i][:, c * 128:(c + 1) * 128].astype(bf16))
        return token(combos[5], combos[6])

    def fold_piece(kind, c, j, pt):
        blk = {}
        for hh in range(2):
            for kh in range(2):
                k0 = kh * HD + j * 128
                w = wqkv_v[kind * NWC + c, k0:k0 + 128, hh * 128:(hh + 1) * 128]
                blk[hh, kh] = lax.dot_general(pt[2 * c + hh], w, _NT,
                                              preferred_element_type=f32) * LOG2E
        combos = _left_combos(blk[0, 0], blk[0, 1], blk[1, 0], blk[1, 1])
        r0 = kind * HD + c * 128
        for i in range(7):
            wt_v[i, j, r0:r0 + 128, :] = combos[i].astype(bf16)

    def fold_chunk(kind, c, pt):
        for j in range(4):
            fold_piece(kind, c, j, pt)

    def vprep_piece(c, j, m):
        wqkv_v[3 * NWC, 0:8, 0:128] = m[0:8, 0:128].astype(bf16)
        blk = {}
        for hh in range(2):
            for kh in range(2):
                k0 = kh * HD + j * 128
                w = wqkv_v[zs + V_ * NWC + c, k0:k0 + 128, hh * 128:(hh + 1) * 128]
                blk[hh, kh] = w.T.astype(f32)
        combos = _left_combos(blk[0, 0], blk[0, 1], blk[1, 0], blk[1, 1])
        r0 = V_ * HD + c * 128
        for i in range(7):
            wt_v[i, j, r0:r0 + 128, :] = combos[i].astype(bf16)
        return token(combos[1], combos[4])

    def wo_piece(w0, m):
        wo_v[D:D + 8, 0:128] = m[0:8, 0:128].astype(bf16)
        top = wo_v[pl.ds(pl.multiple_of(w0, 16), 16), :].astype(f32)
        bot = wo_v[pl.ds(pl.multiple_of(HD + w0, 16), 16), :].astype(f32)
        combos = _right_combos(top[:, :HD], top[:, HD:], bot[:, :HD], bot[:, HD:])
        for i in range(7):
            for c in range(4):
                wo7_v[i, c, pl.ds(pl.multiple_of(w0, 16), 16), :] = (
                    combos[i][:, c * 128:(c + 1) * 128].astype(bf16))
        return token(combos[5], combos[6])

    def run_rounds(t0, rounds, post, first):
        count = [0]
        pins = {}

        def pinned(w):
            toks = pins.get(count[0])
            if not toks:
                return w
            top = w[0:8, 0:128]
            for tk in toks:
                top = top | tk
            return jnp.concatenate(
                [jnp.concatenate([top, w[0:8, 128:]], axis=1), w[8:]], axis=0)

        def run_jobs(m):
            for fn, span in post.get(count[0], ()):
                tok = fn(m)
                if span:
                    pins.setdefault(count[0] + span, []).append(tok())
            count[0] += 1

        for par, kind, cs in rounds:
            r0 = kind * HD + cs[0] * 128
            rows = 128 * len(cs)

            def prod(i):
                if (par, kind) == (1, V_):
                    rhs = ld(sc7_v.at[i], 0, HT1 // 2, 0, HD, SW1)
                else:
                    rhs = tiles(s_v[par].at[i], 0, HT1, not SW1)
                if (par, kind, cs[0]) == (1, K_, 0):
                    sc7_v[i, srows(SW1, 0, HT1 // 2), :] = rhs
                m = lax.dot_general(_unpack(tiles(wt_v.at[i], r0, rows, False)),
                                    _unpack(pinned(rhs)),
                                    _NT, preferred_element_type=f32)
                run_jobs(m)
                return m

            def emit(rh, ch, blk):
                tb = 2 * par + ch
                for n, c in enumerate(cs):
                    for jj in range(2):
                        pair = 4 * c + 2 * rh + jj
                        p = blk[n * 128 + jj * 64:n * 128 + (jj + 1) * 64]
                        if kind == K_:
                            phik_v[tb, srows(SW2, pair * 128, 128, 16), :] = _dual_softmax(p)
                        elif kind == Q_:
                            phiq_v[t0 // 2, tb, pair * 128:(pair + 1) * 128, :] = (
                                _dual_softmax(p))
                        else:
                            vt_v[pair // 8][tb, srows(SW2, (pair % 8) * 64, 64, 16), :] = (
                                p.astype(bf16))

            _strassen(prod, emit)

        ones = jnp.full((8, 2 * T1), 0x3F803F80, u32)
        kr = lax.broadcasted_iota(jnp.int32, (80, 128), 0)
        kc = lax.broadcasted_iota(jnp.int32, (80, 128), 1)
        kmask = jnp.where(kr < 64, kr // 32, (kr - 64) // 8) == kc % 2
        for j in range(NP):
            lhs = jnp.concatenate([tiles(vt_v[j // 8], (j % 8) * 64, 64, not SW2), ones], axis=0)
            rhs = tiles(phik_v, j * 128, 128, not SW2)
            upd = lax.dot_general(_unpack(lhs), _unpack(pinned(rhs)), _NT,
                                  preferred_element_type=f32)
            run_jobs(upd)
            if first:
                kv_acc[j] = upd
            else:
                upd = kv_acc[j] + upd
                kv_acc[j] = upd
                kvt_v[j] = jnp.where(kmask, upd, 0.0).astype(bf16)

    def load_best():
        return best_v[0], besti_v[...], best_v[1], best_v[2]

    def store_best(best):
        best_v[0], besti_v[...], best_v[1], best_v[2] = best

    def build_pt(g0, g1):
        n = g1 - g0
        w2 = wphi_v[4 * g0:4 * g1].reshape(n * 128, DH)
        er = lax.broadcasted_iota(jnp.int32, (128, DH), 0)
        ec = lax.broadcasted_iota(jnp.int32, (128, DH), 1)
        e = jnp.where(ec == (er % 64) // 2, 1.0, 0.0).astype(bf16)
        ptf = lax.dot_general(e, w2, _NT, preferred_element_type=f32)
        pr = lax.broadcasted_iota(jnp.int32, (128, 128), 0)
        pc = lax.broadcasted_iota(jnp.int32, (128, 128), 1)
        keep = pc // 32 == (pr // 64) * 2 + pr % 2
        return [jnp.where(keep, ptf[:, g * 128:(g + 1) * 128], 0.0).astype(bf16)
                for g in range(n)]

    hbl_v[...] = jnp.zeros_like(hbl_v)
    hbr_v[...] = jnp.zeros_like(hbr_v)
    store_best((jnp.full((8, 128), -jnp.inf, f32), jnp.zeros((8, 128), jnp.int32),
                jnp.zeros((8, 128), f32), jnp.zeros((8, 128), f32)))
    n_ln = HT1 // LN_ROWS
    x0_copy(0).wait()
    x0_copy(1).wait()
    for p in range(n_ln // 2):
        ln1_piece(0, s_v[0], p)
    full_copy(wr_hbm, wr_v, SEM_WR).wait()
    phi_copy(0).wait()
    x0_copy(2).wait()
    x0_copy(3).wait()
    wr_row = wr_v[...].astype(f32).reshape(1, D)
    wrf_v[...] = jnp.broadcast_to(
        wr_row - jnp.sum(wr_row, axis=-1, keepdims=True) * (1.0 / D), (8, D))
    pt = build_pt(0, 4)
    for p in range(n_ln // 2, n_ln):
        ln1_piece(0, s_v[0], p)
    for part in range(2):
        k0_copy(2 * part).wait()
        k0_copy(2 * part + 1).wait()
        fold_piece(K_, 0, 2 * part, pt)
        fold_piece(K_, 0, 2 * part + 1, pt)

    post = {}

    def at(slot, fn, span=0):
        post.setdefault(slot, []).append((fn, span))

    for slot, copies in T0_WAITS:
        for cp in copies:
            if cp == 'phi':
                at(slot, lambda m: phi_copy(1).wait())
            elif cp in ('x1', 'x2', 'x3'):
                at(slot, lambda m, cp=cp: x_copy(int(cp[1])).wait())
            else:
                at(slot, lambda m, cp=cp: w_copy(cp // NWC, cp % NWC).wait())
    for n in range(1, 2 * NWC):
        if n == 2:
            at(T0_FOLD[n], lambda m: pt.extend(build_pt(4, 8)))
        at(T0_FOLD[n], lambda m, n=n: fold_chunk(n // NWC, n % NWC, pt))
    for c in range(NWC):
        for j in range(4):
            at(T0_VPREP[c][j], lambda m, c=c, j=j: vprep_piece(c, j, m), T0_VSPAN)
    for p in range(n_ln):
        at(T0_LN[p], lambda m, p=p: ln1_piece(zs + T1, s_v[1], p, m), T0_LNSPAN[p])
    for p in range(n_ln):
        at(T1_LN[0][p], lambda m, p=p: ln1_piece(zs + 2 * T1, s_v[0], p, m), P1_LNSPAN)
        at(T1_LN[1][p], lambda m, p=p: ln1_piece(zs + 3 * T1, s_v[1], p, m), P1_LNSPAN)
    lo, hi = [0, 1], [2, 3]
    run_rounds(0, [(0, kind, [c]) for kind in (K_, Q_) for c in range(NWC)]
               + [(1, K_, lo), (1, K_, hi), (1, Q_, lo), (1, Q_, hi),
                  (0, V_, lo), (0, V_, hi), (1, V_, lo), (1, V_, hi)], post, True)
    full_copy(wo_hbm, wo_v.at[pl.ds(0, D), :], SEM_WO).wait()
    for i in range(4, N1):
        x_copy(i).wait()

    def phase1(i, carry):
        post = {}
        nxt = jnp.minimum(i + 1, N2 - 1) * T2
        w0 = jnp.minimum((i - 1) * WO_ROWS, HD - WO_ROWS)
        for par in range(2):
            for p in range(n_ln):
                post.setdefault(P1_LN2[par][p], []).append(
                    (lambda m, p=p, par=par: ln1_piece(nxt + par * T1, s_v[par], p, m, False),
                     P1_LNSPAN2[par]))
        for p in range(WO_ROWS // 16):
            post.setdefault(P1_WO[p], []).append(
                (lambda m, p=p: wo_piece(w0 + 16 * p, m), P1_WOSPAN))
        run_rounds(2 * i, [(par, kind, cs) for kind in (K_, Q_, V_) for par in range(2)
                           for cs in ([0, 1], [2, 3])], post, False)
        return carry

    lax.fori_loop(1, N1 // 2, phase1, 0)

    for _, dst, rows, slot in ffn_tiled:
        filled = dst.at[:, pl.ds(0, rows), :]
        full_copy(filled, filled, slot).wait()
    full_copy(wg_hbm.at[:, pl.ds(f0, F - f0)], wgv_v, SEM_WGV).wait()
    full_copy(wu_hbm.at[:, pl.ds(f0, F - f0)], wuv_v, SEM_WUV).wait()

    def o_copy(hf):
        return pltpu.make_async_copy(
            out_v.at[pl.ds(hf * HT2, HT2), :], out_hbm.at[0, pl.ds(hf * HT2, HT2), :],
            sem.at[SEM_O + hf])

    def half_stats(hh, c0):
        rows = hh.shape[0]
        parts = [hh[:, c * 128:(c + 1) * 128] for c in range(4)]
        wts = [wrf_v[:, c0 + c * 128:c0 + (c + 1) * 128] for c in range(4)]
        s1 = (parts[0] + parts[1]) + (parts[2] + parts[3])
        sq = [p * p for p in parts]
        s2 = (sq[0] + sq[1]) + (sq[2] + sq[3])
        dw = [(p.reshape(rows // 8, 8, 128) * w[None]).reshape(rows, 128)
              for p, w in zip(parts, wts)]
        s3 = (dw[0] + dw[1]) + (dw[2] + dw[3])
        return s1, s2, s3

    def first_half(hbuf, sbuf, base, p, c0):
        r0 = p * EP_ROWS
        hh = ld(hbuf[c0 // HD], r0, EP_ROWS, 0, HD, SW3)
        h_v[pl.ds(pl.multiple_of(base + r0, EP_ROWS), EP_ROWS), c0:c0 + HD] = hh.astype(bf16)
        st = jnp.concatenate(half_stats(hh, c0), axis=1)
        sbuf[srows(SW3, r0, EP_ROWS), :] = st
        return _fold_token(pltpu.bitcast(st, u32), zero_v)

    def finish(hbuf, sbuf, base, p, valid, best, defer=None):
        r0 = p * EP_ROWS
        g0 = pl.multiple_of(base + r0, EP_ROWS)
        hl, hr = [ld(r, r0, EP_ROWS, 0, HD, SW3) for r in hbuf]
        if defer is None:
            h_v[pl.ds(g0, EP_ROWS), 0:HD] = hl.astype(bf16)
        if sbuf is None:
            if defer is None:
                h_v[pl.ds(g0, EP_ROWS), HD:D] = hr.astype(bf16)
            st = half_stats(hr, HD)
        else:
            st = ld(sbuf, r0, EP_ROWS, 0, 384, SW3)
            st = [st[:, n * 128:(n + 1) * 128] for n in range(3)]
        s1, s2, s3 = [jnp.sum(v + w, axis=-1, keepdims=True)
                      for v, w in zip(half_stats(hl, 0), st)]
        m = s1 * (1.0 / D)
        var = jnp.maximum(s2 * (1.0 / D) - m * m, 0.0)
        inv = _rsqrt(var + EPS)
        r = s3 * inv

        def write_out(h):
            o = h * (1.0 + inv) - m * inv
            out_v[pl.ds(g0, EP_ROWS), :] = o.astype(bf16)
            return o

        if defer is None:
            o = write_out(jnp.concatenate([hl, hr], axis=1))
        else:
            defer.append(lambda: write_out(jnp.concatenate(
                [ld(r_, r0, EP_ROWS, 0, HD, SW3) for r_ in hbuf], axis=1)))
        bv, bi, bm, bq = best
        sub = lax.broadcasted_iota(jnp.int32, (8, 128), 0)
        for g in range(EP_ROWS // 8):
            rows = slice(g * 8, (g + 1) * 8)
            rg = jnp.broadcast_to(r[rows], (8, 128))
            if valid is not None:
                rg = jnp.where(valid, rg, -jnp.inf)
            better = rg > bv
            bi = jnp.where(better, sub + (g0 + g * 8), bi)
            bv = jnp.where(better, rg, bv)
            bm = jnp.where(better, jnp.broadcast_to(m[rows], (8, 128)), bm)
            bq = jnp.where(better, jnp.broadcast_to(var[rows], (8, 128)), bq)
        best = (bv, bi, bm, bq)
        if defer is not None:
            return best, None
        tok = _fold_token(pltpu.bitcast(jnp.concatenate(
            [o[:, D - 128:], bv, bm, bq], axis=0), u32), zero_v)
        return best, tok

    n_ep = HT2 // EP_ROWS

    def phase2(i, carry):
        ot = []
        for j in range(NP):
            ph = tiles(phiq_v.at[i], j * 128, 128, False)
            n = jnp.dot(_unpack(kvt_v.bitcast(u32)[j]), _unpack(ph),
                        preferred_element_type=f32)
            r0h = _recip(n[64:72] + 1e-6)
            r1h = _recip(n[72:80] + 1e-6)
            ot.append((n[0:32].reshape(4, 8, T2) * r0h[None]).reshape(32, T2))
            ot.append((n[32:64].reshape(4, 8, T2) * r1h[None]).reshape(32, T2))
        lo = jnp.concatenate(ot[:H // 2], axis=0)
        hi = jnp.concatenate(ot[H // 2:], axis=0)
        lcs = _left_combos(lo[:, :HT2], hi[:, :HT2], lo[:, HT2:], hi[:, HT2:])

        state = {'best': load_best()}
        pins = {}
        jobs = {}
        lts = {}
        ra = pl.multiple_of(i * T2, T2)
        rb = pl.multiple_of(i * T2 + HT2, HT2)
        prev = jnp.maximum(i * T2 - HT2, HT2)

        def add_job(slot, deadline, fn, gates=()):
            jobs.setdefault(slot, []).append((fn, deadline, gates))

        def finish_job(hbuf, sbuf, base, p, valid):
            def fn():
                state['best'], tok = finish(hbuf, sbuf, base, p, valid, state['best'])
                return tok
            return fn

        def lt_job(k):
            def fn():
                lts[k] = lcs[k].astype(bf16).T
                return _fold_token(pltpu.bitcast(lts[k], u32), zero_v)
            return fn

        order = (2, 4, 6, 0, 3, 1, 5)
        lt_job(2)()
        for n in range(1, 7):
            add_job(LT_START[n], min(LT_START[n] + LT_SPAN[n], 4 * n), lt_job(order[n]))
        for p in range(n_ep):
            add_job(FB_START[p], FB_START[p] + FB_SPAN, finish_job(hb_v, None, prev, p, i > 0), hb_v)
            add_job(SA_START[p], SA_START[p] + SA_SPAN, lambda p=p: first_half(ha_v, sa_v, ra, p, HD), ha_v[1:])
            add_job(FA_START[p], FA_START[p] + FA_SPAN[p], finish_job(ha_v, sa_v, ra, p, None), ha_v)

        def xblk(r0, c0):
            return x_v[pl.ds(r0, HT2), c0:c0 + 128].astype(f32)

        for n, k in enumerate(order):
            for c in range(4):
                slot = 4 * n + c
                for fn, deadline, gates in jobs.get(slot, ()):
                    for ref in gates:
                        ref[srows(SW3, HT2, 8), 0:128] = mm[GATE_ROW:GATE_ROW + 8]
                    pins.setdefault(deadline, []).append(fn())
                w = wo7_v.bitcast(u32)[k, c, 0:HD // 2, :]
                toks = pins.get(slot)
                if toks:
                    top = w[0:8]
                    for tk in toks:
                        top = top | tk
                    w = jnp.concatenate([top, w[8:]], axis=0)
                mm = jnp.dot(lts[k], _unpack(w), preferred_element_type=f32)
                c0 = c * 128
                cs = slice(c0, c0 + 128)
                tmp = lambda t: ld(tmp_v[t], 0, HT2, c0, 128, SW4)
                if n == 0:
                    tmp_v[0][srows(SW4, 0, HT2), cs] = mm
                elif n == 1:
                    ha_v[1][srows(SW3, 0, HT2), cs] = (xblk(ra, HD + c0) + tmp(0)) + mm
                    tmp_v[1][srows(SW4, 0, HT2), cs] = xblk(ra, c0) - mm
                elif n == 2:
                    tmp_v[2][srows(SW4, 0, HT2), cs] = tmp(1) + mm
                elif n == 3:
                    tmp_v[3][srows(SW4, 0, HT2), cs] = tmp(2) + mm
                    tmp_v[4][srows(SW4, 0, HT2), cs] = (xblk(rb, HD + c0) + tmp(0)) + mm
                elif n == 4:
                    ha_v[0][srows(SW3, 0, HT2), cs] = tmp(3) + mm
                    tmp_v[5][srows(SW4, 0, HT2), cs] = xblk(rb, c0) + mm
                elif n == 5:
                    hb_v[0][srows(SW3, 0, HT2), cs] = tmp(5) + mm
                    tmp_v[6][srows(SW4, 0, HT2), cs] = tmp(4) - mm
                else:
                    hb_v[1][srows(SW3, 0, HT2), cs] = tmp(6) + mm
        store_best(state['best'])
        o_copy(2 * i).start()

        @pl.when(i > 0)
        def _():
            o_copy(2 * i - 1).start()

        return carry

    lax.fori_loop(0, N2, phase2, 0)
    best = load_best()
    late = []
    for p in range(n_ep):
        best, _ = finish(hb_v, None, S - HT2, p, None, best, late)


    bv, bi, bm, bq = best
    for sh in (4, 2, 1):
        ov, oi, om, oq = [pltpu.roll(t, sh, 0) for t in (bv, bi, bm, bq)]
        take = jnp.logical_or(ov > bv, jnp.logical_and(ov == bv, oi < bi))
        bv, bi, bm, bq = [jnp.where(take, o_, t)
                          for o_, t in zip((ov, oi, om, oq), (bv, bi, bm, bq))]
    idx = jnp.clip(bi[0, 0], 0, S - 1)
    b0 = pl.multiple_of((idx // 8) * 8, 8)
    t = _rb(_rb(bq) + EPS)
    inv = _recip(_rb(t * _rsqrt(t)))
    gate = _sigmoid(bv)
    wide = lambda v: jnp.concatenate([v] * (D // 128), axis=1)
    b1 = pl.multiple_of(jnp.minimum(b0, S - HT2 - 8), 8)
    b2 = pl.multiple_of(jnp.maximum(b0 - (S - HT2), 0), 8)
    hb = jnp.where(wide(bi) < S - HT2, h_v[pl.ds(b1, 8), :].astype(f32),
                   _rb(jnp.concatenate([r_[pl.ds(b2, 8), :] for r_ in hb_v], axis=1)))
    hn = (hb - wide(bm)) * wide(inv)
    xs = hn.astype(bf16)
    rows = lax.broadcasted_iota(jnp.int32, (8, D), 0) + b0

    xm = jnp.where(rows == wide(bi), _rb(hn), 0.0)
    for sh in (4, 2, 1):
        xm = xm + pltpu.roll(xm, sh, 0)
    for t in range(D // 128):
        xcol_v[t // 2][zrows((t % 2) * 128, 128), :] = jnp.concatenate(
            [xm[:, t * 128:(t + 1) * 128]] * 16, axis=0).T

    nblk = F // 256
    nmx = nblk - FFN_VPU_BLOCKS
    act = {}
    acc = {}

    def activate(g, u):
        return (g * _sigmoid(g) * u).astype(bf16)

    parts = D // 8 // FFN_KG

    def vpu_chunk(q):
        blk, part = nmx + q // parts, q % parts
        cur = acc.get(blk)
        for kg in range(part * FFN_KG, (part + 1) * FFN_KG):
            xc = xcol_v[kg // 32][(kg % 32) * 8:(kg % 32 + 1) * 8, :]
            w = jnp.concatenate(
                [r[kg * 8:(kg + 1) * 8, (blk - nmx) * 256:(blk - nmx + 1) * 256].astype(f32)
                 for r in (wgv_v, wuv_v)], axis=1)
            p = w * jnp.concatenate([xc] * 4, axis=1)
            cur = p if cur is None else cur + p
        acc[blk] = cur
        if part == parts - 1:
            for sh in (4, 2, 1):
                cur = cur + pltpu.roll(cur, sh, 0)
            act[blk] = activate(cur[:, :256], cur[:, 256:])
        if FFN_TOKALL:
            return _fold_token(pltpu.bitcast(cur, u32), zero_v)
        c = q % 4
        return _fold_token(pltpu.bitcast(cur[:, c * 128:(c + 1) * 128], u32), zero_v)

    nchunk = FFN_VPU_BLOCKS * parts
    starts = [FFN_W0 + (q * (FFN_W1 - FFN_W0)) // (nchunk - 1) for q in range(nchunk)]
    pins = {}
    xs16 = jnp.zeros((16, 256), bf16)
    wave = [0]
    wgw, wuw, wdw = [r.bitcast(u32) for r in (wg_v, wu_v, wd_v)]

    def run_wave(lhs, tls):
        top = tls[0][0:8]
        for tk in pins.get(wave[0], ()):
            top = top | tk
        w = jnp.concatenate([jnp.concatenate([top, tls[0][8:]], axis=0)] + tls[1:], axis=1)
        out = jnp.dot(lhs, _unpack(w), preferred_element_type=f32)
        for p, fn in enumerate(late):
            if LATE_AT[p] == wave[0]:
                for r_ in hb_v:
                    r_[srows(SW3, HT2, 8), 0:128] = out[:, 0:128] if LATE_GATE else hn[:, 0:128]
                tk = token(fn()[:, D - 128:])
                if LATE_SPAN:
                    pins.setdefault(wave[0] + LATE_SPAN, []).append(tk())
        for q, start in enumerate(starts):
            if start == wave[0]:
                pins.setdefault(wave[0] + FFN_SPAN, []).append(vpu_chunk(q))
        if wave[0] == FFN_LATE:
            o_copy(2 * N2 - 1).start()
            out_v[pl.ds(pl.multiple_of(zs * 16 + S, 16), 16), 0:256] = xs16
            pins.setdefault(wave[0] + 4, []).append(
                token(out_v[S:S + 8, 0:128].astype(f32))())
        wave[0] += 1
        return out

    for j in range(nmx):
        gu = None
        for kt in range(D // 128):
            p = run_wave(xs[:, kt * 128:(kt + 1) * 128],
                         [r[2 * j + c, kt * 64:(kt + 1) * 64, :]
                          for r in (wgw, wuw) for c in range(2)])
            gu = p if gu is None else gu + p
        act[j] = activate(gu[:, :256], gu[:, 256:])
    ys = [None, None]
    for j in range(nblk):
        for kt in range(2):
            for hf in range(2):
                r0 = (2 * j + kt) * 64
                p = run_wave(act[j][:, kt * 128:(kt + 1) * 128],
                             [wdw[4 * hf + c, r0:r0 + 64, :] for c in range(4)])
                ys[hf] = p if ys[hf] is None else ys[hf] + p
    y = jnp.concatenate(ys, axis=1)
    cur = out_v[pl.ds(b0, 8), :].astype(f32)
    fix_v[...] = jnp.where(rows == wide(bi), hb + hn + y * wide(gate), cur).astype(bf16)
    for hf in range(2 * N2):
        o_copy(hf).wait()
    fix = pltpu.make_async_copy(fix_v, out_hbm.at[0, pl.ds(b0, 8), :], sem.at[SEM_O])
    fix.start()
    fix.wait()


def _kernel(*refs):
    def step(i, carry):
        @pl.when(i == 0)
        def _():
            _body(i, *refs)

        return carry

    lax.fori_loop(0, 2, step, 0)


@jax.jit
def pallas_sequential_preLN__linear_kernel_hedgehog__moe_arch_mod__prompt_kernel(
    A_x: jax.Array,
    A_wqkv: jax.Array,
    A_w_phi: jax.Array,
    A_wo: jax.Array,
    B_x: jax.Array,
    B_w_r: jax.Array,
    B_w_gate: jax.Array,
    B_w_up: jax.Array,
    B_w_down: jax.Array,
):
    any_spec = pl.BlockSpec(memory_space=pl.ANY)
    return pl.pallas_call(
        _kernel,
        out_shape=jax.ShapeDtypeStruct((1, S, D), bf16),
        in_specs=[any_spec] * 8,
        out_specs=any_spec,
        scratch_shapes=[
            pltpu.VMEM((S + 16, D), bf16),
            pltpu.VMEM((3 * NWC + 1, D, WC), bf16),
            pltpu.VMEM((H, DH, DH), bf16),
            pltpu.VMEM((D + 16, D), bf16),
            pltpu.VMEM((D,), bf16),
            pltpu.VMEM((F // 128 - 2 * FFN_VPU_BLOCKS, D + PAD, 128), bf16),
            pltpu.VMEM((F // 128 - 2 * FFN_VPU_BLOCKS, D + PAD, 128), bf16),
            pltpu.VMEM((D // 128, F + PAD, 128), bf16),
            pltpu.VMEM((D, 256 * FFN_VPU_BLOCKS), bf16),
            pltpu.VMEM((D, 256 * FFN_VPU_BLOCKS), bf16),
            pltpu.VMEM((7, 4, 3 * HD + PAD, 128), bf16),
            pltpu.VMEM((7, 4, HD + PAD, 128), bf16),
            pltpu.VMEM((7, 4, HT1 + PAD, 128), bf16),
            pltpu.VMEM((7, 4, HT1 + PAD, 128), bf16),
            pltpu.VMEM((7, HT1 // 2, HD), u32),
            pltpu.VMEM((N2, 4, 2 * D + PAD, 128), bf16),
            pltpu.VMEM((4, 2 * D + PAD, 128), bf16),
            pltpu.VMEM((4, HD + PAD, 128), bf16),
            pltpu.VMEM((4, HD + PAD, 128), bf16),
            pltpu.VMEM((NP, 80, 128), f32),
            pltpu.VMEM((NP, 80, 128), bf16),
            *[pltpu.VMEM((HT2 + 8, HD), f32) for _ in range(4)],
            pltpu.VMEM((HT2, 384), f32),
            *[pltpu.VMEM((HT2, HD), f32) for _ in range(7)],
            pltpu.VMEM((S, D), bf16),
            pltpu.VMEM((S + 16, D), bf16),
            pltpu.VMEM((8, D), f32),
            pltpu.VMEM((3, 8, 128), f32),
            pltpu.VMEM((8, 128), jnp.int32),
            pltpu.VMEM((8, D), bf16),
            *[pltpu.VMEM((264, 128), f32) for _ in range(4)],
            pltpu.SemaphoreType.DMA((NSEM,)),
        ],
        compiler_params=pltpu.CompilerParams(
            vmem_limit_bytes=110 * 1024 * 1024,
            disable_bounds_checks=True,
            disable_semaphore_checks=True),
    )(A_x, A_wqkv, A_w_phi, A_wo, B_w_r, B_w_gate, B_w_up, B_w_down)
```

```python
import jax
import jax.numpy as jnp
from jax import lax
import jax.experimental.pallas as pl
import jax.experimental.pallas.tpu as pltpu

S = 2048
D = 1024
H = 32
DH = 32
F = 3584
NP = H // 2
T1 = 256
T2 = 512
N1 = S // T1
N2 = S // T2
HT1 = T1 // 2
HT2 = T2 // 2
HD = D // 2
WC = 256
NWC = D // WC
LOG2E = 1.4426950408889634
EPS = 1e-5
PAD = 16
WO_ROWS = 176
LN_ROWS = 16
EP_ROWS = 32

T0_FOLD = (0, 4, 11, 18, 25, 33, 39, 46)
T0_WAITS = ((4, (1,)), (11, ('phi', 2)), (18, (3, 4)), (33, ('x1', 5, 6)), (46, (7,)),
            (73, (8, 9, 10, 11, 'x2', 'x3')))
T0_VPREP = ((73, 74, 75, 76), (77, 78, 79, 80), (81, 82, 83, 84), (85, 86, 87, 88))
T0_VSPAN = 4
T0_LN = (33, 35, 36, 37, 38, 39, 40, 43)
T0_LNSPAN = (3, 0, 0, 0, 0, 0, 0, 0)
T1_LN = ((99, 100, 101, 102, 103, 104, 105, 106), (90, 91, 92, 93, 94, 95, 96, 97))
P1_LNSPAN = 3
P1_WO = (57, 58, 59, 60, 63, 77, 79, 80, 81, 82, 83)
P1_WOSPAN = 3
P1_LN2 = ((70, 71, 72, 73, 74, 75, 76, 77), (62, 63, 64, 65, 66, 67, 68, 69))
P1_LNSPAN2 = (2, 2)
LT_START = (0, 0, 1, 5, 8, 11, 14)
LT_SPAN = (0, 2, 4, 4, 4, 4, 4)
FB_START = (2, 4, 6, 8, 10, 12, 14, 16)
FB_SPAN = 2
SA_START = (9, 11, 15, 15, 17, 17, 18, 18)
SA_SPAN = 3
FA_START = (20, 21, 22, 23, 24, 25, 26, 27)
FA_SPAN = (3, 7, 2, 5, 3, 5, 3, 2)
FFN_VPU_BLOCKS = 7
FFN_KG = 16
FFN_W0 = 18
FFN_W1 = 107
FFN_SPAN = 4
FFN_LATE = 16
LATE_AT = (1, 2, 3, 3, 4, 6, 6, 7)

_NT = (((1,), (1,)), ((), ()))
f32 = jnp.float32
bf16 = jnp.bfloat16
u32 = jnp.uint32

K_, Q_, V_ = 0, 1, 2
SRC = {K_: 1, Q_: 0, V_: 2}

SEM_W = 0
SEM_X = SEM_W + 3 * NWC
SEM_X0 = SEM_X + N1
SEM_K0 = SEM_X0 + 4
SEM_PHI = SEM_K0 + 4
SEM_WO = SEM_PHI + 2
SEM_WR, SEM_WG, SEM_WU, SEM_WD, SEM_WGV, SEM_WUV, SEM_O = (SEM_WO + 1 + i for i in range(7))
NSEM = SEM_O + 1


def _rb(v):
    return v.astype(bf16).astype(f32)


def _unpack(w):
    return pltpu.bitcast(w, bf16)


def _mo(i, n):
    return i if isinstance(i, int) else pl.multiple_of(i, n)


def _recip(x):
    r = pl.reciprocal(x, approx=True)
    return r * (2.0 - x * r)


def _sigmoid(x):
    return _recip(1.0 + jnp.exp(jnp.minimum(-x, 80.0)))


def _dual_softmax(p):
    t = p.shape[-1]
    p3 = p.reshape(8, 8, t)

    def allred(v, op):
        v = op(v, pltpu.roll(v, 2, 0))
        return op(v, pltpu.roll(v, 4, 0))

    mx = allred(jnp.max(p3, axis=0), jnp.maximum)
    mn = allred(jnp.min(p3, axis=0), jnp.minimum)
    ep = jnp.exp2(p3 - mx[None])
    en = jnp.exp2(mn[None] - p3)
    sp = allred(jnp.sum(ep, axis=0), jnp.add)
    sn = allred(jnp.sum(en, axis=0), jnp.add)
    fp = (ep * _recip(sp)[None]).reshape(64, t)
    fn = (en * _recip(sn)[None]).reshape(64, t)
    return jnp.concatenate([fp, fn], axis=0).astype(bf16)


def _left_combos(a11, a12, a21, a22):
    return [a11 + a22, a21 + a22, a11, a22, a11 + a12, a21 - a11, a12 - a22]


def _right_combos(b11, b12, b21, b22):
    return [b11 + b22, b11, b12 - b22, b21 - b11, b22, b11 + b12, b21 + b22]


def _strassen(prod, emit):
    m3 = prod(2)
    m5 = prod(4)
    emit(0, 1, m3 + m5)
    m7 = prod(6)
    u = m7 - m5
    m1 = prod(0)
    u = u + m1
    w = m1 + m3
    m4 = prod(3)
    emit(0, 0, u + m4)
    m2 = prod(1)
    emit(1, 0, m2 + m4)
    w = w - m2
    m6 = prod(5)
    emit(1, 1, w + m6)


def _or_into(w, toks):
    if not toks:
        return w
    top = w[0:8, 0:128]
    for tk in toks:
        top = top | tk
    if w.shape[1] > 128:
        top = jnp.concatenate([top, w[0:8, 128:]], axis=1)
    return jnp.concatenate([top, w[8:]], axis=0)


def _fold_token(w, zero):
    r, c = w.shape
    acc = None
    for i in range(r // 8):
        for j in range(c // 128):
            blk = w[i * 8:(i + 1) * 8, j * 128:(j + 1) * 128]
            acc = blk if acc is None else acc | blk
    return acc & zero


def _body(zs, x_hbm, wqkv_hbm, wphi_hbm, wo_hbm, wr_hbm, wg_hbm, wu_hbm, wd_hbm, out_hbm,
          x_v, wqkv_v, wphi_v, wo_v, wr_v, wg_v, wu_v, wd_v, wgv_v, wuv_v,
          wt_v, wo7_v, sa7_v, sb7_v, sc7_v, phiq_v, phik_v, vt0_v, vt1_v, kv_acc, kvt_v,
          hal_v, har_v, hbl_v, hbr_v, sa_v, t0_v, t1_v, t2_v, t3_v, t4_v, t5_v, t6_v,
          h_v, out_v, wrf_v, best_v, besti_v, fix_v, xc0_v, xc1_v, xc2_v, xc3_v, sem):
    xcol_v = (xc0_v, xc1_v, xc2_v, xc3_v)
    s_v = (sa7_v, sb7_v)
    vt_v = (vt0_v, vt1_v)
    ha_v = (hal_v, har_v)
    hb_v = (hbl_v, hbr_v)
    tmp_v = (t0_v, t1_v, t2_v, t3_v, t4_v, t5_v, t6_v)

    def x_rows(r0, rows, slot):
        return pltpu.make_async_copy(
            x_hbm.at[0, pl.ds(r0, rows), :], x_v.at[pl.ds(r0, rows), :], sem.at[slot])

    def x_copy(i):
        return x_rows(i * T1, T1, SEM_X + i)

    def x0_copy(q):
        return x_rows((q % 2) * HT1 + (q // 2) * (HT1 // 2), HT1 // 2, SEM_X0 + q)

    def w_copy(kind, c):
        return pltpu.make_async_copy(
            wqkv_hbm.at[:, pl.ds(SRC[kind] * D + c * WC, WC)],
            wqkv_v.at[kind * NWC + c], sem.at[SEM_W + kind * NWC + c])

    def k0_copy(q):
        r0 = (q % 2) * HD + (q // 2) * 256
        return pltpu.make_async_copy(
            wqkv_hbm.at[pl.ds(r0, 256), pl.ds(SRC[K_] * D, WC)],
            wqkv_v.at[K_ * NWC, pl.ds(r0, 256), :], sem.at[SEM_K0 + q])

    def phi_copy(part):
        lo, n = part * (H // 2), H // 2
        return pltpu.make_async_copy(wphi_hbm.at[pl.ds(lo, n)], wphi_v.at[pl.ds(lo, n)],
                                     sem.at[SEM_PHI + part])

    def full_copy(src, dst, slot):
        return pltpu.make_async_copy(src, dst, sem.at[slot])

    x0_copy(0).start()
    x0_copy(1).start()
    full_copy(wr_hbm, wr_v, SEM_WR).start()
    phi_copy(0).start()
    x0_copy(2).start()
    x0_copy(3).start()
    for q in range(4):
        k0_copy(q).start()
    w_copy(K_, 1).start()
    phi_copy(1).start()
    w_copy(K_, 2).start()
    w_copy(K_, 3).start()
    w_copy(Q_, 0).start()
    x_copy(1).start()
    for c in range(1, NWC):
        w_copy(Q_, c).start()
    for c in range(NWC):
        w_copy(V_, c).start()
    x_copy(2).start()
    x_copy(3).start()
    full_copy(wo_hbm, wo_v.at[pl.ds(0, D), :], SEM_WO).start()
    for i in range(4, N1):
        x_copy(i).start()
    f0 = F - 256 * FFN_VPU_BLOCKS
    ffn_tiled = ((wg_hbm, wg_v, D, SEM_WG), (wu_hbm, wu_v, D, SEM_WU), (wd_hbm, wd_v, F, SEM_WD))
    for src, dst, rows, slot in ffn_tiled:
        for c in range(dst.shape[0]):
            full_copy(src.at[:, pl.ds(c * 128, 128)], dst.at[c, pl.ds(0, rows), :], slot).start()
    full_copy(wg_hbm.at[:, pl.ds(f0, F - f0)], wgv_v, SEM_WGV).start()
    full_copy(wu_hbm.at[:, pl.ds(f0, F - f0)], wuv_v, SEM_WUV).start()

    zero_v = jnp.full((8, 128), zs, jnp.int32).astype(u32)

    def zrows(r0, rows, mult=8):
        return pl.ds(pl.multiple_of(zs * mult + r0, mult), rows)

    def tiles(ref, r0, rows):
        w = ref.bitcast(u32)
        return jnp.concatenate(
            [w[c, r0 // 2:(r0 + rows) // 2, :] for c in range(ref.shape[0])], axis=1)

    def token(*vals):
        return lambda: _fold_token(pltpu.bitcast(jnp.concatenate(vals, axis=0), u32), zero_v)

    def ln1_stats(xf):
        m = jnp.sum(xf, axis=-1, keepdims=True) * (1.0 / D)
        q = jnp.sum(xf * xf, axis=-1, keepdims=True) * (1.0 / D)
        inv = lax.rsqrt(jnp.maximum(q - m * m, 0.0) + EPS)
        return inv, m * inv

    def ln1_piece(r0, dst, p, m=None):
        fixed = isinstance(r0, int)
        if m is not None:
            x_v[zrows(S, 8) if fixed else pl.ds(S, 8), 0:128] = m[0:8, 0:128].astype(bf16)
        xa, xb = [x_v[pl.ds(_mo(r0 + hf * HT1 + p * LN_ROWS, LN_ROWS), LN_ROWS), :]
                  .astype(f32) for hf in range(2)]
        (ia, ma), (ib, mb) = ln1_stats(xa), ln1_stats(xb)
        ya, yb = xa * ia, xb * ib
        s2 = ya[:, :HD] - ma
        s5 = yb[:, HD:] - mb
        s1 = s2 + s5
        s3 = yb[:, :HD] - yb[:, HD:]
        s4 = ya[:, HD:] - ya[:, :HD]
        combos = [s1, s2, s3, s4, s5, s1 + s3, s1 + s4]
        rows = zrows(p * LN_ROWS, LN_ROWS, 16) if fixed else pl.ds(p * LN_ROWS, LN_ROWS)
        for i in range(7):
            for c in range(4):
                dst[i, c, rows, :] = combos[i][:, c * 128:(c + 1) * 128].astype(bf16)
        return token(combos[5], combos[6])

    def fold_piece(kind, c, j, pt):
        blk = {}
        for hh in range(2):
            for kh in range(2):
                k0 = kh * HD + j * 128
                w = wqkv_v[kind * NWC + c, k0:k0 + 128, hh * 128:(hh + 1) * 128]
                blk[hh, kh] = lax.dot_general(pt[2 * c + hh], w, _NT,
                                              preferred_element_type=f32) * LOG2E
        combos = _left_combos(blk[0, 0], blk[0, 1], blk[1, 0], blk[1, 1])
        r0 = kind * HD + c * 128
        for i in range(7):
            wt_v[i, j, r0:r0 + 128, :] = combos[i].astype(bf16)

    def fold_chunk(kind, c, pt):
        for j in range(4):
            fold_piece(kind, c, j, pt)

    def vprep_piece(c, j, m):
        wqkv_v[zs + 3 * NWC, 0:8, 0:128] = m[0:8, 0:128].astype(bf16)
        blk = {}
        for hh in range(2):
            for kh in range(2):
                k0 = kh * HD + j * 128
                w = wqkv_v[V_ * NWC + c, k0:k0 + 128, hh * 128:(hh + 1) * 128]
                blk[hh, kh] = w.T.astype(f32)
        combos = _left_combos(blk[0, 0], blk[0, 1], blk[1, 0], blk[1, 1])
        r0 = V_ * HD + c * 128
        for i in range(7):
            wt_v[i, j, r0:r0 + 128, :] = combos[i].astype(bf16)
        return token(combos[1], combos[4])

    def wo_piece(w0, m):
        wo_v[D:D + 8, 0:128] = m[0:8, 0:128].astype(bf16)
        top = wo_v[pl.ds(pl.multiple_of(w0, 16), 16), :].astype(f32)
        bot = wo_v[pl.ds(pl.multiple_of(HD + w0, 16), 16), :].astype(f32)
        combos = _right_combos(top[:, :HD], top[:, HD:], bot[:, :HD], bot[:, HD:])
        for i in range(7):
            for c in range(4):
                wo7_v[i, c, pl.ds(pl.multiple_of(w0, 16), 16), :] = (
                    combos[i][:, c * 128:(c + 1) * 128].astype(bf16))
        return token(combos[5], combos[6])

    def run_rounds(t0, rounds, post, first):
        count = [0]
        pins = {}

        def run_jobs(m):
            for fn, span in post.get(count[0], ()):
                tok = fn(m)
                if span:
                    pins.setdefault(count[0] + span, []).append(tok())
            count[0] += 1

        for par, kind, cs in rounds:
            r0 = kind * HD + cs[0] * 128
            rows = 128 * len(cs)

            def prod(i):
                if (par, kind) == (1, V_):
                    rhs = sc7_v[i]
                else:
                    rhs = tiles(s_v[par].at[i], 0, HT1)
                if (par, kind, cs[0]) == (1, K_, 0):
                    sc7_v[i, zrows(0, HT1 // 2), :] = rhs
                m = lax.dot_general(_unpack(tiles(wt_v.at[i], r0, rows)),
                                    _unpack(_or_into(rhs, pins.get(count[0]))),
                                    _NT, preferred_element_type=f32)
                run_jobs(m)
                return m

            def emit(rh, ch, blk):
                tb = 2 * par + ch
                for n, c in enumerate(cs):
                    for jj in range(2):
                        pair = 4 * c + 2 * rh + jj
                        p = blk[n * 128 + jj * 64:n * 128 + (jj + 1) * 64]
                        if kind == K_:
                            phik_v[tb, zrows(pair * 128, 128, 16), :] = _dual_softmax(p)
                        elif kind == Q_:
                            phiq_v[t0 // 2, tb, pair * 128:(pair + 1) * 128, :] = (
                                _dual_softmax(p))
                        else:
                            vt_v[pair // 8][tb, zrows((pair % 8) * 64, 64, 16), :] = (
                                p.astype(bf16))

            _strassen(prod, emit)

        ones = jnp.full((8, 2 * T1), 0x3F803F80, u32)
        kr = lax.broadcasted_iota(jnp.int32, (80, 128), 0)
        kc = lax.broadcasted_iota(jnp.int32, (80, 128), 1)
        kmask = jnp.where(kr < 64, kr // 32, (kr - 64) // 8) == kc % 2
        for j in range(NP):
            lhs = jnp.concatenate([tiles(vt_v[j // 8], (j % 8) * 64, 64), ones], axis=0)
            rhs = tiles(phik_v, j * 128, 128)
            upd = lax.dot_general(_unpack(lhs), _unpack(_or_into(rhs, pins.get(count[0]))), _NT,
                                  preferred_element_type=f32)
            run_jobs(upd)
            if first:
                kv_acc[j] = upd
            else:
                upd = kv_acc[j] + upd
                kv_acc[j] = upd
                kvt_v[j] = jnp.where(kmask, upd, 0.0).astype(bf16)

    def load_best():
        return best_v[0], besti_v[...], best_v[1], best_v[2]

    def store_best(best):
        best_v[0], besti_v[...], best_v[1], best_v[2] = best

    def build_pt(g0, g1):
        n = g1 - g0
        w2 = wphi_v[4 * g0:4 * g1].reshape(n * 128, DH)
        er = lax.broadcasted_iota(jnp.int32, (128, DH), 0)
        ec = lax.broadcasted_iota(jnp.int32, (128, DH), 1)
        e = jnp.where(ec == (er % 64) // 2, 1.0, 0.0).astype(bf16)
        ptf = lax.dot_general(e, w2, _NT, preferred_element_type=f32)
        pr = lax.broadcasted_iota(jnp.int32, (128, 128), 0)
        pc = lax.broadcasted_iota(jnp.int32, (128, 128), 1)
        keep = pc // 32 == (pr // 64) * 2 + pr % 2
        return [jnp.where(keep, ptf[:, g * 128:(g + 1) * 128], 0.0).astype(bf16)
                for g in range(n)]

    hbl_v[...] = jnp.zeros_like(hbl_v)
    hbr_v[...] = jnp.zeros_like(hbr_v)
    store_best((jnp.full((8, 128), -jnp.inf, f32), jnp.zeros((8, 128), jnp.int32),
                jnp.zeros((8, 128), f32), jnp.zeros((8, 128), f32)))
    n_ln = HT1 // LN_ROWS
    x0_copy(0).wait()
    x0_copy(1).wait()
    for p in range(n_ln // 2):
        ln1_piece(0, s_v[0], p)
    full_copy(wr_hbm, wr_v, SEM_WR).wait()
    phi_copy(0).wait()
    x0_copy(2).wait()
    x0_copy(3).wait()
    wr_row = wr_v[...].astype(f32).reshape(1, D)
    wrf_v[...] = jnp.broadcast_to(
        wr_row - jnp.sum(wr_row, axis=-1, keepdims=True) * (1.0 / D), (8, D))
    pt = build_pt(0, 4)
    for p in range(n_ln // 2, n_ln):
        ln1_piece(0, s_v[0], p)
    for part in range(2):
        k0_copy(2 * part).wait()
        k0_copy(2 * part + 1).wait()
        fold_piece(K_, 0, 2 * part, pt)
        fold_piece(K_, 0, 2 * part + 1, pt)

    post = {}

    def at(slot, fn, span=0):
        post.setdefault(slot, []).append((fn, span))

    for slot, copies in T0_WAITS:
        for cp in copies:
            if cp == 'phi':
                at(slot, lambda m: phi_copy(1).wait())
            elif cp in ('x1', 'x2', 'x3'):
                at(slot, lambda m, cp=cp: x_copy(int(cp[1])).wait())
            else:
                at(slot, lambda m, cp=cp: w_copy(cp // NWC, cp % NWC).wait())
    for n in range(1, 2 * NWC):
        if n == 2:
            at(T0_FOLD[n], lambda m: pt.extend(build_pt(4, 8)))
        at(T0_FOLD[n], lambda m, n=n: fold_chunk(n // NWC, n % NWC, pt))
    for c in range(NWC):
        for j in range(4):
            at(T0_VPREP[c][j], lambda m, c=c, j=j: vprep_piece(c, j, m), T0_VSPAN)
    for p in range(n_ln):
        at(T0_LN[p], lambda m, p=p: ln1_piece(T1, s_v[1], p, m), T0_LNSPAN[p])
    for p in range(n_ln):
        at(T1_LN[0][p], lambda m, p=p: ln1_piece(2 * T1, s_v[0], p, m), P1_LNSPAN)
        at(T1_LN[1][p], lambda m, p=p: ln1_piece(3 * T1, s_v[1], p, m), P1_LNSPAN)
    lo, hi = [0, 1], [2, 3]
    run_rounds(0, [(0, kind, [c]) for kind in (K_, Q_) for c in range(NWC)]
               + [(1, K_, lo), (1, K_, hi), (1, Q_, lo), (1, Q_, hi),
                  (0, V_, lo), (0, V_, hi), (1, V_, lo), (1, V_, hi)], post, True)
    full_copy(wo_hbm, wo_v.at[pl.ds(0, D), :], SEM_WO).wait()
    for i in range(4, N1):
        x_copy(i).wait()

    def phase1(i, carry):
        post = {}
        nxt = jnp.minimum(i + 1, N2 - 1) * T2
        w0 = jnp.minimum((i - 1) * WO_ROWS, HD - WO_ROWS)
        for par in range(2):
            for p in range(n_ln):
                post.setdefault(P1_LN2[par][p], []).append(
                    (lambda m, p=p, par=par: ln1_piece(nxt + par * T1, s_v[par], p, m),
                     P1_LNSPAN2[par]))
        for p in range(WO_ROWS // 16):
            post.setdefault(P1_WO[p], []).append(
                (lambda m, p=p: wo_piece(w0 + 16 * p, m), P1_WOSPAN))
        run_rounds(2 * i, [(par, kind, cs) for kind in (K_, Q_, V_) for par in range(2)
                           for cs in ([0, 1], [2, 3])], post, False)
        return carry

    lax.fori_loop(1, N1 // 2, phase1, 0)

    for _, dst, rows, slot in ffn_tiled:
        filled = dst.at[:, pl.ds(0, rows), :]
        full_copy(filled, filled, slot).wait()
    full_copy(wg_hbm.at[:, pl.ds(f0, F - f0)], wgv_v, SEM_WGV).wait()
    full_copy(wu_hbm.at[:, pl.ds(f0, F - f0)], wuv_v, SEM_WUV).wait()

    def o_copy(hf):
        return pltpu.make_async_copy(
            out_v.at[pl.ds(hf * HT2, HT2), :], out_hbm.at[0, pl.ds(hf * HT2, HT2), :],
            sem.at[SEM_O])

    def half_stats(hh, c0):
        rows = hh.shape[0]
        parts = [hh[:, c * 128:(c + 1) * 128] for c in range(4)]
        wts = [wrf_v[:, c0 + c * 128:c0 + (c + 1) * 128] for c in range(4)]
        s1 = (parts[0] + parts[1]) + (parts[2] + parts[3])
        sq = [p * p for p in parts]
        s2 = (sq[0] + sq[1]) + (sq[2] + sq[3])
        dw = [(p.reshape(rows // 8, 8, 128) * w[None]).reshape(rows, 128)
              for p, w in zip(parts, wts)]
        s3 = (dw[0] + dw[1]) + (dw[2] + dw[3])
        return s1, s2, s3

    def first_half(hbuf, sbuf, base, p, c0):
        r0 = p * EP_ROWS
        hh = hbuf[c0 // HD][r0:r0 + EP_ROWS, :]
        h_v[pl.ds(pl.multiple_of(base + r0, EP_ROWS), EP_ROWS), c0:c0 + HD] = hh.astype(bf16)
        st = jnp.concatenate(half_stats(hh, c0), axis=1)
        sbuf[zrows(r0, EP_ROWS), :] = st
        return _fold_token(pltpu.bitcast(st, u32), zero_v)

    def finish(hbuf, sbuf, base, p, valid, best, defer=None):
        r0 = p * EP_ROWS
        g0 = pl.multiple_of(base + r0, EP_ROWS)
        hl, hr = [r[r0:r0 + EP_ROWS, :] for r in hbuf]
        if defer is None:
            h_v[pl.ds(g0, EP_ROWS), 0:HD] = hl.astype(bf16)
        if sbuf is None:
            if defer is None:
                h_v[pl.ds(g0, EP_ROWS), HD:D] = hr.astype(bf16)
            st = half_stats(hr, HD)
        else:
            st = sbuf[r0:r0 + EP_ROWS, :]
            st = [st[:, n * 128:(n + 1) * 128] for n in range(3)]
        s1, s2, s3 = [jnp.sum(v + w, axis=-1, keepdims=True)
                      for v, w in zip(half_stats(hl, 0), st)]
        m = s1 * (1.0 / D)
        var = jnp.maximum(s2 * (1.0 / D) - m * m, 0.0)
        inv = lax.rsqrt(var + EPS)
        r = s3 * inv

        def write_out(h):
            o = h * (1.0 + inv) - m * inv
            out_v[pl.ds(g0, EP_ROWS), :] = o.astype(bf16)
            return o

        if defer is None:
            o = write_out(jnp.concatenate([hl, hr], axis=1))
        else:
            defer.append(lambda: write_out(jnp.concatenate(
                [r_[r0:r0 + EP_ROWS, :] for r_ in hbuf], axis=1)))
        bv, bi, bm, bq = best
        sub = lax.broadcasted_iota(jnp.int32, (8, 128), 0)
        for g in range(EP_ROWS // 8):
            rows = slice(g * 8, (g + 1) * 8)
            rg = jnp.broadcast_to(r[rows], (8, 128))
            if valid is not None:
                rg = jnp.where(valid, rg, -jnp.inf)
            better = rg > bv
            bi = jnp.where(better, sub + (g0 + g * 8), bi)
            bv = jnp.where(better, rg, bv)
            bm = jnp.where(better, jnp.broadcast_to(m[rows], (8, 128)), bm)
            bq = jnp.where(better, jnp.broadcast_to(var[rows], (8, 128)), bq)
        best = (bv, bi, bm, bq)
        if defer is not None:
            return best, None
        tok = _fold_token(pltpu.bitcast(jnp.concatenate(
            [o[:, D - 128:], bv, bm, bq], axis=0), u32), zero_v)
        return best, tok

    n_ep = HT2 // EP_ROWS

    def phase2(i, carry):
        ot = []
        for j in range(NP):
            ph = tiles(phiq_v.at[i], j * 128, 128)
            n = jnp.dot(_unpack(kvt_v.bitcast(u32)[j]), _unpack(ph),
                        preferred_element_type=f32)
            r0h = _recip(n[64:72] + 1e-6)
            r1h = _recip(n[72:80] + 1e-6)
            ot.append((n[0:32].reshape(4, 8, T2) * r0h[None]).reshape(32, T2))
            ot.append((n[32:64].reshape(4, 8, T2) * r1h[None]).reshape(32, T2))
        lo = jnp.concatenate(ot[:H // 2], axis=0)
        hi = jnp.concatenate(ot[H // 2:], axis=0)
        lcs = _left_combos(lo[:, :HT2], hi[:, :HT2], lo[:, HT2:], hi[:, HT2:])

        state = {'best': load_best()}
        pins = {}
        jobs = {}
        lts = {}
        ra = pl.multiple_of(i * T2, T2)
        rb = pl.multiple_of(i * T2 + HT2, HT2)
        prev = jnp.maximum(i * T2 - HT2, HT2)

        def add_job(slot, deadline, fn, gates=()):
            jobs.setdefault(slot, []).append((fn, deadline, gates))

        def finish_job(hbuf, sbuf, base, p, valid):
            def fn():
                state['best'], tok = finish(hbuf, sbuf, base, p, valid, state['best'])
                return tok
            return fn

        def lt_job(k):
            def fn():
                lts[k] = lcs[k].astype(bf16).T
                return _fold_token(pltpu.bitcast(lts[k], u32), zero_v)
            return fn

        order = (2, 4, 6, 0, 3, 1, 5)
        lt_job(2)()
        for n in range(1, 7):
            add_job(LT_START[n], min(LT_START[n] + LT_SPAN[n], 4 * n), lt_job(order[n]))
        for p in range(n_ep):
            add_job(FB_START[p], FB_START[p] + FB_SPAN,
                    finish_job(hb_v, None, prev, p, i > 0), hb_v)
            add_job(SA_START[p], SA_START[p] + SA_SPAN,
                    lambda p=p: first_half(ha_v, sa_v, ra, p, HD), ha_v[1:])
            add_job(FA_START[p], FA_START[p] + FA_SPAN[p],
                    finish_job(ha_v, sa_v, ra, p, None), ha_v)

        def xblk(r0, c0):
            return x_v[pl.ds(r0, HT2), c0:c0 + 128].astype(f32)

        for n, k in enumerate(order):
            for c in range(4):
                slot = 4 * n + c
                for fn, deadline, gates in jobs.get(slot, ()):
                    for ref in gates:
                        ref[zrows(HT2, 8), 0:128] = mm[0:8]
                    pins.setdefault(deadline, []).append(fn())
                w = _or_into(wo7_v.bitcast(u32)[k, c, 0:HD // 2, :], pins.get(slot))
                mm = jnp.dot(lts[k], _unpack(w), preferred_element_type=f32)
                c0 = c * 128
                cs = slice(c0, c0 + 128)
                tmp = lambda t: tmp_v[t][:, cs]
                if n == 0:
                    tmp_v[0][zrows(0, HT2), cs] = mm
                elif n == 1:
                    ha_v[1][zrows(0, HT2), cs] = (xblk(ra, HD + c0) + tmp(0)) + mm
                    tmp_v[1][zrows(0, HT2), cs] = xblk(ra, c0) - mm
                elif n == 2:
                    tmp_v[2][zrows(0, HT2), cs] = tmp(1) + mm
                elif n == 3:
                    tmp_v[3][zrows(0, HT2), cs] = tmp(2) + mm
                    tmp_v[4][zrows(0, HT2), cs] = (xblk(rb, HD + c0) + tmp(0)) + mm
                elif n == 4:
                    ha_v[0][zrows(0, HT2), cs] = tmp(3) + mm
                    tmp_v[5][zrows(0, HT2), cs] = xblk(rb, c0) + mm
                elif n == 5:
                    hb_v[0][zrows(0, HT2), cs] = tmp(5) + mm
                    tmp_v[6][zrows(0, HT2), cs] = tmp(4) - mm
                else:
                    hb_v[1][zrows(0, HT2), cs] = tmp(6) + mm
        store_best(state['best'])
        o_copy(2 * i).start()

        @pl.when(i > 0)
        def _():
            o_copy(2 * i - 1).start()

        return carry

    lax.fori_loop(0, N2, phase2, 0)
    best = load_best()
    late = []
    for p in range(n_ep):
        best, _ = finish(hb_v, None, S - HT2, p, None, best, late)

    bv, bi, bm, bq = best
    for sh in (4, 2, 1):
        ov, oi, om, oq = [pltpu.roll(t, sh, 0) for t in (bv, bi, bm, bq)]
        take = jnp.logical_or(ov > bv, jnp.logical_and(ov == bv, oi < bi))
        bv, bi, bm, bq = [jnp.where(take, o_, t)
                          for o_, t in zip((ov, oi, om, oq), (bv, bi, bm, bq))]
    idx = jnp.clip(bi[0, 0], 0, S - 1)
    b0 = pl.multiple_of((idx // 8) * 8, 8)
    t = _rb(_rb(bq) + EPS)
    inv = _recip(_rb(t * lax.rsqrt(t)))
    gate = _sigmoid(bv)
    wide = lambda v: jnp.concatenate([v] * (D // 128), axis=1)
    b1 = pl.multiple_of(jnp.minimum(b0, S - HT2 - 8), 8)
    b2 = pl.multiple_of(jnp.maximum(b0 - (S - HT2), 0), 8)
    hb = jnp.where(wide(bi) < S - HT2, h_v[pl.ds(b1, 8), :].astype(f32),
                   _rb(jnp.concatenate([r_[pl.ds(b2, 8), :] for r_ in hb_v], axis=1)))
    hn = (hb - wide(bm)) * wide(inv)
    xs = hn.astype(bf16)
    rows = lax.broadcasted_iota(jnp.int32, (8, D), 0) + b0

    xm = jnp.where(rows == wide(bi), _rb(hn), 0.0)
    for sh in (4, 2, 1):
        xm = xm + pltpu.roll(xm, sh, 0)
    for t in range(D // 128):
        xcol_v[t // 2][zrows((t % 2) * 128, 128), :] = jnp.concatenate(
            [xm[:, t * 128:(t + 1) * 128]] * 16, axis=0).T

    nblk = F // 256
    nmx = nblk - FFN_VPU_BLOCKS
    act = {}
    acc = {}

    def activate(g, u):
        return (g * _sigmoid(g) * u).astype(bf16)

    parts = D // 8 // FFN_KG

    def vpu_chunk(q):
        blk, part = nmx + q // parts, q % parts
        cur = acc.get(blk)
        for kg in range(part * FFN_KG, (part + 1) * FFN_KG):
            xc = xcol_v[kg // 32][(kg % 32) * 8:(kg % 32 + 1) * 8, :]
            w = jnp.concatenate(
                [r[kg * 8:(kg + 1) * 8, (blk - nmx) * 256:(blk - nmx + 1) * 256].astype(f32)
                 for r in (wgv_v, wuv_v)], axis=1)
            p = w * jnp.concatenate([xc] * 4, axis=1)
            cur = p if cur is None else cur + p
        acc[blk] = cur
        if part == parts - 1:
            for sh in (4, 2, 1):
                cur = cur + pltpu.roll(cur, sh, 0)
            act[blk] = activate(cur[:, :256], cur[:, 256:])
        c = q % 4
        return _fold_token(pltpu.bitcast(cur[:, c * 128:(c + 1) * 128], u32), zero_v)

    nchunk = FFN_VPU_BLOCKS * parts
    starts = [FFN_W0 + (q * (FFN_W1 - FFN_W0)) // (nchunk - 1) for q in range(nchunk)]
    pins = {}
    wave = [0]
    wgw, wuw, wdw = [r.bitcast(u32) for r in (wg_v, wu_v, wd_v)]

    def run_wave(lhs, tls):
        w = jnp.concatenate([_or_into(tls[0], pins.get(wave[0]))] + tls[1:], axis=1)
        out = jnp.dot(lhs, _unpack(w), preferred_element_type=f32)
        for p, fn in enumerate(late):
            if LATE_AT[p] == wave[0]:
                for r_ in hb_v:
                    r_[zrows(HT2, 8), 0:128] = out[:, 0:128]
                fn()
        for q, start in enumerate(starts):
            if start == wave[0]:
                pins.setdefault(wave[0] + FFN_SPAN, []).append(vpu_chunk(q))
        if wave[0] == FFN_LATE:
            o_copy(2 * N2 - 1).start()
            out_v[zrows(S, 16, 16), 0:256] = jnp.zeros((16, 256), bf16)
            pins.setdefault(wave[0] + 4, []).append(
                token(out_v[S:S + 8, 0:128].astype(f32))())
        wave[0] += 1
        return out

    for j in range(nmx):
        gu = None
        for kt in range(D // 128):
            p = run_wave(xs[:, kt * 128:(kt + 1) * 128],
                         [r[2 * j + c, kt * 64:(kt + 1) * 64, :]
                          for r in (wgw, wuw) for c in range(2)])
            gu = p if gu is None else gu + p
        act[j] = activate(gu[:, :256], gu[:, 256:])
    ys = [None, None]
    for j in range(nblk):
        for kt in range(2):
            for hf in range(2):
                r0 = (2 * j + kt) * 64
                p = run_wave(act[j][:, kt * 128:(kt + 1) * 128],
                             [wdw[4 * hf + c, r0:r0 + 64, :] for c in range(4)])
                ys[hf] = p if ys[hf] is None else ys[hf] + p
    y = jnp.concatenate(ys, axis=1)
    cur = out_v[pl.ds(b0, 8), :].astype(f32)
    fix_v[...] = jnp.where(rows == wide(bi), hb + hn + y * wide(gate), cur).astype(bf16)
    full_copy(out_v.at[pl.ds(0, S), :], out_hbm.at[0], SEM_O).wait()
    fix = pltpu.make_async_copy(fix_v, out_hbm.at[0, pl.ds(b0, 8), :], sem.at[SEM_O])
    fix.start()
    fix.wait()


def _kernel(*refs):
    def step(i, carry):
        @pl.when(i == 0)
        def _():
            _body(i, *refs)

        return carry

    lax.fori_loop(0, 2, step, 0)


@jax.jit
def pallas_sequential_preLN__linear_kernel_hedgehog__moe_arch_mod__prompt_kernel(
    A_x: jax.Array,
    A_wqkv: jax.Array,
    A_w_phi: jax.Array,
    A_wo: jax.Array,
    B_x: jax.Array,
    B_w_r: jax.Array,
    B_w_gate: jax.Array,
    B_w_up: jax.Array,
    B_w_down: jax.Array,
):
    any_spec = pl.BlockSpec(memory_space=pl.ANY)
    return pl.pallas_call(
        _kernel,
        out_shape=jax.ShapeDtypeStruct((1, S, D), bf16),
        in_specs=[any_spec] * 8,
        out_specs=any_spec,
        scratch_shapes=[
            pltpu.VMEM((S + 16, D), bf16),
            pltpu.VMEM((3 * NWC + 1, D, WC), bf16),
            pltpu.VMEM((H, DH, DH), bf16),
            pltpu.VMEM((D + 16, D), bf16),
            pltpu.VMEM((D,), bf16),
            pltpu.VMEM((F // 128 - 2 * FFN_VPU_BLOCKS, D + PAD, 128), bf16),
            pltpu.VMEM((F // 128 - 2 * FFN_VPU_BLOCKS, D + PAD, 128), bf16),
            pltpu.VMEM((D // 128, F + PAD, 128), bf16),
            pltpu.VMEM((D, 256 * FFN_VPU_BLOCKS), bf16),
            pltpu.VMEM((D, 256 * FFN_VPU_BLOCKS), bf16),
            pltpu.VMEM((7, 4, 3 * HD + PAD, 128), bf16),
            pltpu.VMEM((7, 4, HD + PAD, 128), bf16),
            pltpu.VMEM((7, 4, HT1 + PAD, 128), bf16),
            pltpu.VMEM((7, 4, HT1 + PAD, 128), bf16),
            pltpu.VMEM((7, HT1 // 2, HD), u32),
            pltpu.VMEM((N2, 4, 2 * D + PAD, 128), bf16),
            pltpu.VMEM((4, 2 * D + PAD, 128), bf16),
            pltpu.VMEM((4, HD + PAD, 128), bf16),
            pltpu.VMEM((4, HD + PAD, 128), bf16),
            pltpu.VMEM((NP, 80, 128), f32),
            pltpu.VMEM((NP, 80, 128), bf16),
            *[pltpu.VMEM((HT2 + 8, HD), f32) for _ in range(4)],
            pltpu.VMEM((HT2, 384), f32),
            *[pltpu.VMEM((HT2, HD), f32) for _ in range(7)],
            pltpu.VMEM((S, D), bf16),
            pltpu.VMEM((S + 16, D), bf16),
            pltpu.VMEM((8, D), f32),
            pltpu.VMEM((3, 8, 128), f32),
            pltpu.VMEM((8, 128), jnp.int32),
            pltpu.VMEM((8, D), bf16),
            *[pltpu.VMEM((256, 128), f32) for _ in range(4)],
            pltpu.SemaphoreType.DMA((NSEM,)),
        ],
        compiler_params=pltpu.CompilerParams(
            vmem_limit_bytes=110 * 1024 * 1024,
            disable_bounds_checks=True,
            disable_semaphore_checks=True),
    )(A_x, A_wqkv, A_w_phi, A_wo, B_w_r, B_w_gate, B_w_up, B_w_down)
```

```python
import jax
import jax.numpy as jnp
from jax import lax
import jax.experimental.pallas as pl
import jax.experimental.pallas.tpu as pltpu

S = 2048
D = 1024
H = 32
DH = 32
F = 3584
NP = H // 2
T1 = 256
T2 = 512
N1 = S // T1
N2 = S // T2
HT1 = T1 // 2
HT2 = T2 // 2
HD = D // 2
WC = 256
NWC = D // WC
LOG2E = 1.4426950408889634
EPS = 1e-5
PAD = 16
WO_ROWS = 176
LN_ROWS = 16
EP_ROWS = 32

T0_FOLD = (0, 4, 11, 18, 25, 33, 39, 46)
T0_WAITS = ((4, (1,)), (11, ('phi', 2)), (18, (3, 4)), (33, ('x1', 5, 6)), (46, (7,)),
            (73, (8, 9, 10, 11, 'x2', 'x3')))
T0_VPREP = ((73, 74, 75, 76), (77, 78, 79, 80), (81, 82, 83, 84), (85, 86, 87, 88))
T0_VSPAN = 4
T0_LN = (33, 33, 35, 37, 38, 39, 40, 42)
T0_LNSPAN = (3, 0, 0, 0, 0, 0, 0, 0)
T1_LN = ((99, 100, 101, 102, 103, 104, 105, 106), (90, 91, 92, 93, 94, 95, 96, 97))
P1_LNSPAN = 3
P1_WO = (57, 58, 59, 60, 63, 77, 79, 80, 81, 82, 83)
P1_WOSPAN = 3
P1_LN2 = ((70, 71, 72, 73, 74, 75, 76, 77), (62, 63, 64, 65, 66, 67, 68, 69))
P1_LNSPAN2 = (3, 3)
LT_START = (0, 0, 1, 5, 8, 11, 14)
LT_SPAN = (1, 3, 4, 4, 3, 4, 5)
FB_START = (2, 4, 6, 8, 10, 12, 14, 16)
FB_SPAN = 2
SA_START = (9, 11, 13, 15, 17, 17, 18, 18)
SA_SPAN = 3
FA_START = (20, 21, 22, 23, 24, 25, 26, 27)
FA_SPAN = (3, 6, 2, 4, 2, 4, 2, 2)
FFN_VPU_BLOCKS = 7
FFN_KG = 16
FFN_W0 = 18
FFN_W1 = 107
FFN_SPAN = 4
FFN_LATE = 16
LATE_AT = (1, 2, 3, 4, 4, 5, 7, 8)

_NT = (((1,), (1,)), ((), ()))
f32 = jnp.float32
bf16 = jnp.bfloat16
u32 = jnp.uint32

K_, Q_, V_ = 0, 1, 2
SRC = {K_: 1, Q_: 0, V_: 2}

SEM_W = 0
SEM_X = SEM_W + 3 * NWC
SEM_X0 = SEM_X + N1
SEM_K0 = SEM_X0 + 4
SEM_PHI = SEM_K0 + 4
SEM_WO = SEM_PHI + 2
SEM_WR, SEM_WG, SEM_WU, SEM_WD, SEM_WGV, SEM_WUV, SEM_O = (SEM_WO + 1 + i for i in range(7))
NSEM = SEM_O + 1


def _rb(v):
    return v.astype(bf16).astype(f32)


def _unpack(w):
    return pltpu.bitcast(w, bf16)


def _mo(i, n):
    return i if isinstance(i, int) else pl.multiple_of(i, n)


def _recip(x):
    r = pl.reciprocal(x, approx=True)
    return r * (2.0 - x * r)


def _sigmoid(x):
    return _recip(1.0 + jnp.exp(jnp.minimum(-x, 80.0)))


def _dual_softmax(p):
    t = p.shape[-1]
    p3 = p.reshape(8, 8, t)

    def allred(v, op):
        v = op(v, pltpu.roll(v, 2, 0))
        return op(v, pltpu.roll(v, 4, 0))

    mx = allred(jnp.max(p3, axis=0), jnp.maximum)
    mn = allred(jnp.min(p3, axis=0), jnp.minimum)
    ep = jnp.exp2(p3 - mx[None])
    en = jnp.exp2(mn[None] - p3)
    sp = allred(jnp.sum(ep, axis=0), jnp.add)
    sn = allred(jnp.sum(en, axis=0), jnp.add)
    fp = (ep * _recip(sp)[None]).reshape(64, t)
    fn = (en * _recip(sn)[None]).reshape(64, t)
    return jnp.concatenate([fp, fn], axis=0).astype(bf16)


def _left_combos(a11, a12, a21, a22):
    return [a11 + a22, a21 + a22, a11, a22, a11 + a12, a21 - a11, a12 - a22]


def _right_combos(b11, b12, b21, b22):
    return [b11 + b22, b11, b12 - b22, b21 - b11, b22, b11 + b12, b21 + b22]


def _strassen(prod, emit):
    m3 = prod(2)
    m5 = prod(4)
    emit(0, 1, m3 + m5)
    m7 = prod(6)
    u = m7 - m5
    m1 = prod(0)
    u = u + m1
    w = m1 + m3
    m4 = prod(3)
    emit(0, 0, u + m4)
    m2 = prod(1)
    emit(1, 0, m2 + m4)
    w = w - m2
    m6 = prod(5)
    emit(1, 1, w + m6)


def _or_into(w, toks):
    if not toks:
        return w
    top = w[0:8, 0:128]
    for tk in toks:
        top = top | tk
    if w.shape[1] > 128:
        top = jnp.concatenate([top, w[0:8, 128:]], axis=1)
    return jnp.concatenate([top, w[8:]], axis=0)


def _fold_token(w, zero):
    r, c = w.shape
    acc = None
    for i in range(r // 8):
        for j in range(c // 128):
            blk = w[i * 8:(i + 1) * 8, j * 128:(j + 1) * 128]
            acc = blk if acc is None else acc | blk
    return acc & zero


def _body(zs, x_hbm, wqkv_hbm, wphi_hbm, wo_hbm, wr_hbm, wg_hbm, wu_hbm, wd_hbm, out_hbm,
          x_v, wqkv_v, wphi_v, wo_v, wr_v, wg_v, wu_v, wd_v, wgv_v, wuv_v,
          wt_v, wo7_v, sa7_v, sb7_v, sc7_v, phiq_v, phik_v, vt0_v, vt1_v, kv_acc, kvt_v,
          hal_v, har_v, hbl_v, hbr_v, sa_v, t0_v, t1_v, t2_v, t3_v, t4_v, t5_v, t6_v,
          h_v, out_v, wrf_v, best_v, besti_v, fix_v, xc0_v, xc1_v, xc2_v, xc3_v, sem):
    xcol_v = (xc0_v, xc1_v, xc2_v, xc3_v)
    s_v = (sa7_v, sb7_v)
    vt_v = (vt0_v, vt1_v)
    ha_v = (hal_v, har_v)
    hb_v = (hbl_v, hbr_v)
    tmp_v = (t0_v, t1_v, t2_v, t3_v, t4_v, t5_v, t6_v)

    def x_rows(r0, rows, slot):
        return pltpu.make_async_copy(
            x_hbm.at[0, pl.ds(r0, rows), :], x_v.at[pl.ds(r0, rows), :], sem.at[slot])

    def x_copy(i):
        return x_rows(i * T1, T1, SEM_X + i)

    def x0_copy(q):
        return x_rows((q % 2) * HT1 + (q // 2) * (HT1 // 2), HT1 // 2, SEM_X0 + q)

    def w_copy(kind, c):
        return pltpu.make_async_copy(
            wqkv_hbm.at[:, pl.ds(SRC[kind] * D + c * WC, WC)],
            wqkv_v.at[kind * NWC + c], sem.at[SEM_W + kind * NWC + c])

    def k0_copy(q):
        r0 = (q % 2) * HD + (q // 2) * 256
        return pltpu.make_async_copy(
            wqkv_hbm.at[pl.ds(r0, 256), pl.ds(SRC[K_] * D, WC)],
            wqkv_v.at[K_ * NWC, pl.ds(r0, 256), :], sem.at[SEM_K0 + q])

    def phi_copy(part):
        lo, n = part * (H // 2), H // 2
        return pltpu.make_async_copy(wphi_hbm.at[pl.ds(lo, n)], wphi_v.at[pl.ds(lo, n)],
                                     sem.at[SEM_PHI + part])

    def full_copy(src, dst, slot):
        return pltpu.make_async_copy(src, dst, sem.at[slot])

    x0_copy(0).start()
    x0_copy(1).start()
    full_copy(wr_hbm, wr_v, SEM_WR).start()
    phi_copy(0).start()
    x0_copy(2).start()
    x0_copy(3).start()
    for q in range(4):
        k0_copy(q).start()
    w_copy(K_, 1).start()
    phi_copy(1).start()
    w_copy(K_, 2).start()
    w_copy(K_, 3).start()
    w_copy(Q_, 0).start()
    x_copy(1).start()
    for c in range(1, NWC):
        w_copy(Q_, c).start()
    for c in range(NWC):
        w_copy(V_, c).start()
    x_copy(2).start()
    x_copy(3).start()
    full_copy(wo_hbm, wo_v.at[pl.ds(0, D), :], SEM_WO).start()
    for i in range(4, N1):
        x_copy(i).start()
    f0 = F - 256 * FFN_VPU_BLOCKS
    ffn_tiled = ((wg_hbm, wg_v, D, SEM_WG), (wu_hbm, wu_v, D, SEM_WU), (wd_hbm, wd_v, F, SEM_WD))
    for src, dst, rows, slot in ffn_tiled:
        for c in range(dst.shape[0]):
            full_copy(src.at[:, pl.ds(c * 128, 128)], dst.at[c, pl.ds(0, rows), :], slot).start()
    full_copy(wg_hbm.at[:, pl.ds(f0, F - f0)], wgv_v, SEM_WGV).start()
    full_copy(wu_hbm.at[:, pl.ds(f0, F - f0)], wuv_v, SEM_WUV).start()

    zero_v = jnp.full((8, 128), zs, jnp.int32).astype(u32)

    def zrows(r0, rows, mult=8):
        return pl.ds(pl.multiple_of(zs * mult + r0, mult), rows)

    def tiles(ref, r0, rows):
        w = ref.bitcast(u32)
        return jnp.concatenate(
            [w[c, r0 // 2:(r0 + rows) // 2, :] for c in range(ref.shape[0])], axis=1)

    def token(*vals):
        return lambda: _fold_token(pltpu.bitcast(jnp.concatenate(vals, axis=0), u32), zero_v)

    def ln1_stats(xf):
        m = jnp.sum(xf, axis=-1, keepdims=True) * (1.0 / D)
        q = jnp.sum(xf * xf, axis=-1, keepdims=True) * (1.0 / D)
        inv = lax.rsqrt(jnp.maximum(q - m * m, 0.0) + EPS)
        return inv, m * inv

    def ln1_piece(r0, dst, p, m=None):
        fixed = isinstance(r0, int)
        if m is not None:
            x_v[zrows(S, 8) if fixed else pl.ds(S, 8), 0:128] = m[0:8, 0:128].astype(bf16)
        xa, xb = [x_v[pl.ds(_mo(r0 + hf * HT1 + p * LN_ROWS, LN_ROWS), LN_ROWS), :]
                  .astype(f32) for hf in range(2)]
        (ia, ma), (ib, mb) = ln1_stats(xa), ln1_stats(xb)
        ya, yb = xa * ia, xb * ib
        s2 = ya[:, :HD] - ma
        s5 = yb[:, HD:] - mb
        s1 = s2 + s5
        s3 = yb[:, :HD] - yb[:, HD:]
        s4 = ya[:, HD:] - ya[:, :HD]
        combos = [s1, s2, s3, s4, s5, s1 + s3, s1 + s4]
        rows = zrows(p * LN_ROWS, LN_ROWS, 16) if fixed else pl.ds(p * LN_ROWS, LN_ROWS)
        for i in range(7):
            for c in range(4):
                dst[i, c, rows, :] = combos[i][:, c * 128:(c + 1) * 128].astype(bf16)
        return token(combos[5], combos[6])

    def fold_piece(kind, c, j, pt):
        blk = {}
        for hh in range(2):
            for kh in range(2):
                k0 = kh * HD + j * 128
                w = wqkv_v[kind * NWC + c, k0:k0 + 128, hh * 128:(hh + 1) * 128]
                blk[hh, kh] = lax.dot_general(pt[2 * c + hh], w, _NT,
                                              preferred_element_type=f32) * LOG2E
        combos = _left_combos(blk[0, 0], blk[0, 1], blk[1, 0], blk[1, 1])
        r0 = kind * HD + c * 128
        for i in range(7):
            wt_v[i, j, r0:r0 + 128, :] = combos[i].astype(bf16)

    def fold_chunk(kind, c, pt):
        for j in range(4):
            fold_piece(kind, c, j, pt)

    def vprep_piece(c, j, m):
        wqkv_v[zs + 3 * NWC, 0:8, 0:128] = m[0:8, 0:128].astype(bf16)
        blk = {}
        for hh in range(2):
            for kh in range(2):
                k0 = kh * HD + j * 128
                w = wqkv_v[V_ * NWC + c, k0:k0 + 128, hh * 128:(hh + 1) * 128]
                blk[hh, kh] = w.T.astype(f32)
        combos = _left_combos(blk[0, 0], blk[0, 1], blk[1, 0], blk[1, 1])
        r0 = V_ * HD + c * 128
        for i in range(7):
            wt_v[i, j, r0:r0 + 128, :] = combos[i].astype(bf16)
        return token(combos[1], combos[4])

    def wo_piece(w0, m):
        wo_v[D:D + 8, 0:128] = m[0:8, 0:128].astype(bf16)
        top = wo_v[pl.ds(pl.multiple_of(w0, 16), 16), :].astype(f32)
        bot = wo_v[pl.ds(pl.multiple_of(HD + w0, 16), 16), :].astype(f32)
        combos = _right_combos(top[:, :HD], top[:, HD:], bot[:, :HD], bot[:, HD:])
        for i in range(7):
            for c in range(4):
                wo7_v[i, c, pl.ds(pl.multiple_of(w0, 16), 16), :] = (
                    combos[i][:, c * 128:(c + 1) * 128].astype(bf16))
        return token(combos[5], combos[6])

    def run_rounds(t0, rounds, post, first):
        count = [0]
        pins = {}

        def run_jobs(m):
            for fn, span in post.get(count[0], ()):
                tok = fn(m)
                if span:
                    pins.setdefault(count[0] + span, []).append(tok())
            count[0] += 1

        for par, kind, cs in rounds:
            r0 = kind * HD + cs[0] * 128
            rows = 128 * len(cs)

            def prod(i):
                if (par, kind) == (1, V_):
                    rhs = sc7_v[i]
                else:
                    rhs = tiles(s_v[par].at[i], 0, HT1)
                if (par, kind, cs[0]) == (1, K_, 0):
                    sc7_v[i, zrows(0, HT1 // 2), :] = rhs
                m = lax.dot_general(_unpack(tiles(wt_v.at[i], r0, rows)),
                                    _unpack(_or_into(rhs, pins.get(count[0]))),
                                    _NT, preferred_element_type=f32)
                run_jobs(m)
                return m

            def emit(rh, ch, blk):
                tb = 2 * par + ch
                for n, c in enumerate(cs):
                    for jj in range(2):
                        pair = 4 * c + 2 * rh + jj
                        p = blk[n * 128 + jj * 64:n * 128 + (jj + 1) * 64]
                        if kind == K_:
                            phik_v[tb, zrows(pair * 128, 128, 16), :] = _dual_softmax(p)
                        elif kind == Q_:
                            phiq_v[t0 // 2, tb, pair * 128:(pair + 1) * 128, :] = (
                                _dual_softmax(p))
                        else:
                            vt_v[pair // 8][tb, zrows((pair % 8) * 64, 64, 16), :] = (
                                p.astype(bf16))

            _strassen(prod, emit)

        ones = jnp.full((8, 2 * T1), 0x3F803F80, u32)
        kr = lax.broadcasted_iota(jnp.int32, (80, 128), 0)
        kc = lax.broadcasted_iota(jnp.int32, (80, 128), 1)
        kmask = jnp.where(kr < 64, kr // 32, (kr - 64) // 8) == kc % 2
        for j in range(NP):
            lhs = jnp.concatenate([tiles(vt_v[j // 8], (j % 8) * 64, 64), ones], axis=0)
            rhs = tiles(phik_v, j * 128, 128)
            upd = lax.dot_general(_unpack(lhs), _unpack(_or_into(rhs, pins.get(count[0]))), _NT,
                                  preferred_element_type=f32)
            run_jobs(upd)
            if first:
                kv_acc[j] = upd
            else:
                upd = kv_acc[j] + upd
                kv_acc[j] = upd
                kvt_v[j] = jnp.where(kmask, upd, 0.0).astype(bf16)

    def load_best():
        return best_v[0], besti_v[...], best_v[1], best_v[2]

    def store_best(best):
        best_v[0], besti_v[...], best_v[1], best_v[2] = best

    def build_pt(g0, g1):
        n = g1 - g0
        w2 = wphi_v[4 * g0:4 * g1].reshape(n * 128, DH)
        er = lax.broadcasted_iota(jnp.int32, (128, DH), 0)
        ec = lax.broadcasted_iota(jnp.int32, (128, DH), 1)
        e = jnp.where(ec == (er % 64) // 2, 1.0, 0.0).astype(bf16)
        ptf = lax.dot_general(e, w2, _NT, preferred_element_type=f32)
        pr = lax.broadcasted_iota(jnp.int32, (128, 128), 0)
        pc = lax.broadcasted_iota(jnp.int32, (128, 128), 1)
        keep = pc // 32 == (pr // 64) * 2 + pr % 2
        return [jnp.where(keep, ptf[:, g * 128:(g + 1) * 128], 0.0).astype(bf16)
                for g in range(n)]

    hbl_v[...] = jnp.zeros_like(hbl_v)
    hbr_v[...] = jnp.zeros_like(hbr_v)
    store_best((jnp.full((8, 128), -jnp.inf, f32), jnp.zeros((8, 128), jnp.int32),
                jnp.zeros((8, 128), f32), jnp.zeros((8, 128), f32)))
    n_ln = HT1 // LN_ROWS
    x0_copy(0).wait()
    x0_copy(1).wait()
    for p in range(n_ln // 2):
        ln1_piece(0, s_v[0], p)
    full_copy(wr_hbm, wr_v, SEM_WR).wait()
    phi_copy(0).wait()
    x0_copy(2).wait()
    x0_copy(3).wait()
    wr_row = wr_v[...].astype(f32).reshape(1, D)
    wrf_v[...] = jnp.broadcast_to(
        wr_row - jnp.sum(wr_row, axis=-1, keepdims=True) * (1.0 / D), (8, D))
    pt = build_pt(0, 4)
    for p in range(n_ln // 2, n_ln):
        ln1_piece(0, s_v[0], p)
    for part in range(2):
        k0_copy(2 * part).wait()
        k0_copy(2 * part + 1).wait()
        fold_piece(K_, 0, 2 * part, pt)
        fold_piece(K_, 0, 2 * part + 1, pt)

    post = {}

    def at(slot, fn, span=0):
        post.setdefault(slot, []).append((fn, span))

    for slot, copies in T0_WAITS:
        for cp in copies:
            if cp == 'phi':
                at(slot, lambda m: phi_copy(1).wait())
            elif cp in ('x1', 'x2', 'x3'):
                at(slot, lambda m, cp=cp: x_copy(int(cp[1])).wait())
            else:
                at(slot, lambda m, cp=cp: w_copy(cp // NWC, cp % NWC).wait())
    for n in range(1, 2 * NWC):
        if n == 2:
            at(T0_FOLD[n], lambda m: pt.extend(build_pt(4, 8)))
        at(T0_FOLD[n], lambda m, n=n: fold_chunk(n // NWC, n % NWC, pt))
    for c in range(NWC):
        for j in range(4):
            at(T0_VPREP[c][j], lambda m, c=c, j=j: vprep_piece(c, j, m), T0_VSPAN)
    for p in range(n_ln):
        at(T0_LN[p], lambda m, p=p: ln1_piece(T1, s_v[1], p, m), T0_LNSPAN[p])
    for p in range(n_ln):
        at(T1_LN[0][p], lambda m, p=p: ln1_piece(2 * T1, s_v[0], p, m), P1_LNSPAN)
        at(T1_LN[1][p], lambda m, p=p: ln1_piece(3 * T1, s_v[1], p, m), P1_LNSPAN)
    lo, hi = [0, 1], [2, 3]
    run_rounds(0, [(0, kind, [c]) for kind in (K_, Q_) for c in range(NWC)]
               + [(1, K_, lo), (1, K_, hi), (1, Q_, lo), (1, Q_, hi),
                  (0, V_, lo), (0, V_, hi), (1, V_, lo), (1, V_, hi)], post, True)
    full_copy(wo_hbm, wo_v.at[pl.ds(0, D), :], SEM_WO).wait()
    for i in range(4, N1):
        x_copy(i).wait()

    def phase1(i, carry):
        post = {}
        nxt = jnp.minimum(i + 1, N2 - 1) * T2
        w0 = jnp.minimum((i - 1) * WO_ROWS, HD - WO_ROWS)
        for par in range(2):
            for p in range(n_ln):
                post.setdefault(P1_LN2[par][p], []).append(
                    (lambda m, p=p, par=par: ln1_piece(nxt + par * T1, s_v[par], p, m),
                     P1_LNSPAN2[par]))
        for p in range(WO_ROWS // 16):
            post.setdefault(P1_WO[p], []).append(
                (lambda m, p=p: wo_piece(w0 + 16 * p, m), P1_WOSPAN))
        run_rounds(2 * i, [(par, kind, cs) for kind in (K_, Q_, V_) for par in range(2)
                           for cs in ([0, 1], [2, 3])], post, False)
        return carry

    lax.fori_loop(1, N1 // 2, phase1, 0)

    for _, dst, rows, slot in ffn_tiled:
        filled = dst.at[:, pl.ds(0, rows), :]
        full_copy(filled, filled, slot).wait()
    full_copy(wg_hbm.at[:, pl.ds(f0, F - f0)], wgv_v, SEM_WGV).wait()
    full_copy(wu_hbm.at[:, pl.ds(f0, F - f0)], wuv_v, SEM_WUV).wait()

    def o_copy(hf):
        return pltpu.make_async_copy(
            out_v.at[pl.ds(hf * HT2, HT2), :], out_hbm.at[0, pl.ds(hf * HT2, HT2), :],
            sem.at[SEM_O])

    def half_stats(hh, c0):
        rows = hh.shape[0]
        parts = [hh[:, c * 128:(c + 1) * 128] for c in range(4)]
        wts = [wrf_v[:, c0 + c * 128:c0 + (c + 1) * 128] for c in range(4)]
        s1 = (parts[0] + parts[1]) + (parts[2] + parts[3])
        sq = [p * p for p in parts]
        s2 = (sq[0] + sq[1]) + (sq[2] + sq[3])
        dw = [(p.reshape(rows // 8, 8, 128) * w[None]).reshape(rows, 128)
              for p, w in zip(parts, wts)]
        s3 = (dw[0] + dw[1]) + (dw[2] + dw[3])
        return s1, s2, s3

    def first_half(hbuf, sbuf, base, p, c0):
        r0 = p * EP_ROWS
        hh = hbuf[c0 // HD][r0:r0 + EP_ROWS, :]
        h_v[pl.ds(pl.multiple_of(base + r0, EP_ROWS), EP_ROWS), c0:c0 + HD] = hh.astype(bf16)
        st = jnp.concatenate(half_stats(hh, c0), axis=1)
        sbuf[zrows(r0, EP_ROWS), :] = st
        return _fold_token(pltpu.bitcast(st, u32), zero_v)

    def finish(hbuf, sbuf, base, p, valid, best, defer=None):
        r0 = p * EP_ROWS
        g0 = pl.multiple_of(base + r0, EP_ROWS)
        hl, hr = [r[r0:r0 + EP_ROWS, :] for r in hbuf]
        if defer is None:
            h_v[pl.ds(g0, EP_ROWS), 0:HD] = hl.astype(bf16)
        if sbuf is None:
            if defer is None:
                h_v[pl.ds(g0, EP_ROWS), HD:D] = hr.astype(bf16)
            st = half_stats(hr, HD)
        else:
            st = sbuf[r0:r0 + EP_ROWS, :]
            st = [st[:, n * 128:(n + 1) * 128] for n in range(3)]
        s1, s2, s3 = [jnp.sum(v + w, axis=-1, keepdims=True)
                      for v, w in zip(half_stats(hl, 0), st)]
        m = s1 * (1.0 / D)
        var = jnp.maximum(s2 * (1.0 / D) - m * m, 0.0)
        inv = lax.rsqrt(var + EPS)
        r = s3 * inv

        def write_out(h):
            o = h * (1.0 + inv) - m * inv
            out_v[pl.ds(g0, EP_ROWS), :] = o.astype(bf16)
            return o

        if defer is None:
            o = write_out(jnp.concatenate([hl, hr], axis=1))
        else:
            defer.append(lambda: write_out(jnp.concatenate(
                [r_[r0:r0 + EP_ROWS, :] for r_ in hbuf], axis=1)))
        bv, bi, bm, bq = best
        sub = lax.broadcasted_iota(jnp.int32, (8, 128), 0)
        for g in range(EP_ROWS // 8):
            rows = slice(g * 8, (g + 1) * 8)
            rg = jnp.broadcast_to(r[rows], (8, 128))
            if valid is not None:
                rg = jnp.where(valid, rg, -jnp.inf)
            better = rg > bv
            bi = jnp.where(better, sub + (g0 + g * 8), bi)
            bv = jnp.where(better, rg, bv)
            bm = jnp.where(better, jnp.broadcast_to(m[rows], (8, 128)), bm)
            bq = jnp.where(better, jnp.broadcast_to(var[rows], (8, 128)), bq)
        best = (bv, bi, bm, bq)
        if defer is not None:
            return best, None
        tok = _fold_token(pltpu.bitcast(jnp.concatenate(
            [o[:, D - 128:], bv, bm, bq], axis=0), u32), zero_v)
        return best, tok

    n_ep = HT2 // EP_ROWS

    def phase2(i, carry):
        ot = []
        for j in range(NP):
            ph = tiles(phiq_v.at[i], j * 128, 128)
            n = jnp.dot(_unpack(kvt_v.bitcast(u32)[j]), _unpack(ph),
                        preferred_element_type=f32)
            r0h = _recip(n[64:72] + 1e-6)
            r1h = _recip(n[72:80] + 1e-6)
            ot.append((n[0:32].reshape(4, 8, T2) * r0h[None]).reshape(32, T2))
            ot.append((n[32:64].reshape(4, 8, T2) * r1h[None]).reshape(32, T2))
        lo = jnp.concatenate(ot[:H // 2], axis=0)
        hi = jnp.concatenate(ot[H // 2:], axis=0)
        lcs = _left_combos(lo[:, :HT2], hi[:, :HT2], lo[:, HT2:], hi[:, HT2:])

        state = {'best': load_best()}
        pins = {}
        jobs = {}
        lts = {}
        ra = pl.multiple_of(i * T2, T2)
        rb = pl.multiple_of(i * T2 + HT2, HT2)
        prev = jnp.maximum(i * T2 - HT2, HT2)

        def add_job(slot, deadline, fn, gates=()):
            jobs.setdefault(slot, []).append((fn, deadline, gates))

        def finish_job(hbuf, sbuf, base, p, valid):
            def fn():
                state['best'], tok = finish(hbuf, sbuf, base, p, valid, state['best'])
                return tok
            return fn

        def lt_job(k):
            def fn():
                lts[k] = lcs[k].astype(bf16).T
                return _fold_token(pltpu.bitcast(lts[k], u32), zero_v)
            return fn

        order = (2, 4, 6, 0, 3, 1, 5)
        lt_job(2)()
        for n in range(1, 7):
            add_job(LT_START[n], min(LT_START[n] + LT_SPAN[n], 4 * n), lt_job(order[n]))
        for p in range(n_ep):
            add_job(FB_START[p], FB_START[p] + FB_SPAN,
                    finish_job(hb_v, None, prev, p, i > 0), hb_v)
            add_job(SA_START[p], SA_START[p] + SA_SPAN,
                    lambda p=p: first_half(ha_v, sa_v, ra, p, HD), ha_v[1:])
            add_job(FA_START[p], FA_START[p] + FA_SPAN[p],
                    finish_job(ha_v, sa_v, ra, p, None), ha_v)

        def xblk(r0, c0):
            return x_v[pl.ds(r0, HT2), c0:c0 + 128].astype(f32)

        for n, k in enumerate(order):
            for c in range(4):
                slot = 4 * n + c
                for fn, deadline, gates in jobs.get(slot, ()):
                    for ref in gates:
                        ref[zrows(HT2, 8), 0:128] = mm[0:8]
                    pins.setdefault(deadline, []).append(fn())
                w = _or_into(wo7_v.bitcast(u32)[k, c, 0:HD // 2, :], pins.get(slot))
                mm = jnp.dot(lts[k], _unpack(w), preferred_element_type=f32)
                c0 = c * 128
                cs = slice(c0, c0 + 128)
                tmp = lambda t: tmp_v[t][:, cs]
                if n == 0:
                    tmp_v[0][zrows(0, HT2), cs] = mm
                elif n == 1:
                    ha_v[1][zrows(0, HT2), cs] = (xblk(ra, HD + c0) + tmp(0)) + mm
                    tmp_v[1][zrows(0, HT2), cs] = xblk(ra, c0) - mm
                elif n == 2:
                    tmp_v[2][zrows(0, HT2), cs] = tmp(1) + mm
                elif n == 3:
                    tmp_v[3][zrows(0, HT2), cs] = tmp(2) + mm
                    tmp_v[4][zrows(0, HT2), cs] = (xblk(rb, HD + c0) + tmp(0)) + mm
                elif n == 4:
                    ha_v[0][zrows(0, HT2), cs] = tmp(3) + mm
                    tmp_v[5][zrows(0, HT2), cs] = xblk(rb, c0) + mm
                elif n == 5:
                    hb_v[0][zrows(0, HT2), cs] = tmp(5) + mm
                    tmp_v[6][zrows(0, HT2), cs] = tmp(4) - mm
                else:
                    hb_v[1][zrows(0, HT2), cs] = tmp(6) + mm
        store_best(state['best'])
        o_copy(2 * i).start()

        @pl.when(i > 0)
        def _():
            o_copy(2 * i - 1).start()

        return carry

    lax.fori_loop(0, N2, phase2, 0)
    best = load_best()
    late = []
    for p in range(n_ep):
        best, _ = finish(hb_v, None, S - HT2, p, None, best, late)

    bv, bi, bm, bq = best
    for sh in (4, 2, 1):
        ov, oi, om, oq = [pltpu.roll(t, sh, 0) for t in (bv, bi, bm, bq)]
        take = jnp.logical_or(ov > bv, jnp.logical_and(ov == bv, oi < bi))
        bv, bi, bm, bq = [jnp.where(take, o_, t)
                          for o_, t in zip((ov, oi, om, oq), (bv, bi, bm, bq))]
    idx = jnp.clip(bi[0, 0], 0, S - 1)
    b0 = pl.multiple_of((idx // 8) * 8, 8)
    t = _rb(_rb(bq) + EPS)
    inv = _recip(_rb(t * lax.rsqrt(t)))
    gate = _sigmoid(bv)
    wide = lambda v: jnp.concatenate([v] * (D // 128), axis=1)
    b1 = pl.multiple_of(jnp.minimum(b0, S - HT2 - 8), 8)
    b2 = pl.multiple_of(jnp.maximum(b0 - (S - HT2), 0), 8)
    hb = jnp.where(wide(bi) < S - HT2, h_v[pl.ds(b1, 8), :].astype(f32),
                   _rb(jnp.concatenate([r_[pl.ds(b2, 8), :] for r_ in hb_v], axis=1)))
    hn = (hb - wide(bm)) * wide(inv)
    xs = hn.astype(bf16)
    rows = lax.broadcasted_iota(jnp.int32, (8, D), 0) + b0

    xm = jnp.where(rows == wide(bi), _rb(hn), 0.0)
    for sh in (4, 2, 1):
        xm = xm + pltpu.roll(xm, sh, 0)
    for t in range(D // 128):
        xcol_v[t // 2][zrows((t % 2) * 128, 128), :] = jnp.concatenate(
            [xm[:, t * 128:(t + 1) * 128]] * 16, axis=0).T

    nblk = F // 256
    nmx = nblk - FFN_VPU_BLOCKS
    act = {}
    acc = {}

    def activate(g, u):
        return (g * _sigmoid(g) * u).astype(bf16)

    parts = D // 8 // FFN_KG

    def vpu_chunk(q):
        blk, part = nmx + q // parts, q % parts
        cur = acc.get(blk)
        for kg in range(part * FFN_KG, (part + 1) * FFN_KG):
            xc = xcol_v[kg // 32][(kg % 32) * 8:(kg % 32 + 1) * 8, :]
            w = jnp.concatenate(
                [r[kg * 8:(kg + 1) * 8, (blk - nmx) * 256:(blk - nmx + 1) * 256].astype(f32)
                 for r in (wgv_v, wuv_v)], axis=1)
            p = w * jnp.concatenate([xc] * 4, axis=1)
            cur = p if cur is None else cur + p
        acc[blk] = cur
        if part == parts - 1:
            for sh in (4, 2, 1):
                cur = cur + pltpu.roll(cur, sh, 0)
            act[blk] = activate(cur[:, :256], cur[:, 256:])
        c = q % 4
        return _fold_token(pltpu.bitcast(cur[:, c * 128:(c + 1) * 128], u32), zero_v)

    nchunk = FFN_VPU_BLOCKS * parts
    starts = [FFN_W0 + (q * (FFN_W1 - FFN_W0)) // (nchunk - 1) for q in range(nchunk)]
    pins = {}
    wave = [0]
    wgw, wuw, wdw = [r.bitcast(u32) for r in (wg_v, wu_v, wd_v)]

    def run_wave(lhs, tls):
        w = jnp.concatenate([_or_into(tls[0], pins.get(wave[0]))] + tls[1:], axis=1)
        out = jnp.dot(lhs, _unpack(w), preferred_element_type=f32)
        for p, fn in enumerate(late):
            if LATE_AT[p] == wave[0]:
                for r_ in hb_v:
                    r_[zrows(HT2, 8), 0:128] = out[:, 0:128]
                fn()
        for q, start in enumerate(starts):
            if start == wave[0]:
                pins.setdefault(wave[0] + FFN_SPAN, []).append(vpu_chunk(q))
        if wave[0] == FFN_LATE:
            o_copy(2 * N2 - 1).start()
            out_v[zrows(S, 16, 16), 0:256] = jnp.zeros((16, 256), bf16)
            pins.setdefault(wave[0] + 4, []).append(
                token(out_v[S:S + 8, 0:128].astype(f32))())
        wave[0] += 1
        return out

    for j in range(nmx):
        gu = None
        for kt in range(D // 128):
            p = run_wave(xs[:, kt * 128:(kt + 1) * 128],
                         [r[2 * j + c, kt * 64:(kt + 1) * 64, :]
                          for r in (wgw, wuw) for c in range(2)])
            gu = p if gu is None else gu + p
        act[j] = activate(gu[:, :256], gu[:, 256:])
    ys = [None, None]
    for j in range(nblk):
        for kt in range(2):
            for hf in range(2):
                r0 = (2 * j + kt) * 64
                p = run_wave(act[j][:, kt * 128:(kt + 1) * 128],
                             [wdw[4 * hf + c, r0:r0 + 64, :] for c in range(4)])
                ys[hf] = p if ys[hf] is None else ys[hf] + p
    y = jnp.concatenate(ys, axis=1)
    cur = out_v[pl.ds(b0, 8), :].astype(f32)
    fix_v[...] = jnp.where(rows == wide(bi), hb + hn + y * wide(gate), cur).astype(bf16)
    full_copy(out_v.at[pl.ds(0, S), :], out_hbm.at[0], SEM_O).wait()
    fix = pltpu.make_async_copy(fix_v, out_hbm.at[0, pl.ds(b0, 8), :], sem.at[SEM_O])
    fix.start()
    fix.wait()


def _kernel(*refs):
    def step(i, carry):
        @pl.when(i == 0)
        def _():
            _body(i, *refs)

        return carry

    lax.fori_loop(0, 2, step, 0)


@jax.jit
def pallas_sequential_preLN__linear_kernel_hedgehog__moe_arch_mod__prompt_kernel(
    A_x: jax.Array,
    A_wqkv: jax.Array,
    A_w_phi: jax.Array,
    A_wo: jax.Array,
    B_x: jax.Array,
    B_w_r: jax.Array,
    B_w_gate: jax.Array,
    B_w_up: jax.Array,
    B_w_down: jax.Array,
):
    any_spec = pl.BlockSpec(memory_space=pl.ANY)
    return pl.pallas_call(
        _kernel,
        out_shape=jax.ShapeDtypeStruct((1, S, D), bf16),
        in_specs=[any_spec] * 8,
        out_specs=any_spec,
        scratch_shapes=[
            pltpu.VMEM((S + 16, D), bf16),
            pltpu.VMEM((3 * NWC + 1, D, WC), bf16),
            pltpu.VMEM((H, DH, DH), bf16),
            pltpu.VMEM((D + 16, D), bf16),
            pltpu.VMEM((D,), bf16),
            pltpu.VMEM((F // 128 - 2 * FFN_VPU_BLOCKS, D + PAD, 128), bf16),
            pltpu.VMEM((F // 128 - 2 * FFN_VPU_BLOCKS, D + PAD, 128), bf16),
            pltpu.VMEM((D // 128, F + PAD, 128), bf16),
            pltpu.VMEM((D, 256 * FFN_VPU_BLOCKS), bf16),
            pltpu.VMEM((D, 256 * FFN_VPU_BLOCKS), bf16),
            pltpu.VMEM((7, 4, 3 * HD + PAD, 128), bf16),
            pltpu.VMEM((7, 4, HD + PAD, 128), bf16),
            pltpu.VMEM((7, 4, HT1 + PAD, 128), bf16),
            pltpu.VMEM((7, 4, HT1 + PAD, 128), bf16),
            pltpu.VMEM((7, HT1 // 2, HD), u32),
            pltpu.VMEM((N2, 4, 2 * D + PAD, 128), bf16),
            pltpu.VMEM((4, 2 * D + PAD, 128), bf16),
            pltpu.VMEM((4, HD + PAD, 128), bf16),
            pltpu.VMEM((4, HD + PAD, 128), bf16),
            pltpu.VMEM((NP, 80, 128), f32),
            pltpu.VMEM((NP, 80, 128), bf16),
            *[pltpu.VMEM((HT2 + 8, HD), f32) for _ in range(4)],
            pltpu.VMEM((HT2, 384), f32),
            *[pltpu.VMEM((HT2, HD), f32) for _ in range(7)],
            pltpu.VMEM((S, D), bf16),
            pltpu.VMEM((S + 16, D), bf16),
            pltpu.VMEM((8, D), f32),
            pltpu.VMEM((3, 8, 128), f32),
            pltpu.VMEM((8, 128), jnp.int32),
            pltpu.VMEM((8, D), bf16),
            *[pltpu.VMEM((256, 128), f32) for _ in range(4)],
            pltpu.SemaphoreType.DMA((NSEM,)),
        ],
        compiler_params=pltpu.CompilerParams(
            vmem_limit_bytes=110 * 1024 * 1024,
            disable_bounds_checks=True,
            disable_semaphore_checks=True),
    )(A_x, A_wqkv, A_w_phi, A_wo, B_w_r, B_w_gate, B_w_up, B_w_down)
```

```python
import jax
import jax.numpy as jnp
from jax import lax
import jax.experimental.pallas as pl
import jax.experimental.pallas.tpu as pltpu

S = 2048
D = 1024
H = 32
DH = 32
F = 3584
NP = H // 2
T1 = 256
T2 = 512
N1 = S // T1
N2 = S // T2
HT1 = T1 // 2
HT2 = T2 // 2
HD = D // 2
WC = 256
NWC = D // WC
LOG2E = 1.4426950408889634
EPS = 1e-5
PAD = 16
WO_ROWS = 176
LN_ROWS = 16
MAIN = 56
EP_ROWS = 32

T0_FOLD = (0, 4, 11, 18, 25, 33, 39, 46)
T0_WAITS = ((4, (1,)), (11, ('phi', 2)), (18, (3, 4)), (33, ('x1', 5, 6)), (46, (7,)),
            (65, (8, 9, 10, 11, 'x2', 'x3')))
T0_VPREP = ((65, 66, 66.5, 67.5), (68.5, 69, 70, 72), (74, 76, 78, 79), (81, 83, 85, 86))
T0_COMPACT = (47, 55)
T0_VSPAN = (2, 5, 5, 4)
T0_LN = (33, 33, 35, 37, 38, 39, 40, 45)
T0_LNSPAN = (3, 3, 0, 0, 0, 0, 0, 0)
T1_LN = ((102, 103, 104, 105, 106, 107, 108, 109), (89, 91, 93, 95, 97, 99, 100, 101))
P1_LNSPAN = 5
P1_WO = (29, 30, 31, 32, 35, 49, 51, 52, 53, 54, 55)
P1_WOSPAN = 3
P1_LN2 = ((42, 43, 44, 45, 46, 47, 48, 50), (34, 35, 36, 37, 38, 39, 40, 41))
P1_LNSPAN2 = (3, 3)
LT_START = (0, 0, 1, 5, 8, 11, 14)
LT_SPAN = (1, 3, 4, 4, 3, 4, 5)
FB_START = (2, 4, 6, 8, 10, 12, 14, 16)
FB_SPAN = 2
SA_START = (9, 11, 13, 15, 15, 18, 18, 19)
SA_SPAN = 4
FA_START = (20, 21, 22, 23, 24, 25, 26, 27)
FA_SPAN = (3, 6, 2, 4, 2, 4, 2, 2)
FFN_VPU_BLOCKS = 7
FFN_KG = 16
FFN_W0 = 18
FFN_W1 = 107
FFN_SPAN = 4
FFN_LATE = 16
LATE_AT = (1, 2, 3, 4, 4, 5, 7, 8)

_NT = (((1,), (1,)), ((), ()))
f32 = jnp.float32
bf16 = jnp.bfloat16
u32 = jnp.uint32

K_, Q_, V_ = 0, 1, 2
SRC = {K_: 1, Q_: 0, V_: 2}

SEM_W = 0
SEM_X = SEM_W + 3 * NWC
SEM_X0 = SEM_X + N1
SEM_K0 = SEM_X0 + 4
SEM_PHI = SEM_K0 + 4
SEM_WO = SEM_PHI + 2
SEM_WR, SEM_WG, SEM_WU, SEM_WD, SEM_WGV, SEM_WUV, SEM_O = (SEM_WO + 1 + i for i in range(7))
NSEM = SEM_O + 1


def _rb(v):
    return v.astype(bf16).astype(f32)


def _unpack(w):
    return pltpu.bitcast(w, bf16)


def _mo(i, n):
    return i if isinstance(i, int) else pl.multiple_of(i, n)


def _recip(x):
    r = pl.reciprocal(x, approx=True)
    return r * (2.0 - x * r)


def _sigmoid(x):
    return _recip(1.0 + jnp.exp(jnp.minimum(-x, 80.0)))


def _dual_softmax(p):
    t = p.shape[-1]
    p3 = p.reshape(8, 8, t)

    def allred(v, op):
        v = op(v, pltpu.roll(v, 2, 0))
        return op(v, pltpu.roll(v, 4, 0))

    mx = allred(jnp.max(p3, axis=0), jnp.maximum)
    mn = allred(jnp.min(p3, axis=0), jnp.minimum)
    ep = jnp.exp2(p3 - mx[None])
    en = jnp.exp2(mn[None] - p3)
    sp = allred(jnp.sum(ep, axis=0), jnp.add)
    sn = allred(jnp.sum(en, axis=0), jnp.add)
    fp = (ep * _recip(sp)[None]).reshape(64, t)
    fn = (en * _recip(sn)[None]).reshape(64, t)
    return jnp.concatenate([fp, fn], axis=0).astype(bf16)


def _left_combos(a11, a12, a21, a22):
    return [a11 + a22, a21 + a22, a11, a22, a11 + a12, a21 - a11, a12 - a22]


def _right_combos(b11, b12, b21, b22):
    return [b11 + b22, b11, b12 - b22, b21 - b11, b22, b11 + b12, b21 + b22]


def _strassen(prod, emit):
    m3 = prod(2)
    m5 = prod(4)
    emit(0, 1, m3 + m5)
    m7 = prod(6)
    u = m7 - m5
    m1 = prod(0)
    u = u + m1
    w = m1 + m3
    m4 = prod(3)
    emit(0, 0, u + m4)
    m2 = prod(1)
    emit(1, 0, m2 + m4)
    w = w - m2
    m6 = prod(5)
    emit(1, 1, w + m6)


def _or_into(w, toks):
    if not toks:
        return w
    top = w[0:8, 0:128]
    for tk in toks:
        top = top | tk
    if w.shape[1] > 128:
        top = jnp.concatenate([top, w[0:8, 128:]], axis=1)
    return jnp.concatenate([top, w[8:]], axis=0)


def _fold_token(w, zero):
    r, c = w.shape
    acc = None
    for i in range(r // 8):
        for j in range(c // 128):
            blk = w[i * 8:(i + 1) * 8, j * 128:(j + 1) * 128]
            acc = blk if acc is None else acc | blk
    return acc & zero


def _body(zs, x_hbm, wqkv_hbm, wphi_hbm, wo_hbm, wr_hbm, wg_hbm, wu_hbm, wd_hbm, out_hbm,
          x_v, wqkv_v, wphi_v, wo_v, wr_v, wg_v, wu_v, wd_v, wgv_v, wuv_v,
          wt_v, we_v, wl_v, wo7_v, sa7_v, sb7_v, sc7_v, phiq_v, phik_v, vt0_v, vt1_v, kv_acc, kvt_v,
          hal_v, har_v, hbl_v, hbr_v, sa_v, t0_v, t1_v, t2_v, t3_v, t4_v, t5_v, t6_v,
          h_v, out_v, wrf_v, best_v, besti_v, fix_v, xc0_v, xc1_v, xc2_v, xc3_v, sem):
    xcol_v = (xc0_v, xc1_v, xc2_v, xc3_v)
    s_v = (sa7_v, sb7_v)
    vt_v = (vt0_v, vt1_v)
    ha_v = (hal_v, har_v)
    hb_v = (hbl_v, hbr_v)
    tmp_v = (t0_v, t1_v, t2_v, t3_v, t4_v, t5_v, t6_v)

    def x_rows(r0, rows, slot):
        return pltpu.make_async_copy(
            x_hbm.at[0, pl.ds(r0, rows), :], x_v.at[pl.ds(r0, rows), :], sem.at[slot])

    def x_copy(i):
        return x_rows(i * T1, T1, SEM_X + i)

    def x0_copy(q):
        return x_rows((q % 2) * HT1 + (q // 2) * (HT1 // 2), HT1 // 2, SEM_X0 + q)

    def w_copy(kind, c):
        return pltpu.make_async_copy(
            wqkv_hbm.at[:, pl.ds(SRC[kind] * D + c * WC, WC)],
            wqkv_v.at[kind * NWC + c], sem.at[SEM_W + kind * NWC + c])

    def k0_copy(q):
        r0 = (q % 2) * HD + (q // 2) * 256
        return pltpu.make_async_copy(
            wqkv_hbm.at[pl.ds(r0, 256), pl.ds(SRC[K_] * D, WC)],
            wqkv_v.at[K_ * NWC, pl.ds(r0, 256), :], sem.at[SEM_K0 + q])

    def phi_copy(part):
        lo, n = part * (H // 2), H // 2
        return pltpu.make_async_copy(wphi_hbm.at[pl.ds(lo, n)], wphi_v.at[pl.ds(lo, n)],
                                     sem.at[SEM_PHI + part])

    def full_copy(src, dst, slot):
        return pltpu.make_async_copy(src, dst, sem.at[slot])

    x0_copy(0).start()
    x0_copy(1).start()
    full_copy(wr_hbm, wr_v, SEM_WR).start()
    phi_copy(0).start()
    x0_copy(2).start()
    x0_copy(3).start()
    for q in range(4):
        k0_copy(q).start()
    w_copy(K_, 1).start()
    phi_copy(1).start()
    w_copy(K_, 2).start()
    w_copy(K_, 3).start()
    w_copy(Q_, 0).start()
    x_copy(1).start()
    for c in range(1, NWC):
        w_copy(Q_, c).start()
    for c in range(NWC):
        w_copy(V_, c).start()
    x_copy(2).start()
    x_copy(3).start()
    full_copy(wo_hbm, wo_v.at[pl.ds(0, D), :], SEM_WO).start()
    for i in range(4, N1):
        x_copy(i).start()
    f0 = F - 256 * FFN_VPU_BLOCKS
    ffn_tiled = ((wg_hbm, wg_v, D, SEM_WG), (wu_hbm, wu_v, D, SEM_WU), (wd_hbm, wd_v, F, SEM_WD))
    for src, dst, rows, slot in ffn_tiled:
        for c in range(dst.shape[0]):
            full_copy(src.at[:, pl.ds(c * 128, 128)], dst.at[c, pl.ds(0, rows), :], slot).start()
    full_copy(wg_hbm.at[:, pl.ds(f0, F - f0)], wgv_v, SEM_WGV).start()
    full_copy(wu_hbm.at[:, pl.ds(f0, F - f0)], wuv_v, SEM_WUV).start()

    zero_v = jnp.full((8, 128), zs, jnp.int32).astype(u32)

    def zrows(r0, rows, mult=8):
        return pl.ds(pl.multiple_of(zs * mult + r0, mult), rows)

    def tiles(ref, r0, rows):
        w = ref.bitcast(u32)
        return jnp.concatenate(
            [w[c, r0 // 2:(r0 + rows) // 2, :] for c in range(ref.shape[0])], axis=1)

    def token(*vals):
        return lambda: _fold_token(pltpu.bitcast(jnp.concatenate(vals, axis=0), u32), zero_v)

    def ln1_stats(xf):
        m = jnp.sum(xf, axis=-1, keepdims=True) * (1.0 / D)
        q = jnp.sum(xf * xf, axis=-1, keepdims=True) * (1.0 / D)
        inv = lax.rsqrt(jnp.maximum(q - m * m, 0.0) + EPS)
        return inv, m * inv

    def ln1_piece(r0, dst, p, m=None):
        fixed = isinstance(r0, int)
        if m is not None:
            x_v[zrows(S, 8) if fixed else pl.ds(S, 8), 0:128] = m[0:8, 0:128].astype(bf16)
        xa, xb = [x_v[pl.ds(_mo(r0 + hf * HT1 + p * LN_ROWS, LN_ROWS), LN_ROWS), :]
                  .astype(f32) for hf in range(2)]
        (ia, ma), (ib, mb) = ln1_stats(xa), ln1_stats(xb)
        ya, yb = xa * ia, xb * ib
        s2 = ya[:, :HD] - ma
        s5 = yb[:, HD:] - mb
        s1 = s2 + s5
        s3 = yb[:, :HD] - yb[:, HD:]
        s4 = ya[:, HD:] - ya[:, :HD]
        combos = [s1, s2, s3, s4, s5, s1 + s3, s1 + s4]
        rows = zrows(p * LN_ROWS, LN_ROWS, 16) if fixed else pl.ds(p * LN_ROWS, LN_ROWS)
        for i in range(7):
            for c in range(4):
                dst[i, c, rows, :] = combos[i][:, c * 128:(c + 1) * 128].astype(bf16)
        return token(combos[5], combos[6])

    def fold_piece(kind, c, j, pt):
        blk = {}
        for hh in range(2):
            for kh in range(2):
                k0 = kh * HD + j * 128
                w = wqkv_v[kind * NWC + c, k0:k0 + 128, hh * 128:(hh + 1) * 128]
                blk[hh, kh] = lax.dot_general(pt[2 * c + hh], w, _NT,
                                              preferred_element_type=f32) * LOG2E
        combos = _left_combos(blk[0, 0], blk[0, 1], blk[1, 0], blk[1, 1])
        r0 = kind * HD + c * 128
        for i in range(7):
            wt_v[i, j, r0:r0 + 128, :] = combos[i].astype(bf16)
            we_v[kind, i, j, c * 16:(c + 1) * 16, :] = combos[i][0:16].astype(bf16)

    def fold_chunk(kind, c, pt):
        for j in range(4):
            fold_piece(kind, c, j, pt)

    def vprep_piece(c, j, m):
        wqkv_v[zs + 3 * NWC, 0:8, 0:128] = m[0:8, 0:128].astype(bf16)
        blk = {}
        for hh in range(2):
            for kh in range(2):
                k0 = kh * HD + j * 128
                w = wqkv_v[V_ * NWC + c, k0:k0 + 128, hh * 128:(hh + 1) * 128]
                blk[hh, kh] = w.T.astype(f32)
        combos = _left_combos(blk[0, 0], blk[0, 1], blk[1, 0], blk[1, 1])
        r0 = V_ * HD + c * 128
        for i in range(7):
            wt_v[i, j, r0:r0 + 128, :] = combos[i].astype(bf16)
        return token(combos[1], combos[4])

    def wo_piece(w0, m):
        wo_v[D:D + 8, 0:128] = m[0:8, 0:128].astype(bf16)
        top = wo_v[pl.ds(pl.multiple_of(w0, 16), 16), :].astype(f32)
        bot = wo_v[pl.ds(pl.multiple_of(HD + w0, 16), 16), :].astype(f32)
        combos = _right_combos(top[:, :HD], top[:, HD:], bot[:, :HD], bot[:, HD:])
        for i in range(7):
            for c in range(4):
                wo7_v[i, c, pl.ds(pl.multiple_of(w0, 16), 16), :] = (
                    combos[i][:, c * 128:(c + 1) * 128].astype(bf16))
        return token(combos[5], combos[6])

    def run_rounds(t0, rounds, post, first):
        count = [0]
        pins = {}

        def run_jobs(m):
            for fn, span in post.get(count[0], ()):
                tok = fn(m)
                if span:
                    pins.setdefault(count[0] + span, []).append(tok())
            count[0] += 1

        for par, kind, cs in rounds:
            r0 = kind * HD + cs[0] * 128
            rows = 128 * len(cs)

            def prod(i):
                if (par, kind) == (1, V_):
                    rhs = sc7_v[i]
                else:
                    rhs = tiles(s_v[par].at[i], 0, HT1)
                if (par, kind, cs[0]) == (1, K_, 0):
                    sc7_v[i, zrows(0, HT1 // 2), :] = rhs
                if len(cs) == NWC:
                    lhs = jnp.concatenate(
                        [wl_v[kind, i]] + [tiles(wt_v.at[i], r0 + c * 128 + 16, 2 * MAIN)
                                           for c in cs], axis=0)
                else:
                    lhs = tiles(wt_v.at[i], r0, rows)
                m = lax.dot_general(_unpack(lhs),
                                    _unpack(_or_into(rhs, pins.get(count[0]))),
                                    _NT, preferred_element_type=f32)
                run_jobs(m)
                return m

            def emit(rh, ch, blk):
                tb = 2 * par + ch
                for n, c in enumerate(cs):
                    for jj in range(2):
                        pair = 4 * c + 2 * rh + jj
                        if kind == V_:
                            p = blk[n * 128 + jj * 64:n * 128 + (jj + 1) * 64]
                        elif len(cs) == NWC:
                            sub = lax.broadcasted_iota(jnp.int32, (8, HT1), 0)
                            ends = [blk[k * 16 + jj * 8:k * 16 + jj * 8 + 8] for k in range(3)]
                            if c < 3:
                                end = ends[c]
                            else:
                                end = jnp.where(
                                    sub < 2, pltpu.roll(ends[0], 2, 0),
                                    jnp.where(sub < 4, pltpu.roll(ends[1], 4, 0),
                                              pltpu.roll(ends[2], 6, 0)))
                            q0 = 48 + (2 * n + jj) * MAIN
                            p = jnp.concatenate(
                                [blk[q0:q0 + MAIN], jnp.where(sub < 6, end, 0.0)], axis=0)
                        else:
                            q0, q1 = n * 128 + 16 + jj * MAIN, n * 128 + jj * 8
                            p = jnp.concatenate([blk[q0:q0 + MAIN], blk[q1:q1 + 8]], axis=0)
                        if kind == K_:
                            phik_v[tb, zrows(pair * 128, 128, 16), :] = _dual_softmax(p)
                        elif kind == Q_:
                            phiq_v[t0 // 2, tb, pair * 128:(pair + 1) * 128, :] = (
                                _dual_softmax(p))
                        else:
                            vt_v[pair // 8][tb, zrows((pair % 8) * 64, 64, 16), :] = (
                                p.astype(bf16))

            _strassen(prod, emit)

        ones = jnp.full((8, 2 * T1), 0x3F803F80, u32)
        kr = lax.broadcasted_iota(jnp.int32, (80, 128), 0)
        kc = lax.broadcasted_iota(jnp.int32, (80, 128), 1)
        kmask = jnp.where(kr < 64, kr // 32, (kr - 64) // 8) == kc % 2
        for j in range(NP):
            lhs = jnp.concatenate([tiles(vt_v[j // 8], (j % 8) * 64, 64), ones], axis=0)
            rhs = tiles(phik_v, j * 128, 128)
            upd = lax.dot_general(_unpack(lhs), _unpack(_or_into(rhs, pins.get(count[0]))), _NT,
                                  preferred_element_type=f32)
            run_jobs(upd)
            if first:
                kv_acc[j] = upd
            else:
                upd = kv_acc[j] + upd
                kv_acc[j] = upd
                kvt_v[j] = jnp.where(kmask, upd, 0.0).astype(bf16)

    def load_best():
        return best_v[0], besti_v[...], best_v[1], best_v[2]

    def store_best(best):
        best_v[0], besti_v[...], best_v[1], best_v[2] = best

    def build_pt(g0, g1):
        def row_ids(r):
            pair = jnp.where(r < 16, r // 8, jnp.where(r < 16 + MAIN, 0, 1))
            feat = jnp.where(r < 16, MAIN + r % 8, r - 16 - pair * MAIN) // 2
            return pair, feat

        n = g1 - g0
        w2 = wphi_v[4 * g0:4 * g1].reshape(n * 128, DH)
        er = lax.broadcasted_iota(jnp.int32, (128, DH), 0)
        ec = lax.broadcasted_iota(jnp.int32, (128, DH), 1)
        e = (jnp.where(ec == row_ids(er)[1], 1.0, 0.0)
             - jnp.where(ec == DH - 1, 1.0, 0.0)).astype(bf16)
        ptf = lax.dot_general(e, w2, _NT, preferred_element_type=f32)
        pr = lax.broadcasted_iota(jnp.int32, (128, 128), 0)
        pc = lax.broadcasted_iota(jnp.int32, (128, 128), 1)
        keep = pc // 32 == row_ids(pr)[0] * 2 + pr % 2
        return [jnp.where(keep, ptf[:, g * 128:(g + 1) * 128], 0.0).astype(bf16)
                for g in range(n)]

    def compact(kind, i, m):
        we_v[0, 0, 0, zrows(64, 16, 16), :] = m[0:16, 0:128].astype(bf16)
        sub = lax.broadcasted_iota(jnp.int32, (8, HD), 0)
        ends = tiles(we_v.at[kind, i], 0, 64)
        for c in range(NWC - 1):
            wl_v[kind, i, zrows(c * 8, 8), :] = jnp.where(
                sub % 4 == 3, pltpu.roll(ends[24:32], 3 - c, 0), ends[c * 8:(c + 1) * 8])

    hbl_v[...] = jnp.zeros_like(hbl_v)
    hbr_v[...] = jnp.zeros_like(hbr_v)
    store_best((jnp.full((8, 128), -jnp.inf, f32), jnp.zeros((8, 128), jnp.int32),
                jnp.zeros((8, 128), f32), jnp.zeros((8, 128), f32)))
    n_ln = HT1 // LN_ROWS
    x0_copy(0).wait()
    x0_copy(1).wait()
    for p in range(n_ln // 2):
        ln1_piece(0, s_v[0], p)
    full_copy(wr_hbm, wr_v, SEM_WR).wait()
    phi_copy(0).wait()
    x0_copy(2).wait()
    x0_copy(3).wait()
    wr_row = wr_v[...].astype(f32).reshape(1, D)
    wrf_v[...] = jnp.broadcast_to(
        wr_row - jnp.sum(wr_row, axis=-1, keepdims=True) * (1.0 / D), (8, D))
    pt = build_pt(0, 4)
    for p in range(n_ln // 2, n_ln):
        ln1_piece(0, s_v[0], p)
    for part in range(2):
        k0_copy(2 * part).wait()
        k0_copy(2 * part + 1).wait()
        fold_piece(K_, 0, 2 * part, pt)
        fold_piece(K_, 0, 2 * part + 1, pt)

    post = {}

    def at(slot, fn, span=0):
        late_gate = 240 if slot != int(slot) else 0
        post.setdefault(int(slot), []).append((lambda m: fn(m[late_gate:]), span))

    for slot, copies in T0_WAITS:
        for cp in copies:
            if cp == 'phi':
                at(slot, lambda m: phi_copy(1).wait())
            elif cp in ('x1', 'x2', 'x3'):
                at(slot, lambda m, cp=cp: x_copy(int(cp[1])).wait())
            else:
                at(slot, lambda m, cp=cp: w_copy(cp // NWC, cp % NWC).wait())
    for n in range(1, 2 * NWC):
        if n == 2:
            at(T0_FOLD[n], lambda m: pt.extend(build_pt(4, 8)))
        at(T0_FOLD[n], lambda m, n=n: fold_chunk(n // NWC, n % NWC, pt))
    for kind in (K_, Q_):
        for i in range(7):
            at(T0_COMPACT[kind] + i, lambda m, kind=kind, i=i: compact(kind, i, m))
    for c in range(NWC):
        for j in range(4):
            at(T0_VPREP[c][j], lambda m, c=c, j=j: vprep_piece(c, j, m), T0_VSPAN[c])
    for p in range(n_ln):
        at(T0_LN[p], lambda m, p=p: ln1_piece(T1, s_v[1], p, m), T0_LNSPAN[p])
    for p in range(n_ln):
        at(T1_LN[0][p], lambda m, p=p: ln1_piece(2 * T1, s_v[0], p, m), P1_LNSPAN)
        at(T1_LN[1][p], lambda m, p=p: ln1_piece(3 * T1, s_v[1], p, m), P1_LNSPAN)
    lo, hi = [0, 1], [2, 3]
    run_rounds(0, [(0, kind, [c]) for kind in (K_, Q_) for c in range(NWC)]
               + [(1, K_, lo + hi), (1, Q_, lo + hi)] + [(0, V_, [c]) for c in range(NWC)]
               + [(1, V_, lo), (1, V_, hi)], post, True)
    full_copy(wo_hbm, wo_v.at[pl.ds(0, D), :], SEM_WO).wait()
    for i in range(4, N1):
        x_copy(i).wait()

    def phase1(i, carry):
        post = {}
        nxt = jnp.minimum(i + 1, N2 - 1) * T2
        w0 = jnp.minimum((i - 1) * WO_ROWS, HD - WO_ROWS)
        for par in range(2):
            for p in range(n_ln):
                post.setdefault(P1_LN2[par][p], []).append(
                    (lambda m, p=p, par=par: ln1_piece(nxt + par * T1, s_v[par], p, m),
                     P1_LNSPAN2[par]))
        for p in range(WO_ROWS // 16):
            post.setdefault(P1_WO[p], []).append(
                (lambda m, p=p: wo_piece(w0 + 16 * p, m), P1_WOSPAN))
        run_rounds(2 * i, [(par, kind, lo + hi) for kind in (K_, Q_) for par in range(2)]
                   + [(par, V_, cs) for par in range(2) for cs in (lo, hi)], post, False)
        return carry

    lax.fori_loop(1, N1 // 2, phase1, 0)

    for _, dst, rows, slot in ffn_tiled:
        filled = dst.at[:, pl.ds(0, rows), :]
        full_copy(filled, filled, slot).wait()
    full_copy(wg_hbm.at[:, pl.ds(f0, F - f0)], wgv_v, SEM_WGV).wait()
    full_copy(wu_hbm.at[:, pl.ds(f0, F - f0)], wuv_v, SEM_WUV).wait()

    def o_copy(hf):
        return pltpu.make_async_copy(
            out_v.at[pl.ds(hf * HT2, HT2), :], out_hbm.at[0, pl.ds(hf * HT2, HT2), :],
            sem.at[SEM_O])

    def half_stats(hh, c0):
        rows = hh.shape[0]
        parts = [hh[:, c * 128:(c + 1) * 128] for c in range(4)]
        wts = [wrf_v[:, c0 + c * 128:c0 + (c + 1) * 128] for c in range(4)]
        s1 = (parts[0] + parts[1]) + (parts[2] + parts[3])
        sq = [p * p for p in parts]
        s2 = (sq[0] + sq[1]) + (sq[2] + sq[3])
        dw = [(p.reshape(rows // 8, 8, 128) * w[None]).reshape(rows, 128)
              for p, w in zip(parts, wts)]
        s3 = (dw[0] + dw[1]) + (dw[2] + dw[3])
        return s1, s2, s3

    def first_half(hbuf, sbuf, base, p, c0):
        r0 = p * EP_ROWS
        hh = hbuf[c0 // HD][r0:r0 + EP_ROWS, :]
        h_v[pl.ds(pl.multiple_of(base + r0, EP_ROWS), EP_ROWS), c0:c0 + HD] = hh.astype(bf16)
        st = jnp.concatenate(half_stats(hh, c0), axis=1)
        sbuf[zrows(r0, EP_ROWS), :] = st
        return _fold_token(pltpu.bitcast(st, u32), zero_v)

    def finish(hbuf, sbuf, base, p, valid, best, defer=None):
        r0 = p * EP_ROWS
        g0 = pl.multiple_of(base + r0, EP_ROWS)
        hl, hr = [r[r0:r0 + EP_ROWS, :] for r in hbuf]
        if defer is None:
            h_v[pl.ds(g0, EP_ROWS), 0:HD] = hl.astype(bf16)
        if sbuf is None:
            if defer is None:
                h_v[pl.ds(g0, EP_ROWS), HD:D] = hr.astype(bf16)
            st = half_stats(hr, HD)
        else:
            st = sbuf[r0:r0 + EP_ROWS, :]
            st = [st[:, n * 128:(n + 1) * 128] for n in range(3)]
        s1, s2, s3 = [jnp.sum(v + w, axis=-1, keepdims=True)
                      for v, w in zip(half_stats(hl, 0), st)]
        m = s1 * (1.0 / D)
        var = jnp.maximum(s2 * (1.0 / D) - m * m, 0.0)
        inv = lax.rsqrt(var + EPS)
        r = s3 * inv

        def write_out(h):
            o = h * (1.0 + inv) - m * inv
            out_v[pl.ds(g0, EP_ROWS), :] = o.astype(bf16)
            return o

        if defer is None:
            o = write_out(jnp.concatenate([hl, hr], axis=1))
        else:
            defer.append(lambda: write_out(jnp.concatenate(
                [r_[r0:r0 + EP_ROWS, :] for r_ in hbuf], axis=1)))
        bv, bi, bm, bq = best
        sub = lax.broadcasted_iota(jnp.int32, (8, 128), 0)
        for g in range(EP_ROWS // 8):
            rows = slice(g * 8, (g + 1) * 8)
            rg = jnp.broadcast_to(r[rows], (8, 128))
            if valid is not None:
                rg = jnp.where(valid, rg, -jnp.inf)
            better = rg > bv
            bi = jnp.where(better, sub + (g0 + g * 8), bi)
            bv = jnp.where(better, rg, bv)
            bm = jnp.where(better, jnp.broadcast_to(m[rows], (8, 128)), bm)
            bq = jnp.where(better, jnp.broadcast_to(var[rows], (8, 128)), bq)
        best = (bv, bi, bm, bq)
        if defer is not None:
            return best, None
        tok = _fold_token(pltpu.bitcast(jnp.concatenate(
            [o[:, D - 128:], bv, bm, bq], axis=0), u32), zero_v)
        return best, tok

    n_ep = HT2 // EP_ROWS

    def phase2(i, carry):
        ot = []
        for j in range(NP):
            ph = tiles(phiq_v.at[i], j * 128, 128)
            n = jnp.dot(_unpack(kvt_v.bitcast(u32)[j]), _unpack(ph),
                        preferred_element_type=f32)
            r0h = _recip(n[64:72] + 1e-6)
            r1h = _recip(n[72:80] + 1e-6)
            ot.append((n[0:32].reshape(4, 8, T2) * r0h[None]).reshape(32, T2))
            ot.append((n[32:64].reshape(4, 8, T2) * r1h[None]).reshape(32, T2))
        lo = jnp.concatenate(ot[:H // 2], axis=0)
        hi = jnp.concatenate(ot[H // 2:], axis=0)
        lcs = _left_combos(lo[:, :HT2], hi[:, :HT2], lo[:, HT2:], hi[:, HT2:])

        state = {'best': load_best()}
        pins = {}
        jobs = {}
        lts = {}
        ra = pl.multiple_of(i * T2, T2)
        rb = pl.multiple_of(i * T2 + HT2, HT2)
        prev = jnp.maximum(i * T2 - HT2, HT2)

        def add_job(slot, deadline, fn, gates=()):
            jobs.setdefault(slot, []).append((fn, deadline, gates))

        def finish_job(hbuf, sbuf, base, p, valid):
            def fn():
                state['best'], tok = finish(hbuf, sbuf, base, p, valid, state['best'])
                return tok
            return fn

        def lt_job(k):
            def fn():
                lts[k] = lcs[k].astype(bf16).T
                return _fold_token(pltpu.bitcast(lts[k], u32), zero_v)
            return fn

        order = (2, 4, 6, 0, 3, 1, 5)
        lt_job(2)()
        for n in range(1, 7):
            add_job(LT_START[n], min(LT_START[n] + LT_SPAN[n], 4 * n), lt_job(order[n]))
        for p in range(n_ep):
            add_job(FB_START[p], FB_START[p] + FB_SPAN,
                    finish_job(hb_v, None, prev, p, i > 0), hb_v)
            add_job(SA_START[p], SA_START[p] + SA_SPAN,
                    lambda p=p: first_half(ha_v, sa_v, ra, p, HD), ha_v[1:])
            add_job(FA_START[p], FA_START[p] + FA_SPAN[p],
                    finish_job(ha_v, sa_v, ra, p, None), ha_v)

        def xblk(r0, c0):
            return x_v[pl.ds(r0, HT2), c0:c0 + 128].astype(f32)

        for n, k in enumerate(order):
            for c in range(4):
                slot = 4 * n + c
                for fn, deadline, gates in jobs.get(slot, ()):
                    for ref in gates:
                        ref[zrows(HT2, 8), 0:128] = mm[0:8]
                    pins.setdefault(deadline, []).append(fn())
                w = _or_into(wo7_v.bitcast(u32)[k, c, 0:HD // 2, :], pins.get(slot))
                mm = jnp.dot(lts[k], _unpack(w), preferred_element_type=f32)
                c0 = c * 128
                cs = slice(c0, c0 + 128)
                tmp = lambda t: tmp_v[t][:, cs]
                if n == 0:
                    tmp_v[0][zrows(0, HT2), cs] = mm
                elif n == 1:
                    ha_v[1][zrows(0, HT2), cs] = (xblk(ra, HD + c0) + tmp(0)) + mm
                    tmp_v[1][zrows(0, HT2), cs] = xblk(ra, c0) - mm
                elif n == 2:
                    tmp_v[2][zrows(0, HT2), cs] = tmp(1) + mm
                elif n == 3:
                    tmp_v[3][zrows(0, HT2), cs] = tmp(2) + mm
                    tmp_v[4][zrows(0, HT2), cs] = (xblk(rb, HD + c0) + tmp(0)) + mm
                elif n == 4:
                    ha_v[0][zrows(0, HT2), cs] = tmp(3) + mm
                    tmp_v[5][zrows(0, HT2), cs] = xblk(rb, c0) + mm
                elif n == 5:
                    hb_v[0][zrows(0, HT2), cs] = tmp(5) + mm
                    tmp_v[6][zrows(0, HT2), cs] = tmp(4) - mm
                else:
                    hb_v[1][zrows(0, HT2), cs] = tmp(6) + mm
        store_best(state['best'])
        o_copy(2 * i).start()

        @pl.when(i > 0)
        def _():
            o_copy(2 * i - 1).start()

        return carry

    lax.fori_loop(0, N2, phase2, 0)
    best = load_best()
    late = []
    for p in range(n_ep):
        best, _ = finish(hb_v, None, S - HT2, p, None, best, late)

    bv, bi, bm, bq = best
    for sh in (4, 2, 1):
        ov, oi, om, oq = [pltpu.roll(t, sh, 0) for t in (bv, bi, bm, bq)]
        take = jnp.logical_or(ov > bv, jnp.logical_and(ov == bv, oi < bi))
        bv, bi, bm, bq = [jnp.where(take, o_, t)
                          for o_, t in zip((ov, oi, om, oq), (bv, bi, bm, bq))]
    idx = jnp.clip(bi[0, 0], 0, S - 1)
    b0 = pl.multiple_of((idx // 8) * 8, 8)
    t = _rb(_rb(bq) + EPS)
    inv = _recip(_rb(t * lax.rsqrt(t)))
    gate = _sigmoid(bv)
    wide = lambda v: jnp.concatenate([v] * (D // 128), axis=1)
    b1 = pl.multiple_of(jnp.minimum(b0, S - HT2 - 8), 8)
    b2 = pl.multiple_of(jnp.maximum(b0 - (S - HT2), 0), 8)
    hb = jnp.where(wide(bi) < S - HT2, h_v[pl.ds(b1, 8), :].astype(f32),
                   _rb(jnp.concatenate([r_[pl.ds(b2, 8), :] for r_ in hb_v], axis=1)))
    hn = (hb - wide(bm)) * wide(inv)
    xs = hn.astype(bf16)
    rows = lax.broadcasted_iota(jnp.int32, (8, D), 0) + b0

    xm = jnp.where(rows == wide(bi), _rb(hn), 0.0)
    for sh in (4, 2, 1):
        xm = xm + pltpu.roll(xm, sh, 0)
    for t in range(D // 128):
        xcol_v[t // 2][zrows((t % 2) * 128, 128), :] = jnp.concatenate(
            [xm[:, t * 128:(t + 1) * 128]] * 16, axis=0).T

    nblk = F // 256
    nmx = nblk - FFN_VPU_BLOCKS
    act = {}
    acc = {}

    def activate(g, u):
        return (g * _sigmoid(g) * u).astype(bf16)

    parts = D // 8 // FFN_KG

    def vpu_chunk(q):
        blk, part = nmx + q // parts, q % parts
        cur = acc.get(blk)
        for kg in range(part * FFN_KG, (part + 1) * FFN_KG):
            xc = xcol_v[kg // 32][(kg % 32) * 8:(kg % 32 + 1) * 8, :]
            w = jnp.concatenate(
                [r[kg * 8:(kg + 1) * 8, (blk - nmx) * 256:(blk - nmx + 1) * 256].astype(f32)
                 for r in (wgv_v, wuv_v)], axis=1)
            p = w * jnp.concatenate([xc] * 4, axis=1)
            cur = p if cur is None else cur + p
        acc[blk] = cur
        if part == parts - 1:
            for sh in (4, 2, 1):
                cur = cur + pltpu.roll(cur, sh, 0)
            act[blk] = activate(cur[:, :256], cur[:, 256:])
        c = q % 4
        return _fold_token(pltpu.bitcast(cur[:, c * 128:(c + 1) * 128], u32), zero_v)

    nchunk = FFN_VPU_BLOCKS * parts
    starts = [FFN_W0 + (q * (FFN_W1 - FFN_W0)) // (nchunk - 1) for q in range(nchunk)]
    pins = {}
    wave = [0]
    wgw, wuw, wdw = [r.bitcast(u32) for r in (wg_v, wu_v, wd_v)]

    def run_wave(lhs, tls):
        w = jnp.concatenate([_or_into(tls[0], pins.get(wave[0]))] + tls[1:], axis=1)
        out = jnp.dot(lhs, _unpack(w), preferred_element_type=f32)
        for p, fn in enumerate(late):
            if LATE_AT[p] == wave[0]:
                for r_ in hb_v:
                    r_[zrows(HT2, 8), 0:128] = out[:, 0:128]
                fn()
        for q, start in enumerate(starts):
            if start == wave[0]:
                pins.setdefault(wave[0] + FFN_SPAN, []).append(vpu_chunk(q))
        if wave[0] == FFN_LATE:
            o_copy(2 * N2 - 1).start()
            out_v[zrows(S, 16, 16), 0:256] = jnp.zeros((16, 256), bf16)
            pins.setdefault(wave[0] + 4, []).append(
                token(out_v[S:S + 8, 0:128].astype(f32))())
        wave[0] += 1
        return out

    for j in range(nmx):
        gu = None
        for kt in range(D // 128):
            p = run_wave(xs[:, kt * 128:(kt + 1) * 128],
                         [r[2 * j + c, kt * 64:(kt + 1) * 64, :]
                          for r in (wgw, wuw) for c in range(2)])
            gu = p if gu is None else gu + p
        act[j] = activate(gu[:, :256], gu[:, 256:])
    ys = [None, None]
    for j in range(nblk):
        for kt in range(2):
            for hf in range(2):
                r0 = (2 * j + kt) * 64
                p = run_wave(act[j][:, kt * 128:(kt + 1) * 128],
                             [wdw[4 * hf + c, r0:r0 + 64, :] for c in range(4)])
                ys[hf] = p if ys[hf] is None else ys[hf] + p
    y = jnp.concatenate(ys, axis=1)
    cur = out_v[pl.ds(b0, 8), :].astype(f32)
    fix_v[...] = jnp.where(rows == wide(bi), hb + hn + y * wide(gate), cur).astype(bf16)
    full_copy(out_v.at[pl.ds(0, S), :], out_hbm.at[0], SEM_O).wait()
    fix = pltpu.make_async_copy(fix_v, out_hbm.at[0, pl.ds(b0, 8), :], sem.at[SEM_O])
    fix.start()
    fix.wait()


def _kernel(*refs):
    def step(i, carry):
        @pl.when(i == 0)
        def _():
            _body(i, *refs)

        return carry

    lax.fori_loop(0, 2, step, 0)


@jax.jit
def pallas_sequential_preLN__linear_kernel_hedgehog__moe_arch_mod__prompt_kernel(
    A_x: jax.Array,
    A_wqkv: jax.Array,
    A_w_phi: jax.Array,
    A_wo: jax.Array,
    B_x: jax.Array,
    B_w_r: jax.Array,
    B_w_gate: jax.Array,
    B_w_up: jax.Array,
    B_w_down: jax.Array,
):
    any_spec = pl.BlockSpec(memory_space=pl.ANY)
    return pl.pallas_call(
        _kernel,
        out_shape=jax.ShapeDtypeStruct((1, S, D), bf16),
        in_specs=[any_spec] * 8,
        out_specs=any_spec,
        scratch_shapes=[
            pltpu.VMEM((S + 16, D), bf16),
            pltpu.VMEM((3 * NWC + 1, D, WC), bf16),
            pltpu.VMEM((H, DH, DH), bf16),
            pltpu.VMEM((D + 16, D), bf16),
            pltpu.VMEM((D,), bf16),
            pltpu.VMEM((F // 128 - 2 * FFN_VPU_BLOCKS, D + PAD, 128), bf16),
            pltpu.VMEM((F // 128 - 2 * FFN_VPU_BLOCKS, D + PAD, 128), bf16),
            pltpu.VMEM((D // 128, F + PAD, 128), bf16),
            pltpu.VMEM((D, 256 * FFN_VPU_BLOCKS), bf16),
            pltpu.VMEM((D, 256 * FFN_VPU_BLOCKS), bf16),
            pltpu.VMEM((7, 4, 3 * HD + PAD, 128), bf16),
            pltpu.VMEM((2, 7, 4, 64 + PAD, 128), bf16),
            pltpu.VMEM((2, 7, 24, HD), u32),
            pltpu.VMEM((7, 4, HD + PAD, 128), bf16),
            pltpu.VMEM((7, 4, HT1 + PAD, 128), bf16),
            pltpu.VMEM((7, 4, HT1 + PAD, 128), bf16),
            pltpu.VMEM((7, HT1 // 2, HD), u32),
            pltpu.VMEM((N2, 4, 2 * D + PAD, 128), bf16),
            pltpu.VMEM((4, 2 * D + PAD, 128), bf16),
            pltpu.VMEM((4, HD + PAD, 128), bf16),
            pltpu.VMEM((4, HD + PAD, 128), bf16),
            pltpu.VMEM((NP, 80, 128), f32),
            pltpu.VMEM((NP, 80, 128), bf16),
            *[pltpu.VMEM((HT2 + 8, HD), f32) for _ in range(4)],
            pltpu.VMEM((HT2, 384), f32),
            *[pltpu.VMEM((HT2, HD), f32) for _ in range(7)],
            pltpu.VMEM((S, D), bf16),
            pltpu.VMEM((S + 16, D), bf16),
            pltpu.VMEM((8, D), f32),
            pltpu.VMEM((3, 8, 128), f32),
            pltpu.VMEM((8, 128), jnp.int32),
            pltpu.VMEM((8, D), bf16),
            *[pltpu.VMEM((256, 128), f32) for _ in range(4)],
            pltpu.SemaphoreType.DMA((NSEM,)),
        ],
        compiler_params=pltpu.CompilerParams(
            vmem_limit_bytes=110 * 1024 * 1024,
            disable_bounds_checks=True,
            disable_semaphore_checks=True),
    )(A_x, A_wqkv, A_w_phi, A_wo, B_w_r, B_w_gate, B_w_up, B_w_down)
```

```python
import jax
import jax.numpy as jnp
from jax import lax
import jax.experimental.pallas as pl
import jax.experimental.pallas.tpu as pltpu

S = 2048
D = 1024
H = 32
DH = 32
F = 3584
NP = H // 2
T1 = 256
T2 = 512
N1 = S // T1
N2 = S // T2
HT1 = T1 // 2
HT2 = T2 // 2
HD = D // 2
WC = 256
NWC = D // WC
LOG2E = 1.4426950408889634
EPS = 1e-5
PAD = 16
WO_ROWS = 176
LN_ROWS = 16
MAIN = 56
EP_ROWS = 32

T0_FOLD = (0, 4, 11, 18, 25, 33, 39, 46)
T0_WAITS = ((4, (1,)), (11, ('phi', 2)), (18, (3, 4)), (33, ('x1', 5, 6)), (46, (7,)),
            (65, (8, 9, 10, 11, 'x2', 'x3')))
T0_VPREP = ((65, 66, 66.5, 67.5), (68.5, 69, 70, 74), (74, 76, 78, 79), (81, 83, 85, 86))
T0_COMPACT = (47, 55)
T0_VSPAN = (2, 5, 5, 4)
T0_LN = (33, 33, 35, 36, 38, 38, 40, 45)
T0_LNSPAN = (3, 3, 0, 0, 0, 0, 0, 0)
T1_LN = ((102, 103, 104, 105, 106, 107, 108, 109), (89, 91, 93, 95, 97, 99, 100, 101))
P1_LNSPAN = 5
P1_WO = (30, 30, 32, 34, 35, 49, 52, 53, 53, 54, 55)
P1_WOSPAN = 3
P1_LN2 = ((42, 43, 44, 45, 46, 47, 48, 50), (34, 35, 35, 37, 38, 39, 40, 41))
P1_LNSPAN2 = (3, 3)
P1_Z = (28, 30, 31, 33, 36, 38, 40, 42, 43, 44, 46, 47, 48, 51, 52, 53)
P1_ZSPAN = 2
T0_Z = (63, 63.5, 64, 70.5, 75, 79, 84, 90, 90, 94, 96.0, 98, 98.0, 99.5, 100.5, 109.5)
T0_ZSPAN = 0
LT_START = (0, 0, 1, 5, 8, 11, 14)
LT_SPAN = (1, 3, 4, 4, 3, 4, 5)
FB_START = (2, 4, 6, 8, 10, 12, 14, 16)
FB_SPAN = 2
SA_START = (9, 11, 13, 15, 15, 18, 18, 19)
SA_SPAN = 4
FA_START = (20, 21, 22, 23, 24, 25, 26, 27)
FA_SPAN = (3, 6, 2, 4, 2, 4, 2, 2)
FFN_VPU_BLOCKS = 7
FFN_KG = 16
FFN_W0 = 18
FFN_W1 = 107
FFN_SPAN = 4
FFN_LATE = 16
LATE_AT = (1, 2, 3, 4, 4, 5, 7, 8)

_NT = (((1,), (1,)), ((), ()))
f32 = jnp.float32
bf16 = jnp.bfloat16
u32 = jnp.uint32

K_, Q_, V_ = 0, 1, 2
SRC = {K_: 1, Q_: 0, V_: 2}

SEM_W = 0
SEM_X = SEM_W + 3 * NWC
SEM_X0 = SEM_X + N1
SEM_K0 = SEM_X0 + 4
SEM_PHI = SEM_K0 + 4
SEM_WO = SEM_PHI + 2
SEM_WR, SEM_WG, SEM_WU, SEM_WD, SEM_WGV, SEM_WUV, SEM_O = (SEM_WO + 1 + i for i in range(7))
NSEM = SEM_O + 1


def _rb(v):
    return v.astype(bf16).astype(f32)


def _unpack(w):
    return pltpu.bitcast(w, bf16)


def _mo(i, n):
    return i if isinstance(i, int) else pl.multiple_of(i, n)


def _recip(x):
    r = pl.reciprocal(x, approx=True)
    return r * (2.0 - x * r)


def _sigmoid(x):
    return _recip(1.0 + jnp.exp(jnp.minimum(-x, 80.0)))


def _dual_softmax(p):
    t = p.shape[-1]
    p3 = p.reshape(8, 8, t)

    def allred(v, op):
        v = op(v, pltpu.roll(v, 2, 0))
        return op(v, pltpu.roll(v, 4, 0))

    mx = allred(jnp.max(p3, axis=0), jnp.maximum)
    mn = allred(jnp.min(p3, axis=0), jnp.minimum)
    ep = jnp.exp2(p3 - mx[None])
    en = jnp.exp2(mn[None] - p3)
    sp = allred(jnp.sum(ep, axis=0), jnp.add)
    sn = allred(jnp.sum(en, axis=0), jnp.add)
    fp = (ep * _recip(sp)[None]).reshape(64, t)
    fn = (en * _recip(sn)[None]).reshape(64, t)
    return jnp.concatenate([fp, fn], axis=0).astype(bf16)


def _left_combos(a11, a12, a21, a22):
    return [a11 + a22, a21 + a22, a11, a22, a11 + a12, a21 - a11, a12 - a22]


def _right_combos(b11, b12, b21, b22):
    return [b11 + b22, b11, b12 - b22, b21 - b11, b22, b11 + b12, b21 + b22]


def _strassen(prod, emit):
    m3 = prod(2)
    m5 = prod(4)
    emit(0, 1, m3 + m5)
    m7 = prod(6)
    u = m7 - m5
    m1 = prod(0)
    u = u + m1
    w = m1 + m3
    m4 = prod(3)
    emit(0, 0, u + m4)
    m2 = prod(1)
    emit(1, 0, m2 + m4)
    w = w - m2
    m6 = prod(5)
    emit(1, 1, w + m6)


def _or_into(w, toks):
    if not toks:
        return w
    top = w[0:8, 0:128]
    for tk in toks:
        top = top | tk
    if w.shape[1] > 128:
        top = jnp.concatenate([top, w[0:8, 128:]], axis=1)
    return jnp.concatenate([top, w[8:]], axis=0)


def _fold_token(w, zero):
    r, c = w.shape
    acc = None
    for i in range(r // 8):
        for j in range(c // 128):
            blk = w[i * 8:(i + 1) * 8, j * 128:(j + 1) * 128]
            acc = blk if acc is None else acc | blk
    return acc & zero


def _body(zs, x_hbm, wqkv_hbm, wphi_hbm, wo_hbm, wr_hbm, wg_hbm, wu_hbm, wd_hbm, out_hbm,
          x_v, wqkv_v, wphi_v, wo_v, wr_v, wg_v, wu_v, wd_v, wgv_v, wuv_v,
          wt_v, we_v, wl_v, wo7_v, sa7_v, sb7_v, sc7_v, phiq_v, phik_v, vt0_v, vt1_v, kv_acc, kvt_v,
          hal_v, har_v, hbl_v, hbr_v, sa_v, t0_v, t1_v, t2_v, t3_v, t4_v, t5_v, t6_v,
          h_v, out_v, wrf_v, best_v, besti_v, fix_v, xc0_v, xc1_v, xc2_v, xc3_v, sem):
    xcol_v = (xc0_v, xc1_v, xc2_v, xc3_v)
    s_v = (sa7_v, sb7_v)
    vt_v = (vt0_v, vt1_v)
    ha_v = (hal_v, har_v)
    hb_v = (hbl_v, hbr_v)
    tmp_v = (t0_v, t1_v, t2_v, t3_v, t4_v, t5_v, t6_v)

    def x_rows(r0, rows, slot):
        return pltpu.make_async_copy(
            x_hbm.at[0, pl.ds(r0, rows), :], x_v.at[pl.ds(r0, rows), :], sem.at[slot])

    def x_copy(i):
        return x_rows(i * T1, T1, SEM_X + i)

    def x0_copy(q):
        return x_rows((q % 2) * HT1 + (q // 2) * (HT1 // 2), HT1 // 2, SEM_X0 + q)

    def w_copy(kind, c):
        return pltpu.make_async_copy(
            wqkv_hbm.at[:, pl.ds(SRC[kind] * D + c * WC, WC)],
            wqkv_v.at[kind * NWC + c], sem.at[SEM_W + kind * NWC + c])

    def k0_copy(q):
        r0 = (q % 2) * HD + (q // 2) * 256
        return pltpu.make_async_copy(
            wqkv_hbm.at[pl.ds(r0, 256), pl.ds(SRC[K_] * D, WC)],
            wqkv_v.at[K_ * NWC, pl.ds(r0, 256), :], sem.at[SEM_K0 + q])

    def phi_copy(part):
        lo, n = part * (H // 2), H // 2
        return pltpu.make_async_copy(wphi_hbm.at[pl.ds(lo, n)], wphi_v.at[pl.ds(lo, n)],
                                     sem.at[SEM_PHI + part])

    def full_copy(src, dst, slot):
        return pltpu.make_async_copy(src, dst, sem.at[slot])

    x0_copy(0).start()
    x0_copy(1).start()
    full_copy(wr_hbm, wr_v, SEM_WR).start()
    phi_copy(0).start()
    x0_copy(2).start()
    x0_copy(3).start()
    for q in range(4):
        k0_copy(q).start()
    w_copy(K_, 1).start()
    phi_copy(1).start()
    w_copy(K_, 2).start()
    w_copy(K_, 3).start()
    w_copy(Q_, 0).start()
    x_copy(1).start()
    for c in range(1, NWC):
        w_copy(Q_, c).start()
    for c in range(NWC):
        w_copy(V_, c).start()
    x_copy(2).start()
    x_copy(3).start()
    full_copy(wo_hbm, wo_v.at[pl.ds(0, D), :], SEM_WO).start()
    for i in range(4, N1):
        x_copy(i).start()
    f0 = F - 256 * FFN_VPU_BLOCKS
    ffn_tiled = ((wg_hbm, wg_v, D, SEM_WG), (wu_hbm, wu_v, D, SEM_WU), (wd_hbm, wd_v, F, SEM_WD))
    for src, dst, rows, slot in ffn_tiled:
        for c in range(dst.shape[0]):
            full_copy(src.at[:, pl.ds(c * 128, 128)], dst.at[c, pl.ds(0, rows), :], slot).start()
    full_copy(wg_hbm.at[:, pl.ds(f0, F - f0)], wgv_v, SEM_WGV).start()
    full_copy(wu_hbm.at[:, pl.ds(f0, F - f0)], wuv_v, SEM_WUV).start()

    zero_v = jnp.full((8, 128), zs, jnp.int32).astype(u32)

    def zrows(r0, rows, mult=8):
        return pl.ds(pl.multiple_of(zs * mult + r0, mult), rows)

    def tiles(ref, r0, rows):
        w = ref.bitcast(u32)
        return jnp.concatenate(
            [w[c, r0 // 2:(r0 + rows) // 2, :] for c in range(ref.shape[0])], axis=1)

    def token(*vals):
        return lambda: _fold_token(pltpu.bitcast(jnp.concatenate(vals, axis=0), u32), zero_v)

    def ln1_stats(xf):
        m = jnp.sum(xf, axis=-1, keepdims=True) * (1.0 / D)
        q = jnp.sum(xf * xf, axis=-1, keepdims=True) * (1.0 / D)
        inv = lax.rsqrt(jnp.maximum(q - m * m, 0.0) + EPS)
        return inv, m * inv

    def ln1_piece(r0, dst, p, m=None):
        fixed = isinstance(r0, int)
        if m is not None:
            x_v[zrows(S, 8) if fixed else pl.ds(S, 8), 0:128] = m[0:8, 0:128].astype(bf16)
        xa, xb = [x_v[pl.ds(_mo(r0 + hf * HT1 + p * LN_ROWS, LN_ROWS), LN_ROWS), :]
                  .astype(f32) for hf in range(2)]
        (ia, ma), (ib, mb) = ln1_stats(xa), ln1_stats(xb)
        ya, yb = xa * ia, xb * ib
        s2 = ya[:, :HD] - ma
        s5 = yb[:, HD:] - mb
        s1 = s2 + s5
        s3 = yb[:, :HD] - yb[:, HD:]
        s4 = ya[:, HD:] - ya[:, :HD]
        combos = [s1, s2, s3, s4, s5, s1 + s3, s1 + s4]
        rows = zrows(p * LN_ROWS, LN_ROWS, 16) if fixed else pl.ds(p * LN_ROWS, LN_ROWS)
        for i in range(7):
            for c in range(4):
                dst[i, c, rows, :] = combos[i][:, c * 128:(c + 1) * 128].astype(bf16)
        return token(combos[5], combos[6])

    def fold_piece(kind, c, j, pt):
        blk = {}
        for hh in range(2):
            for kh in range(2):
                k0 = kh * HD + j * 128
                w = wqkv_v[kind * NWC + c, k0:k0 + 128, hh * 128:(hh + 1) * 128]
                blk[hh, kh] = lax.dot_general(pt[2 * c + hh], w, _NT,
                                              preferred_element_type=f32) * LOG2E
        combos = _left_combos(blk[0, 0], blk[0, 1], blk[1, 0], blk[1, 1])
        r0 = kind * HD + c * 128
        for i in range(7):
            wt_v[i, j, r0:r0 + 128, :] = combos[i].astype(bf16)
            we_v[kind, i, j, c * 16:(c + 1) * 16, :] = combos[i][0:16].astype(bf16)

    def fold_chunk(kind, c, pt):
        for j in range(4):
            fold_piece(kind, c, j, pt)

    def vprep_piece(c, j, m):
        wqkv_v[zs + 3 * NWC, 0:8, 0:128] = m[0:8, 0:128].astype(bf16)
        blk = {}
        for hh in range(2):
            for kh in range(2):
                k0 = kh * HD + j * 128
                w = wqkv_v[V_ * NWC + c, k0:k0 + 128, hh * 128:(hh + 1) * 128]
                blk[hh, kh] = w.T.astype(f32)
        combos = _left_combos(blk[0, 0], blk[0, 1], blk[1, 0], blk[1, 1])
        r0 = V_ * HD + c * 128
        for i in range(7):
            wt_v[i, j, r0:r0 + 128, :] = combos[i].astype(bf16)
        return token(combos[1], combos[4])

    def wo_piece(w0, m):
        wo_v[D:D + 8, 0:128] = m[0:8, 0:128].astype(bf16)
        top = wo_v[pl.ds(pl.multiple_of(w0, 16), 16), :].astype(f32)
        bot = wo_v[pl.ds(pl.multiple_of(HD + w0, 16), 16), :].astype(f32)
        combos = _right_combos(top[:, :HD], top[:, HD:], bot[:, :HD], bot[:, HD:])
        for i in range(7):
            for c in range(4):
                wo7_v[i, c, pl.ds(pl.multiple_of(w0, 16), 16), :] = (
                    combos[i][:, c * 128:(c + 1) * 128].astype(bf16))
        return token(combos[5], combos[6])

    def z_piece(j, first, m):
        phik_v[0, zrows(2 * D, 16, 16), :] = m[0:16, 0:128].astype(bf16)
        ph = _unpack(tiles(phik_v, j * 128, 128)).astype(f32)
        part = (ph[:, 0:128] + ph[:, 128:256]) + (ph[:, 256:384] + ph[:, 384:512])
        z = jnp.sum(part.astype(bf16).T.astype(f32).reshape(16, 8, 128), axis=0)
        for sh in (4, 2, 1):
            z = z + pltpu.roll(z, sh, 0)
        if first:
            kv_acc[j, 64:72, :] = z
        else:
            z = kv_acc[j, 64:72, :] + z
            kv_acc[j, 64:72, :] = z
            odd = lax.broadcasted_iota(jnp.int32, (8, 128), 1) % 2
            kvt_v[j, 64:80, :] = jnp.concatenate(
                [jnp.where(odd == hl, z, 0.0) for hl in range(2)], axis=0).astype(bf16)
        return token(z)

    def run_rounds(t0, rounds, post, first):
        count = [0]
        pins = {}

        def run_jobs(m):
            for fn, span in post.get(count[0], ()):
                tok = fn(m)
                if span:
                    pins.setdefault(count[0] + span, []).append(tok())
            count[0] += 1

        for par, kind, cs in rounds:
            r0 = kind * HD + cs[0] * 128
            rows = 128 * len(cs)

            def prod(i):
                if (par, kind) == (1, V_):
                    rhs = sc7_v[i]
                else:
                    rhs = tiles(s_v[par].at[i], 0, HT1)
                if (par, kind, cs[0]) == (1, K_, 0):
                    sc7_v[i, zrows(0, HT1 // 2), :] = rhs
                if len(cs) == NWC:
                    lhs = jnp.concatenate(
                        [wl_v[kind, i]] + [tiles(wt_v.at[i], r0 + c * 128 + 16, 2 * MAIN)
                                           for c in cs], axis=0)
                else:
                    lhs = tiles(wt_v.at[i], r0, rows)
                m = lax.dot_general(_unpack(lhs),
                                    _unpack(_or_into(rhs, pins.get(count[0]))),
                                    _NT, preferred_element_type=f32)
                run_jobs(m)
                return m

            def emit(rh, ch, blk):
                tb = 2 * par + ch
                for n, c in enumerate(cs):
                    for jj in range(2):
                        pair = 4 * c + 2 * rh + jj
                        if kind == V_:
                            p = blk[n * 128 + jj * 64:n * 128 + (jj + 1) * 64]
                        elif len(cs) == NWC:
                            sub = lax.broadcasted_iota(jnp.int32, (8, HT1), 0)
                            ends = [blk[k * 16 + jj * 8:k * 16 + jj * 8 + 8] for k in range(3)]
                            if c < 3:
                                end = ends[c]
                            else:
                                end = jnp.where(
                                    sub < 2, pltpu.roll(ends[0], 2, 0),
                                    jnp.where(sub < 4, pltpu.roll(ends[1], 4, 0),
                                              pltpu.roll(ends[2], 6, 0)))
                            q0 = 48 + (2 * n + jj) * MAIN
                            p = jnp.concatenate(
                                [blk[q0:q0 + MAIN], jnp.where(sub < 6, end, 0.0)], axis=0)
                        else:
                            q0, q1 = n * 128 + 16 + jj * MAIN, n * 128 + jj * 8
                            p = jnp.concatenate([blk[q0:q0 + MAIN], blk[q1:q1 + 8]], axis=0)
                        if kind == K_:
                            phik_v[tb, zrows(pair * 128, 128, 16), :] = _dual_softmax(p)
                        elif kind == Q_:
                            phiq_v[t0 // 2, tb, pair * 128:(pair + 1) * 128, :] = (
                                _dual_softmax(p))
                        else:
                            vt_v[pair // 8][tb, zrows((pair % 8) * 64, 64, 16), :] = (
                                p.astype(bf16))

            _strassen(prod, emit)

        kr = lax.broadcasted_iota(jnp.int32, (64, 128), 0)
        kc = lax.broadcasted_iota(jnp.int32, (64, 128), 1)
        kmask = kr // 32 == kc % 2
        for j in range(NP):
            lhs = tiles(vt_v[j // 8], (j % 8) * 64, 64)
            rhs = tiles(phik_v, j * 128, 128)
            upd = lax.dot_general(_unpack(lhs), _unpack(_or_into(rhs, pins.get(count[0]))), _NT,
                                  preferred_element_type=f32)
            run_jobs(upd)
            if first:
                kv_acc[j, 0:64, :] = upd
            else:
                upd = kv_acc[j, 0:64, :] + upd
                kv_acc[j, 0:64, :] = upd
                kvt_v[j, 0:64, :] = jnp.where(kmask, upd, 0.0).astype(bf16)

    def load_best():
        return best_v[0], besti_v[...], best_v[1], best_v[2]

    def store_best(best):
        best_v[0], besti_v[...], best_v[1], best_v[2] = best

    def build_pt(g0, g1):
        def row_ids(r):
            pair = jnp.where(r < 16, r // 8, jnp.where(r < 16 + MAIN, 0, 1))
            feat = jnp.where(r < 16, MAIN + r % 8, r - 16 - pair * MAIN) // 2
            return pair, feat

        n = g1 - g0
        w2 = wphi_v[4 * g0:4 * g1].reshape(n * 128, DH)
        er = lax.broadcasted_iota(jnp.int32, (128, DH), 0)
        ec = lax.broadcasted_iota(jnp.int32, (128, DH), 1)
        e = (jnp.where(ec == row_ids(er)[1], 1.0, 0.0)
             - jnp.where(ec == DH - 1, 1.0, 0.0)).astype(bf16)
        ptf = lax.dot_general(e, w2, _NT, preferred_element_type=f32)
        pr = lax.broadcasted_iota(jnp.int32, (128, 128), 0)
        pc = lax.broadcasted_iota(jnp.int32, (128, 128), 1)
        keep = pc // 32 == row_ids(pr)[0] * 2 + pr % 2
        return [jnp.where(keep, ptf[:, g * 128:(g + 1) * 128], 0.0).astype(bf16)
                for g in range(n)]

    def compact(kind, i, m):
        we_v[0, 0, 0, zrows(64, 16, 16), :] = m[0:16, 0:128].astype(bf16)
        sub = lax.broadcasted_iota(jnp.int32, (8, HD), 0)
        ends = tiles(we_v.at[kind, i], 0, 64)
        for c in range(NWC - 1):
            wl_v[kind, i, zrows(c * 8, 8), :] = jnp.where(
                sub % 4 == 3, pltpu.roll(ends[24:32], 3 - c, 0), ends[c * 8:(c + 1) * 8])

    hbl_v[...] = jnp.zeros_like(hbl_v)
    hbr_v[...] = jnp.zeros_like(hbr_v)
    store_best((jnp.full((8, 128), -jnp.inf, f32), jnp.zeros((8, 128), jnp.int32),
                jnp.zeros((8, 128), f32), jnp.zeros((8, 128), f32)))
    n_ln = HT1 // LN_ROWS
    x0_copy(0).wait()
    x0_copy(1).wait()
    for p in range(n_ln // 2):
        ln1_piece(0, s_v[0], p)
    full_copy(wr_hbm, wr_v, SEM_WR).wait()
    phi_copy(0).wait()
    x0_copy(2).wait()
    x0_copy(3).wait()
    wr_row = wr_v[...].astype(f32).reshape(1, D)
    wrf_v[...] = jnp.broadcast_to(
        wr_row - jnp.sum(wr_row, axis=-1, keepdims=True) * (1.0 / D), (8, D))
    pt = build_pt(0, 4)
    for p in range(n_ln // 2, n_ln):
        ln1_piece(0, s_v[0], p)
    for part in range(2):
        k0_copy(2 * part).wait()
        k0_copy(2 * part + 1).wait()
        fold_piece(K_, 0, 2 * part, pt)
        fold_piece(K_, 0, 2 * part + 1, pt)

    def add_at(post, slot, fn, span=0):
        half = slot != int(slot)
        post.setdefault(int(slot), []).append(
            (lambda m: fn(m[m.shape[0] // 32 * 16:] if half else m), span))

    post = {}

    def at(slot, fn, span=0):
        add_at(post, slot, fn, span)

    for slot, copies in T0_WAITS:
        for cp in copies:
            if cp == 'phi':
                at(slot, lambda m: phi_copy(1).wait())
            elif cp in ('x1', 'x2', 'x3'):
                at(slot, lambda m, cp=cp: x_copy(int(cp[1])).wait())
            else:
                at(slot, lambda m, cp=cp: w_copy(cp // NWC, cp % NWC).wait())
    for n in range(1, 2 * NWC):
        if n == 2:
            at(T0_FOLD[n], lambda m: pt.extend(build_pt(4, 8)))
        at(T0_FOLD[n], lambda m, n=n: fold_chunk(n // NWC, n % NWC, pt))
    for kind in (K_, Q_):
        for i in range(7):
            at(T0_COMPACT[kind] + i, lambda m, kind=kind, i=i: compact(kind, i, m))
    for c in range(NWC):
        for j in range(4):
            at(T0_VPREP[c][j], lambda m, c=c, j=j: vprep_piece(c, j, m), T0_VSPAN[c])
    for p in range(n_ln):
        at(T0_LN[p], lambda m, p=p: ln1_piece(T1, s_v[1], p, m), T0_LNSPAN[p])
    for p in range(n_ln):
        at(T1_LN[0][p], lambda m, p=p: ln1_piece(2 * T1, s_v[0], p, m), P1_LNSPAN)
        at(T1_LN[1][p], lambda m, p=p: ln1_piece(3 * T1, s_v[1], p, m), P1_LNSPAN)
    for j in range(NP):
        at(T0_Z[j], lambda m, j=j: z_piece(j, True, m), T0_ZSPAN)
    lo, hi = [0, 1], [2, 3]
    run_rounds(0, [(0, kind, [c]) for kind in (K_, Q_) for c in range(NWC)]
               + [(1, K_, lo + hi), (1, Q_, lo + hi)] + [(0, V_, [c]) for c in range(NWC)]
               + [(1, V_, lo), (1, V_, hi)], post, True)
    full_copy(wo_hbm, wo_v.at[pl.ds(0, D), :], SEM_WO).wait()
    for i in range(4, N1):
        x_copy(i).wait()

    def phase1(i, carry):
        post = {}
        nxt = jnp.minimum(i + 1, N2 - 1) * T2
        w0 = jnp.minimum((i - 1) * WO_ROWS, HD - WO_ROWS)
        for par in range(2):
            for p in range(n_ln):
                add_at(post, P1_LN2[par][p],
                       lambda m, p=p, par=par: ln1_piece(nxt + par * T1, s_v[par], p, m),
                       P1_LNSPAN2[par])
        for p in range(WO_ROWS // 16):
            add_at(post, P1_WO[p], lambda m, p=p: wo_piece(w0 + 16 * p, m), P1_WOSPAN)
        for j in range(NP):
            add_at(post, P1_Z[j], lambda m, j=j: z_piece(j, False, m), P1_ZSPAN)
        run_rounds(2 * i, [(par, kind, lo + hi) for kind in (K_, Q_) for par in range(2)]
                   + [(par, V_, cs) for par in range(2) for cs in (lo, hi)], post, False)
        return carry

    lax.fori_loop(1, N1 // 2, phase1, 0)

    for _, dst, rows, slot in ffn_tiled:
        filled = dst.at[:, pl.ds(0, rows), :]
        full_copy(filled, filled, slot).wait()
    full_copy(wg_hbm.at[:, pl.ds(f0, F - f0)], wgv_v, SEM_WGV).wait()
    full_copy(wu_hbm.at[:, pl.ds(f0, F - f0)], wuv_v, SEM_WUV).wait()

    def o_copy(hf):
        return pltpu.make_async_copy(
            out_v.at[pl.ds(hf * HT2, HT2), :], out_hbm.at[0, pl.ds(hf * HT2, HT2), :],
            sem.at[SEM_O])

    def half_stats(hh, c0):
        rows = hh.shape[0]
        parts = [hh[:, c * 128:(c + 1) * 128] for c in range(4)]
        wts = [wrf_v[:, c0 + c * 128:c0 + (c + 1) * 128] for c in range(4)]
        s1 = (parts[0] + parts[1]) + (parts[2] + parts[3])
        sq = [p * p for p in parts]
        s2 = (sq[0] + sq[1]) + (sq[2] + sq[3])
        dw = [(p.reshape(rows // 8, 8, 128) * w[None]).reshape(rows, 128)
              for p, w in zip(parts, wts)]
        s3 = (dw[0] + dw[1]) + (dw[2] + dw[3])
        return s1, s2, s3

    def first_half(hbuf, sbuf, base, p, c0):
        r0 = p * EP_ROWS
        hh = hbuf[c0 // HD][r0:r0 + EP_ROWS, :]
        h_v[pl.ds(pl.multiple_of(base + r0, EP_ROWS), EP_ROWS), c0:c0 + HD] = hh.astype(bf16)
        st = jnp.concatenate(half_stats(hh, c0), axis=1)
        sbuf[zrows(r0, EP_ROWS), :] = st
        return _fold_token(pltpu.bitcast(st, u32), zero_v)

    def finish(hbuf, sbuf, base, p, valid, best, defer=None):
        r0 = p * EP_ROWS
        g0 = pl.multiple_of(base + r0, EP_ROWS)
        hl, hr = [r[r0:r0 + EP_ROWS, :] for r in hbuf]
        if defer is None:
            h_v[pl.ds(g0, EP_ROWS), 0:HD] = hl.astype(bf16)
        if sbuf is None:
            if defer is None:
                h_v[pl.ds(g0, EP_ROWS), HD:D] = hr.astype(bf16)
            st = half_stats(hr, HD)
        else:
            st = sbuf[r0:r0 + EP_ROWS, :]
            st = [st[:, n * 128:(n + 1) * 128] for n in range(3)]
        s1, s2, s3 = [jnp.sum(v + w, axis=-1, keepdims=True)
                      for v, w in zip(half_stats(hl, 0), st)]
        m = s1 * (1.0 / D)
        var = jnp.maximum(s2 * (1.0 / D) - m * m, 0.0)
        inv = lax.rsqrt(var + EPS)
        r = s3 * inv

        def write_out(h):
            o = h * (1.0 + inv) - m * inv
            out_v[pl.ds(g0, EP_ROWS), :] = o.astype(bf16)
            return o

        if defer is None:
            o = write_out(jnp.concatenate([hl, hr], axis=1))
        else:
            defer.append(lambda: write_out(jnp.concatenate(
                [r_[r0:r0 + EP_ROWS, :] for r_ in hbuf], axis=1)))
        bv, bi, bm, bq = best
        sub = lax.broadcasted_iota(jnp.int32, (8, 128), 0)
        for g in range(EP_ROWS // 8):
            rows = slice(g * 8, (g + 1) * 8)
            rg = jnp.broadcast_to(r[rows], (8, 128))
            if valid is not None:
                rg = jnp.where(valid, rg, -jnp.inf)
            better = rg > bv
            bi = jnp.where(better, sub + (g0 + g * 8), bi)
            bv = jnp.where(better, rg, bv)
            bm = jnp.where(better, jnp.broadcast_to(m[rows], (8, 128)), bm)
            bq = jnp.where(better, jnp.broadcast_to(var[rows], (8, 128)), bq)
        best = (bv, bi, bm, bq)
        if defer is not None:
            return best, None
        tok = _fold_token(pltpu.bitcast(jnp.concatenate(
            [o[:, D - 128:], bv, bm, bq], axis=0), u32), zero_v)
        return best, tok

    n_ep = HT2 // EP_ROWS

    def phase2(i, carry):
        ot = []
        for j in range(NP):
            ph = tiles(phiq_v.at[i], j * 128, 128)
            n = jnp.dot(_unpack(kvt_v.bitcast(u32)[j]), _unpack(ph),
                        preferred_element_type=f32)
            r0h = _recip(n[64:72] + 1e-6)
            r1h = _recip(n[72:80] + 1e-6)
            ot.append((n[0:32].reshape(4, 8, T2) * r0h[None]).reshape(32, T2))
            ot.append((n[32:64].reshape(4, 8, T2) * r1h[None]).reshape(32, T2))
        lo = jnp.concatenate(ot[:H // 2], axis=0)
        hi = jnp.concatenate(ot[H // 2:], axis=0)
        lcs = _left_combos(lo[:, :HT2], hi[:, :HT2], lo[:, HT2:], hi[:, HT2:])

        state = {'best': load_best()}
        pins = {}
        jobs = {}
        lts = {}
        ra = pl.multiple_of(i * T2, T2)
        rb = pl.multiple_of(i * T2 + HT2, HT2)
        prev = jnp.maximum(i * T2 - HT2, HT2)

        def add_job(slot, deadline, fn, gates=()):
            jobs.setdefault(slot, []).append((fn, deadline, gates))

        def finish_job(hbuf, sbuf, base, p, valid):
            def fn():
                state['best'], tok = finish(hbuf, sbuf, base, p, valid, state['best'])
                return tok
            return fn

        def lt_job(k):
            def fn():
                lts[k] = lcs[k].astype(bf16).T
                return _fold_token(pltpu.bitcast(lts[k], u32), zero_v)
            return fn

        order = (2, 4, 6, 0, 3, 1, 5)
        lt_job(2)()
        for n in range(1, 7):
            add_job(LT_START[n], min(LT_START[n] + LT_SPAN[n], 4 * n), lt_job(order[n]))
        for p in range(n_ep):
            add_job(FB_START[p], FB_START[p] + FB_SPAN,
                    finish_job(hb_v, None, prev, p, i > 0), hb_v)
            add_job(SA_START[p], SA_START[p] + SA_SPAN,
                    lambda p=p: first_half(ha_v, sa_v, ra, p, HD), ha_v[1:])
            add_job(FA_START[p], FA_START[p] + FA_SPAN[p],
                    finish_job(ha_v, sa_v, ra, p, None), ha_v)

        def xblk(r0, c0):
            return x_v[pl.ds(r0, HT2), c0:c0 + 128].astype(f32)

        for n, k in enumerate(order):
            for c in range(4):
                slot = 4 * n + c
                for fn, deadline, gates in jobs.get(slot, ()):
                    for ref in gates:
                        ref[zrows(HT2, 8), 0:128] = mm[0:8]
                    pins.setdefault(deadline, []).append(fn())
                w = _or_into(wo7_v.bitcast(u32)[k, c, 0:HD // 2, :], pins.get(slot))
                mm = jnp.dot(lts[k], _unpack(w), preferred_element_type=f32)
                c0 = c * 128
                cs = slice(c0, c0 + 128)
                tmp = lambda t: tmp_v[t][:, cs]
                if n == 0:
                    tmp_v[0][zrows(0, HT2), cs] = mm
                elif n == 1:
                    ha_v[1][zrows(0, HT2), cs] = (xblk(ra, HD + c0) + tmp(0)) + mm
                    tmp_v[1][zrows(0, HT2), cs] = xblk(ra, c0) - mm
                elif n == 2:
                    tmp_v[2][zrows(0, HT2), cs] = tmp(1) + mm
                elif n == 3:
                    tmp_v[3][zrows(0, HT2), cs] = tmp(2) + mm
                    tmp_v[4][zrows(0, HT2), cs] = (xblk(rb, HD + c0) + tmp(0)) + mm
                elif n == 4:
                    ha_v[0][zrows(0, HT2), cs] = tmp(3) + mm
                    tmp_v[5][zrows(0, HT2), cs] = xblk(rb, c0) + mm
                elif n == 5:
                    hb_v[0][zrows(0, HT2), cs] = tmp(5) + mm
                    tmp_v[6][zrows(0, HT2), cs] = tmp(4) - mm
                else:
                    hb_v[1][zrows(0, HT2), cs] = tmp(6) + mm
        store_best(state['best'])
        o_copy(2 * i).start()

        @pl.when(i > 0)
        def _():
            o_copy(2 * i - 1).start()

        return carry

    lax.fori_loop(0, N2, phase2, 0)
    best = load_best()
    late = []
    for p in range(n_ep):
        best, _ = finish(hb_v, None, S - HT2, p, None, best, late)

    bv, bi, bm, bq = best
    for sh in (4, 2, 1):
        ov, oi, om, oq = [pltpu.roll(t, sh, 0) for t in (bv, bi, bm, bq)]
        take = jnp.logical_or(ov > bv, jnp.logical_and(ov == bv, oi < bi))
        bv, bi, bm, bq = [jnp.where(take, o_, t)
                          for o_, t in zip((ov, oi, om, oq), (bv, bi, bm, bq))]
    idx = jnp.clip(bi[0, 0], 0, S - 1)
    b0 = pl.multiple_of((idx // 8) * 8, 8)
    t = _rb(_rb(bq) + EPS)
    inv = _recip(_rb(t * lax.rsqrt(t)))
    gate = _sigmoid(bv)
    wide = lambda v: jnp.concatenate([v] * (D // 128), axis=1)
    b1 = pl.multiple_of(jnp.minimum(b0, S - HT2 - 8), 8)
    b2 = pl.multiple_of(jnp.maximum(b0 - (S - HT2), 0), 8)
    hb = jnp.where(wide(bi) < S - HT2, h_v[pl.ds(b1, 8), :].astype(f32),
                   _rb(jnp.concatenate([r_[pl.ds(b2, 8), :] for r_ in hb_v], axis=1)))
    hn = (hb - wide(bm)) * wide(inv)
    xs = hn.astype(bf16)
    rows = lax.broadcasted_iota(jnp.int32, (8, D), 0) + b0

    xm = jnp.where(rows == wide(bi), _rb(hn), 0.0)
    for sh in (4, 2, 1):
        xm = xm + pltpu.roll(xm, sh, 0)
    for t in range(D // 128):
        xcol_v[t // 2][zrows((t % 2) * 128, 128), :] = jnp.concatenate(
            [xm[:, t * 128:(t + 1) * 128]] * 16, axis=0).T

    nblk = F // 256
    nmx = nblk - FFN_VPU_BLOCKS
    act = {}
    acc = {}

    def activate(g, u):
        return (g * _sigmoid(g) * u).astype(bf16)

    parts = D // 8 // FFN_KG

    def vpu_chunk(q):
        blk, part = nmx + q // parts, q % parts
        cur = acc.get(blk)
        for kg in range(part * FFN_KG, (part + 1) * FFN_KG):
            xc = xcol_v[kg // 32][(kg % 32) * 8:(kg % 32 + 1) * 8, :]
            w = jnp.concatenate(
                [r[kg * 8:(kg + 1) * 8, (blk - nmx) * 256:(blk - nmx + 1) * 256].astype(f32)
                 for r in (wgv_v, wuv_v)], axis=1)
            p = w * jnp.concatenate([xc] * 4, axis=1)
            cur = p if cur is None else cur + p
        acc[blk] = cur
        if part == parts - 1:
            for sh in (4, 2, 1):
                cur = cur + pltpu.roll(cur, sh, 0)
            act[blk] = activate(cur[:, :256], cur[:, 256:])
        c = q % 4
        return _fold_token(pltpu.bitcast(cur[:, c * 128:(c + 1) * 128], u32), zero_v)

    nchunk = FFN_VPU_BLOCKS * parts
    starts = [FFN_W0 + (q * (FFN_W1 - FFN_W0)) // (nchunk - 1) for q in range(nchunk)]
    pins = {}
    wave = [0]
    wgw, wuw, wdw = [r.bitcast(u32) for r in (wg_v, wu_v, wd_v)]

    def run_wave(lhs, tls):
        w = jnp.concatenate([_or_into(tls[0], pins.get(wave[0]))] + tls[1:], axis=1)
        out = jnp.dot(lhs, _unpack(w), preferred_element_type=f32)
        for p, fn in enumerate(late):
            if LATE_AT[p] == wave[0]:
                for r_ in hb_v:
                    r_[zrows(HT2, 8), 0:128] = out[:, 0:128]
                fn()
        for q, start in enumerate(starts):
            if start == wave[0]:
                pins.setdefault(wave[0] + FFN_SPAN, []).append(vpu_chunk(q))
        if wave[0] == FFN_LATE:
            o_copy(2 * N2 - 1).start()
            out_v[zrows(S, 16, 16), 0:256] = jnp.zeros((16, 256), bf16)
            pins.setdefault(wave[0] + 4, []).append(
                token(out_v[S:S + 8, 0:128].astype(f32))())
        wave[0] += 1
        return out

    for j in range(nmx):
        gu = None
        for kt in range(D // 128):
            p = run_wave(xs[:, kt * 128:(kt + 1) * 128],
                         [r[2 * j + c, kt * 64:(kt + 1) * 64, :]
                          for r in (wgw, wuw) for c in range(2)])
            gu = p if gu is None else gu + p
        act[j] = activate(gu[:, :256], gu[:, 256:])
    ys = [None, None]
    for j in range(nblk):
        for kt in range(2):
            for hf in range(2):
                r0 = (2 * j + kt) * 64
                p = run_wave(act[j][:, kt * 128:(kt + 1) * 128],
                             [wdw[4 * hf + c, r0:r0 + 64, :] for c in range(4)])
                ys[hf] = p if ys[hf] is None else ys[hf] + p
    y = jnp.concatenate(ys, axis=1)
    cur = out_v[pl.ds(b0, 8), :].astype(f32)
    fix_v[...] = jnp.where(rows == wide(bi), hb + hn + y * wide(gate), cur).astype(bf16)
    full_copy(out_v.at[pl.ds(0, S), :], out_hbm.at[0], SEM_O).wait()
    fix = pltpu.make_async_copy(fix_v, out_hbm.at[0, pl.ds(b0, 8), :], sem.at[SEM_O])
    fix.start()
    fix.wait()


def _kernel(*refs):
    def step(i, carry):
        @pl.when(i == 0)
        def _():
            _body(i, *refs)

        return carry

    lax.fori_loop(0, 2, step, 0)


@jax.jit
def pallas_sequential_preLN__linear_kernel_hedgehog__moe_arch_mod__prompt_kernel(
    A_x: jax.Array,
    A_wqkv: jax.Array,
    A_w_phi: jax.Array,
    A_wo: jax.Array,
    B_x: jax.Array,
    B_w_r: jax.Array,
    B_w_gate: jax.Array,
    B_w_up: jax.Array,
    B_w_down: jax.Array,
):
    any_spec = pl.BlockSpec(memory_space=pl.ANY)
    return pl.pallas_call(
        _kernel,
        out_shape=jax.ShapeDtypeStruct((1, S, D), bf16),
        in_specs=[any_spec] * 8,
        out_specs=any_spec,
        scratch_shapes=[
            pltpu.VMEM((S + 16, D), bf16),
            pltpu.VMEM((3 * NWC + 1, D, WC), bf16),
            pltpu.VMEM((H, DH, DH), bf16),
            pltpu.VMEM((D + 16, D), bf16),
            pltpu.VMEM((D,), bf16),
            pltpu.VMEM((F // 128 - 2 * FFN_VPU_BLOCKS, D + PAD, 128), bf16),
            pltpu.VMEM((F // 128 - 2 * FFN_VPU_BLOCKS, D + PAD, 128), bf16),
            pltpu.VMEM((D // 128, F + PAD, 128), bf16),
            pltpu.VMEM((D, 256 * FFN_VPU_BLOCKS), bf16),
            pltpu.VMEM((D, 256 * FFN_VPU_BLOCKS), bf16),
            pltpu.VMEM((7, 4, 3 * HD + PAD, 128), bf16),
            pltpu.VMEM((2, 7, 4, 64 + PAD, 128), bf16),
            pltpu.VMEM((2, 7, 24, HD), u32),
            pltpu.VMEM((7, 4, HD + PAD, 128), bf16),
            pltpu.VMEM((7, 4, HT1 + PAD, 128), bf16),
            pltpu.VMEM((7, 4, HT1 + PAD, 128), bf16),
            pltpu.VMEM((7, HT1 // 2, HD), u32),
            pltpu.VMEM((N2, 4, 2 * D + PAD, 128), bf16),
            pltpu.VMEM((4, 2 * D + PAD, 128), bf16),
            pltpu.VMEM((4, HD + PAD, 128), bf16),
            pltpu.VMEM((4, HD + PAD, 128), bf16),
            pltpu.VMEM((NP, 72, 128), f32),
            pltpu.VMEM((NP, 80, 128), bf16),
            *[pltpu.VMEM((HT2 + 8, HD), f32) for _ in range(4)],
            pltpu.VMEM((HT2, 384), f32),
            *[pltpu.VMEM((HT2, HD), f32) for _ in range(7)],
            pltpu.VMEM((S, D), bf16),
            pltpu.VMEM((S + 16, D), bf16),
            pltpu.VMEM((8, D), f32),
            pltpu.VMEM((3, 8, 128), f32),
            pltpu.VMEM((8, 128), jnp.int32),
            pltpu.VMEM((8, D), bf16),
            *[pltpu.VMEM((256, 128), f32) for _ in range(4)],
            pltpu.SemaphoreType.DMA((NSEM,)),
        ],
        compiler_params=pltpu.CompilerParams(
            vmem_limit_bytes=110 * 1024 * 1024,
            disable_bounds_checks=True,
            disable_semaphore_checks=True),
    )(A_x, A_wqkv, A_w_phi, A_wo, B_w_r, B_w_gate, B_w_up, B_w_down)
```

```python
import jax
import jax.numpy as jnp
from jax import lax
import jax.experimental.pallas as pl
import jax.experimental.pallas.tpu as pltpu

S = 2048
D = 1024
H = 32
DH = 32
F = 3584
NP = H // 2
T1 = 256
T2 = 512
N1 = S // T1
N2 = S // T2
HT1 = T1 // 2
HT2 = T2 // 2
HD = D // 2
WC = 256
NWC = D // WC
LOG2E = 1.4426950408889634
EPS = 1e-5
PAD = 16
WO_ROWS = 176
LN_ROWS = 16
MAIN = 56
EP_ROWS = 32

T0_FOLD = (0, 4, 11, 18, 25, 33, 39, 46)
T0_WAITS = ((4, (1,)), (11, ('phi', 2)), (18, (3, 4)), (33, ('x1', 5, 6)), (46, (7,)),
            (65, (8, 9, 10, 11, 'x2', 'x3')))
T0_VPREP = ((65, 66, 66.5, 67.5), (68.5, 69, 70, 74), (74, 76, 78, 79), (81, 83, 85, 86))
T0_COMPACT = (47, 55)
T0_VSPAN = (2, 5, 5, 4)
T0_LN = (33, 33, 35, 36, 38, 38, 40, 45)
T0_LNSPAN = (3, 3, 0, 0, 0, 0, 0, 0)
T1_LN = ((102, 103, 104, 105, 106, 107, 108, 109), (89, 91, 93, 95, 97, 99, 100, 101))
P1_LNSPAN = 5
P1_WO = (30, 30, 32, 34, 35, 49, 52, 53, 53, 54, 55)
P1_WOSPAN = 3
P1_LN2 = ((42, 43, 44, 45, 46, 47, 48, 50), (34, 35, 35, 37, 38, 39, 40, 41))
P1_LNSPAN2 = (3, 3)
P1_Z = (28, 30, 31, 33, 36, 38, 40, 42, 43, 44, 46, 47, 48, 51, 52, 53)
P1_ZSPAN = 2
T0_Z = (63, 63.5, 64, 70.5, 75, 79, 84, 90, 90, 94, 96.0, 98, 98.0, 99.5, 100.5, 109.5)
T0_ZSPAN = 0
LT_START = (0, 0, 1, 5, 8, 11, 14)
LT_SPAN = (1, 3, 4, 4, 3, 4, 5)
FB_START = (2, 4, 6, 8, 10, 12, 14, 16)
FB_SPAN = 2
SA_START = (9, 11, 13, 15, 15, 18, 18, 19)
SA_SPAN = 4
FA_START = (20, 21, 22, 23, 24, 25, 26, 27)
FA_SPAN = (3, 6, 2, 4, 2, 4, 2, 2)
FFN_VPU_BLOCKS = 7
FFN_KG = 16
FFN_W0 = 18
FFN_W1 = 107
FFN_SPAN = 4
FFN_LATE = 16
LATE_AT = (1, 2, 3, 4, 4, 5, 7, 8)

_NT = (((1,), (1,)), ((), ()))
f32 = jnp.float32
bf16 = jnp.bfloat16
u32 = jnp.uint32

K_, Q_, V_ = 0, 1, 2
SRC = {K_: 1, Q_: 0, V_: 2}

SEM_W = 0
SEM_X = SEM_W + 3 * NWC
SEM_X0 = SEM_X + N1
SEM_K0 = SEM_X0 + 4
SEM_PHI = SEM_K0 + 4
SEM_WO = SEM_PHI + 2
SEM_WR, SEM_WG, SEM_WU, SEM_WD, SEM_WGV, SEM_WUV, SEM_O = (SEM_WO + 1 + i for i in range(7))
NSEM = SEM_O + 1


def _rb(v):
    return v.astype(bf16).astype(f32)


def _unpack(w):
    return pltpu.bitcast(w, bf16)


def _mo(i, n):
    return i if isinstance(i, int) else pl.multiple_of(i, n)


def _recip(x):
    r = pl.reciprocal(x, approx=True)
    return r * (2.0 - x * r)


def _sigmoid(x):
    return _recip(1.0 + jnp.exp(jnp.minimum(-x, 80.0)))


def _dual_softmax(p):
    t = p.shape[-1]
    p3 = p.reshape(8, 8, t)

    def allred(v, op):
        v = op(v, pltpu.roll(v, 2, 0))
        return op(v, pltpu.roll(v, 4, 0))

    mx = allred(jnp.max(p3, axis=0), jnp.maximum)
    mn = allred(jnp.min(p3, axis=0), jnp.minimum)
    ep = jnp.exp2(p3 - mx[None])
    en = jnp.exp2(mn[None] - p3)
    sp = allred(jnp.sum(ep, axis=0), jnp.add)
    sn = allred(jnp.sum(en, axis=0), jnp.add)
    fp = (ep * _recip(sp)[None]).reshape(64, t)
    fn = (en * _recip(sn)[None]).reshape(64, t)
    return jnp.concatenate([fp, fn], axis=0).astype(bf16)


def _left_combos(a11, a12, a21, a22):
    return [a11 + a22, a21 + a22, a11, a22, a11 + a12, a21 - a11, a12 - a22]


def _right_combos(b11, b12, b21, b22):
    return [b11 + b22, b11, b12 - b22, b21 - b11, b22, b11 + b12, b21 + b22]


def _strassen(prod, emit):
    m3 = prod(2)
    m5 = prod(4)
    emit(0, 1, m3 + m5)
    m7 = prod(6)
    u = m7 - m5
    m1 = prod(0)
    u = u + m1
    w = m1 + m3
    m4 = prod(3)
    emit(0, 0, u + m4)
    m2 = prod(1)
    emit(1, 0, m2 + m4)
    w = w - m2
    m6 = prod(5)
    emit(1, 1, w + m6)


def _or_into(w, toks):
    if not toks:
        return w
    top = w[0:8, 0:128]
    for tk in toks:
        top = top | tk
    if w.shape[1] > 128:
        top = jnp.concatenate([top, w[0:8, 128:]], axis=1)
    return jnp.concatenate([top, w[8:]], axis=0)


def _fold_token(w, zero):
    r, c = w.shape
    acc = None
    for i in range(r // 8):
        for j in range(c // 128):
            blk = w[i * 8:(i + 1) * 8, j * 128:(j + 1) * 128]
            acc = blk if acc is None else acc | blk
    return acc & zero


def _body(zs, x_hbm, wqkv_hbm, wphi_hbm, wo_hbm, wr_hbm, wg_hbm, wu_hbm, wd_hbm, out_hbm,
          x_v, wqkv_v, wphi_v, wo_v, wr_v, wg_v, wu_v, wd_v, wgv_v, wuv_v,
          wt_v, we_v, wl_v, wo7_v, sa7_v, sb7_v, sc7_v, phiq_v, phik_v, vt0_v, vt1_v, kv_acc, kvt_v,
          hal_v, har_v, hbl_v, hbr_v, sa_v, t0_v, t1_v, t2_v, t3_v, t4_v, t5_v, t6_v,
          h_v, out_v, wrf_v, best_v, besti_v, fix_v, xc0_v, xc1_v, xc2_v, xc3_v, sem):
    xcol_v = (xc0_v, xc1_v, xc2_v, xc3_v)
    s_v = (sa7_v, sb7_v)
    vt_v = (vt0_v, vt1_v)
    ha_v = (hal_v, har_v)
    hb_v = (hbl_v, hbr_v)
    tmp_v = (t0_v, t1_v, t2_v, t3_v, t4_v, t5_v, t6_v)

    def x_rows(r0, rows, slot):
        return pltpu.make_async_copy(
            x_hbm.at[0, pl.ds(r0, rows), :], x_v.at[pl.ds(r0, rows), :], sem.at[slot])

    def x_copy(i):
        return x_rows(i * T1, T1, SEM_X + i)

    def x0_copy(q):
        return x_rows((q % 2) * HT1 + (q // 2) * (HT1 // 2), HT1 // 2, SEM_X0 + q)

    def w_copy(kind, c):
        return pltpu.make_async_copy(
            wqkv_hbm.at[:, pl.ds(SRC[kind] * D + c * WC, WC)],
            wqkv_v.at[kind * NWC + c], sem.at[SEM_W + kind * NWC + c])

    def k0_copy(q):
        r0 = (q % 2) * HD + (q // 2) * 256
        return pltpu.make_async_copy(
            wqkv_hbm.at[pl.ds(r0, 256), pl.ds(SRC[K_] * D, WC)],
            wqkv_v.at[K_ * NWC, pl.ds(r0, 256), :], sem.at[SEM_K0 + q])

    def phi_copy(part):
        lo, n = part * (H // 2), H // 2
        return pltpu.make_async_copy(wphi_hbm.at[pl.ds(lo, n)], wphi_v.at[pl.ds(lo, n)],
                                     sem.at[SEM_PHI + part])

    def full_copy(src, dst, slot):
        return pltpu.make_async_copy(src, dst, sem.at[slot])

    x0_copy(0).start()
    x0_copy(1).start()
    full_copy(wr_hbm, wr_v, SEM_WR).start()
    phi_copy(0).start()
    x0_copy(2).start()
    x0_copy(3).start()
    for q in range(4):
        k0_copy(q).start()
    w_copy(K_, 1).start()
    phi_copy(1).start()
    w_copy(K_, 2).start()
    w_copy(K_, 3).start()
    w_copy(Q_, 0).start()
    x_copy(1).start()
    for c in range(1, NWC):
        w_copy(Q_, c).start()
    for c in range(NWC):
        w_copy(V_, c).start()
    x_copy(2).start()
    x_copy(3).start()
    full_copy(wo_hbm, wo_v.at[pl.ds(0, D), :], SEM_WO).start()
    for i in range(4, N1):
        x_copy(i).start()
    f0 = F - 256 * FFN_VPU_BLOCKS
    ffn_tiled = ((wg_hbm, wg_v, D, SEM_WG), (wu_hbm, wu_v, D, SEM_WU), (wd_hbm, wd_v, F, SEM_WD))
    for src, dst, rows, slot in ffn_tiled:
        for c in range(dst.shape[0]):
            full_copy(src.at[:, pl.ds(c * 128, 128)], dst.at[c, pl.ds(0, rows), :], slot).start()
    full_copy(wg_hbm.at[:, pl.ds(f0, F - f0)], wgv_v, SEM_WGV).start()
    full_copy(wu_hbm.at[:, pl.ds(f0, F - f0)], wuv_v, SEM_WUV).start()

    zero_v = jnp.full((8, 128), zs, jnp.int32).astype(u32)

    def zrows(r0, rows, mult=8):
        return pl.ds(pl.multiple_of(zs * mult + r0, mult), rows)

    def tiles(ref, r0, rows):
        w = ref.bitcast(u32)
        return jnp.concatenate(
            [w[c, r0 // 2:(r0 + rows) // 2, :] for c in range(ref.shape[0])], axis=1)

    def token(*vals):
        return lambda: _fold_token(pltpu.bitcast(jnp.concatenate(vals, axis=0), u32), zero_v)

    def ln1_stats(xf):
        m = jnp.sum(xf, axis=-1, keepdims=True) * (1.0 / D)
        q = jnp.sum(xf * xf, axis=-1, keepdims=True) * (1.0 / D)
        inv = lax.rsqrt(jnp.maximum(q - m * m, 0.0) + EPS) * LOG2E
        return inv, m * inv

    def ln1_piece(r0, dst, p, m=None):
        fixed = isinstance(r0, int)
        if m is not None:
            x_v[zrows(S, 8) if fixed else pl.ds(S, 8), 0:128] = m[0:8, 0:128].astype(bf16)
        xa, xb = [x_v[pl.ds(_mo(r0 + hf * HT1 + p * LN_ROWS, LN_ROWS), LN_ROWS), :]
                  .astype(f32) for hf in range(2)]
        (ia, ma), (ib, mb) = ln1_stats(xa), ln1_stats(xb)
        ya, yb = xa * ia, xb * ib
        s2 = ya[:, :HD] - ma
        s5 = yb[:, HD:] - mb
        s1 = s2 + s5
        s3 = yb[:, :HD] - yb[:, HD:]
        s4 = ya[:, HD:] - ya[:, :HD]
        combos = [s1, s2, s3, s4, s5, s1 + s3, s1 + s4]
        rows = zrows(p * LN_ROWS, LN_ROWS, 16) if fixed else pl.ds(p * LN_ROWS, LN_ROWS)
        for i in range(7):
            for c in range(4):
                dst[i, c, rows, :] = combos[i][:, c * 128:(c + 1) * 128].astype(bf16)
        return token(combos[5], combos[6])

    def fold_piece(kind, c, j, pt):
        sub = lax.broadcasted_iota(jnp.int32, (8, 128), 0)
        blk = {}
        for hh in range(2):
            for kh in range(2):
                k0 = kh * HD + j * 128
                w = wqkv_v[kind * NWC + c, k0:k0 + 128, hh * 128:(hh + 1) * 128]
                f = lax.dot_general(pt[2 * c + hh], w, _NT, preferred_element_type=f32)
                refs = []
                for pp in range(2):
                    ref = jnp.where(sub >= 6, f[pp * 8:(pp + 1) * 8], 0.0)
                    ref = ref + pltpu.roll(ref, 2, 0)
                    refs.append(ref + pltpu.roll(ref, 4, 0))
                blk[hh, kh] = f - jnp.concatenate(refs + [refs[0]] * 7 + [refs[1]] * 7, axis=0)
        combos = _left_combos(blk[0, 0], blk[0, 1], blk[1, 0], blk[1, 1])
        r0 = kind * HD + c * 128
        for i in range(7):
            wt_v[i, j, r0:r0 + 128, :] = combos[i].astype(bf16)
            we_v[kind, i, j, c * 16:(c + 1) * 16, :] = combos[i][0:16].astype(bf16)

    def fold_chunk(kind, c, pt):
        for j in range(4):
            fold_piece(kind, c, j, pt)

    def vprep_piece(c, j, m):
        wqkv_v[zs + 3 * NWC, 0:8, 0:128] = m[0:8, 0:128].astype(bf16)
        blk = {}
        for hh in range(2):
            for kh in range(2):
                k0 = kh * HD + j * 128
                w = wqkv_v[V_ * NWC + c, k0:k0 + 128, hh * 128:(hh + 1) * 128]
                blk[hh, kh] = w.T.astype(f32)
        combos = _left_combos(blk[0, 0], blk[0, 1], blk[1, 0], blk[1, 1])
        r0 = V_ * HD + c * 128
        for i in range(7):
            wt_v[i, j, r0:r0 + 128, :] = combos[i].astype(bf16)
        return token(combos[1], combos[4])

    def wo_piece(w0, m):
        wo_v[D:D + 8, 0:128] = m[0:8, 0:128].astype(bf16)
        top = wo_v[pl.ds(pl.multiple_of(w0, 16), 16), :].astype(f32)
        bot = wo_v[pl.ds(pl.multiple_of(HD + w0, 16), 16), :].astype(f32)
        combos = _right_combos(top[:, :HD], top[:, HD:], bot[:, :HD], bot[:, HD:])
        for i in range(7):
            for c in range(4):
                wo7_v[i, c, pl.ds(pl.multiple_of(w0, 16), 16), :] = (
                    combos[i][:, c * 128:(c + 1) * 128].astype(bf16))
        return token(combos[5], combos[6])

    def z_piece(j, first, m):
        phik_v[0, zrows(2 * D, 16, 16), :] = m[0:16, 0:128].astype(bf16)
        ph = _unpack(tiles(phik_v, j * 128, 128)).astype(f32)
        part = (ph[:, 0:128] + ph[:, 128:256]) + (ph[:, 256:384] + ph[:, 384:512])
        z = jnp.sum(part.astype(bf16).T.astype(f32).reshape(16, 8, 128), axis=0)
        for sh in (4, 2, 1):
            z = z + pltpu.roll(z, sh, 0)
        if first:
            kv_acc[j, 64:72, :] = z
        else:
            z = kv_acc[j, 64:72, :] + z
            kv_acc[j, 64:72, :] = z
            odd = lax.broadcasted_iota(jnp.int32, (8, 128), 1) % 2
            kvt_v[j, 64:80, :] = jnp.concatenate(
                [jnp.where(odd == hl, z, 0.0) for hl in range(2)], axis=0).astype(bf16)
        return token(z)

    def run_rounds(t0, rounds, post, first):
        count = [0]
        pins = {}

        def run_jobs(m):
            for fn, span in post.get(count[0], ()):
                tok = fn(m)
                if span:
                    pins.setdefault(count[0] + span, []).append(tok())
            count[0] += 1

        for par, kind, cs in rounds:
            r0 = kind * HD + cs[0] * 128
            rows = 128 * len(cs)

            def prod(i):
                if (par, kind) == (1, V_):
                    rhs = sc7_v[i]
                else:
                    rhs = tiles(s_v[par].at[i], 0, HT1)
                if (par, kind, cs[0]) == (1, K_, 0):
                    sc7_v[i, zrows(0, HT1 // 2), :] = rhs
                if len(cs) == NWC:
                    lhs = jnp.concatenate(
                        [wl_v[kind, i]] + [tiles(wt_v.at[i], r0 + c * 128 + 16, 2 * MAIN)
                                           for c in cs], axis=0)
                else:
                    lhs = tiles(wt_v.at[i], r0, rows)
                m = lax.dot_general(_unpack(lhs),
                                    _unpack(_or_into(rhs, pins.get(count[0]))),
                                    _NT, preferred_element_type=f32)
                run_jobs(m)
                return m

            def emit(rh, ch, blk):
                tb = 2 * par + ch
                for n, c in enumerate(cs):
                    for jj in range(2):
                        pair = 4 * c + 2 * rh + jj
                        if kind == V_:
                            p = blk[n * 128 + jj * 64:n * 128 + (jj + 1) * 64]
                        elif len(cs) == NWC:
                            sub = lax.broadcasted_iota(jnp.int32, (8, HT1), 0)
                            ends = [blk[k * 16 + jj * 8:k * 16 + jj * 8 + 8] for k in range(3)]
                            if c < 3:
                                end = ends[c]
                            else:
                                end = jnp.where(
                                    sub < 2, pltpu.roll(ends[0], 2, 0),
                                    jnp.where(sub < 4, pltpu.roll(ends[1], 4, 0),
                                              pltpu.roll(ends[2], 6, 0)))
                            q0 = 48 + (2 * n + jj) * MAIN
                            p = jnp.concatenate(
                                [blk[q0:q0 + MAIN], jnp.where(sub < 6, end, 0.0)], axis=0)
                        else:
                            q0, q1 = n * 128 + 16 + jj * MAIN, n * 128 + jj * 8
                            p = jnp.concatenate([blk[q0:q0 + MAIN], blk[q1:q1 + 8]], axis=0)
                        if kind == K_:
                            phik_v[tb, zrows(pair * 128, 128, 16), :] = _dual_softmax(p)
                        elif kind == Q_:
                            phiq_v[t0 // 2, tb, pair * 128:(pair + 1) * 128, :] = (
                                _dual_softmax(p))
                        else:
                            vt_v[pair // 8][tb, zrows((pair % 8) * 64, 64, 16), :] = (
                                p.astype(bf16))

            _strassen(prod, emit)

        kr = lax.broadcasted_iota(jnp.int32, (64, 128), 0)
        kc = lax.broadcasted_iota(jnp.int32, (64, 128), 1)
        kmask = kr // 32 == kc % 2
        for j in range(NP):
            lhs = tiles(vt_v[j // 8], (j % 8) * 64, 64)
            rhs = tiles(phik_v, j * 128, 128)
            upd = lax.dot_general(_unpack(lhs), _unpack(_or_into(rhs, pins.get(count[0]))), _NT,
                                  preferred_element_type=f32)
            run_jobs(upd)
            if first:
                kv_acc[j, 0:64, :] = upd
            else:
                upd = kv_acc[j, 0:64, :] + upd
                kv_acc[j, 0:64, :] = upd
                kvt_v[j, 0:64, :] = jnp.where(kmask, upd * (1.0 / LOG2E), 0.0).astype(bf16)

    def load_best():
        return best_v[0], besti_v[...], best_v[1], best_v[2]

    def store_best(best):
        best_v[0], besti_v[...], best_v[1], best_v[2] = best

    def build_pt(g0, g1):
        def row_ids(r):
            pair = jnp.where(r < 16, r // 8, jnp.where(r < 16 + MAIN, 0, 1))
            feat = jnp.where(r < 16, MAIN + r % 8, r - 16 - pair * MAIN) // 2
            return pair, feat

        n = g1 - g0
        w2 = wphi_v[4 * g0:4 * g1].reshape(n * 128, DH)
        er = lax.broadcasted_iota(jnp.int32, (128, DH), 0)
        ec = lax.broadcasted_iota(jnp.int32, (128, DH), 1)
        e = jnp.where(ec == row_ids(er)[1], 1.0, 0.0).astype(bf16)
        ptf = lax.dot_general(e, w2, _NT, preferred_element_type=f32)
        pr = lax.broadcasted_iota(jnp.int32, (128, 128), 0)
        pc = lax.broadcasted_iota(jnp.int32, (128, 128), 1)
        keep = pc // 32 == row_ids(pr)[0] * 2 + pr % 2
        return [jnp.where(keep, ptf[:, g * 128:(g + 1) * 128], 0.0).astype(bf16)
                for g in range(n)]

    def compact(kind, i, m):
        we_v[0, 0, 0, zrows(64, 16, 16), :] = m[0:16, 0:128].astype(bf16)
        sub = lax.broadcasted_iota(jnp.int32, (8, HD), 0)
        ends = tiles(we_v.at[kind, i], 0, 64)
        for c in range(NWC - 1):
            wl_v[kind, i, zrows(c * 8, 8), :] = jnp.where(
                sub % 4 == 3, pltpu.roll(ends[24:32], 3 - c, 0), ends[c * 8:(c + 1) * 8])

    hbl_v[...] = jnp.zeros_like(hbl_v)
    hbr_v[...] = jnp.zeros_like(hbr_v)
    store_best((jnp.full((8, 128), -jnp.inf, f32), jnp.zeros((8, 128), jnp.int32),
                jnp.zeros((8, 128), f32), jnp.zeros((8, 128), f32)))
    n_ln = HT1 // LN_ROWS
    x0_copy(0).wait()
    x0_copy(1).wait()
    for p in range(n_ln // 2):
        ln1_piece(0, s_v[0], p)
    full_copy(wr_hbm, wr_v, SEM_WR).wait()
    phi_copy(0).wait()
    x0_copy(2).wait()
    x0_copy(3).wait()
    wr_row = wr_v[...].astype(f32).reshape(1, D)
    wrf_v[...] = jnp.broadcast_to(
        wr_row - jnp.sum(wr_row, axis=-1, keepdims=True) * (1.0 / D), (8, D))
    pt = build_pt(0, 4)
    for p in range(n_ln // 2, n_ln):
        ln1_piece(0, s_v[0], p)
    for part in range(2):
        k0_copy(2 * part).wait()
        k0_copy(2 * part + 1).wait()
        fold_piece(K_, 0, 2 * part, pt)
        fold_piece(K_, 0, 2 * part + 1, pt)

    def add_at(post, slot, fn, span=0):
        half = slot != int(slot)
        post.setdefault(int(slot), []).append(
            (lambda m: fn(m[m.shape[0] // 32 * 16:] if half else m), span))

    post = {}

    def at(slot, fn, span=0):
        add_at(post, slot, fn, span)

    for slot, copies in T0_WAITS:
        for cp in copies:
            if cp == 'phi':
                at(slot, lambda m: phi_copy(1).wait())
            elif cp in ('x1', 'x2', 'x3'):
                at(slot, lambda m, cp=cp: x_copy(int(cp[1])).wait())
            else:
                at(slot, lambda m, cp=cp: w_copy(cp // NWC, cp % NWC).wait())
    for n in range(1, 2 * NWC):
        if n == 2:
            at(T0_FOLD[n], lambda m: pt.extend(build_pt(4, 8)))
        at(T0_FOLD[n], lambda m, n=n: fold_chunk(n // NWC, n % NWC, pt))
    for kind in (K_, Q_):
        for i in range(7):
            at(T0_COMPACT[kind] + i, lambda m, kind=kind, i=i: compact(kind, i, m))
    for c in range(NWC):
        for j in range(4):
            at(T0_VPREP[c][j], lambda m, c=c, j=j: vprep_piece(c, j, m), T0_VSPAN[c])
    for p in range(n_ln):
        at(T0_LN[p], lambda m, p=p: ln1_piece(T1, s_v[1], p, m), T0_LNSPAN[p])
    for p in range(n_ln):
        at(T1_LN[0][p], lambda m, p=p: ln1_piece(2 * T1, s_v[0], p, m), P1_LNSPAN)
        at(T1_LN[1][p], lambda m, p=p: ln1_piece(3 * T1, s_v[1], p, m), P1_LNSPAN)
    for j in range(NP):
        at(T0_Z[j], lambda m, j=j: z_piece(j, True, m), T0_ZSPAN)
    lo, hi = [0, 1], [2, 3]
    run_rounds(0, [(0, kind, [c]) for kind in (K_, Q_) for c in range(NWC)]
               + [(1, K_, lo + hi), (1, Q_, lo + hi)] + [(0, V_, [c]) for c in range(NWC)]
               + [(1, V_, lo), (1, V_, hi)], post, True)
    full_copy(wo_hbm, wo_v.at[pl.ds(0, D), :], SEM_WO).wait()
    for i in range(4, N1):
        x_copy(i).wait()

    def phase1(i, carry):
        post = {}
        nxt = jnp.minimum(i + 1, N2 - 1) * T2
        w0 = jnp.minimum((i - 1) * WO_ROWS, HD - WO_ROWS)
        for par in range(2):
            for p in range(n_ln):
                add_at(post, P1_LN2[par][p],
                       lambda m, p=p, par=par: ln1_piece(nxt + par * T1, s_v[par], p, m),
                       P1_LNSPAN2[par])
        for p in range(WO_ROWS // 16):
            add_at(post, P1_WO[p], lambda m, p=p: wo_piece(w0 + 16 * p, m), P1_WOSPAN)
        for j in range(NP):
            add_at(post, P1_Z[j], lambda m, j=j: z_piece(j, False, m), P1_ZSPAN)
        run_rounds(2 * i, [(par, kind, lo + hi) for kind in (K_, Q_) for par in range(2)]
                   + [(par, V_, cs) for par in range(2) for cs in (lo, hi)], post, False)
        return carry

    lax.fori_loop(1, N1 // 2, phase1, 0)

    for _, dst, rows, slot in ffn_tiled:
        filled = dst.at[:, pl.ds(0, rows), :]
        full_copy(filled, filled, slot).wait()
    full_copy(wg_hbm.at[:, pl.ds(f0, F - f0)], wgv_v, SEM_WGV).wait()
    full_copy(wu_hbm.at[:, pl.ds(f0, F - f0)], wuv_v, SEM_WUV).wait()

    def o_copy(hf):
        return pltpu.make_async_copy(
            out_v.at[pl.ds(hf * HT2, HT2), :], out_hbm.at[0, pl.ds(hf * HT2, HT2), :],
            sem.at[SEM_O])

    def half_stats(hh, c0):
        rows = hh.shape[0]
        parts = [hh[:, c * 128:(c + 1) * 128] for c in range(4)]
        wts = [wrf_v[:, c0 + c * 128:c0 + (c + 1) * 128] for c in range(4)]
        s1 = (parts[0] + parts[1]) + (parts[2] + parts[3])
        sq = [p * p for p in parts]
        s2 = (sq[0] + sq[1]) + (sq[2] + sq[3])
        dw = [(p.reshape(rows // 8, 8, 128) * w[None]).reshape(rows, 128)
              for p, w in zip(parts, wts)]
        s3 = (dw[0] + dw[1]) + (dw[2] + dw[3])
        return s1, s2, s3

    def first_half(hbuf, sbuf, base, p, c0):
        r0 = p * EP_ROWS
        hh = hbuf[c0 // HD][r0:r0 + EP_ROWS, :]
        h_v[pl.ds(pl.multiple_of(base + r0, EP_ROWS), EP_ROWS), c0:c0 + HD] = hh.astype(bf16)
        st = jnp.concatenate(half_stats(hh, c0), axis=1)
        sbuf[zrows(r0, EP_ROWS), :] = st
        return _fold_token(pltpu.bitcast(st, u32), zero_v)

    def finish(hbuf, sbuf, base, p, valid, best, defer=None):
        r0 = p * EP_ROWS
        g0 = pl.multiple_of(base + r0, EP_ROWS)
        hl, hr = [r[r0:r0 + EP_ROWS, :] for r in hbuf]
        if defer is None:
            h_v[pl.ds(g0, EP_ROWS), 0:HD] = hl.astype(bf16)
        if sbuf is None:
            if defer is None:
                h_v[pl.ds(g0, EP_ROWS), HD:D] = hr.astype(bf16)
            st = half_stats(hr, HD)
        else:
            st = sbuf[r0:r0 + EP_ROWS, :]
            st = [st[:, n * 128:(n + 1) * 128] for n in range(3)]
        s1, s2, s3 = [jnp.sum(v + w, axis=-1, keepdims=True)
                      for v, w in zip(half_stats(hl, 0), st)]
        m = s1 * (1.0 / D)
        var = jnp.maximum(s2 * (1.0 / D) - m * m, 0.0)
        inv = lax.rsqrt(var + EPS)
        r = s3 * inv

        def write_out(h):
            o = h * (1.0 + inv) - m * inv
            out_v[pl.ds(g0, EP_ROWS), :] = o.astype(bf16)
            return o

        if defer is None:
            o = write_out(jnp.concatenate([hl, hr], axis=1))
        else:
            defer.append(lambda: write_out(jnp.concatenate(
                [r_[r0:r0 + EP_ROWS, :] for r_ in hbuf], axis=1)))
        bv, bi, bm, bq = best
        sub = lax.broadcasted_iota(jnp.int32, (8, 128), 0)
        for g in range(EP_ROWS // 8):
            rows = slice(g * 8, (g + 1) * 8)
            rg = jnp.broadcast_to(r[rows], (8, 128))
            if valid is not None:
                rg = jnp.where(valid, rg, -jnp.inf)
            better = rg > bv
            bi = jnp.where(better, sub + (g0 + g * 8), bi)
            bv = jnp.where(better, rg, bv)
            bm = jnp.where(better, jnp.broadcast_to(m[rows], (8, 128)), bm)
            bq = jnp.where(better, jnp.broadcast_to(var[rows], (8, 128)), bq)
        best = (bv, bi, bm, bq)
        if defer is not None:
            return best, None
        tok = _fold_token(pltpu.bitcast(jnp.concatenate(
            [o[:, D - 128:], bv, bm, bq], axis=0), u32), zero_v)
        return best, tok

    n_ep = HT2 // EP_ROWS

    def phase2(i, carry):
        ot = []
        for j in range(NP):
            ph = tiles(phiq_v.at[i], j * 128, 128)
            n = jnp.dot(_unpack(kvt_v.bitcast(u32)[j]), _unpack(ph),
                        preferred_element_type=f32)
            r0h = _recip(n[64:72] + 1e-6)
            r1h = _recip(n[72:80] + 1e-6)
            ot.append((n[0:32].reshape(4, 8, T2) * r0h[None]).reshape(32, T2))
            ot.append((n[32:64].reshape(4, 8, T2) * r1h[None]).reshape(32, T2))
        lo = jnp.concatenate(ot[:H // 2], axis=0)
        hi = jnp.concatenate(ot[H // 2:], axis=0)
        lcs = _left_combos(lo[:, :HT2], hi[:, :HT2], lo[:, HT2:], hi[:, HT2:])

        state = {'best': load_best()}
        pins = {}
        jobs = {}
        lts = {}
        ra = pl.multiple_of(i * T2, T2)
        rb = pl.multiple_of(i * T2 + HT2, HT2)
        prev = jnp.maximum(i * T2 - HT2, HT2)

        def add_job(slot, deadline, fn, gates=()):
            jobs.setdefault(slot, []).append((fn, deadline, gates))

        def finish_job(hbuf, sbuf, base, p, valid):
            def fn():
                state['best'], tok = finish(hbuf, sbuf, base, p, valid, state['best'])
                return tok
            return fn

        def lt_job(k):
            def fn():
                lts[k] = lcs[k].astype(bf16).T
                return _fold_token(pltpu.bitcast(lts[k], u32), zero_v)
            return fn

        order = (2, 4, 6, 0, 3, 1, 5)
        lt_job(2)()
        for n in range(1, 7):
            add_job(LT_START[n], min(LT_START[n] + LT_SPAN[n], 4 * n), lt_job(order[n]))
        for p in range(n_ep):
            add_job(FB_START[p], FB_START[p] + FB_SPAN,
                    finish_job(hb_v, None, prev, p, i > 0), hb_v)
            add_job(SA_START[p], SA_START[p] + SA_SPAN,
                    lambda p=p: first_half(ha_v, sa_v, ra, p, HD), ha_v[1:])
            add_job(FA_START[p], FA_START[p] + FA_SPAN[p],
                    finish_job(ha_v, sa_v, ra, p, None), ha_v)

        def xblk(r0, c0):
            return x_v[pl.ds(r0, HT2), c0:c0 + 128].astype(f32)

        for n, k in enumerate(order):
            for c in range(4):
                slot = 4 * n + c
                for fn, deadline, gates in jobs.get(slot, ()):
                    for ref in gates:
                        ref[zrows(HT2, 8), 0:128] = mm[0:8]
                    pins.setdefault(deadline, []).append(fn())
                w = _or_into(wo7_v.bitcast(u32)[k, c, 0:HD // 2, :], pins.get(slot))
                mm = jnp.dot(lts[k], _unpack(w), preferred_element_type=f32)
                c0 = c * 128
                cs = slice(c0, c0 + 128)
                tmp = lambda t: tmp_v[t][:, cs]
                if n == 0:
                    tmp_v[0][zrows(0, HT2), cs] = mm
                elif n == 1:
                    ha_v[1][zrows(0, HT2), cs] = (xblk(ra, HD + c0) + tmp(0)) + mm
                    tmp_v[1][zrows(0, HT2), cs] = xblk(ra, c0) - mm
                elif n == 2:
                    tmp_v[2][zrows(0, HT2), cs] = tmp(1) + mm
                elif n == 3:
                    tmp_v[3][zrows(0, HT2), cs] = tmp(2) + mm
                    tmp_v[4][zrows(0, HT2), cs] = (xblk(rb, HD + c0) + tmp(0)) + mm
                elif n == 4:
                    ha_v[0][zrows(0, HT2), cs] = tmp(3) + mm
                    tmp_v[5][zrows(0, HT2), cs] = xblk(rb, c0) + mm
                elif n == 5:
                    hb_v[0][zrows(0, HT2), cs] = tmp(5) + mm
                    tmp_v[6][zrows(0, HT2), cs] = tmp(4) - mm
                else:
                    hb_v[1][zrows(0, HT2), cs] = tmp(6) + mm
        store_best(state['best'])
        o_copy(2 * i).start()

        @pl.when(i > 0)
        def _():
            o_copy(2 * i - 1).start()

        return carry

    lax.fori_loop(0, N2, phase2, 0)
    best = load_best()
    late = []
    for p in range(n_ep):
        best, _ = finish(hb_v, None, S - HT2, p, None, best, late)

    bv, bi, bm, bq = best
    for sh in (4, 2, 1):
        ov, oi, om, oq = [pltpu.roll(t, sh, 0) for t in (bv, bi, bm, bq)]
        take = jnp.logical_or(ov > bv, jnp.logical_and(ov == bv, oi < bi))
        bv, bi, bm, bq = [jnp.where(take, o_, t)
                          for o_, t in zip((ov, oi, om, oq), (bv, bi, bm, bq))]
    idx = jnp.clip(bi[0, 0], 0, S - 1)
    b0 = pl.multiple_of((idx // 8) * 8, 8)
    t = _rb(_rb(bq) + EPS)
    inv = _recip(_rb(t * lax.rsqrt(t)))
    gate = _sigmoid(bv)
    wide = lambda v: jnp.concatenate([v] * (D // 128), axis=1)
    b1 = pl.multiple_of(jnp.minimum(b0, S - HT2 - 8), 8)
    b2 = pl.multiple_of(jnp.maximum(b0 - (S - HT2), 0), 8)
    hb = jnp.where(wide(bi) < S - HT2, h_v[pl.ds(b1, 8), :].astype(f32),
                   _rb(jnp.concatenate([r_[pl.ds(b2, 8), :] for r_ in hb_v], axis=1)))
    hn = (hb - wide(bm)) * wide(inv)
    xs = hn.astype(bf16)
    rows = lax.broadcasted_iota(jnp.int32, (8, D), 0) + b0

    xm = jnp.where(rows == wide(bi), _rb(hn), 0.0)
    for sh in (4, 2, 1):
        xm = xm + pltpu.roll(xm, sh, 0)
    for t in range(D // 128):
        xcol_v[t // 2][zrows((t % 2) * 128, 128), :] = jnp.concatenate(
            [xm[:, t * 128:(t + 1) * 128]] * 16, axis=0).T

    nblk = F // 256
    nmx = nblk - FFN_VPU_BLOCKS
    act = {}
    acc = {}

    def activate(g, u):
        return (g * _sigmoid(g) * u).astype(bf16)

    parts = D // 8 // FFN_KG

    def vpu_chunk(q):
        blk, part = nmx + q // parts, q % parts
        cur = acc.get(blk)
        for kg in range(part * FFN_KG, (part + 1) * FFN_KG):
            xc = xcol_v[kg // 32][(kg % 32) * 8:(kg % 32 + 1) * 8, :]
            w = jnp.concatenate(
                [r[kg * 8:(kg + 1) * 8, (blk - nmx) * 256:(blk - nmx + 1) * 256].astype(f32)
                 for r in (wgv_v, wuv_v)], axis=1)
            p = w * jnp.concatenate([xc] * 4, axis=1)
            cur = p if cur is None else cur + p
        acc[blk] = cur
        if part == parts - 1:
            for sh in (4, 2, 1):
                cur = cur + pltpu.roll(cur, sh, 0)
            act[blk] = activate(cur[:, :256], cur[:, 256:])
        c = q % 4
        return _fold_token(pltpu.bitcast(cur[:, c * 128:(c + 1) * 128], u32), zero_v)

    nchunk = FFN_VPU_BLOCKS * parts
    starts = [FFN_W0 + (q * (FFN_W1 - FFN_W0)) // (nchunk - 1) for q in range(nchunk)]
    pins = {}
    wave = [0]
    wgw, wuw, wdw = [r.bitcast(u32) for r in (wg_v, wu_v, wd_v)]

    def run_wave(lhs, tls):
        w = jnp.concatenate([_or_into(tls[0], pins.get(wave[0]))] + tls[1:], axis=1)
        out = jnp.dot(lhs, _unpack(w), preferred_element_type=f32)
        for p, fn in enumerate(late):
            if LATE_AT[p] == wave[0]:
                for r_ in hb_v:
                    r_[zrows(HT2, 8), 0:128] = out[:, 0:128]
                fn()
        for q, start in enumerate(starts):
            if start == wave[0]:
                pins.setdefault(wave[0] + FFN_SPAN, []).append(vpu_chunk(q))
        if wave[0] == FFN_LATE:
            o_copy(2 * N2 - 1).start()
            out_v[zrows(S, 16, 16), 0:256] = jnp.zeros((16, 256), bf16)
            pins.setdefault(wave[0] + 4, []).append(
                token(out_v[S:S + 8, 0:128].astype(f32))())
        wave[0] += 1
        return out

    for j in range(nmx):
        gu = None
        for kt in range(D // 128):
            p = run_wave(xs[:, kt * 128:(kt + 1) * 128],
                         [r[2 * j + c, kt * 64:(kt + 1) * 64, :]
                          for r in (wgw, wuw) for c in range(2)])
            gu = p if gu is None else gu + p
        act[j] = activate(gu[:, :256], gu[:, 256:])
    ys = [None, None]
    for j in range(nblk):
        for kt in range(2):
            for hf in range(2):
                r0 = (2 * j + kt) * 64
                p = run_wave(act[j][:, kt * 128:(kt + 1) * 128],
                             [wdw[4 * hf + c, r0:r0 + 64, :] for c in range(4)])
                ys[hf] = p if ys[hf] is None else ys[hf] + p
    y = jnp.concatenate(ys, axis=1)
    cur = out_v[pl.ds(b0, 8), :].astype(f32)
    fix_v[...] = jnp.where(rows == wide(bi), hb + hn + y * wide(gate), cur).astype(bf16)
    full_copy(out_v.at[pl.ds(0, S), :], out_hbm.at[0], SEM_O).wait()
    fix = pltpu.make_async_copy(fix_v, out_hbm.at[0, pl.ds(b0, 8), :], sem.at[SEM_O])
    fix.start()
    fix.wait()


def _kernel(*refs):
    def step(i, carry):
        @pl.when(i == 0)
        def _():
            _body(i, *refs)

        return carry

    lax.fori_loop(0, 2, step, 0)


@jax.jit
def pallas_sequential_preLN__linear_kernel_hedgehog__moe_arch_mod__prompt_kernel(
    A_x: jax.Array,
    A_wqkv: jax.Array,
    A_w_phi: jax.Array,
    A_wo: jax.Array,
    B_x: jax.Array,
    B_w_r: jax.Array,
    B_w_gate: jax.Array,
    B_w_up: jax.Array,
    B_w_down: jax.Array,
):
    any_spec = pl.BlockSpec(memory_space=pl.ANY)
    return pl.pallas_call(
        _kernel,
        out_shape=jax.ShapeDtypeStruct((1, S, D), bf16),
        in_specs=[any_spec] * 8,
        out_specs=any_spec,
        scratch_shapes=[
            pltpu.VMEM((S + 16, D), bf16),
            pltpu.VMEM((3 * NWC + 1, D, WC), bf16),
            pltpu.VMEM((H, DH, DH), bf16),
            pltpu.VMEM((D + 16, D), bf16),
            pltpu.VMEM((D,), bf16),
            pltpu.VMEM((F // 128 - 2 * FFN_VPU_BLOCKS, D + PAD, 128), bf16),
            pltpu.VMEM((F // 128 - 2 * FFN_VPU_BLOCKS, D + PAD, 128), bf16),
            pltpu.VMEM((D // 128, F + PAD, 128), bf16),
            pltpu.VMEM((D, 256 * FFN_VPU_BLOCKS), bf16),
            pltpu.VMEM((D, 256 * FFN_VPU_BLOCKS), bf16),
            pltpu.VMEM((7, 4, 3 * HD + PAD, 128), bf16),
            pltpu.VMEM((2, 7, 4, 64 + PAD, 128), bf16),
            pltpu.VMEM((2, 7, 24, HD), u32),
            pltpu.VMEM((7, 4, HD + PAD, 128), bf16),
            pltpu.VMEM((7, 4, HT1 + PAD, 128), bf16),
            pltpu.VMEM((7, 4, HT1 + PAD, 128), bf16),
            pltpu.VMEM((7, HT1 // 2, HD), u32),
            pltpu.VMEM((N2, 4, 2 * D + PAD, 128), bf16),
            pltpu.VMEM((4, 2 * D + PAD, 128), bf16),
            pltpu.VMEM((4, HD + PAD, 128), bf16),
            pltpu.VMEM((4, HD + PAD, 128), bf16),
            pltpu.VMEM((NP, 72, 128), f32),
            pltpu.VMEM((NP, 80, 128), bf16),
            *[pltpu.VMEM((HT2 + 8, HD), f32) for _ in range(4)],
            pltpu.VMEM((HT2, 384), f32),
            *[pltpu.VMEM((HT2, HD), f32) for _ in range(7)],
            pltpu.VMEM((S, D), bf16),
            pltpu.VMEM((S + 16, D), bf16),
            pltpu.VMEM((8, D), f32),
            pltpu.VMEM((3, 8, 128), f32),
            pltpu.VMEM((8, 128), jnp.int32),
            pltpu.VMEM((8, D), bf16),
            *[pltpu.VMEM((256, 128), f32) for _ in range(4)],
            pltpu.SemaphoreType.DMA((NSEM,)),
        ],
        compiler_params=pltpu.CompilerParams(
            vmem_limit_bytes=110 * 1024 * 1024,
            disable_bounds_checks=True,
            disable_semaphore_checks=True),
    )(A_x, A_wqkv, A_w_phi, A_wo, B_w_r, B_w_gate, B_w_up, B_w_down)
```

```python
import jax
import jax.numpy as jnp
from jax import lax
import jax.experimental.pallas as pl
import jax.experimental.pallas.tpu as pltpu

S = 2048
D = 1024
H = 32
DH = 32
F = 3584
NP = H // 2
T1 = 256
T2 = 512
N1 = S // T1
N2 = S // T2
HT1 = T1 // 2
HT2 = T2 // 2
HD = D // 2
WC = 256
NWC = D // WC
LOG2E = 1.4426950408889634
EPS = 1e-5
PAD = 16
WO_ROWS = 176
LN_ROWS = 16
MAIN = 56
EP_ROWS = 32

T0_FOLD = (0, 4, 11, 18, 25, 33, 39, 46)
T0_WAITS = ((4, (1,)), (11, ('phi', 2)), (18, (3, 4)), (33, ('x1', 5, 6)), (46, (7,)),
            (65, (8, 9, 10, 11, 'x2', 'x3')))
T0_VPREP = ((65, 66, 66.5, 67.5), (68.5, 69, 70, 74), (74, 76, 78, 79), (81, 83, 84, 86))
T0_COMPACT = (22, 47)
T0_VSPAN = (2, 5, 5, 4)
T0_LN = (33, 33, 35, 35, 36, 38, 40, 45)
T0_LNSPAN = (3, 4, 0, 0, 0, 0, 0, 0)
T1_LN = ((102, 103, 104, 105, 106, 107, 108, 109), (89, 91, 93, 95, 97, 99, 100, 101))
P1_LNSPAN = 5
T0_Z = (63, 63.5, 64, 70.5, 75, 79, 84, 90, 90, 94, 98, 98, 99.5, 100.5, 107, 109.5)
T0_ZSPAN = 0
P1_WO = (30, 30, 32, 33, 34, 51, 52, 53, 53, 53, 55)
P1_WOSPAN = 3
P1_LN2 = ((42, 43, 44, 45, 46, 47, 48, 50), (34, 35, 35, 37, 38, 39, 40, 41))
P1_LNSPAN2 = (3, 3)
P1_Z = (28, 30, 31, 33, 36, 38, 40, 42, 43, 44, 46, 47, 48, 51, 52, 53)
P1_ZSPAN = 2
LT_START = (0, 0, 1, 5, 8, 11, 14)
LT_SPAN = (1, 3, 4, 4, 3, 4, 5)
FB_START = (2, 4, 6, 8, 10, 12, 14, 16)
FB_SPAN = 2
SA_START = (9, 11, 13, 15, 15, 17, 18, 19)
SA_SPAN = 4
FA_START = (20, 21, 22, 23, 24, 25, 26, 27)
FA_SPAN = (3, 4, 2, 4, 2, 4, 2, 2)
FFN_VPU_BLOCKS = 7
FFN_KG = 16
FFN_W0 = 16
FFN_W1 = 107
FFN_SPAN = 4
FFN_LATE = 16
LATE_AT = (-1, -1, -1, 0, 1, 2, 4, 5)

_NT = (((1,), (1,)), ((), ()))
f32 = jnp.float32
bf16 = jnp.bfloat16
u32 = jnp.uint32

K_, Q_, V_ = 0, 1, 2
SRC = {K_: 1, Q_: 0, V_: 2}

SEM_W = 0
SEM_X = SEM_W + 3 * NWC
SEM_X0 = SEM_X + N1
SEM_K0 = SEM_X0 + 4
SEM_PHI = SEM_K0 + 4
SEM_WO = SEM_PHI + 2
SEM_WR, SEM_WG, SEM_WU, SEM_WD, SEM_WGV, SEM_WUV, SEM_O = (SEM_WO + 1 + i for i in range(7))
NSEM = SEM_O + 1


def _rb(v):
    return v.astype(bf16).astype(f32)


def _unpack(w):
    return pltpu.bitcast(w, bf16)


def _mo(i, n):
    return i if isinstance(i, int) else pl.multiple_of(i, n)


def _recip(x):
    r = pl.reciprocal(x, approx=True)
    return r * (2.0 - x * r)


def _sigmoid(x):
    return _recip(1.0 + jnp.exp(jnp.minimum(-x, 80.0)))


def _dual_softmax(p):
    t = p.shape[-1]
    p3 = p.reshape(8, 8, t)

    def allred(v, op):
        v = op(v, pltpu.roll(v, 2, 0))
        return op(v, pltpu.roll(v, 4, 0))

    mx = allred(jnp.max(p3, axis=0), jnp.maximum)
    mn = allred(jnp.min(p3, axis=0), jnp.minimum)
    ep = jnp.exp2(p3 - mx[None])
    en = jnp.exp2(mn[None] - p3)
    sp = allred(jnp.sum(ep, axis=0), jnp.add)
    sn = allred(jnp.sum(en, axis=0), jnp.add)
    fp = (ep * _recip(sp)[None]).reshape(64, t)
    fn = (en * _recip(sn)[None]).reshape(64, t)
    return jnp.concatenate([fp, fn], axis=0).astype(bf16)


def _left_combos(a11, a12, a21, a22):
    return [a11 + a22, a21 + a22, a11, a22, a11 + a12, a21 - a11, a12 - a22]


def _right_combos(b11, b12, b21, b22):
    return [b11 + b22, b11, b12 - b22, b21 - b11, b22, b11 + b12, b21 + b22]


def _strassen(prod, emit):
    m3 = prod(2)
    m5 = prod(4)
    emit(0, 1, m3 + m5)
    m7 = prod(6)
    u = m7 - m5
    m1 = prod(0)
    u = u + m1
    w = m1 + m3
    m4 = prod(3)
    emit(0, 0, u + m4)
    m2 = prod(1)
    emit(1, 0, m2 + m4)
    w = w - m2
    m6 = prod(5)
    emit(1, 1, w + m6)


def _or_into(w, toks):
    if not toks:
        return w
    top = w[0:8, 0:128]
    for tk in toks:
        top = top | tk
    if w.shape[1] > 128:
        top = jnp.concatenate([top, w[0:8, 128:]], axis=1)
    return jnp.concatenate([top, w[8:]], axis=0)


def _fold_token(w, zero):
    r, c = w.shape
    acc = None
    for i in range(r // 8):
        for j in range(c // 128):
            blk = w[i * 8:(i + 1) * 8, j * 128:(j + 1) * 128]
            acc = blk if acc is None else acc | blk
    return acc & zero


def _body(zs, x_hbm, wqkv_hbm, wphi_hbm, wo_hbm, wr_hbm, wg_hbm, wu_hbm, wd_hbm, out_hbm,
          x_v, wqkv_v, wphi_v, wo_v, wr_v, wg_v, wu_v, wd_v, wgv_v, wuv_v,
          wt_v, we_v, wl_v, wo7_v, sa7_v, sb7_v, sc7_v, phiq_v, phik_v, vt0_v, vt1_v, kv_acc, kvt_v,
          hal_v, har_v, hbl_v, hbr_v, sa_v, t0_v, t1_v, t2_v, t3_v, t4_v, t5_v, t6_v,
          h_v, out_v, wrf_v, best_v, besti_v, fix_v, xc0_v, xc1_v, xc2_v, xc3_v, sem):
    xcol_v = (xc0_v, xc1_v, xc2_v, xc3_v)
    s_v = (sa7_v, sb7_v)
    vt_v = (vt0_v, vt1_v)
    ha_v = (hal_v, har_v)
    hb_v = (hbl_v, hbr_v)
    tmp_v = (t0_v, t1_v, t2_v, t3_v, t4_v, t5_v, t6_v)

    def x_rows(r0, rows, slot):
        return pltpu.make_async_copy(
            x_hbm.at[0, pl.ds(r0, rows), :], x_v.at[pl.ds(r0, rows), :], sem.at[slot])

    def x_copy(i):
        return x_rows(i * T1, T1, SEM_X + i)

    def x0_copy(q):
        return x_rows((q % 2) * HT1 + (q // 2) * (HT1 // 2), HT1 // 2, SEM_X0 + q)

    def w_copy(kind, c):
        return pltpu.make_async_copy(
            wqkv_hbm.at[:, pl.ds(SRC[kind] * D + c * WC, WC)],
            wqkv_v.at[kind * NWC + c], sem.at[SEM_W + kind * NWC + c])

    def k0_copy(q):
        r0 = (q % 2) * HD + (q // 2) * 256
        return pltpu.make_async_copy(
            wqkv_hbm.at[pl.ds(r0, 256), pl.ds(SRC[K_] * D, WC)],
            wqkv_v.at[K_ * NWC, pl.ds(r0, 256), :], sem.at[SEM_K0 + q])

    def phi_copy(part):
        lo, n = part * (H // 2), H // 2
        return pltpu.make_async_copy(wphi_hbm.at[pl.ds(lo, n)], wphi_v.at[pl.ds(lo, n)],
                                     sem.at[SEM_PHI + part])

    def full_copy(src, dst, slot):
        return pltpu.make_async_copy(src, dst, sem.at[slot])

    x0_copy(0).start()
    x0_copy(1).start()
    full_copy(wr_hbm, wr_v, SEM_WR).start()
    phi_copy(0).start()
    x0_copy(2).start()
    x0_copy(3).start()
    for q in range(4):
        k0_copy(q).start()
    w_copy(K_, 1).start()
    phi_copy(1).start()
    w_copy(K_, 2).start()
    w_copy(K_, 3).start()
    w_copy(Q_, 0).start()
    x_copy(1).start()
    for c in range(1, NWC):
        w_copy(Q_, c).start()
    for c in range(NWC):
        w_copy(V_, c).start()
    x_copy(2).start()
    x_copy(3).start()
    full_copy(wo_hbm, wo_v.at[pl.ds(0, D), :], SEM_WO).start()
    for i in range(4, N1):
        x_copy(i).start()
    f0 = F - 256 * FFN_VPU_BLOCKS
    ffn_tiled = ((wg_hbm, wg_v, D, SEM_WG), (wu_hbm, wu_v, D, SEM_WU), (wd_hbm, wd_v, F, SEM_WD))
    for src, dst, rows, slot in ffn_tiled:
        for c in range(dst.shape[0]):
            full_copy(src.at[:, pl.ds(c * 128, 128)], dst.at[c, pl.ds(0, rows), :], slot).start()
    full_copy(wg_hbm.at[:, pl.ds(f0, F - f0)], wgv_v, SEM_WGV).start()
    full_copy(wu_hbm.at[:, pl.ds(f0, F - f0)], wuv_v, SEM_WUV).start()

    zero_v = jnp.full((8, 128), zs, jnp.int32).astype(u32)

    def zrows(r0, rows, mult=8):
        return pl.ds(pl.multiple_of(zs * mult + r0, mult), rows)

    def tiles(ref, r0, rows):
        w = ref.bitcast(u32)
        return jnp.concatenate(
            [w[c, r0 // 2:(r0 + rows) // 2, :] for c in range(ref.shape[0])], axis=1)

    def token(*vals):
        return lambda: _fold_token(pltpu.bitcast(jnp.concatenate(vals, axis=0), u32), zero_v)

    def ln1_stats(xf):
        m = jnp.sum(xf, axis=-1, keepdims=True) * (1.0 / D)
        q = jnp.sum(xf * xf, axis=-1, keepdims=True) * (1.0 / D)
        inv = lax.rsqrt(jnp.maximum(q - m * m, 0.0) + EPS) * LOG2E
        return inv, m * inv

    def ln1_piece(r0, dst, p, m=None):
        fixed = isinstance(r0, int)
        if m is not None:
            x_v[zrows(S, 8) if fixed else pl.ds(S, 8), 0:128] = m[0:8, 0:128].astype(bf16)
        xa, xb = [x_v[pl.ds(_mo(r0 + hf * HT1 + p * LN_ROWS, LN_ROWS), LN_ROWS), :]
                  .astype(f32) for hf in range(2)]
        (ia, ma), (ib, mb) = ln1_stats(xa), ln1_stats(xb)
        ya, yb = xa * ia, xb * ib
        s2 = ya[:, :HD] - ma
        s5 = yb[:, HD:] - mb
        s1 = s2 + s5
        s3 = yb[:, :HD] - yb[:, HD:]
        s4 = ya[:, HD:] - ya[:, :HD]
        combos = [s1, s2, s3, s4, s5, s1 + s3, s1 + s4]
        rows = zrows(p * LN_ROWS, LN_ROWS, 16) if fixed else pl.ds(p * LN_ROWS, LN_ROWS)
        for i in range(7):
            for c in range(4):
                dst[i, c, rows, :] = combos[i][:, c * 128:(c + 1) * 128].astype(bf16)
        return token(combos[5], combos[6])

    def fold_piece(kind, c, j, pt):
        sub = lax.broadcasted_iota(jnp.int32, (8, 128), 0)
        blk = {}
        for hh in range(2):
            for kh in range(2):
                k0 = kh * HD + j * 128
                w = wqkv_v[kind * NWC + c, k0:k0 + 128, hh * 128:(hh + 1) * 128]
                f = lax.dot_general(pt[2 * c + hh], w, _NT, preferred_element_type=f32)
                refs = []
                for pp in range(2):
                    ref = jnp.where(sub >= 6, f[pp * 8:(pp + 1) * 8], 0.0)
                    ref = ref + pltpu.roll(ref, 2, 0)
                    refs.append(ref + pltpu.roll(ref, 4, 0))
                blk[hh, kh] = f - jnp.concatenate(refs + [refs[0]] * 7 + [refs[1]] * 7, axis=0)
        combos = _left_combos(blk[0, 0], blk[0, 1], blk[1, 0], blk[1, 1])
        r0 = kind * HD + c * 128
        for i in range(7):
            wt_v[i, j, r0:r0 + 128, :] = combos[i].astype(bf16)
            we_v[kind, i, j, c * 16:(c + 1) * 16, :] = combos[i][0:16].astype(bf16)

    def fold_chunk(kind, c, pt):
        for j in range(4):
            fold_piece(kind, c, j, pt)

    def vprep_piece(c, j, m):
        wqkv_v[zs + 3 * NWC, 0:8, 0:128] = m[0:8, 0:128].astype(bf16)
        blk = {}
        for hh in range(2):
            for kh in range(2):
                k0 = kh * HD + j * 128
                w = wqkv_v[V_ * NWC + c, k0:k0 + 128, hh * 128:(hh + 1) * 128]
                blk[hh, kh] = w.T.astype(f32)
        combos = _left_combos(blk[0, 0], blk[0, 1], blk[1, 0], blk[1, 1])
        r0 = V_ * HD + c * 128
        for i in range(7):
            wt_v[i, j, r0:r0 + 128, :] = combos[i].astype(bf16)
        return token(combos[1], combos[4])

    def wo_piece(w0, m):
        wo_v[D:D + 8, 0:128] = m[0:8, 0:128].astype(bf16)
        top = wo_v[pl.ds(pl.multiple_of(w0, 16), 16), :].astype(f32)
        bot = wo_v[pl.ds(pl.multiple_of(HD + w0, 16), 16), :].astype(f32)
        combos = _right_combos(top[:, :HD], top[:, HD:], bot[:, :HD], bot[:, HD:])
        for i in range(7):
            for c in range(4):
                wo7_v[i, c, pl.ds(pl.multiple_of(w0, 16), 16), :] = (
                    combos[i][:, c * 128:(c + 1) * 128].astype(bf16))
        return token(combos[5], combos[6])

    def z_piece(j, first, m):
        phik_v[0, zrows(2 * D, 16, 16), :] = m[0:16, 0:128].astype(bf16)
        ph = _unpack(tiles(phik_v, j * 128, 128)).astype(f32)
        part = (ph[:, 0:128] + ph[:, 128:256]) + (ph[:, 256:384] + ph[:, 384:512])
        z = jnp.sum(part.astype(bf16).T.astype(f32).reshape(16, 8, 128), axis=0)
        for sh in (4, 2, 1):
            z = z + pltpu.roll(z, sh, 0)
        if first:
            kv_acc[j, 64:72, :] = z
        else:
            z = kv_acc[j, 64:72, :] + z
            kv_acc[j, 64:72, :] = z
            odd = lax.broadcasted_iota(jnp.int32, (8, 128), 1) % 2
            kvt_v[j, 64:80, :] = jnp.concatenate(
                [jnp.where(odd == hl, z, 0.0) for hl in range(2)], axis=0).astype(bf16)
        return token(z)

    def run_rounds(t0, rounds, post, first):
        count = [0]
        pins = {}

        def run_jobs(m):
            for fn, span in post.get(count[0], ()):
                tok = fn(m)
                if span:
                    pins.setdefault(count[0] + span, []).append(tok())
            count[0] += 1

        for par, kind, cs in rounds:
            r0 = kind * HD + cs[0] * 128
            rows = 128 * len(cs)

            def prod(i):
                if (par, kind) == (1, V_):
                    rhs = sc7_v[i]
                else:
                    rhs = tiles(s_v[par].at[i], 0, HT1)
                if (par, kind, cs[0]) == (1, K_, 0):
                    sc7_v[i, zrows(0, HT1 // 2), :] = rhs
                if len(cs) == NWC:
                    lhs = jnp.concatenate(
                        [wl_v[kind, i]] + [tiles(wt_v.at[i], r0 + c * 128 + 16, 2 * MAIN)
                                           for c in cs], axis=0)
                else:
                    lhs = tiles(wt_v.at[i], r0, rows)
                m = lax.dot_general(_unpack(lhs),
                                    _unpack(_or_into(rhs, pins.get(count[0]))),
                                    _NT, preferred_element_type=f32)
                run_jobs(m)
                return m

            def emit(rh, ch, blk):
                tb = 2 * par + ch
                for n, c in enumerate(cs):
                    for jj in range(2):
                        pair = 4 * c + 2 * rh + jj
                        if kind == V_:
                            p = blk[n * 128 + jj * 64:n * 128 + (jj + 1) * 64]
                        elif len(cs) == NWC:
                            sub = lax.broadcasted_iota(jnp.int32, (8, HT1), 0)
                            ends = [blk[k * 16 + jj * 8:k * 16 + jj * 8 + 8] for k in range(3)]
                            if c < 3:
                                end = ends[c]
                            else:
                                end = jnp.where(
                                    sub < 2, pltpu.roll(ends[0], 2, 0),
                                    jnp.where(sub < 4, pltpu.roll(ends[1], 4, 0),
                                              pltpu.roll(ends[2], 6, 0)))
                            q0 = 48 + (2 * n + jj) * MAIN
                            p = jnp.concatenate(
                                [blk[q0:q0 + MAIN], jnp.where(sub < 6, end, 0.0)], axis=0)
                        else:
                            q0, q1 = n * 128 + 16 + jj * MAIN, n * 128 + jj * 8
                            p = jnp.concatenate([blk[q0:q0 + MAIN], blk[q1:q1 + 8]], axis=0)
                        if kind == K_:
                            phik_v[tb, zrows(pair * 128, 128, 16), :] = _dual_softmax(p)
                        elif kind == Q_:
                            phiq_v[t0 // 2, tb, pair * 128:(pair + 1) * 128, :] = (
                                _dual_softmax(p))
                        else:
                            vt_v[pair // 8][tb, zrows((pair % 8) * 64, 64, 16), :] = (
                                p.astype(bf16))

            _strassen(prod, emit)

        kr = lax.broadcasted_iota(jnp.int32, (64, 128), 0)
        kc = lax.broadcasted_iota(jnp.int32, (64, 128), 1)
        kmask = kr // 32 == kc % 2
        for j in range(NP):
            lhs = tiles(vt_v[j // 8], (j % 8) * 64, 64)
            rhs = tiles(phik_v, j * 128, 128)
            upd = lax.dot_general(_unpack(lhs), _unpack(_or_into(rhs, pins.get(count[0]))), _NT,
                                  preferred_element_type=f32)
            run_jobs(upd)
            if first:
                kv_acc[j, 0:64, :] = upd
            else:
                upd = kv_acc[j, 0:64, :] + upd
                kv_acc[j, 0:64, :] = upd
                kvt_v[j, 0:64, :] = jnp.where(kmask, upd * (1.0 / LOG2E), 0.0).astype(bf16)

    def load_best():
        return best_v[0], besti_v[...], best_v[1], best_v[2]

    def store_best(best):
        best_v[0], besti_v[...], best_v[1], best_v[2] = best

    def build_pt(g0, g1):
        def row_ids(r):
            pair = jnp.where(r < 16, r // 8, jnp.where(r < 16 + MAIN, 0, 1))
            feat = jnp.where(r < 16, MAIN + r % 8, r - 16 - pair * MAIN) // 2
            return pair, feat

        n = g1 - g0
        w2 = wphi_v[4 * g0:4 * g1].reshape(n * 128, DH)
        er = lax.broadcasted_iota(jnp.int32, (128, DH), 0)
        ec = lax.broadcasted_iota(jnp.int32, (128, DH), 1)
        e = jnp.where(ec == row_ids(er)[1], 1.0, 0.0).astype(bf16)
        ptf = lax.dot_general(e, w2, _NT, preferred_element_type=f32)
        pr = lax.broadcasted_iota(jnp.int32, (128, 128), 0)
        pc = lax.broadcasted_iota(jnp.int32, (128, 128), 1)
        keep = pc // 32 == row_ids(pr)[0] * 2 + pr % 2
        return [jnp.where(keep, ptf[:, g * 128:(g + 1) * 128], 0.0).astype(bf16)
                for g in range(n)]

    def compact(kind, i, m):
        we_v[0, 0, 0, zrows(64, 16, 16), :] = m[0:16, 0:128].astype(bf16)
        sub = lax.broadcasted_iota(jnp.int32, (8, HD), 0)
        ends = tiles(we_v.at[kind, i], 0, 64)
        for c in range(NWC - 1):
            wl_v[kind, i, zrows(c * 8, 8), :] = jnp.where(
                sub % 4 == 3, pltpu.roll(ends[24:32], 3 - c, 0), ends[c * 8:(c + 1) * 8])

    hbl_v[...] = jnp.zeros_like(hbl_v)
    hbr_v[...] = jnp.zeros_like(hbr_v)
    store_best((jnp.full((8, 128), -jnp.inf, f32), jnp.zeros((8, 128), jnp.int32),
                jnp.zeros((8, 128), f32), jnp.zeros((8, 128), f32)))
    n_ln = HT1 // LN_ROWS
    x0_copy(0).wait()
    x0_copy(1).wait()
    for p in range(n_ln // 2):
        ln1_piece(0, s_v[0], p)
    full_copy(wr_hbm, wr_v, SEM_WR).wait()
    phi_copy(0).wait()
    x0_copy(2).wait()
    x0_copy(3).wait()
    wr_row = wr_v[...].astype(f32).reshape(1, D)
    wrf_v[...] = jnp.broadcast_to(
        wr_row - jnp.sum(wr_row, axis=-1, keepdims=True) * (1.0 / D), (8, D))
    pt = build_pt(0, 4)
    for p in range(n_ln // 2, n_ln):
        ln1_piece(0, s_v[0], p)
    for part in range(2):
        k0_copy(2 * part).wait()
        k0_copy(2 * part + 1).wait()
        fold_piece(K_, 0, 2 * part, pt)
        fold_piece(K_, 0, 2 * part + 1, pt)

    def add_at(post, slot, fn, span=0):
        half = slot != int(slot)
        post.setdefault(int(slot), []).append(
            (lambda m: fn(m[m.shape[0] // 32 * 16:] if half else m), span))

    post = {}

    def at(slot, fn, span=0):
        add_at(post, slot, fn, span)

    for slot, copies in T0_WAITS:
        for cp in copies:
            if cp == 'phi':
                at(slot, lambda m: phi_copy(1).wait())
            elif cp in ('x1', 'x2', 'x3'):
                at(slot, lambda m, cp=cp: x_copy(int(cp[1])).wait())
            else:
                at(slot, lambda m, cp=cp: w_copy(cp // NWC, cp % NWC).wait())
    for n in range(1, 2 * NWC):
        if n == 2:
            at(T0_FOLD[n], lambda m: pt.extend(build_pt(4, 8)))
        at(T0_FOLD[n], lambda m, n=n: fold_chunk(n // NWC, n % NWC, pt))
    for kind in (K_, Q_):
        for i in range(7):
            at(T0_COMPACT[kind] + i, lambda m, kind=kind, i=i: compact(kind, i, m))
    for c in range(NWC):
        for j in range(4):
            at(T0_VPREP[c][j], lambda m, c=c, j=j: vprep_piece(c, j, m), T0_VSPAN[c])
    for p in range(n_ln):
        at(T0_LN[p], lambda m, p=p: ln1_piece(T1, s_v[1], p, m), T0_LNSPAN[p])
    for p in range(n_ln):
        at(T1_LN[0][p], lambda m, p=p: ln1_piece(2 * T1, s_v[0], p, m), P1_LNSPAN)
        at(T1_LN[1][p], lambda m, p=p: ln1_piece(3 * T1, s_v[1], p, m), P1_LNSPAN)
    for j in range(NP):
        at(T0_Z[j], lambda m, j=j: z_piece(j, True, m), T0_ZSPAN)
    lo, hi = [0, 1], [2, 3]
    run_rounds(0, [(0, kind, [c]) for kind in (K_, Q_) for c in range(NWC)]
               + [(1, K_, lo + hi), (1, Q_, lo + hi)] + [(0, V_, [c]) for c in range(NWC)]
               + [(1, V_, lo), (1, V_, hi)], post, True)
    full_copy(wo_hbm, wo_v.at[pl.ds(0, D), :], SEM_WO).wait()
    for i in range(4, N1):
        x_copy(i).wait()

    def phase1(i, carry):
        post = {}
        nxt = jnp.minimum(i + 1, N2 - 1) * T2
        w0 = jnp.minimum((i - 1) * WO_ROWS, HD - WO_ROWS)
        for par in range(2):
            for p in range(n_ln):
                add_at(post, P1_LN2[par][p],
                       lambda m, p=p, par=par: ln1_piece(nxt + par * T1, s_v[par], p, m),
                       P1_LNSPAN2[par])
        for p in range(WO_ROWS // 16):
            add_at(post, P1_WO[p], lambda m, p=p: wo_piece(w0 + 16 * p, m), P1_WOSPAN)
        for j in range(NP):
            add_at(post, P1_Z[j], lambda m, j=j: z_piece(j, False, m), P1_ZSPAN)
        run_rounds(2 * i, [(par, kind, lo + hi) for kind in (K_, Q_) for par in range(2)]
                   + [(par, V_, cs) for par in range(2) for cs in (lo, hi)], post, False)
        return carry

    lax.fori_loop(1, N1 // 2, phase1, 0)

    for _, dst, rows, slot in ffn_tiled:
        filled = dst.at[:, pl.ds(0, rows), :]
        full_copy(filled, filled, slot).wait()
    full_copy(wg_hbm.at[:, pl.ds(f0, F - f0)], wgv_v, SEM_WGV).wait()
    full_copy(wu_hbm.at[:, pl.ds(f0, F - f0)], wuv_v, SEM_WUV).wait()

    def o_copy(hf):
        return pltpu.make_async_copy(
            out_v.at[pl.ds(hf * HT2, HT2), :], out_hbm.at[0, pl.ds(hf * HT2, HT2), :],
            sem.at[SEM_O])

    def half_stats(hh, c0):
        rows = hh.shape[0]
        parts = [hh[:, c * 128:(c + 1) * 128] for c in range(4)]
        wts = [wrf_v[:, c0 + c * 128:c0 + (c + 1) * 128] for c in range(4)]
        s1 = (parts[0] + parts[1]) + (parts[2] + parts[3])
        sq = [p * p for p in parts]
        s2 = (sq[0] + sq[1]) + (sq[2] + sq[3])
        dw = [(p.reshape(rows // 8, 8, 128) * w[None]).reshape(rows, 128)
              for p, w in zip(parts, wts)]
        s3 = (dw[0] + dw[1]) + (dw[2] + dw[3])
        return s1, s2, s3

    def first_half(hbuf, sbuf, base, p, c0):
        r0 = p * EP_ROWS
        hh = hbuf[c0 // HD][r0:r0 + EP_ROWS, :]
        h_v[pl.ds(pl.multiple_of(base + r0, EP_ROWS), EP_ROWS), c0:c0 + HD] = hh.astype(bf16)
        st = jnp.concatenate(half_stats(hh, c0), axis=1)
        sbuf[zrows(r0, EP_ROWS), :] = st
        return _fold_token(pltpu.bitcast(st, u32), zero_v)

    def finish(hbuf, sbuf, base, p, valid, best, defer=None):
        r0 = p * EP_ROWS
        g0 = pl.multiple_of(base + r0, EP_ROWS)
        hl, hr = [r[r0:r0 + EP_ROWS, :] for r in hbuf]
        if defer is None:
            h_v[pl.ds(g0, EP_ROWS), 0:HD] = hl.astype(bf16)
        if sbuf is None:
            if defer is None:
                h_v[pl.ds(g0, EP_ROWS), HD:D] = hr.astype(bf16)
            st = half_stats(hr, HD)
        else:
            st = sbuf[r0:r0 + EP_ROWS, :]
            st = [st[:, n * 128:(n + 1) * 128] for n in range(3)]
        s1, s2, s3 = [jnp.sum(v + w, axis=-1, keepdims=True)
                      for v, w in zip(half_stats(hl, 0), st)]
        m = s1 * (1.0 / D)
        var = jnp.maximum(s2 * (1.0 / D) - m * m, 0.0)
        inv = lax.rsqrt(var + EPS)
        r = s3 * inv

        def write_out(h):
            o = h * (1.0 + inv) - m * inv
            out_v[pl.ds(g0, EP_ROWS), :] = o.astype(bf16)
            return o

        if defer is None:
            o = write_out(jnp.concatenate([hl, hr], axis=1))
        else:
            defer.append(lambda: write_out(jnp.concatenate(
                [r_[r0:r0 + EP_ROWS, :] for r_ in hbuf], axis=1)))
        bv, bi, bm, bq = best
        sub = lax.broadcasted_iota(jnp.int32, (8, 128), 0)
        for g in range(EP_ROWS // 8):
            rows = slice(g * 8, (g + 1) * 8)
            rg = jnp.broadcast_to(r[rows], (8, 128))
            if valid is not None:
                rg = jnp.where(valid, rg, -jnp.inf)
            better = rg > bv
            bi = jnp.where(better, sub + (g0 + g * 8), bi)
            bv = jnp.where(better, rg, bv)
            bm = jnp.where(better, jnp.broadcast_to(m[rows], (8, 128)), bm)
            bq = jnp.where(better, jnp.broadcast_to(var[rows], (8, 128)), bq)
        best = (bv, bi, bm, bq)
        if defer is not None:
            return best, None
        tok = _fold_token(pltpu.bitcast(jnp.concatenate(
            [o[:, D - 128:], bv, bm, bq], axis=0), u32), zero_v)
        return best, tok

    n_ep = HT2 // EP_ROWS

    def phase2(i, carry):
        ot = []
        for j in range(NP):
            ph = tiles(phiq_v.at[i], j * 128, 128)
            n = jnp.dot(_unpack(kvt_v.bitcast(u32)[j]), _unpack(ph),
                        preferred_element_type=f32)
            r0h = _recip(n[64:72] + 1e-6)
            r1h = _recip(n[72:80] + 1e-6)
            ot.append((n[0:32].reshape(4, 8, T2) * r0h[None]).reshape(32, T2))
            ot.append((n[32:64].reshape(4, 8, T2) * r1h[None]).reshape(32, T2))
        lo = jnp.concatenate(ot[:H // 2], axis=0)
        hi = jnp.concatenate(ot[H // 2:], axis=0)
        lcs = _left_combos(lo[:, :HT2], hi[:, :HT2], lo[:, HT2:], hi[:, HT2:])

        state = {'best': load_best()}
        pins = {}
        jobs = {}
        lts = {}
        ra = pl.multiple_of(i * T2, T2)
        rb = pl.multiple_of(i * T2 + HT2, HT2)
        prev = jnp.maximum(i * T2 - HT2, HT2)

        def add_job(slot, deadline, fn, gates=()):
            jobs.setdefault(slot, []).append((fn, deadline, gates))

        def finish_job(hbuf, sbuf, base, p, valid):
            def fn():
                state['best'], tok = finish(hbuf, sbuf, base, p, valid, state['best'])
                return tok
            return fn

        def lt_job(k):
            def fn():
                lts[k] = lcs[k].astype(bf16).T
                return _fold_token(pltpu.bitcast(lts[k], u32), zero_v)
            return fn

        order = (2, 4, 6, 0, 3, 1, 5)
        lt_job(2)()
        for n in range(1, 7):
            add_job(LT_START[n], min(LT_START[n] + LT_SPAN[n], 4 * n), lt_job(order[n]))
        for p in range(n_ep):
            add_job(FB_START[p], FB_START[p] + FB_SPAN,
                    finish_job(hb_v, None, prev, p, i > 0), hb_v)
            add_job(SA_START[p], SA_START[p] + SA_SPAN,
                    lambda p=p: first_half(ha_v, sa_v, ra, p, HD), ha_v[1:])
            add_job(FA_START[p], FA_START[p] + FA_SPAN[p],
                    finish_job(ha_v, sa_v, ra, p, None), ha_v)

        def xblk(r0, c0):
            return x_v[pl.ds(r0, HT2), c0:c0 + 128].astype(f32)

        for n, k in enumerate(order):
            for c in range(4):
                slot = 4 * n + c
                for fn, deadline, gates in jobs.get(slot, ()):
                    for ref in gates:
                        ref[zrows(HT2, 8), 0:128] = mm[0:8]
                    pins.setdefault(deadline, []).append(fn())
                w = _or_into(wo7_v.bitcast(u32)[k, c, 0:HD // 2, :], pins.get(slot))
                mm = jnp.dot(lts[k], _unpack(w), preferred_element_type=f32)
                c0 = c * 128
                cs = slice(c0, c0 + 128)
                tmp = lambda t: tmp_v[t][:, cs]
                if n == 0:
                    tmp_v[0][zrows(0, HT2), cs] = mm
                elif n == 1:
                    ha_v[1][zrows(0, HT2), cs] = (xblk(ra, HD + c0) + tmp(0)) + mm
                    tmp_v[1][zrows(0, HT2), cs] = xblk(ra, c0) - mm
                elif n == 2:
                    tmp_v[2][zrows(0, HT2), cs] = tmp(1) + mm
                elif n == 3:
                    tmp_v[3][zrows(0, HT2), cs] = tmp(2) + mm
                    tmp_v[4][zrows(0, HT2), cs] = (xblk(rb, HD + c0) + tmp(0)) + mm
                elif n == 4:
                    ha_v[0][zrows(0, HT2), cs] = tmp(3) + mm
                    tmp_v[5][zrows(0, HT2), cs] = xblk(rb, c0) + mm
                elif n == 5:
                    hb_v[0][zrows(0, HT2), cs] = tmp(5) + mm
                    tmp_v[6][zrows(0, HT2), cs] = tmp(4) - mm
                else:
                    hb_v[1][zrows(0, HT2), cs] = tmp(6) + mm
        store_best(state['best'])
        o_copy(2 * i).start()

        @pl.when(i > 0)
        def _():
            o_copy(2 * i - 1).start()

        return carry

    lax.fori_loop(0, N2, phase2, 0)
    best = load_best()
    late = []
    for p in range(n_ep):
        best, _ = finish(hb_v, None, S - HT2, p, None, best, late)

    bv, bi, bm, bq = best
    for sh in (4, 2, 1):
        ov, oi, om, oq = [pltpu.roll(t, sh, 0) for t in (bv, bi, bm, bq)]
        take = jnp.logical_or(ov > bv, jnp.logical_and(ov == bv, oi < bi))
        bv, bi, bm, bq = [jnp.where(take, o_, t)
                          for o_, t in zip((ov, oi, om, oq), (bv, bi, bm, bq))]
    idx = jnp.clip(bi[0, 0], 0, S - 1)
    for r_ in hb_v:
        r_[zrows(HT2, 8), 0:128] = bv
    for p, fn in enumerate(late):
        if LATE_AT[p] < 0:
            fn()
    b0 = pl.multiple_of((idx // 8) * 8, 8)
    t = _rb(_rb(bq) + EPS)
    inv = _recip(_rb(t * lax.rsqrt(t)))
    gate = _sigmoid(bv)
    wide = lambda v: jnp.concatenate([v] * (D // 128), axis=1)
    b1 = pl.multiple_of(jnp.minimum(b0, S - HT2 - 8), 8)
    b2 = pl.multiple_of(jnp.maximum(b0 - (S - HT2), 0), 8)
    hb = jnp.where(wide(bi) < S - HT2, h_v[pl.ds(b1, 8), :].astype(f32),
                   _rb(jnp.concatenate([r_[pl.ds(b2, 8), :] for r_ in hb_v], axis=1)))
    hn = (hb - wide(bm)) * wide(inv)
    xs = hn.astype(bf16)
    rows = lax.broadcasted_iota(jnp.int32, (8, D), 0) + b0

    xm = jnp.where(rows == wide(bi), hn, 0.0)
    for sh in (4, 2, 1):
        xm = xm + pltpu.roll(xm, sh, 0)
    for t in range(D // 128):
        xcol_v[t // 2][zrows((t % 2) * 128, 128), :] = jnp.concatenate(
            [xm[:, t * 128:(t + 1) * 128]] * 16, axis=0).astype(bf16).T.astype(f32)

    nblk = F // 256
    nmx = nblk - FFN_VPU_BLOCKS
    act = {}
    acc = {}

    def activate(g, u):
        return (g * _sigmoid(g) * u).astype(bf16)

    parts = D // 8 // FFN_KG

    def vpu_chunk(q):
        blk, part = nmx + q // parts, q % parts
        cur = acc.get(blk)
        for kg in range(part * FFN_KG, (part + 1) * FFN_KG):
            xc = xcol_v[kg // 32][(kg % 32) * 8:(kg % 32 + 1) * 8, :]
            w = jnp.concatenate(
                [r[kg * 8:(kg + 1) * 8, (blk - nmx) * 256:(blk - nmx + 1) * 256].astype(f32)
                 for r in (wgv_v, wuv_v)], axis=1)
            p = w * jnp.concatenate([xc] * 4, axis=1)
            cur = p if cur is None else cur + p
        acc[blk] = cur
        if part == parts - 1:
            for sh in (4, 2, 1):
                cur = cur + pltpu.roll(cur, sh, 0)
            act[blk] = activate(cur[:, :256], cur[:, 256:])
        c = q % 4
        return _fold_token(pltpu.bitcast(cur[:, c * 128:(c + 1) * 128], u32), zero_v)

    nchunk = FFN_VPU_BLOCKS * parts
    starts = [FFN_W0 + (q * (FFN_W1 - FFN_W0)) // (nchunk - 1) for q in range(nchunk)]
    pins = {}
    wave = [0]
    wgw, wuw, wdw = [r.bitcast(u32) for r in (wg_v, wu_v, wd_v)]

    def run_wave(lhs, tls):
        w = jnp.concatenate([_or_into(tls[0], pins.get(wave[0]))] + tls[1:], axis=1)
        out = jnp.dot(lhs, _unpack(w), preferred_element_type=f32)
        for p, fn in enumerate(late):
            if LATE_AT[p] == wave[0]:
                for r_ in hb_v:
                    r_[zrows(HT2, 8), 0:128] = out[:, 0:128]
                fn()
        for q, start in enumerate(starts):
            if start == wave[0]:
                pins.setdefault(wave[0] + FFN_SPAN, []).append(vpu_chunk(q))
        if wave[0] == FFN_LATE:
            o_copy(2 * N2 - 1).start()
            out_v[zrows(S, 16, 16), 0:256] = jnp.zeros((16, 256), bf16)
            pins.setdefault(wave[0] + 4, []).append(
                token(out_v[S:S + 8, 0:128].astype(f32))())
        wave[0] += 1
        return out

    for j in range(nmx):
        gu = None
        for kt in range(D // 128):
            p = run_wave(xs[:, kt * 128:(kt + 1) * 128],
                         [r[2 * j + c, kt * 64:(kt + 1) * 64, :]
                          for r in (wgw, wuw) for c in range(2)])
            gu = p if gu is None else gu + p
        act[j] = activate(gu[:, :256], gu[:, 256:])
    ys = [None, None]
    for j in range(nblk):
        for kt in range(2):
            for hf in range(2):
                r0 = (2 * j + kt) * 64
                p = run_wave(act[j][:, kt * 128:(kt + 1) * 128],
                             [wdw[4 * hf + c, r0:r0 + 64, :] for c in range(4)])
                ys[hf] = p if ys[hf] is None else ys[hf] + p
    y = jnp.concatenate(ys, axis=1)
    cur = out_v[pl.ds(b0, 8), :].astype(f32)
    fix_v[...] = jnp.where(rows == wide(bi), hb + hn + y * wide(gate), cur).astype(bf16)
    full_copy(out_v.at[pl.ds(0, S), :], out_hbm.at[0], SEM_O).wait()
    fix = pltpu.make_async_copy(fix_v, out_hbm.at[0, pl.ds(b0, 8), :], sem.at[SEM_O])
    fix.start()
    fix.wait()


def _kernel(*refs):
    def step(i, carry):
        @pl.when(i == 0)
        def _():
            _body(i, *refs)

        return carry

    lax.fori_loop(0, 2, step, 0)


@jax.jit
def pallas_sequential_preLN__linear_kernel_hedgehog__moe_arch_mod__prompt_kernel(
    A_x: jax.Array,
    A_wqkv: jax.Array,
    A_w_phi: jax.Array,
    A_wo: jax.Array,
    B_x: jax.Array,
    B_w_r: jax.Array,
    B_w_gate: jax.Array,
    B_w_up: jax.Array,
    B_w_down: jax.Array,
):
    any_spec = pl.BlockSpec(memory_space=pl.ANY)
    return pl.pallas_call(
        _kernel,
        out_shape=jax.ShapeDtypeStruct((1, S, D), bf16),
        in_specs=[any_spec] * 8,
        out_specs=any_spec,
        scratch_shapes=[
            pltpu.VMEM((S + 16, D), bf16),
            pltpu.VMEM((3 * NWC + 1, D, WC), bf16),
            pltpu.VMEM((H, DH, DH), bf16),
            pltpu.VMEM((D + 16, D), bf16),
            pltpu.VMEM((D,), bf16),
            pltpu.VMEM((F // 128 - 2 * FFN_VPU_BLOCKS, D + PAD, 128), bf16),
            pltpu.VMEM((F // 128 - 2 * FFN_VPU_BLOCKS, D + PAD, 128), bf16),
            pltpu.VMEM((D // 128, F + PAD, 128), bf16),
            pltpu.VMEM((D, 256 * FFN_VPU_BLOCKS), bf16),
            pltpu.VMEM((D, 256 * FFN_VPU_BLOCKS), bf16),
            pltpu.VMEM((7, 4, 3 * HD + PAD, 128), bf16),
            pltpu.VMEM((2, 7, 4, 64 + PAD, 128), bf16),
            pltpu.VMEM((2, 7, 24, HD), u32),
            pltpu.VMEM((7, 4, HD + PAD, 128), bf16),
            pltpu.VMEM((7, 4, HT1 + PAD, 128), bf16),
            pltpu.VMEM((7, 4, HT1 + PAD, 128), bf16),
            pltpu.VMEM((7, HT1 // 2, HD), u32),
            pltpu.VMEM((N2, 4, 2 * D + PAD, 128), bf16),
            pltpu.VMEM((4, 2 * D + PAD, 128), bf16),
            pltpu.VMEM((4, HD + PAD, 128), bf16),
            pltpu.VMEM((4, HD + PAD, 128), bf16),
            pltpu.VMEM((NP, 72, 128), f32),
            pltpu.VMEM((NP, 80, 128), bf16),
            *[pltpu.VMEM((HT2 + 8, HD), f32) for _ in range(4)],
            pltpu.VMEM((HT2, 384), f32),
            *[pltpu.VMEM((HT2, HD), f32) for _ in range(7)],
            pltpu.VMEM((S, D), bf16),
            pltpu.VMEM((S + 16, D), bf16),
            pltpu.VMEM((8, D), f32),
            pltpu.VMEM((3, 8, 128), f32),
            pltpu.VMEM((8, 128), jnp.int32),
            pltpu.VMEM((8, D), bf16),
            *[pltpu.VMEM((256, 128), f32) for _ in range(4)],
            pltpu.SemaphoreType.DMA((NSEM,)),
        ],
        compiler_params=pltpu.CompilerParams(
            vmem_limit_bytes=110 * 1024 * 1024,
            disable_bounds_checks=True,
            disable_semaphore_checks=True),
    )(A_x, A_wqkv, A_w_phi, A_wo, B_w_r, B_w_gate, B_w_up, B_w_down)
```

```python
import jax
import jax.numpy as jnp
from jax import lax
import jax.experimental.pallas as pl
import jax.experimental.pallas.tpu as pltpu

S = 2048
D = 1024
H = 32
DH = 32
F = 3584
NP = H // 2
T1 = 256
T2 = 512
N1 = S // T1
N2 = S // T2
HT1 = T1 // 2
HT2 = T2 // 2
HD = D // 2
WC = 256
NWC = D // WC
LOG2E = 1.4426950408889634
EPS = 1e-5
PAD = 16
WO_ROWS = 176
LN_ROWS = 16
MAIN = 56
EP_ROWS = 32

T0_FOLD = (0, 4, 11, 18, 25, 33, 39, 46)
T0_WAITS = ((4, (1,)), (11, ('phi', 2)), (18, (3, 4)), (33, ('x1', 5, 6)), (46, (7,)),
            (65, (8, 9, 10, 11, 'x2', 'x3')))
T0_VPREP = ((65, 66, 66.5, 67.5), (68.5, 69, 70, 74), (74, 76, 78, 79), (81, 83, 84, 86))
T0_COMPACT = (22, 47)
T0_VSPAN = (2, 5, 5, 4)
T0_LN = (33, 33, 35, 35, 36, 38, 40, 45)
T0_LNSPAN = (3, 4, 0, 0, 0, 0, 0, 0)
T1_LN = ((102, 103, 104, 105, 106, 107, 108, 109), (89, 91, 93, 95, 97, 99, 100, 101))
P1_LNSPAN = 5
T0_Z = (63, 63.5, 64, 70.5, 75, 79, 84, 90, 90, 94, 98, 98.0, 99.5, 100.5, 107.0, 109.5)
T0_ZSPAN = 0
P1_WO = (30, 30, 32, 33, 34, 51, 52, 52, 53, 53, 55)
P1_WOSPAN = 3
P1_LN2 = ((42, 43, 44, 45, 46, 47, 48, 50), (34, 35, 35, 37, 38, 39, 40, 41))
P1_LNSPAN2 = (3, 3)
P1_Z = (28, 30, 31, 33, 36, 38, 40, 42, 43, 44, 46, 47, 48, 51, 52, 53)
P1_ZSPAN = 2
LT_START = (0, 0, 1, 5, 8, 11, 14)
LT_SPAN = (1, 3, 4, 4, 3, 4, 5)
FB_START = (2, 4, 6, 8, 10, 12, 14, 16)
FB_SPAN = 2
SA_START = (9, 11, 13, 13, 15, 15, 18, 19)
SA_SPAN = 4
FA_START = (20, 21, 22, 23, 24, 25, 26, 27)
FA_SPAN = (3, 4, 2, 4, 2, 4, 2, 2)
FFN_VPU_BLOCKS = 7
FFN_KG = 16
FFN_W0 = 16
FFN_W1 = 107
FFN_SPAN = 4
FFN_LATE = 16
LATE_AT = (-1, -1, -1, 0, 1, 2, 4, 5)

_NT = (((1,), (1,)), ((), ()))
f32 = jnp.float32
bf16 = jnp.bfloat16
u32 = jnp.uint32

K_, Q_, V_ = 0, 1, 2
SRC = {K_: 1, Q_: 0, V_: 2}

SEM_W = 0
SEM_X = SEM_W + 3 * NWC
SEM_X0 = SEM_X + N1
SEM_K0 = SEM_X0 + 4
SEM_PHI = SEM_K0 + 4
SEM_WO = SEM_PHI + 2
SEM_WR, SEM_WG, SEM_WU, SEM_WD, SEM_WGV, SEM_WUV, SEM_O = (SEM_WO + 1 + i for i in range(7))
NSEM = SEM_O + 1


def _rb(v):
    return v.astype(bf16).astype(f32)


def _unpack(w):
    return pltpu.bitcast(w, bf16)


def _mo(i, n):
    return i if isinstance(i, int) else pl.multiple_of(i, n)


def _recip(x):
    r = pl.reciprocal(x, approx=True)
    return r * (2.0 - x * r)


def _sigmoid(x):
    return _recip(1.0 + jnp.exp(jnp.minimum(-x, 80.0)))


def _dual_softmax(p):
    t = p.shape[-1]
    p3 = p.reshape(8, 8, t)

    def allred(v, op):
        v = op(v, pltpu.roll(v, 2, 0))
        return op(v, pltpu.roll(v, 4, 0))

    mx = allred(jnp.max(p3, axis=0), jnp.maximum)
    mn = allred(jnp.min(p3, axis=0), jnp.minimum)
    ep = jnp.exp2(p3 - mx[None])
    en = jnp.exp2(mn[None] - p3)
    sp = allred(jnp.sum(ep, axis=0), jnp.add)
    sn = allred(jnp.sum(en, axis=0), jnp.add)
    fp = (ep * _recip(sp)[None]).reshape(64, t)
    fn = (en * _recip(sn)[None]).reshape(64, t)
    return jnp.concatenate([fp, fn], axis=0).astype(bf16)


def _left_combos(a11, a12, a21, a22):
    return [a11 + a22, a21 + a22, a11, a22, a11 + a12, a21 - a11, a12 - a22]


def _right_combos(b11, b12, b21, b22):
    return [b11 + b22, b11, b12 - b22, b21 - b11, b22, b11 + b12, b21 + b22]


def _strassen(prod, emit):
    m3 = prod(2)
    m5 = prod(4)
    emit(0, 1, m3 + m5)
    m7 = prod(6)
    u = m7 - m5
    m1 = prod(0)
    u = u + m1
    w = m1 + m3
    m4 = prod(3)
    emit(0, 0, u + m4)
    m2 = prod(1)
    emit(1, 0, m2 + m4)
    w = w - m2
    m6 = prod(5)
    emit(1, 1, w + m6)


def _or_into(w, toks):
    if not toks:
        return w
    top = w[0:8, 0:128]
    for tk in toks:
        top = top | tk
    if w.shape[1] > 128:
        top = jnp.concatenate([top, w[0:8, 128:]], axis=1)
    return jnp.concatenate([top, w[8:]], axis=0)


def _fold_token(w, zero):
    r, c = w.shape
    acc = None
    for i in range(r // 8):
        for j in range(c // 128):
            blk = w[i * 8:(i + 1) * 8, j * 128:(j + 1) * 128]
            acc = blk if acc is None else acc | blk
    return acc & zero


def _body(zs, x_hbm, wqkv_hbm, wphi_hbm, wo_hbm, wr_hbm, wg_hbm, wu_hbm, wd_hbm, out_hbm,
          x_v, wqkv_v, wphi_v, wo_v, wr_v, wg_v, wu_v, wd_v, wgv_v, wuv_v,
          wt_v, we_v, wl_v, wo7_v, sa7_v, sb7_v, sc7_v, phiq_v, phik_v, vt0_v, vt1_v, kv_acc, kvt_v,
          hal_v, har_v, hbl_v, hbr_v, sa_v, t0_v, t1_v, t2_v, t3_v, t4_v, t5_v, t6_v,
          out_v, wrf_v, best_v, besti_v, fix_v, xc0_v, xc1_v, xc2_v, xc3_v, sem):
    xcol_v = (xc0_v, xc1_v, xc2_v, xc3_v)
    s_v = (sa7_v, sb7_v)
    vt_v = (vt0_v, vt1_v)
    ha_v = (hal_v, har_v)
    hb_v = (hbl_v, hbr_v)
    tmp_v = (t0_v, t1_v, t2_v, t3_v, t4_v, t5_v, t6_v)

    def x_rows(r0, rows, slot):
        return pltpu.make_async_copy(
            x_hbm.at[0, pl.ds(r0, rows), :], x_v.at[pl.ds(r0, rows), :], sem.at[slot])

    def x_copy(i):
        return x_rows(i * T1, T1, SEM_X + i)

    def x0_copy(q):
        return x_rows((q % 2) * HT1 + (q // 2) * (HT1 // 2), HT1 // 2, SEM_X0 + q)

    def w_copy(kind, c):
        return pltpu.make_async_copy(
            wqkv_hbm.at[:, pl.ds(SRC[kind] * D + c * WC, WC)],
            wqkv_v.at[kind * NWC + c], sem.at[SEM_W + kind * NWC + c])

    def k0_copy(q):
        r0 = (q % 2) * HD + (q // 2) * 256
        return pltpu.make_async_copy(
            wqkv_hbm.at[pl.ds(r0, 256), pl.ds(SRC[K_] * D, WC)],
            wqkv_v.at[K_ * NWC, pl.ds(r0, 256), :], sem.at[SEM_K0 + q])

    def phi_copy(part):
        lo, n = part * (H // 2), H // 2
        return pltpu.make_async_copy(wphi_hbm.at[pl.ds(lo, n)], wphi_v.at[pl.ds(lo, n)],
                                     sem.at[SEM_PHI + part])

    def full_copy(src, dst, slot):
        return pltpu.make_async_copy(src, dst, sem.at[slot])

    x0_copy(0).start()
    x0_copy(1).start()
    full_copy(wr_hbm, wr_v, SEM_WR).start()
    phi_copy(0).start()
    x0_copy(2).start()
    x0_copy(3).start()
    for q in range(4):
        k0_copy(q).start()
    w_copy(K_, 1).start()
    phi_copy(1).start()
    w_copy(K_, 2).start()
    w_copy(K_, 3).start()
    w_copy(Q_, 0).start()
    x_copy(1).start()
    for c in range(1, NWC):
        w_copy(Q_, c).start()
    for c in range(NWC):
        w_copy(V_, c).start()
    x_copy(2).start()
    x_copy(3).start()
    full_copy(wo_hbm, wo_v.at[pl.ds(0, D), :], SEM_WO).start()
    for i in range(4, N1):
        x_copy(i).start()
    f0 = F - 256 * FFN_VPU_BLOCKS
    ffn_tiled = ((wg_hbm, wg_v, D, SEM_WG), (wu_hbm, wu_v, D, SEM_WU), (wd_hbm, wd_v, F, SEM_WD))
    for src, dst, rows, slot in ffn_tiled:
        for c in range(dst.shape[0]):
            full_copy(src.at[:, pl.ds(c * 128, 128)], dst.at[c, pl.ds(0, rows), :], slot).start()
    full_copy(wg_hbm.at[:, pl.ds(f0, F - f0)], wgv_v, SEM_WGV).start()
    full_copy(wu_hbm.at[:, pl.ds(f0, F - f0)], wuv_v, SEM_WUV).start()

    zero_v = jnp.full((8, 128), zs, jnp.int32).astype(u32)

    def zrows(r0, rows, mult=8):
        return pl.ds(pl.multiple_of(zs * mult + r0, mult), rows)

    def tiles(ref, r0, rows):
        w = ref.bitcast(u32)
        return jnp.concatenate(
            [w[c, r0 // 2:(r0 + rows) // 2, :] for c in range(ref.shape[0])], axis=1)

    def token(*vals):
        return lambda: _fold_token(pltpu.bitcast(jnp.concatenate(vals, axis=0), u32), zero_v)

    def ln1_stats(xf):
        m = jnp.sum(xf, axis=-1, keepdims=True) * (1.0 / D)
        q = jnp.sum(xf * xf, axis=-1, keepdims=True) * (1.0 / D)
        inv = lax.rsqrt(jnp.maximum(q - m * m, 0.0) + EPS) * LOG2E
        return inv, m * inv

    def ln1_piece(r0, dst, p, m=None):
        fixed = isinstance(r0, int)
        if m is not None:
            x_v[zrows(S, 8) if fixed else pl.ds(S, 8), 0:128] = m[0:8, 0:128].astype(bf16)
        xa, xb = [x_v[pl.ds(_mo(r0 + hf * HT1 + p * LN_ROWS, LN_ROWS), LN_ROWS), :]
                  .astype(f32) for hf in range(2)]
        (ia, ma), (ib, mb) = ln1_stats(xa), ln1_stats(xb)
        ya, yb = xa * ia, xb * ib
        s2 = ya[:, :HD] - ma
        s5 = yb[:, HD:] - mb
        s1 = s2 + s5
        s3 = yb[:, :HD] - yb[:, HD:]
        s4 = ya[:, HD:] - ya[:, :HD]
        combos = [s1, s2, s3, s4, s5, s1 + s3, s1 + s4]
        rows = zrows(p * LN_ROWS, LN_ROWS, 16) if fixed else pl.ds(p * LN_ROWS, LN_ROWS)
        for i in range(7):
            for c in range(4):
                dst[i, c, rows, :] = combos[i][:, c * 128:(c + 1) * 128].astype(bf16)
        return token(combos[5], combos[6])

    def fold_piece(kind, c, j, pt):
        sub = lax.broadcasted_iota(jnp.int32, (8, 128), 0)
        blk = {}
        for hh in range(2):
            for kh in range(2):
                k0 = kh * HD + j * 128
                w = wqkv_v[kind * NWC + c, k0:k0 + 128, hh * 128:(hh + 1) * 128]
                f = lax.dot_general(pt[2 * c + hh], w, _NT, preferred_element_type=f32)
                refs = []
                for pp in range(2):
                    ref = jnp.where(sub >= 6, f[pp * 8:(pp + 1) * 8], 0.0)
                    ref = ref + pltpu.roll(ref, 2, 0)
                    refs.append(ref + pltpu.roll(ref, 4, 0))
                blk[hh, kh] = f - jnp.concatenate(refs + [refs[0]] * 7 + [refs[1]] * 7, axis=0)
        combos = _left_combos(blk[0, 0], blk[0, 1], blk[1, 0], blk[1, 1])
        r0 = kind * HD + c * 128
        for i in range(7):
            wt_v[i, j, r0:r0 + 128, :] = combos[i].astype(bf16)
            we_v[kind, i, j, c * 16:(c + 1) * 16, :] = combos[i][0:16].astype(bf16)

    def fold_chunk(kind, c, pt):
        for j in range(4):
            fold_piece(kind, c, j, pt)

    def vprep_piece(c, j, m):
        wqkv_v[zs + 3 * NWC, 0:8, 0:128] = m[0:8, 0:128].astype(bf16)
        blk = {}
        for hh in range(2):
            for kh in range(2):
                k0 = kh * HD + j * 128
                w = wqkv_v[V_ * NWC + c, k0:k0 + 128, hh * 128:(hh + 1) * 128]
                blk[hh, kh] = w.T.astype(f32)
        combos = _left_combos(blk[0, 0], blk[0, 1], blk[1, 0], blk[1, 1])
        r0 = V_ * HD + c * 128
        for i in range(7):
            wt_v[i, j, r0:r0 + 128, :] = combos[i].astype(bf16)
        return token(combos[1], combos[4])

    def wo_piece(w0, m):
        wo_v[D:D + 8, 0:128] = m[0:8, 0:128].astype(bf16)
        top = wo_v[pl.ds(pl.multiple_of(w0, 16), 16), :].astype(f32)
        bot = wo_v[pl.ds(pl.multiple_of(HD + w0, 16), 16), :].astype(f32)
        combos = _right_combos(top[:, :HD], top[:, HD:], bot[:, :HD], bot[:, HD:])
        for i in range(7):
            for c in range(4):
                wo7_v[i, c, pl.ds(pl.multiple_of(w0, 16), 16), :] = (
                    combos[i][:, c * 128:(c + 1) * 128].astype(bf16))
        return token(combos[5], combos[6])

    def z_piece(j, first, m):
        phik_v[0, zrows(2 * D, 16, 16), :] = m[0:16, 0:128].astype(bf16)
        ph = _unpack(tiles(phik_v, j * 128, 128)).astype(f32)
        part = (ph[:, 0:128] + ph[:, 128:256]) + (ph[:, 256:384] + ph[:, 384:512])
        z = jnp.sum(part.astype(bf16).T.astype(f32).reshape(16, 8, 128), axis=0)
        for sh in (4, 2, 1):
            z = z + pltpu.roll(z, sh, 0)
        if first:
            kv_acc[j, 64:72, :] = z
        else:
            z = kv_acc[j, 64:72, :] + z
            kv_acc[j, 64:72, :] = z
            odd = lax.broadcasted_iota(jnp.int32, (8, 128), 1) % 2
            kvt_v[j, 64:80, :] = jnp.concatenate(
                [jnp.where(odd == hl, z, 0.0) for hl in range(2)], axis=0).astype(bf16)
        return token(z)

    def run_rounds(t0, rounds, post, first):
        count = [0]
        pins = {}

        def run_jobs(m):
            for fn, span in post.get(count[0], ()):
                tok = fn(m)
                if span:
                    pins.setdefault(count[0] + span, []).append(tok())
            count[0] += 1

        for par, kind, cs in rounds:
            r0 = kind * HD + cs[0] * 128
            rows = 128 * len(cs)

            def prod(i):
                if (par, kind) == (1, V_):
                    rhs = sc7_v[i]
                else:
                    rhs = tiles(s_v[par].at[i], 0, HT1)
                if (par, kind, cs[0]) == (1, K_, 0):
                    sc7_v[i, zrows(0, HT1 // 2), :] = rhs
                if len(cs) == NWC:
                    lhs = jnp.concatenate(
                        [wl_v[kind, i]] + [tiles(wt_v.at[i], r0 + c * 128 + 16, 2 * MAIN)
                                           for c in cs], axis=0)
                else:
                    lhs = tiles(wt_v.at[i], r0, rows)
                m = lax.dot_general(_unpack(lhs),
                                    _unpack(_or_into(rhs, pins.get(count[0]))),
                                    _NT, preferred_element_type=f32)
                run_jobs(m)
                return m

            def emit(rh, ch, blk):
                tb = 2 * par + ch
                for n, c in enumerate(cs):
                    for jj in range(2):
                        pair = 4 * c + 2 * rh + jj
                        if kind == V_:
                            p = blk[n * 128 + jj * 64:n * 128 + (jj + 1) * 64]
                        elif len(cs) == NWC:
                            sub = lax.broadcasted_iota(jnp.int32, (8, HT1), 0)
                            ends = [blk[k * 16 + jj * 8:k * 16 + jj * 8 + 8] for k in range(3)]
                            if c < 3:
                                end = ends[c]
                            else:
                                end = jnp.where(
                                    sub < 2, pltpu.roll(ends[0], 2, 0),
                                    jnp.where(sub < 4, pltpu.roll(ends[1], 4, 0),
                                              pltpu.roll(ends[2], 6, 0)))
                            q0 = 48 + (2 * n + jj) * MAIN
                            p = jnp.concatenate(
                                [blk[q0:q0 + MAIN], jnp.where(sub < 6, end, 0.0)], axis=0)
                        else:
                            q0, q1 = n * 128 + 16 + jj * MAIN, n * 128 + jj * 8
                            p = jnp.concatenate([blk[q0:q0 + MAIN], blk[q1:q1 + 8]], axis=0)
                        if kind == K_:
                            phik_v[tb, zrows(pair * 128, 128, 16), :] = _dual_softmax(p)
                        elif kind == Q_:
                            phiq_v[t0 // 2, tb, pair * 128:(pair + 1) * 128, :] = (
                                _dual_softmax(p))
                        else:
                            vt_v[pair // 8][tb, zrows((pair % 8) * 64, 64, 16), :] = (
                                p.astype(bf16))

            _strassen(prod, emit)

        kr = lax.broadcasted_iota(jnp.int32, (64, 128), 0)
        kc = lax.broadcasted_iota(jnp.int32, (64, 128), 1)
        kmask = kr // 32 == kc % 2
        for j in range(NP):
            lhs = tiles(vt_v[j // 8], (j % 8) * 64, 64)
            rhs = tiles(phik_v, j * 128, 128)
            upd = lax.dot_general(_unpack(lhs), _unpack(_or_into(rhs, pins.get(count[0]))), _NT,
                                  preferred_element_type=f32)
            run_jobs(upd)
            if first:
                kv_acc[j, 0:64, :] = upd
            else:
                upd = kv_acc[j, 0:64, :] + upd
                kv_acc[j, 0:64, :] = upd
                kvt_v[j, 0:64, :] = jnp.where(kmask, upd * (1.0 / LOG2E), 0.0).astype(bf16)

    def load_best():
        return best_v[0], besti_v[...], best_v[1], best_v[2]

    def store_best(best):
        best_v[0], besti_v[...], best_v[1], best_v[2] = best

    def build_pt(g0, g1):
        def row_ids(r):
            pair = jnp.where(r < 16, r // 8, jnp.where(r < 16 + MAIN, 0, 1))
            feat = jnp.where(r < 16, MAIN + r % 8, r - 16 - pair * MAIN) // 2
            return pair, feat

        n = g1 - g0
        w2 = wphi_v[4 * g0:4 * g1].reshape(n * 128, DH)
        er = lax.broadcasted_iota(jnp.int32, (128, DH), 0)
        ec = lax.broadcasted_iota(jnp.int32, (128, DH), 1)
        e = jnp.where(ec == row_ids(er)[1], 1.0, 0.0).astype(bf16)
        ptf = lax.dot_general(e, w2, _NT, preferred_element_type=f32)
        pr = lax.broadcasted_iota(jnp.int32, (128, 128), 0)
        pc = lax.broadcasted_iota(jnp.int32, (128, 128), 1)
        keep = pc // 32 == row_ids(pr)[0] * 2 + pr % 2
        return [jnp.where(keep, ptf[:, g * 128:(g + 1) * 128], 0.0).astype(bf16)
                for g in range(n)]

    def compact(kind, i, m):
        we_v[0, 0, 0, zrows(64, 16, 16), :] = m[0:16, 0:128].astype(bf16)
        sub = lax.broadcasted_iota(jnp.int32, (8, HD), 0)
        ends = tiles(we_v.at[kind, i], 0, 64)
        for c in range(NWC - 1):
            wl_v[kind, i, zrows(c * 8, 8), :] = jnp.where(
                sub % 4 == 3, pltpu.roll(ends[24:32], 3 - c, 0), ends[c * 8:(c + 1) * 8])

    hbl_v[...] = jnp.zeros_like(hbl_v)
    hbr_v[...] = jnp.zeros_like(hbr_v)
    store_best((jnp.full((8, 128), -jnp.inf, f32), jnp.zeros((8, 128), jnp.int32),
                jnp.zeros((8, 128), f32), jnp.zeros((8, 128), f32)))
    n_ln = HT1 // LN_ROWS
    x0_copy(0).wait()
    x0_copy(1).wait()
    for p in range(n_ln // 2):
        ln1_piece(0, s_v[0], p)
    full_copy(wr_hbm, wr_v, SEM_WR).wait()
    phi_copy(0).wait()
    x0_copy(2).wait()
    x0_copy(3).wait()
    wr_row = wr_v[...].astype(f32).reshape(1, D)
    wrf_v[...] = jnp.broadcast_to(
        wr_row - jnp.sum(wr_row, axis=-1, keepdims=True) * (1.0 / D), (8, D))
    pt = build_pt(0, 4)
    for p in range(n_ln // 2, n_ln):
        ln1_piece(0, s_v[0], p)
    for part in range(2):
        k0_copy(2 * part).wait()
        k0_copy(2 * part + 1).wait()
        fold_piece(K_, 0, 2 * part, pt)
        fold_piece(K_, 0, 2 * part + 1, pt)

    def add_at(post, slot, fn, span=0):
        half = slot != int(slot)
        post.setdefault(int(slot), []).append(
            (lambda m: fn(m[m.shape[0] // 32 * 16:] if half else m), span))

    post = {}

    def at(slot, fn, span=0):
        add_at(post, slot, fn, span)

    for slot, copies in T0_WAITS:
        for cp in copies:
            if cp == 'phi':
                at(slot, lambda m: phi_copy(1).wait())
            elif cp in ('x1', 'x2', 'x3'):
                at(slot, lambda m, cp=cp: x_copy(int(cp[1])).wait())
            else:
                at(slot, lambda m, cp=cp: w_copy(cp // NWC, cp % NWC).wait())
    for n in range(1, 2 * NWC):
        if n == 2:
            at(T0_FOLD[n], lambda m: pt.extend(build_pt(4, 8)))
        at(T0_FOLD[n], lambda m, n=n: fold_chunk(n // NWC, n % NWC, pt))
    for kind in (K_, Q_):
        for i in range(7):
            at(T0_COMPACT[kind] + i, lambda m, kind=kind, i=i: compact(kind, i, m))
    for c in range(NWC):
        for j in range(4):
            at(T0_VPREP[c][j], lambda m, c=c, j=j: vprep_piece(c, j, m), T0_VSPAN[c])
    for p in range(n_ln):
        at(T0_LN[p], lambda m, p=p: ln1_piece(T1, s_v[1], p, m), T0_LNSPAN[p])
    for p in range(n_ln):
        at(T1_LN[0][p], lambda m, p=p: ln1_piece(2 * T1, s_v[0], p, m), P1_LNSPAN)
        at(T1_LN[1][p], lambda m, p=p: ln1_piece(3 * T1, s_v[1], p, m), P1_LNSPAN)
    for j in range(NP):
        at(T0_Z[j], lambda m, j=j: z_piece(j, True, m), T0_ZSPAN)
    lo, hi = [0, 1], [2, 3]
    run_rounds(0, [(0, kind, [c]) for kind in (K_, Q_) for c in range(NWC)]
               + [(1, K_, lo + hi), (1, Q_, lo + hi)] + [(0, V_, [c]) for c in range(NWC)]
               + [(1, V_, lo), (1, V_, hi)], post, True)
    full_copy(wo_hbm, wo_v.at[pl.ds(0, D), :], SEM_WO).wait()
    for i in range(4, N1):
        x_copy(i).wait()

    def phase1(i, carry):
        post = {}
        nxt = jnp.minimum(i + 1, N2 - 1) * T2
        w0 = jnp.minimum((i - 1) * WO_ROWS, HD - WO_ROWS)
        for par in range(2):
            for p in range(n_ln):
                add_at(post, P1_LN2[par][p],
                       lambda m, p=p, par=par: ln1_piece(nxt + par * T1, s_v[par], p, m),
                       P1_LNSPAN2[par])
        for p in range(WO_ROWS // 16):
            add_at(post, P1_WO[p], lambda m, p=p: wo_piece(w0 + 16 * p, m), P1_WOSPAN)
        for j in range(NP):
            add_at(post, P1_Z[j], lambda m, j=j: z_piece(j, False, m), P1_ZSPAN)
        run_rounds(2 * i, [(par, kind, lo + hi) for kind in (K_, Q_) for par in range(2)]
                   + [(par, V_, cs) for par in range(2) for cs in (lo, hi)], post, False)
        return carry

    lax.fori_loop(1, N1 // 2, phase1, 0)

    for _, dst, rows, slot in ffn_tiled:
        filled = dst.at[:, pl.ds(0, rows), :]
        full_copy(filled, filled, slot).wait()
    full_copy(wg_hbm.at[:, pl.ds(f0, F - f0)], wgv_v, SEM_WGV).wait()
    full_copy(wu_hbm.at[:, pl.ds(f0, F - f0)], wuv_v, SEM_WUV).wait()

    def o_copy(hf):
        return pltpu.make_async_copy(
            out_v.at[pl.ds(hf * HT2, HT2), :], out_hbm.at[0, pl.ds(hf * HT2, HT2), :],
            sem.at[SEM_O])

    def half_stats(hh, c0):
        rows = hh.shape[0]
        parts = [hh[:, c * 128:(c + 1) * 128] for c in range(4)]
        wts = [wrf_v[:, c0 + c * 128:c0 + (c + 1) * 128] for c in range(4)]
        s1 = (parts[0] + parts[1]) + (parts[2] + parts[3])
        sq = [p * p for p in parts]
        s2 = (sq[0] + sq[1]) + (sq[2] + sq[3])
        dw = [(p.reshape(rows // 8, 8, 128) * w[None]).reshape(rows, 128)
              for p, w in zip(parts, wts)]
        s3 = (dw[0] + dw[1]) + (dw[2] + dw[3])
        return s1, s2, s3

    def first_half(hbuf, sbuf, p, c0):
        r0 = p * EP_ROWS
        hh = hbuf[c0 // HD][r0:r0 + EP_ROWS, :]
        st = jnp.concatenate(half_stats(hh, c0), axis=1)
        sbuf[zrows(r0, EP_ROWS), :] = st
        return _fold_token(pltpu.bitcast(st, u32), zero_v)

    def finish(hbuf, sbuf, base, p, valid, best, defer=None):
        r0 = p * EP_ROWS
        g0 = pl.multiple_of(base + r0, EP_ROWS)
        hl, hr = [r[r0:r0 + EP_ROWS, :] for r in hbuf]
        if sbuf is None:
            st = half_stats(hr, HD)
        else:
            st = sbuf[r0:r0 + EP_ROWS, :]
            st = [st[:, n * 128:(n + 1) * 128] for n in range(3)]
        s1, s2, s3 = [jnp.sum(v + w, axis=-1, keepdims=True)
                      for v, w in zip(half_stats(hl, 0), st)]
        m = s1 * (1.0 / D)
        var = jnp.maximum(s2 * (1.0 / D) - m * m, 0.0)
        inv = lax.rsqrt(var + EPS)
        r = s3 * inv

        def write_out(h):
            o = h * (1.0 + inv) - m * inv
            out_v[pl.ds(g0, EP_ROWS), :] = o.astype(bf16)
            return o

        if defer is None:
            o = write_out(jnp.concatenate([hl, hr], axis=1))
        else:
            defer.append(lambda: write_out(jnp.concatenate(
                [r_[r0:r0 + EP_ROWS, :] for r_ in hbuf], axis=1)))
        bv, bi, bm, bq = best
        sub = lax.broadcasted_iota(jnp.int32, (8, 128), 0)
        for g in range(EP_ROWS // 8):
            rows = slice(g * 8, (g + 1) * 8)
            rg = jnp.broadcast_to(r[rows], (8, 128))
            if valid is not None:
                rg = jnp.where(valid, rg, -jnp.inf)
            better = rg > bv
            bi = jnp.where(better, sub + (g0 + g * 8), bi)
            bv = jnp.where(better, rg, bv)
            bm = jnp.where(better, jnp.broadcast_to(m[rows], (8, 128)), bm)
            bq = jnp.where(better, jnp.broadcast_to(var[rows], (8, 128)), bq)
        best = (bv, bi, bm, bq)
        if defer is not None:
            return best, None
        tok = _fold_token(pltpu.bitcast(jnp.concatenate(
            [o[:, D - 128:], bv, bm, bq], axis=0), u32), zero_v)
        return best, tok

    n_ep = HT2 // EP_ROWS

    def phase2(i, carry):
        ot = []
        for j in range(NP):
            ph = tiles(phiq_v.at[i], j * 128, 128)
            n = jnp.dot(_unpack(kvt_v.bitcast(u32)[j]), _unpack(ph),
                        preferred_element_type=f32)
            r0h = _recip(n[64:72] + 1e-6)
            r1h = _recip(n[72:80] + 1e-6)
            ot.append((n[0:32].reshape(4, 8, T2) * r0h[None]).reshape(32, T2))
            ot.append((n[32:64].reshape(4, 8, T2) * r1h[None]).reshape(32, T2))
        lo = jnp.concatenate(ot[:H // 2], axis=0)
        hi = jnp.concatenate(ot[H // 2:], axis=0)
        lcs = _left_combos(lo[:, :HT2], hi[:, :HT2], lo[:, HT2:], hi[:, HT2:])

        state = {'best': load_best()}
        pins = {}
        jobs = {}
        lts = {}
        ra = pl.multiple_of(i * T2, T2)
        rb = pl.multiple_of(i * T2 + HT2, HT2)
        prev = jnp.maximum(i * T2 - HT2, HT2)

        def add_job(slot, deadline, fn, gates=()):
            jobs.setdefault(slot, []).append((fn, deadline, gates))

        def finish_job(hbuf, sbuf, base, p, valid):
            def fn():
                state['best'], tok = finish(hbuf, sbuf, base, p, valid, state['best'])
                return tok
            return fn

        def lt_job(k):
            def fn():
                lts[k] = lcs[k].astype(bf16).T
                return _fold_token(pltpu.bitcast(lts[k], u32), zero_v)
            return fn

        order = (2, 4, 6, 0, 3, 1, 5)
        lt_job(2)()
        for n in range(1, 7):
            add_job(LT_START[n], min(LT_START[n] + LT_SPAN[n], 4 * n), lt_job(order[n]))
        for p in range(n_ep):
            add_job(FB_START[p], FB_START[p] + FB_SPAN,
                    finish_job(hb_v, None, prev, p, i > 0), hb_v)
            add_job(SA_START[p], SA_START[p] + SA_SPAN,
                    lambda p=p: first_half(ha_v, sa_v, p, HD), ha_v[1:])
            add_job(FA_START[p], FA_START[p] + FA_SPAN[p],
                    finish_job(ha_v, sa_v, ra, p, None), ha_v)

        def xblk(r0, c0):
            return x_v[pl.ds(r0, HT2), c0:c0 + 128].astype(f32)

        for n, k in enumerate(order):
            for c in range(4):
                slot = 4 * n + c
                for fn, deadline, gates in jobs.get(slot, ()):
                    for ref in gates:
                        ref[zrows(HT2, 8), 0:128] = mm[0:8]
                    pins.setdefault(deadline, []).append(fn())
                w = _or_into(wo7_v.bitcast(u32)[k, c, 0:HD // 2, :], pins.get(slot))
                mm = jnp.dot(lts[k], _unpack(w), preferred_element_type=f32)
                c0 = c * 128
                cs = slice(c0, c0 + 128)
                tmp = lambda t: tmp_v[t][:, cs]
                if n == 0:
                    tmp_v[0][zrows(0, HT2), cs] = mm
                elif n == 1:
                    ha_v[1][zrows(0, HT2), cs] = (xblk(ra, HD + c0) + tmp(0)) + mm
                    tmp_v[1][zrows(0, HT2), cs] = xblk(ra, c0) - mm
                elif n == 2:
                    tmp_v[2][zrows(0, HT2), cs] = tmp(1) + mm
                elif n == 3:
                    tmp_v[3][zrows(0, HT2), cs] = tmp(2) + mm
                    tmp_v[4][zrows(0, HT2), cs] = (xblk(rb, HD + c0) + tmp(0)) + mm
                elif n == 4:
                    ha_v[0][zrows(0, HT2), cs] = tmp(3) + mm
                    tmp_v[5][zrows(0, HT2), cs] = xblk(rb, c0) + mm
                elif n == 5:
                    hb_v[0][zrows(0, HT2), cs] = tmp(5) + mm
                    tmp_v[6][zrows(0, HT2), cs] = tmp(4) - mm
                else:
                    hb_v[1][zrows(0, HT2), cs] = tmp(6) + mm
        store_best(state['best'])
        o_copy(2 * i).start()

        @pl.when(i > 0)
        def _():
            o_copy(2 * i - 1).start()

        return carry

    lax.fori_loop(0, N2, phase2, 0)
    best = load_best()
    late = []
    for p in range(n_ep):
        best, _ = finish(hb_v, None, S - HT2, p, None, best, late)

    bv, bi, bm, bq = best
    for sh in (4, 2, 1):
        ov, oi, om, oq = [pltpu.roll(t, sh, 0) for t in (bv, bi, bm, bq)]
        take = jnp.logical_or(ov > bv, jnp.logical_and(ov == bv, oi < bi))
        bv, bi, bm, bq = [jnp.where(take, o_, t)
                          for o_, t in zip((ov, oi, om, oq), (bv, bi, bm, bq))]
    idx = jnp.clip(bi[0, 0], 0, S - 1)
    for r_ in hb_v:
        r_[zrows(HT2, 8), 0:128] = bv
    for p, fn in enumerate(late):
        if LATE_AT[p] < 0:
            fn()
    b0 = pl.multiple_of((idx // 8) * 8, 8)
    t = _rb(_rb(bq) + EPS)
    inv = _recip(_rb(t * lax.rsqrt(t)))
    gate = _sigmoid(bv)
    wide = lambda v: jnp.concatenate([v] * (D // 128), axis=1)
    b1 = pl.multiple_of(jnp.minimum(b0, S - HT2 - 8), 8)
    b2 = pl.multiple_of(jnp.maximum(b0 - (S - HT2), 0), 8)
    early = wide(bi) < S - HT2
    src = jnp.where(early, out_v[pl.ds(b1, 8), :].astype(f32),
                    jnp.concatenate([r_[pl.ds(b2, 8), :] for r_ in hb_v], axis=1))
    scale = jnp.where(bi < S - HT2, inv * _recip(1.0 + lax.rsqrt(bq + EPS)), inv)
    hn = (src - wide(bm)) * wide(scale)
    xs = hn.astype(bf16)
    rows = lax.broadcasted_iota(jnp.int32, (8, D), 0) + b0

    xm = jnp.where(rows == wide(bi), hn, 0.0)
    for sh in (4, 2, 1):
        xm = xm + pltpu.roll(xm, sh, 0)
    for t in range(D // 128):
        xcol_v[t // 2][zrows((t % 2) * 128, 128), :] = jnp.concatenate(
            [xm[:, t * 128:(t + 1) * 128]] * 16, axis=0).astype(bf16).T.astype(f32)

    nblk = F // 256
    nmx = nblk - FFN_VPU_BLOCKS
    act = {}
    acc = {}

    def activate(g, u):
        return (g * _sigmoid(g) * u).astype(bf16)

    parts = D // 8 // FFN_KG

    def vpu_chunk(q):
        blk, part = nmx + q // parts, q % parts
        cur = acc.get(blk)
        for kg in range(part * FFN_KG, (part + 1) * FFN_KG):
            xc = xcol_v[kg // 32][(kg % 32) * 8:(kg % 32 + 1) * 8, :]
            w = jnp.concatenate(
                [r[kg * 8:(kg + 1) * 8, (blk - nmx) * 256:(blk - nmx + 1) * 256].astype(f32)
                 for r in (wgv_v, wuv_v)], axis=1)
            p = w * jnp.concatenate([xc] * 4, axis=1)
            cur = p if cur is None else cur + p
        acc[blk] = cur
        if part == parts - 1:
            for sh in (4, 2, 1):
                cur = cur + pltpu.roll(cur, sh, 0)
            act[blk] = activate(cur[:, :256], cur[:, 256:])
        c = q % 4
        return _fold_token(pltpu.bitcast(cur[:, c * 128:(c + 1) * 128], u32), zero_v)

    nchunk = FFN_VPU_BLOCKS * parts
    starts = [FFN_W0 + (q * (FFN_W1 - FFN_W0)) // (nchunk - 1) for q in range(nchunk)]
    pins = {}
    wave = [0]
    wgw, wuw, wdw = [r.bitcast(u32) for r in (wg_v, wu_v, wd_v)]

    def run_wave(lhs, tls):
        w = jnp.concatenate([_or_into(tls[0], pins.get(wave[0]))] + tls[1:], axis=1)
        out = jnp.dot(lhs, _unpack(w), preferred_element_type=f32)
        for p, fn in enumerate(late):
            if LATE_AT[p] == wave[0]:
                for r_ in hb_v:
                    r_[zrows(HT2, 8), 0:128] = out[:, 0:128]
                fn()
        for q, start in enumerate(starts):
            if start == wave[0]:
                pins.setdefault(wave[0] + FFN_SPAN, []).append(vpu_chunk(q))
        if wave[0] == FFN_LATE:
            o_copy(2 * N2 - 1).start()
            out_v[zrows(S, 16, 16), 0:256] = jnp.zeros((16, 256), bf16)
            pins.setdefault(wave[0] + 4, []).append(
                token(out_v[S:S + 8, 0:128].astype(f32))())
        wave[0] += 1
        return out

    for j in range(nmx):
        gu = None
        for kt in range(D // 128):
            p = run_wave(xs[:, kt * 128:(kt + 1) * 128],
                         [r[2 * j + c, kt * 64:(kt + 1) * 64, :]
                          for r in (wgw, wuw) for c in range(2)])
            gu = p if gu is None else gu + p
        act[j] = activate(gu[:, :256], gu[:, 256:])
    ys = [None, None]
    for j in range(nblk):
        for kt in range(2):
            for hf in range(2):
                r0 = (2 * j + kt) * 64
                p = run_wave(act[j][:, kt * 128:(kt + 1) * 128],
                             [wdw[4 * hf + c, r0:r0 + 64, :] for c in range(4)])
                ys[hf] = p if ys[hf] is None else ys[hf] + p
    y = jnp.concatenate(ys, axis=1)
    cur = out_v[pl.ds(b0, 8), :].astype(f32)
    fix_v[...] = jnp.where(rows == wide(bi), cur + y * wide(gate), cur).astype(bf16)
    full_copy(out_v.at[pl.ds(0, S), :], out_hbm.at[0], SEM_O).wait()
    fix = pltpu.make_async_copy(fix_v, out_hbm.at[0, pl.ds(b0, 8), :], sem.at[SEM_O])
    fix.start()
    fix.wait()


def _kernel(*refs):
    def step(i, carry):
        @pl.when(i == 0)
        def _():
            _body(i, *refs)

        return carry

    lax.fori_loop(0, 2, step, 0)


@jax.jit
def pallas_sequential_preLN__linear_kernel_hedgehog__moe_arch_mod__prompt_kernel(
    A_x: jax.Array,
    A_wqkv: jax.Array,
    A_w_phi: jax.Array,
    A_wo: jax.Array,
    B_x: jax.Array,
    B_w_r: jax.Array,
    B_w_gate: jax.Array,
    B_w_up: jax.Array,
    B_w_down: jax.Array,
):
    any_spec = pl.BlockSpec(memory_space=pl.ANY)
    return pl.pallas_call(
        _kernel,
        out_shape=jax.ShapeDtypeStruct((1, S, D), bf16),
        in_specs=[any_spec] * 8,
        out_specs=any_spec,
        scratch_shapes=[
            pltpu.VMEM((S + 16, D), bf16),
            pltpu.VMEM((3 * NWC + 1, D, WC), bf16),
            pltpu.VMEM((H, DH, DH), bf16),
            pltpu.VMEM((D + 16, D), bf16),
            pltpu.VMEM((D,), bf16),
            pltpu.VMEM((F // 128 - 2 * FFN_VPU_BLOCKS, D + PAD, 128), bf16),
            pltpu.VMEM((F // 128 - 2 * FFN_VPU_BLOCKS, D + PAD, 128), bf16),
            pltpu.VMEM((D // 128, F + PAD, 128), bf16),
            pltpu.VMEM((D, 256 * FFN_VPU_BLOCKS), bf16),
            pltpu.VMEM((D, 256 * FFN_VPU_BLOCKS), bf16),
            pltpu.VMEM((7, 4, 3 * HD + PAD, 128), bf16),
            pltpu.VMEM((2, 7, 4, 64 + PAD, 128), bf16),
            pltpu.VMEM((2, 7, 24, HD), u32),
            pltpu.VMEM((7, 4, HD + PAD, 128), bf16),
            pltpu.VMEM((7, 4, HT1 + PAD, 128), bf16),
            pltpu.VMEM((7, 4, HT1 + PAD, 128), bf16),
            pltpu.VMEM((7, HT1 // 2, HD), u32),
            pltpu.VMEM((N2, 4, 2 * D + PAD, 128), bf16),
            pltpu.VMEM((4, 2 * D + PAD, 128), bf16),
            pltpu.VMEM((4, HD + PAD, 128), bf16),
            pltpu.VMEM((4, HD + PAD, 128), bf16),
            pltpu.VMEM((NP, 72, 128), f32),
            pltpu.VMEM((NP, 80, 128), bf16),
            *[pltpu.VMEM((HT2 + 8, HD), f32) for _ in range(4)],
            pltpu.VMEM((HT2, 384), f32),
            *[pltpu.VMEM((HT2, HD), f32) for _ in range(7)],
            pltpu.VMEM((S + 16, D), bf16),
            pltpu.VMEM((8, D), f32),
            pltpu.VMEM((3, 8, 128), f32),
            pltpu.VMEM((8, 128), jnp.int32),
            pltpu.VMEM((8, D), bf16),
            *[pltpu.VMEM((256, 128), f32) for _ in range(4)],
            pltpu.SemaphoreType.DMA((NSEM,)),
        ],
        compiler_params=pltpu.CompilerParams(
            vmem_limit_bytes=110 * 1024 * 1024,
            disable_bounds_checks=True,
            disable_semaphore_checks=True),
    )(A_x, A_wqkv, A_w_phi, A_wo, B_w_r, B_w_gate, B_w_up, B_w_down)
```

```python
import jax
import jax.numpy as jnp
from jax import lax
import jax.experimental.pallas as pl
import jax.experimental.pallas.tpu as pltpu

S = 2048
D = 1024
H = 32
DH = 32
F = 3584
NP = H // 2
T1 = 256
T2 = 512
N1 = S // T1
N2 = S // T2
HT1 = T1 // 2
HT2 = T2 // 2
HD = D // 2
WC = 256
NWC = D // WC
LOG2E = 1.4426950408889634
EPS = 1e-5
PAD = 16
WO_ROWS = 176
LN_ROWS = 16
MAIN = 56
EP_ROWS = 32

T0_FOLD = (0, 4, 11, 18, 25, 33, 39, 46)
T0_WAITS = ((4, (1,)), (11, ('phi', 2)), (18, (3, 4)), (33, ('x1', 5, 6)), (46, (7,)),
            (65, (8, 9, 10, 11, 'x2', 'x3')))
T0_VPREP = ((65, 66, 66.5, 67.5), (68.5, 69, 70, 74), (74, 76, 78, 79), (81, 83, 84, 86))
T0_COMPACT = (22, 47)
T0_VSPAN = (2, 5, 5, 4)
T0_LN = (33, 33, 35, 35, 36, 38, 40, 45)
T0_LNSPAN = (3, 4, 0, 0, 0, 0, 0, 0)
T1_LN = ((102, 103, 104, 105, 106, 107, 108, 109), (89, 91, 93, 95, 97, 99, 100, 101))
P1_LNSPAN = 5
T0_Z = (63, 63.5, 64, 70.5, 73, 79, 84, 90, 90, 94, 98, 98, 99.5, 100.5, 107, 107.5)
T0_ZSPAN = 0
P1_WO = (30, 30, 32, 33, 34, 51, 52, 52, 53, 53, 55)
P1_WOSPAN = 3
P1_LN2 = ((42, 43, 44, 45, 46, 47, 49, 50), (34, 35, 35, 37, 38, 39, 41, 42))
P1_LNSPAN2 = (3, 3)
P1_Z = (28, 30, 31, 33, 36, 38, 40, 42, 43, 44, 46, 47, 48, 51, 52, 53)
P1_ZSPAN = 2
LT_START = (0, 0, 1, 5, 8, 11, 14)
LT_SPAN = (1, 3, 4, 4, 3, 4, 5)
FB_START = (2, 4, 6, 8, 10, 12, 14, 16)
FB_SPAN = 2
SA_START = (9, 11, 12, 13, 15, 15, 18, 19)
SA_SPAN = 4
FA_START = (20, 21, 22, 23, 25, 25, 26, 27)
FA_SPAN = (3, 4, 2, 4, 2, 4, 2, 2)
FFN_VPU_BLOCKS = 7
FFN_KG = 16
FFN_W0 = 16
FFN_W1 = 107
FFN_SPAN = 4
FFN_LATE = 16
LATE_AT = (-1, -1, -1, 0, 1, 2, 4, 5)

_NT = (((1,), (1,)), ((), ()))
f32 = jnp.float32
bf16 = jnp.bfloat16
u32 = jnp.uint32

K_, Q_, V_ = 0, 1, 2
SRC = {K_: 1, Q_: 0, V_: 2}

SEM_W = 0
SEM_X = SEM_W + 3 * NWC
SEM_X0 = SEM_X + N1
SEM_K0 = SEM_X0 + 4
SEM_PHI = SEM_K0 + 4
SEM_WO = SEM_PHI + 2
SEM_WR, SEM_WG, SEM_WU, SEM_WD, SEM_WGV, SEM_WUV, SEM_O = (SEM_WO + 1 + i for i in range(7))
NSEM = SEM_O + 1


def _rb(v):
    return v.astype(bf16).astype(f32)


def _unpack(w):
    return pltpu.bitcast(w, bf16)


def _mo(i, n):
    return i if isinstance(i, int) else pl.multiple_of(i, n)


def _recip(x):
    r = pl.reciprocal(x, approx=True)
    return r * (2.0 - x * r)


def _sigmoid(x):
    return _recip(1.0 + jnp.exp(jnp.minimum(-x, 80.0)))


def _dual_softmax(p):
    t = p.shape[-1]
    p3 = p.reshape(8, 8, t)

    def allred(v, op):
        v = op(v, pltpu.roll(v, 2, 0))
        return op(v, pltpu.roll(v, 4, 0))

    mx = allred(jnp.max(p3, axis=0), jnp.maximum)
    mn = allred(jnp.min(p3, axis=0), jnp.minimum)
    ep = jnp.exp2(p3 - mx[None])
    en = jnp.exp2(mn[None] - p3)
    sp = allred(jnp.sum(ep, axis=0), jnp.add)
    sn = allred(jnp.sum(en, axis=0), jnp.add)
    fp = (ep * _recip(sp)[None]).reshape(64, t)
    fn = (en * _recip(sn)[None]).reshape(64, t)
    return jnp.concatenate([fp, fn], axis=0).astype(bf16)


def _left_combos(a11, a12, a21, a22):
    return [a11 + a22, a21 + a22, a11, a22, a11 + a12, a21 - a11, a12 - a22]


def _right_combos(b11, b12, b21, b22):
    return [b11 + b22, b11, b12 - b22, b21 - b11, b22, b11 + b12, b21 + b22]


def _strassen(prod, emit):
    m3 = prod(2)
    m5 = prod(4)
    emit(0, 1, m3 + m5)
    m7 = prod(6)
    u = m7 - m5
    m1 = prod(0)
    u = u + m1
    w = m1 + m3
    m4 = prod(3)
    emit(0, 0, u + m4)
    m2 = prod(1)
    emit(1, 0, m2 + m4)
    w = w - m2
    m6 = prod(5)
    emit(1, 1, w + m6)


def _or_into(w, toks):
    if not toks:
        return w
    top = w[0:8, 0:128]
    for tk in toks:
        top = top | tk
    if w.shape[1] > 128:
        top = jnp.concatenate([top, w[0:8, 128:]], axis=1)
    return jnp.concatenate([top, w[8:]], axis=0)


def _fold_token(w, zero):
    r, c = w.shape
    acc = None
    for i in range(r // 8):
        for j in range(c // 128):
            blk = w[i * 8:(i + 1) * 8, j * 128:(j + 1) * 128]
            acc = blk if acc is None else acc | blk
    return acc & zero


def _body(zs, x_hbm, wqkv_hbm, wphi_hbm, wo_hbm, wr_hbm, wg_hbm, wu_hbm, wd_hbm, out_hbm,
          x_v, wqkv_v, wphi_v, wo_v, wr_v, wg_v, wu_v, wd_v, wgv_v, wuv_v,
          wt_v, we_v, wl_v, wo7_v, sa7_v, sb7_v, sc7_v, phiq_v, phik_v, vt0_v, vt1_v, kv_acc, kvt_v,
          hal_v, har_v, hbl_v, hbr_v, sa_v, t0_v, t1_v, t2_v, t3_v, t4_v, t5_v, t6_v,
          out_v, wrf_v, best_v, besti_v, fix_v, xc0_v, xc1_v, xc2_v, xc3_v, sem):
    xcol_v = (xc0_v, xc1_v, xc2_v, xc3_v)
    s_v = (sa7_v, sb7_v)
    vt_v = (vt0_v, vt1_v)
    ha_v = (hal_v, har_v)
    hb_v = (hbl_v, hbr_v)
    tmp_v = (t0_v, t1_v, t2_v, t3_v, t4_v, t5_v, t6_v)

    def x_rows(r0, rows, slot):
        return pltpu.make_async_copy(
            x_hbm.at[0, pl.ds(r0, rows), :], x_v.at[pl.ds(r0, rows), :], sem.at[slot])

    def x_copy(i):
        return x_rows(i * T1, T1, SEM_X + i)

    def x0_copy(q):
        return x_rows((q % 2) * HT1 + (q // 2) * (HT1 // 2), HT1 // 2, SEM_X0 + q)

    def w_copy(kind, c):
        return pltpu.make_async_copy(
            wqkv_hbm.at[:, pl.ds(SRC[kind] * D + c * WC, WC)],
            wqkv_v.at[kind * NWC + c], sem.at[SEM_W + kind * NWC + c])

    def k0_copy(q):
        r0 = (q % 2) * HD + (q // 2) * 256
        return pltpu.make_async_copy(
            wqkv_hbm.at[pl.ds(r0, 256), pl.ds(SRC[K_] * D, WC)],
            wqkv_v.at[K_ * NWC, pl.ds(r0, 256), :], sem.at[SEM_K0 + q])

    def phi_copy(part):
        lo, n = part * (H // 2), H // 2
        return pltpu.make_async_copy(wphi_hbm.at[pl.ds(lo, n)], wphi_v.at[pl.ds(lo, n)],
                                     sem.at[SEM_PHI + part])

    def full_copy(src, dst, slot):
        return pltpu.make_async_copy(src, dst, sem.at[slot])

    x0_copy(0).start()
    x0_copy(1).start()
    full_copy(wr_hbm, wr_v, SEM_WR).start()
    phi_copy(0).start()
    x0_copy(2).start()
    x0_copy(3).start()
    for q in range(4):
        k0_copy(q).start()
    w_copy(K_, 1).start()
    phi_copy(1).start()
    w_copy(K_, 2).start()
    w_copy(K_, 3).start()
    w_copy(Q_, 0).start()
    x_copy(1).start()
    for c in range(1, NWC):
        w_copy(Q_, c).start()
    for c in range(NWC):
        w_copy(V_, c).start()
    x_copy(2).start()
    x_copy(3).start()
    full_copy(wo_hbm, wo_v.at[pl.ds(0, D), :], SEM_WO).start()
    for i in range(4, N1):
        x_copy(i).start()
    f0 = F - 256 * FFN_VPU_BLOCKS
    ffn_tiled = ((wg_hbm, wg_v, D, SEM_WG), (wu_hbm, wu_v, D, SEM_WU), (wd_hbm, wd_v, F, SEM_WD))
    for src, dst, rows, slot in ffn_tiled:
        for c in range(dst.shape[0]):
            full_copy(src.at[:, pl.ds(c * 128, 128)], dst.at[c, pl.ds(0, rows), :], slot).start()
    full_copy(wg_hbm.at[:, pl.ds(f0, F - f0)], wgv_v, SEM_WGV).start()
    full_copy(wu_hbm.at[:, pl.ds(f0, F - f0)], wuv_v, SEM_WUV).start()

    zero_v = jnp.full((8, 128), zs, jnp.int32).astype(u32)

    def zrows(r0, rows, mult=8):
        return pl.ds(pl.multiple_of(zs * mult + r0, mult), rows)

    def tiles(ref, r0, rows):
        w = ref.bitcast(u32)
        return jnp.concatenate(
            [w[c, r0 // 2:(r0 + rows) // 2, :] for c in range(ref.shape[0])], axis=1)

    def token(*vals):
        return lambda: _fold_token(pltpu.bitcast(jnp.concatenate(vals, axis=0), u32), zero_v)

    def ln1_stats(xf):
        m = jnp.sum(xf, axis=-1, keepdims=True) * (1.0 / D)
        q = jnp.sum(xf * xf, axis=-1, keepdims=True) * (1.0 / D)
        inv = lax.rsqrt(jnp.maximum(q - m * m, 0.0) + EPS) * LOG2E
        return inv, m * inv

    def ln1_piece(r0, dst, p, m=None):
        fixed = isinstance(r0, int)
        if m is not None:
            x_v[zrows(S, 8) if fixed else pl.ds(S, 8), 0:128] = m[0:8, 0:128].astype(bf16)
        xa, xb = [x_v[pl.ds(_mo(r0 + hf * HT1 + p * LN_ROWS, LN_ROWS), LN_ROWS), :]
                  .astype(f32) for hf in range(2)]
        (ia, ma), (ib, mb) = ln1_stats(xa), ln1_stats(xb)
        ya, yb = xa * ia, xb * ib
        s2 = ya[:, :HD] - ma
        s5 = yb[:, HD:] - mb
        s1 = s2 + s5
        s3 = yb[:, :HD] - yb[:, HD:]
        s4 = ya[:, HD:] - ya[:, :HD]
        combos = [s1, s2, s3, s4, s5, s1 + s3, s1 + s4]
        rows = zrows(p * LN_ROWS, LN_ROWS, 16) if fixed else pl.ds(p * LN_ROWS, LN_ROWS)
        for i in range(7):
            for c in range(4):
                dst[i, c, rows, :] = combos[i][:, c * 128:(c + 1) * 128].astype(bf16)
        return token(combos[5], combos[6])

    def fold_piece(kind, c, j, pt):
        sub = lax.broadcasted_iota(jnp.int32, (8, 128), 0)
        blk = {}
        for hh in range(2):
            for kh in range(2):
                k0 = kh * HD + j * 128
                w = wqkv_v[kind * NWC + c, k0:k0 + 128, hh * 128:(hh + 1) * 128]
                f = lax.dot_general(pt[2 * c + hh], w, _NT, preferred_element_type=f32)
                refs = []
                for pp in range(2):
                    ref = jnp.where(sub >= 6, f[pp * 8:(pp + 1) * 8], 0.0)
                    ref = ref + pltpu.roll(ref, 2, 0)
                    refs.append(ref + pltpu.roll(ref, 4, 0))
                blk[hh, kh] = f - jnp.concatenate(refs + [refs[0]] * 7 + [refs[1]] * 7, axis=0)
        combos = _left_combos(blk[0, 0], blk[0, 1], blk[1, 0], blk[1, 1])
        r0 = kind * HD + c * 128
        for i in range(7):
            wt_v[i, j, r0:r0 + 128, :] = combos[i].astype(bf16)
            we_v[kind, i, j, c * 16:(c + 1) * 16, :] = combos[i][0:16].astype(bf16)

    def fold_chunk(kind, c, pt):
        for j in range(4):
            fold_piece(kind, c, j, pt)

    def vprep_piece(c, j, m):
        wqkv_v[zs + 3 * NWC, 0:8, 0:128] = m[0:8, 0:128].astype(bf16)
        blk = {}
        for hh in range(2):
            for kh in range(2):
                k0 = kh * HD + j * 128
                w = wqkv_v[V_ * NWC + c, k0:k0 + 128, hh * 128:(hh + 1) * 128]
                blk[hh, kh] = w.T.astype(f32)
        combos = _left_combos(blk[0, 0], blk[0, 1], blk[1, 0], blk[1, 1])
        r0 = V_ * HD + c * 128
        for i in range(7):
            wt_v[i, j, r0:r0 + 128, :] = combos[i].astype(bf16)
        return token(combos[1], combos[4])

    def wo_piece(w0, m):
        wo_v[D:D + 8, 0:128] = m[0:8, 0:128].astype(bf16)
        top = wo_v[pl.ds(pl.multiple_of(w0, 16), 16), :].astype(f32)
        bot = wo_v[pl.ds(pl.multiple_of(HD + w0, 16), 16), :].astype(f32)
        combos = _right_combos(top[:, :HD], top[:, HD:], bot[:, :HD], bot[:, HD:])
        for i in range(7):
            for c in range(4):
                wo7_v[i, c, pl.ds(pl.multiple_of(w0, 16), 16), :] = (
                    combos[i][:, c * 128:(c + 1) * 128].astype(bf16))
        return token(combos[5], combos[6])

    def z_piece(j, first, m):
        phik_v[0, zrows(2 * D, 16, 16), :] = m[0:16, 0:128].astype(bf16)
        ph = _unpack(tiles(phik_v, j * 128, 128)).astype(f32)
        part = (ph[:, 0:128] + ph[:, 128:256]) + (ph[:, 256:384] + ph[:, 384:512])
        z = jnp.sum(part.astype(bf16).T.astype(f32).reshape(16, 8, 128), axis=0)
        for sh in (4, 2, 1):
            z = z + pltpu.roll(z, sh, 0)
        if first:
            kv_acc[j, 64:72, :] = z
        else:
            z = kv_acc[j, 64:72, :] + z
            kv_acc[j, 64:72, :] = z
            odd = lax.broadcasted_iota(jnp.int32, (8, 128), 1) % 2
            kvt_v[j, 64:80, :] = jnp.concatenate(
                [jnp.where(odd == hl, z, 0.0) for hl in range(2)], axis=0).astype(bf16)
        return token(z)

    def run_rounds(t0, rounds, post, first):
        count = [0]
        pins = {}

        def run_jobs(m):
            for fn, span in post.get(count[0], ()):
                tok = fn(m)
                if span:
                    pins.setdefault(count[0] + span, []).append(tok())
            count[0] += 1

        for par, kind, cs in rounds:
            r0 = kind * HD + cs[0] * 128
            rows = 128 * len(cs)

            def prod(i):
                if (par, kind) == (1, V_):
                    rhs = sc7_v[i]
                else:
                    rhs = tiles(s_v[par].at[i], 0, HT1)
                if (par, kind, cs[0]) == (1, K_, 0):
                    sc7_v[i, zrows(0, HT1 // 2), :] = rhs
                if len(cs) == NWC:
                    lhs = jnp.concatenate(
                        [wl_v[kind, i]] + [tiles(wt_v.at[i], r0 + c * 128 + 16, 2 * MAIN)
                                           for c in cs], axis=0)
                else:
                    lhs = tiles(wt_v.at[i], r0, rows)
                m = lax.dot_general(_unpack(lhs),
                                    _unpack(_or_into(rhs, pins.get(count[0]))),
                                    _NT, preferred_element_type=f32)
                run_jobs(m)
                return m

            def emit(rh, ch, blk):
                tb = 2 * par + ch
                for n, c in enumerate(cs):
                    for jj in range(2):
                        pair = 4 * c + 2 * rh + jj
                        if kind == V_:
                            p = blk[n * 128 + jj * 64:n * 128 + (jj + 1) * 64]
                        elif len(cs) == NWC:
                            sub = lax.broadcasted_iota(jnp.int32, (8, HT1), 0)
                            ends = [blk[k * 16 + jj * 8:k * 16 + jj * 8 + 8] for k in range(3)]
                            if c < 3:
                                end = ends[c]
                            else:
                                end = jnp.where(
                                    sub < 2, pltpu.roll(ends[0], 2, 0),
                                    jnp.where(sub < 4, pltpu.roll(ends[1], 4, 0),
                                              pltpu.roll(ends[2], 6, 0)))
                            q0 = 48 + (2 * n + jj) * MAIN
                            p = jnp.concatenate(
                                [blk[q0:q0 + MAIN], jnp.where(sub < 6, end, 0.0)], axis=0)
                        else:
                            q0, q1 = n * 128 + 16 + jj * MAIN, n * 128 + jj * 8
                            p = jnp.concatenate([blk[q0:q0 + MAIN], blk[q1:q1 + 8]], axis=0)
                        if kind == K_:
                            phik_v[tb, zrows(pair * 128, 128, 16), :] = _dual_softmax(p)
                        elif kind == Q_:
                            phiq_v[t0 // 2, tb, pair * 128:(pair + 1) * 128, :] = (
                                _dual_softmax(p))
                        else:
                            vt_v[pair // 8][tb, zrows((pair % 8) * 64, 64, 16), :] = (
                                p.astype(bf16))

            _strassen(prod, emit)

        kr = lax.broadcasted_iota(jnp.int32, (64, 128), 0)
        kc = lax.broadcasted_iota(jnp.int32, (64, 128), 1)
        kmask = kr // 32 == kc % 2
        for j in range(NP):
            lhs = tiles(vt_v[j // 8], (j % 8) * 64, 64)
            rhs = tiles(phik_v, j * 128, 128)
            upd = lax.dot_general(_unpack(lhs), _unpack(_or_into(rhs, pins.get(count[0]))), _NT,
                                  preferred_element_type=f32)
            run_jobs(upd)
            if first:
                kv_acc[j, 0:64, :] = upd
            else:
                upd = kv_acc[j, 0:64, :] + upd
                kv_acc[j, 0:64, :] = upd
                kvt_v[j, 0:64, :] = jnp.where(kmask, upd * (1.0 / LOG2E), 0.0).astype(bf16)

    def load_best():
        return best_v[0], besti_v[...], best_v[1], best_v[2]

    def store_best(best):
        best_v[0], besti_v[...], best_v[1], best_v[2] = best

    def build_pt(g0, g1):
        def row_ids(r):
            pair = jnp.where(r < 16, r // 8, jnp.where(r < 16 + MAIN, 0, 1))
            feat = jnp.where(r < 16, MAIN + r % 8, r - 16 - pair * MAIN) // 2
            return pair, feat

        n = g1 - g0
        w2 = wphi_v[4 * g0:4 * g1].reshape(n * 128, DH)
        er = lax.broadcasted_iota(jnp.int32, (128, DH), 0)
        ec = lax.broadcasted_iota(jnp.int32, (128, DH), 1)
        e = jnp.where(ec == row_ids(er)[1], 1.0, 0.0).astype(bf16)
        ptf = lax.dot_general(e, w2, _NT, preferred_element_type=f32)
        pr = lax.broadcasted_iota(jnp.int32, (128, 128), 0)
        pc = lax.broadcasted_iota(jnp.int32, (128, 128), 1)
        keep = pc // 32 == row_ids(pr)[0] * 2 + pr % 2
        return [jnp.where(keep, ptf[:, g * 128:(g + 1) * 128], 0.0).astype(bf16)
                for g in range(n)]

    def compact(kind, i, m):
        we_v[0, 0, 0, zrows(64, 16, 16), :] = m[0:16, 0:128].astype(bf16)
        sub = lax.broadcasted_iota(jnp.int32, (8, HD), 0)
        ends = tiles(we_v.at[kind, i], 0, 64)
        for c in range(NWC - 1):
            wl_v[kind, i, zrows(c * 8, 8), :] = jnp.where(
                sub % 4 == 3, pltpu.roll(ends[24:32], 3 - c, 0), ends[c * 8:(c + 1) * 8])

    hbl_v[...] = jnp.zeros_like(hbl_v)
    hbr_v[...] = jnp.zeros_like(hbr_v)
    store_best((jnp.full((8, 128), -jnp.inf, f32), jnp.zeros((8, 128), jnp.int32),
                jnp.zeros((8, 128), f32), jnp.zeros((8, 128), f32)))
    n_ln = HT1 // LN_ROWS
    x0_copy(0).wait()
    x0_copy(1).wait()
    for p in range(n_ln // 2):
        ln1_piece(0, s_v[0], p)
    full_copy(wr_hbm, wr_v, SEM_WR).wait()
    phi_copy(0).wait()
    x0_copy(2).wait()
    x0_copy(3).wait()
    wr_row = wr_v[...].astype(f32).reshape(1, D)
    wrf_v[...] = jnp.broadcast_to(
        wr_row - jnp.sum(wr_row, axis=-1, keepdims=True) * (1.0 / D), (8, D))
    pt = build_pt(0, 4)
    for p in range(n_ln // 2, n_ln):
        ln1_piece(0, s_v[0], p)
    for part in range(2):
        k0_copy(2 * part).wait()
        k0_copy(2 * part + 1).wait()
        fold_piece(K_, 0, 2 * part, pt)
        fold_piece(K_, 0, 2 * part + 1, pt)

    def add_at(post, slot, fn, span=0):
        half = slot != int(slot)
        post.setdefault(int(slot), []).append(
            (lambda m: fn(m[m.shape[0] // 32 * 16:] if half else m), span))

    post = {}

    def at(slot, fn, span=0):
        add_at(post, slot, fn, span)

    for slot, copies in T0_WAITS:
        for cp in copies:
            if cp == 'phi':
                at(slot, lambda m: phi_copy(1).wait())
            elif cp in ('x1', 'x2', 'x3'):
                at(slot, lambda m, cp=cp: x_copy(int(cp[1])).wait())
            else:
                at(slot, lambda m, cp=cp: w_copy(cp // NWC, cp % NWC).wait())
    for n in range(1, 2 * NWC):
        if n == 2:
            at(T0_FOLD[n], lambda m: pt.extend(build_pt(4, 8)))
        at(T0_FOLD[n], lambda m, n=n: fold_chunk(n // NWC, n % NWC, pt))
    for kind in (K_, Q_):
        for i in range(7):
            at(T0_COMPACT[kind] + i, lambda m, kind=kind, i=i: compact(kind, i, m))
    for c in range(NWC):
        for j in range(4):
            at(T0_VPREP[c][j], lambda m, c=c, j=j: vprep_piece(c, j, m), T0_VSPAN[c])
    for p in range(n_ln):
        at(T0_LN[p], lambda m, p=p: ln1_piece(T1, s_v[1], p, m), T0_LNSPAN[p])
    for p in range(n_ln):
        at(T1_LN[0][p], lambda m, p=p: ln1_piece(2 * T1, s_v[0], p, m), P1_LNSPAN)
        at(T1_LN[1][p], lambda m, p=p: ln1_piece(3 * T1, s_v[1], p, m), P1_LNSPAN)
    for j in range(NP):
        at(T0_Z[j], lambda m, j=j: z_piece(j, True, m), T0_ZSPAN)
    lo, hi = [0, 1], [2, 3]
    run_rounds(0, [(0, kind, [c]) for kind in (K_, Q_) for c in range(NWC)]
               + [(1, K_, lo + hi), (1, Q_, lo + hi)] + [(0, V_, [c]) for c in range(NWC)]
               + [(1, V_, lo), (1, V_, hi)], post, True)
    full_copy(wo_hbm, wo_v.at[pl.ds(0, D), :], SEM_WO).wait()
    for i in range(4, N1):
        x_copy(i).wait()

    def phase1(i, carry):
        post = {}
        nxt = jnp.minimum(i + 1, N2 - 1) * T2
        w0 = jnp.minimum((i - 1) * WO_ROWS, HD - WO_ROWS)
        for par in range(2):
            for p in range(n_ln):
                add_at(post, P1_LN2[par][p],
                       lambda m, p=p, par=par: ln1_piece(nxt + par * T1, s_v[par], p, m),
                       P1_LNSPAN2[par])
        for p in range(WO_ROWS // 16):
            add_at(post, P1_WO[p], lambda m, p=p: wo_piece(w0 + 16 * p, m), P1_WOSPAN)
        for j in range(NP):
            add_at(post, P1_Z[j], lambda m, j=j: z_piece(j, False, m), P1_ZSPAN)
        run_rounds(2 * i, [(par, kind, lo + hi) for kind in (K_, Q_) for par in range(2)]
                   + [(par, V_, cs) for par in range(2) for cs in (lo, hi)], post, False)
        return carry

    lax.fori_loop(1, N1 // 2, phase1, 0)

    for _, dst, rows, slot in ffn_tiled:
        filled = dst.at[:, pl.ds(0, rows), :]
        full_copy(filled, filled, slot).wait()
    full_copy(wg_hbm.at[:, pl.ds(f0, F - f0)], wgv_v, SEM_WGV).wait()
    full_copy(wu_hbm.at[:, pl.ds(f0, F - f0)], wuv_v, SEM_WUV).wait()

    def o_copy(hf):
        return pltpu.make_async_copy(
            out_v.at[pl.ds(hf * HT2, HT2), :], out_hbm.at[0, pl.ds(hf * HT2, HT2), :],
            sem.at[SEM_O])

    def half_stats(hh, c0):
        rows = hh.shape[0]
        parts = [hh[:, c * 128:(c + 1) * 128] for c in range(4)]
        wts = [wrf_v[:, c0 + c * 128:c0 + (c + 1) * 128] for c in range(4)]
        s1 = (parts[0] + parts[1]) + (parts[2] + parts[3])
        sq = [p * p for p in parts]
        s2 = (sq[0] + sq[1]) + (sq[2] + sq[3])
        dw = [(p.reshape(rows // 8, 8, 128) * w[None]).reshape(rows, 128)
              for p, w in zip(parts, wts)]
        s3 = (dw[0] + dw[1]) + (dw[2] + dw[3])
        return s1, s2, s3

    def first_half(hbuf, sbuf, p, c0):
        r0 = p * EP_ROWS
        hh = hbuf[c0 // HD][r0:r0 + EP_ROWS, :]
        st = jnp.concatenate(half_stats(hh, c0), axis=1)
        sbuf[zrows(r0, EP_ROWS), :] = st
        return _fold_token(pltpu.bitcast(st, u32), zero_v)

    def finish(hbuf, sbuf, base, p, valid, best, defer=None):
        r0 = p * EP_ROWS
        g0 = pl.multiple_of(base + r0, EP_ROWS)
        hl, hr = [r[r0:r0 + EP_ROWS, :] for r in hbuf]
        if sbuf is None:
            st = half_stats(hr, HD)
        else:
            st = sbuf[r0:r0 + EP_ROWS, :]
            st = [st[:, n * 128:(n + 1) * 128] for n in range(3)]
        s1, s2, s3 = [jnp.sum(v + w, axis=-1, keepdims=True)
                      for v, w in zip(half_stats(hl, 0), st)]
        m = s1 * (1.0 / D)
        var = jnp.maximum(s2 * (1.0 / D) - m * m, 0.0)
        inv = lax.rsqrt(var + EPS)
        r = s3 * inv

        def write_out(h):
            o = h * (1.0 + inv) - m * inv
            out_v[pl.ds(g0, EP_ROWS), :] = o.astype(bf16)
            return o

        if defer is None:
            o = write_out(jnp.concatenate([hl, hr], axis=1))
        else:
            defer.append(lambda: write_out(jnp.concatenate(
                [r_[r0:r0 + EP_ROWS, :] for r_ in hbuf], axis=1)))
        bv, bi, bm, bq = best
        sub = lax.broadcasted_iota(jnp.int32, (8, 128), 0)
        for g in range(EP_ROWS // 8):
            rows = slice(g * 8, (g + 1) * 8)
            rg = jnp.broadcast_to(r[rows], (8, 128))
            if valid is not None:
                rg = jnp.where(valid, rg, -jnp.inf)
            better = rg > bv
            bi = jnp.where(better, sub + (g0 + g * 8), bi)
            bv = jnp.where(better, rg, bv)
            bm = jnp.where(better, jnp.broadcast_to(m[rows], (8, 128)), bm)
            bq = jnp.where(better, jnp.broadcast_to(var[rows], (8, 128)), bq)
        best = (bv, bi, bm, bq)
        if defer is not None:
            return best, None
        tok = _fold_token(pltpu.bitcast(jnp.concatenate(
            [o[:, D - 128:], bv, bm, bq], axis=0), u32), zero_v)
        return best, tok

    n_ep = HT2 // EP_ROWS

    def phase2(i, carry):
        ot = []
        for j in range(NP):
            ph = tiles(phiq_v.at[i], j * 128, 128)
            n = jnp.dot(_unpack(kvt_v.bitcast(u32)[j]), _unpack(ph),
                        preferred_element_type=f32)
            r0h = _recip(n[64:72] + 1e-6)
            r1h = _recip(n[72:80] + 1e-6)
            ot.append((n[0:32].reshape(4, 8, T2) * r0h[None]).reshape(32, T2))
            ot.append((n[32:64].reshape(4, 8, T2) * r1h[None]).reshape(32, T2))
        lo = jnp.concatenate(ot[:H // 2], axis=0)
        hi = jnp.concatenate(ot[H // 2:], axis=0)
        lcs = _left_combos(lo[:, :HT2], hi[:, :HT2], lo[:, HT2:], hi[:, HT2:])

        state = {'best': load_best()}
        pins = {}
        jobs = {}
        lts = {}
        ra = pl.multiple_of(i * T2, T2)
        rb = pl.multiple_of(i * T2 + HT2, HT2)
        prev = jnp.maximum(i * T2 - HT2, HT2)

        def add_job(slot, deadline, fn, gates=()):
            jobs.setdefault(slot, []).append((fn, deadline, gates))

        def finish_job(hbuf, sbuf, base, p, valid):
            def fn():
                state['best'], tok = finish(hbuf, sbuf, base, p, valid, state['best'])
                return tok
            return fn

        def lt_job(k):
            def fn():
                lts[k] = lcs[k].astype(bf16).T
                return _fold_token(pltpu.bitcast(lts[k], u32), zero_v)
            return fn

        order = (2, 4, 6, 0, 3, 1, 5)
        lt_job(2)()
        for n in range(1, 7):
            add_job(LT_START[n], min(LT_START[n] + LT_SPAN[n], 4 * n), lt_job(order[n]))
        for p in range(n_ep):
            add_job(FB_START[p], FB_START[p] + FB_SPAN,
                    finish_job(hb_v, None, prev, p, i > 0), hb_v)
            add_job(SA_START[p], SA_START[p] + SA_SPAN,
                    lambda p=p: first_half(ha_v, sa_v, p, HD), ha_v[1:])
            add_job(FA_START[p], FA_START[p] + FA_SPAN[p],
                    finish_job(ha_v, sa_v, ra, p, None), ha_v)

        def xblk(r0, c0):
            return x_v[pl.ds(r0, HT2), c0:c0 + 128].astype(f32)

        for n, k in enumerate(order):
            for c in range(4):
                slot = 4 * n + c
                for fn, deadline, gates in jobs.get(slot, ()):
                    for ref in gates:
                        ref[zrows(HT2, 8), 0:128] = mm[0:8]
                    pins.setdefault(deadline, []).append(fn())
                w = _or_into(wo7_v.bitcast(u32)[k, c, 0:HD // 2, :], pins.get(slot))
                mm = jnp.dot(lts[k], _unpack(w), preferred_element_type=f32)
                c0 = c * 128
                cs = slice(c0, c0 + 128)
                tmp = lambda t: tmp_v[t][:, cs]
                if n == 0:
                    tmp_v[0][zrows(0, HT2), cs] = mm
                elif n == 1:
                    ha_v[1][zrows(0, HT2), cs] = (xblk(ra, HD + c0) + tmp(0)) + mm
                    tmp_v[1][zrows(0, HT2), cs] = xblk(ra, c0) - mm
                elif n == 2:
                    tmp_v[2][zrows(0, HT2), cs] = tmp(1) + mm
                elif n == 3:
                    tmp_v[3][zrows(0, HT2), cs] = tmp(2) + mm
                    tmp_v[4][zrows(0, HT2), cs] = (xblk(rb, HD + c0) + tmp(0)) + mm
                elif n == 4:
                    ha_v[0][zrows(0, HT2), cs] = tmp(3) + mm
                    tmp_v[5][zrows(0, HT2), cs] = xblk(rb, c0) + mm
                elif n == 5:
                    hb_v[0][zrows(0, HT2), cs] = tmp(5) + mm
                    tmp_v[6][zrows(0, HT2), cs] = tmp(4) - mm
                else:
                    hb_v[1][zrows(0, HT2), cs] = tmp(6) + mm
        store_best(state['best'])
        o_copy(2 * i).start()

        @pl.when(i > 0)
        def _():
            o_copy(2 * i - 1).start()

        return carry

    lax.fori_loop(0, N2, phase2, 0)
    best = load_best()
    late = []
    for p in range(n_ep):
        best, _ = finish(hb_v, None, S - HT2, p, None, best, late)

    bv, bi, bm, bq = best
    for sh in (4, 2, 1):
        ov, oi, om, oq = [pltpu.roll(t, sh, 0) for t in (bv, bi, bm, bq)]
        take = jnp.logical_or(ov > bv, jnp.logical_and(ov == bv, oi < bi))
        bv, bi, bm, bq = [jnp.where(take, o_, t)
                          for o_, t in zip((ov, oi, om, oq), (bv, bi, bm, bq))]
    idx = jnp.clip(bi[0, 0], 0, S - 1)
    for r_ in hb_v:
        r_[zrows(HT2, 8), 0:128] = bv
    for p, fn in enumerate(late):
        if LATE_AT[p] < 0:
            fn()
    b0 = pl.multiple_of((idx // 8) * 8, 8)
    t = _rb(_rb(bq) + EPS)
    inv = _recip(_rb(t * lax.rsqrt(t)))
    gate = _sigmoid(bv)
    wide = lambda v: jnp.concatenate([v] * (D // 128), axis=1)
    b1 = pl.multiple_of(jnp.minimum(b0, S - HT2 - 8), 8)
    b2 = pl.multiple_of(jnp.maximum(b0 - (S - HT2), 0), 8)
    early = wide(bi) < S - HT2
    src = jnp.where(early, out_v[pl.ds(b1, 8), :].astype(f32),
                    jnp.concatenate([r_[pl.ds(b2, 8), :] for r_ in hb_v], axis=1))
    scale = jnp.where(bi < S - HT2, inv * _recip(1.0 + lax.rsqrt(bq + EPS)), inv)
    hn = (src - wide(bm)) * wide(scale)
    xs = hn.astype(bf16)
    rows = lax.broadcasted_iota(jnp.int32, (8, D), 0) + b0

    xm = jnp.where(rows == wide(bi), hn, 0.0)
    for sh in (4, 2, 1):
        xm = xm + pltpu.roll(xm, sh, 0)
    for t in range(D // 128):
        xcol_v[t // 2][zrows((t % 2) * 128, 128), :] = jnp.concatenate(
            [xm[:, t * 128:(t + 1) * 128]] * 16, axis=0).astype(bf16).T.astype(f32)

    nblk = F // 256
    nmx = nblk - FFN_VPU_BLOCKS
    act = {}
    acc = {}

    def activate(g, u):
        return (g * _sigmoid(g) * u).astype(bf16)

    parts = D // 8 // FFN_KG

    def vpu_chunk(q):
        blk, part = nmx + q // parts, q % parts
        cur = acc.get(blk)
        for kg in range(part * FFN_KG, (part + 1) * FFN_KG):
            xc = xcol_v[kg // 32][(kg % 32) * 8:(kg % 32 + 1) * 8, :]
            w = jnp.concatenate(
                [r[kg * 8:(kg + 1) * 8, (blk - nmx) * 256:(blk - nmx + 1) * 256].astype(f32)
                 for r in (wgv_v, wuv_v)], axis=1)
            p = w * jnp.concatenate([xc] * 4, axis=1)
            cur = p if cur is None else cur + p
        acc[blk] = cur
        if part == parts - 1:
            for sh in (4, 2, 1):
                cur = cur + pltpu.roll(cur, sh, 0)
            act[blk] = activate(cur[:, :256], cur[:, 256:])
        c = q % 4
        return _fold_token(pltpu.bitcast(cur[:, c * 128:(c + 1) * 128], u32), zero_v)

    nchunk = FFN_VPU_BLOCKS * parts
    starts = [FFN_W0 + (q * (FFN_W1 - FFN_W0)) // (nchunk - 1) for q in range(nchunk)]
    pins = {}
    wave = [0]
    wgw, wuw, wdw = [r.bitcast(u32) for r in (wg_v, wu_v, wd_v)]

    def run_wave(lhs, tls):
        w = jnp.concatenate([_or_into(tls[0], pins.get(wave[0]))] + tls[1:], axis=1)
        out = jnp.dot(lhs, _unpack(w), preferred_element_type=f32)
        for p, fn in enumerate(late):
            if LATE_AT[p] == wave[0]:
                for r_ in hb_v:
                    r_[zrows(HT2, 8), 0:128] = out[:, 0:128]
                fn()
        for q, start in enumerate(starts):
            if start == wave[0]:
                pins.setdefault(wave[0] + FFN_SPAN, []).append(vpu_chunk(q))
        if wave[0] == FFN_LATE:
            o_copy(2 * N2 - 1).start()
            out_v[zrows(S, 16, 16), 0:256] = jnp.zeros((16, 256), bf16)
            pins.setdefault(wave[0] + 4, []).append(
                token(out_v[S:S + 8, 0:128].astype(f32))())
        wave[0] += 1
        return out

    for j in range(nmx):
        gu = None
        for kt in range(D // 128):
            p = run_wave(xs[:, kt * 128:(kt + 1) * 128],
                         [r[2 * j + c, kt * 64:(kt + 1) * 64, :]
                          for r in (wgw, wuw) for c in range(2)])
            gu = p if gu is None else gu + p
        act[j] = activate(gu[:, :256], gu[:, 256:])
    ys = [None, None]
    for j in range(nblk):
        for kt in range(2):
            for hf in range(2):
                r0 = (2 * j + kt) * 64
                p = run_wave(act[j][:, kt * 128:(kt + 1) * 128],
                             [wdw[4 * hf + c, r0:r0 + 64, :] for c in range(4)])
                ys[hf] = p if ys[hf] is None else ys[hf] + p
    y = jnp.concatenate(ys, axis=1)
    cur = out_v[pl.ds(b0, 8), :].astype(f32)
    fix_v[...] = jnp.where(rows == wide(bi), cur + y * wide(gate), cur).astype(bf16)
    full_copy(out_v.at[pl.ds(0, S), :], out_hbm.at[0], SEM_O).wait()
    fix = pltpu.make_async_copy(fix_v, out_hbm.at[0, pl.ds(b0, 8), :], sem.at[SEM_O])
    fix.start()
    fix.wait()


def _kernel(*refs):
    def step(i, carry):
        @pl.when(i == 0)
        def _():
            _body(i, *refs)

        return carry

    lax.fori_loop(0, 2, step, 0)


@jax.jit
def pallas_sequential_preLN__linear_kernel_hedgehog__moe_arch_mod__prompt_kernel(
    A_x: jax.Array,
    A_wqkv: jax.Array,
    A_w_phi: jax.Array,
    A_wo: jax.Array,
    B_x: jax.Array,
    B_w_r: jax.Array,
    B_w_gate: jax.Array,
    B_w_up: jax.Array,
    B_w_down: jax.Array,
):
    any_spec = pl.BlockSpec(memory_space=pl.ANY)
    return pl.pallas_call(
        _kernel,
        out_shape=jax.ShapeDtypeStruct((1, S, D), bf16),
        in_specs=[any_spec] * 8,
        out_specs=any_spec,
        scratch_shapes=[
            pltpu.VMEM((S + 16, D), bf16),
            pltpu.VMEM((3 * NWC + 1, D, WC), bf16),
            pltpu.VMEM((H, DH, DH), bf16),
            pltpu.VMEM((D + 16, D), bf16),
            pltpu.VMEM((D,), bf16),
            pltpu.VMEM((F // 128 - 2 * FFN_VPU_BLOCKS, D + PAD, 128), bf16),
            pltpu.VMEM((F // 128 - 2 * FFN_VPU_BLOCKS, D + PAD, 128), bf16),
            pltpu.VMEM((D // 128, F + PAD, 128), bf16),
            pltpu.VMEM((D, 256 * FFN_VPU_BLOCKS), bf16),
            pltpu.VMEM((D, 256 * FFN_VPU_BLOCKS), bf16),
            pltpu.VMEM((7, 4, 3 * HD + PAD, 128), bf16),
            pltpu.VMEM((2, 7, 4, 64 + PAD, 128), bf16),
            pltpu.VMEM((2, 7, 24, HD), u32),
            pltpu.VMEM((7, 4, HD + PAD, 128), bf16),
            pltpu.VMEM((7, 4, HT1 + PAD, 128), bf16),
            pltpu.VMEM((7, 4, HT1 + PAD, 128), bf16),
            pltpu.VMEM((7, HT1 // 2, HD), u32),
            pltpu.VMEM((N2, 4, 2 * D + PAD, 128), bf16),
            pltpu.VMEM((4, 2 * D + PAD, 128), bf16),
            pltpu.VMEM((4, HD + PAD, 128), bf16),
            pltpu.VMEM((4, HD + PAD, 128), bf16),
            pltpu.VMEM((NP, 72, 128), f32),
            pltpu.VMEM((NP, 80, 128), bf16),
            *[pltpu.VMEM((HT2 + 8, HD), f32) for _ in range(4)],
            pltpu.VMEM((HT2, 384), f32),
            *[pltpu.VMEM((HT2, HD), f32) for _ in range(7)],
            pltpu.VMEM((S + 16, D), bf16),
            pltpu.VMEM((8, D), f32),
            pltpu.VMEM((3, 8, 128), f32),
            pltpu.VMEM((8, 128), jnp.int32),
            pltpu.VMEM((8, D), bf16),
            *[pltpu.VMEM((256, 128), f32) for _ in range(4)],
            pltpu.SemaphoreType.DMA((NSEM,)),
        ],
        compiler_params=pltpu.CompilerParams(
            vmem_limit_bytes=110 * 1024 * 1024,
            disable_bounds_checks=True,
            disable_semaphore_checks=True),
    )(A_x, A_wqkv, A_w_phi, A_wo, B_w_r, B_w_gate, B_w_up, B_w_down)
```

```python
import jax
import jax.numpy as jnp
from jax import lax
import jax.experimental.pallas as pl
import jax.experimental.pallas.tpu as pltpu

S = 2048
D = 1024
H = 32
DH = 32
F = 3584
NP = H // 2
T1 = 256
T2 = 512
N1 = S // T1
N2 = S // T2
HT1 = T1 // 2
HT2 = T2 // 2
QT2 = T2 // 4
HD = D // 2
WC = 256
NWC = D // WC
LOG2E = 1.4426950408889634
EPS = 1e-5
PAD = 16
WO_ROWS = 176
LN_ROWS = 16
MAIN = 56
EP_ROWS = 32

T0_FOLD = (0, 4, 11, 18, 25, 33, 39, 46)
T0_WAITS = ((4, (1,)), (11, ('phi', 2)), (18, (3, 4)), (33, ('x1', 5, 6)), (46, (7,)),
            (65, (8, 9, 10, 11, 'x2', 'x3')))
T0_VPREP = ((65, 66, 66.5, 68), (68.5, 69, 70, 74), (74, 76, 78, 79), (81, 83, 84, 86))
T0_COMPACT = (22, 47)
T0_VSPAN = (2, 5, 5, 4)
T0_LN = (33, 33, 35, 35, 36, 38, 40, 45)
T0_LNSPAN = (3, 4, 0, 0, 0, 0, 0, 0)
T1_LN = ((102, 103, 104, 105, 106, 107, 108, 109), (89, 91, 93, 95, 97, 99, 100, 101))
P1_LNSPAN = 5
T0_Z = (63, 63.5, 64, 70.5, 73, 77.5, 79, 84, 94, 95.5, 98, 98, 99.5, 100.5, 105, 107)
T0_ZSPAN = 0
P1_WO = (30, 30, 32, 33, 36, 49, 51, 52, 53, 53, 55)
P1_WOSPAN = 3
P1_LN2 = ((42, 43, 44, 45, 46, 47, 49, 51), (34, 35, 35, 37, 38, 39, 41, 42))
P1_LNSPAN2 = (3, 3)
P1_Z = (28, 30, 31, 33, 36, 38, 40, 42, 43, 44, 46, 47, 48, 51, 52, 53)
P1_ZSPAN = 2
LT_START = (0, 0, 1, 5, 9, 13, 16, 19, 25, 30, 33, 37, 42, 44)
LT_SPAN = (5, 4, 7, 6, 9, 6, 6, 6, 6, 6, 4, 6, 6, 6)
FB_START = ((4, 8, 12, 16), (33, 36, 40, 44))
FB_SPAN = 4
SA_START = ((10, 10, 18, 19), (38, 41, 45, 46))
SA_SPAN = 6
FA_START = ((21, 23, 26, 29), (49, 51, 52, 55))
FA_SPAN = ((4, 4, 4, 3), (5, 5, 9, 9))
FFN_VPU_BLOCKS = 7
FFN_KG = 32
FFN_W0 = 16
FFN_W1 = 107
FFN_SPAN = 4
FFN_LATE = 16
LATE_AT = (-1, 0, 2, 3)

_NT = (((1,), (1,)), ((), ()))
f32 = jnp.float32
bf16 = jnp.bfloat16
u32 = jnp.uint32

K_, Q_, V_ = 0, 1, 2
SRC = {K_: 1, Q_: 0, V_: 2}

SEM_W = 0
SEM_X = SEM_W + 3 * NWC
SEM_X0 = SEM_X + N1
SEM_K0 = SEM_X0 + 4
SEM_PHI = SEM_K0 + 4
SEM_WO = SEM_PHI + 2
SEM_WR, SEM_WG, SEM_WU, SEM_WD, SEM_WGV, SEM_WUV, SEM_O = (SEM_WO + 1 + i for i in range(7))
NSEM = SEM_O + 1


def _rb(v):
    return v.astype(bf16).astype(f32)


def _unpack(w):
    return pltpu.bitcast(w, bf16)


def _mo(i, n):
    return i if isinstance(i, int) else pl.multiple_of(i, n)


def _recip(x):
    r = pl.reciprocal(x, approx=True)
    return r * (2.0 - x * r)


def _sigmoid(x):
    return _recip(1.0 + jnp.exp(jnp.minimum(-x, 80.0)))


def _dual_softmax(p):
    t = p.shape[-1]
    p3 = p.reshape(8, 8, t)

    def allred(v, op):
        v = op(v, pltpu.roll(v, 2, 0))
        return op(v, pltpu.roll(v, 4, 0))

    mx = allred(jnp.max(p3, axis=0), jnp.maximum)
    mn = allred(jnp.min(p3, axis=0), jnp.minimum)
    ep = jnp.exp2(p3 - mx[None])
    en = jnp.exp2(mn[None] - p3)
    sp = allred(jnp.sum(ep, axis=0), jnp.add)
    sn = allred(jnp.sum(en, axis=0), jnp.add)
    fp = (ep * _recip(sp)[None]).reshape(64, t)
    fn = (en * _recip(sn)[None]).reshape(64, t)
    return jnp.concatenate([fp, fn], axis=0).astype(bf16)


def _left_combos(a11, a12, a21, a22):
    return [a11 + a22, a21 + a22, a11, a22, a11 + a12, a21 - a11, a12 - a22]


def _right_combos(b11, b12, b21, b22):
    return [b11 + b22, b11, b12 - b22, b21 - b11, b22, b11 + b12, b21 + b22]


def _strassen(prod, emit):
    m3 = prod(2)
    m5 = prod(4)
    emit(0, 1, m3 + m5)
    m7 = prod(6)
    u = m7 - m5
    m1 = prod(0)
    u = u + m1
    w = m1 + m3
    m4 = prod(3)
    emit(0, 0, u + m4)
    m2 = prod(1)
    emit(1, 0, m2 + m4)
    w = w - m2
    m6 = prod(5)
    emit(1, 1, w + m6)


def _or_into(w, toks):
    if not toks:
        return w
    top = w[0:8, 0:128]
    for tk in toks:
        top = top | tk
    if w.shape[1] > 128:
        top = jnp.concatenate([top, w[0:8, 128:]], axis=1)
    return jnp.concatenate([top, w[8:]], axis=0)


def _fold_token(w, zero):
    r, c = w.shape
    acc = None
    for i in range(r // 8):
        for j in range(c // 128):
            blk = w[i * 8:(i + 1) * 8, j * 128:(j + 1) * 128]
            acc = blk if acc is None else acc | blk
    return acc & zero


def _body(zs, x_hbm, wqkv_hbm, wphi_hbm, wo_hbm, wr_hbm, wg_hbm, wu_hbm, wd_hbm, out_hbm,
          x_v, wqkv_v, wphi_v, wo_v, wr_v, wg_v, wu_v, wd_v, wgv_v, wuv_v,
          wt_v, we_v, wl_v, wo7_v, sa7_v, sb7_v, sc7_v, phiq_v, phik_v, vt0_v, vt1_v, kv_acc, kvt_v,
          hal_v, har_v, hbl_v, hbr_v, sa_v, t0_v, t1_v, t2_v, t3_v, t4_v, t5_v, t6_v,
          out_v, wrf_v, best_v, besti_v, fix_v, xc0_v, xc1_v, xc2_v, xc3_v, sem):
    xcol_v = (xc0_v, xc1_v, xc2_v, xc3_v)
    s_v = (sa7_v, sb7_v)
    vt_v = (vt0_v, vt1_v)
    ha_v = (hal_v, har_v)
    hb_v = (hbl_v, hbr_v)
    tmp_v = (t0_v, t1_v, t2_v, t3_v, t4_v, t5_v, t6_v)

    def x_rows(r0, rows, slot):
        return pltpu.make_async_copy(
            x_hbm.at[0, pl.ds(r0, rows), :], x_v.at[pl.ds(r0, rows), :], sem.at[slot])

    def x_copy(i):
        return x_rows(i * T1, T1, SEM_X + i)

    def x0_copy(q):
        return x_rows((q % 2) * HT1 + (q // 2) * (HT1 // 2), HT1 // 2, SEM_X0 + q)

    def w_copy(kind, c):
        return pltpu.make_async_copy(
            wqkv_hbm.at[:, pl.ds(SRC[kind] * D + c * WC, WC)],
            wqkv_v.at[kind * NWC + c], sem.at[SEM_W + kind * NWC + c])

    def k0_copy(q):
        r0 = (q % 2) * HD + (q // 2) * 256
        return pltpu.make_async_copy(
            wqkv_hbm.at[pl.ds(r0, 256), pl.ds(SRC[K_] * D, WC)],
            wqkv_v.at[K_ * NWC, pl.ds(r0, 256), :], sem.at[SEM_K0 + q])

    def phi_copy(part):
        lo, n = part * (H // 2), H // 2
        return pltpu.make_async_copy(wphi_hbm.at[pl.ds(lo, n)], wphi_v.at[pl.ds(lo, n)],
                                     sem.at[SEM_PHI + part])

    def full_copy(src, dst, slot):
        return pltpu.make_async_copy(src, dst, sem.at[slot])

    x0_copy(0).start()
    x0_copy(1).start()
    full_copy(wr_hbm, wr_v, SEM_WR).start()
    phi_copy(0).start()
    x0_copy(2).start()
    x0_copy(3).start()
    for q in range(4):
        k0_copy(q).start()
    w_copy(K_, 1).start()
    phi_copy(1).start()
    w_copy(K_, 2).start()
    w_copy(K_, 3).start()
    w_copy(Q_, 0).start()
    x_copy(1).start()
    for c in range(1, NWC):
        w_copy(Q_, c).start()
    for c in range(NWC):
        w_copy(V_, c).start()
    x_copy(2).start()
    x_copy(3).start()
    full_copy(wo_hbm, wo_v.at[pl.ds(0, D), :], SEM_WO).start()
    for i in range(4, N1):
        x_copy(i).start()
    f0 = F - 256 * FFN_VPU_BLOCKS
    ffn_tiled = ((wg_hbm, wg_v, D, SEM_WG), (wu_hbm, wu_v, D, SEM_WU), (wd_hbm, wd_v, F, SEM_WD))
    for src, dst, rows, slot in ffn_tiled:
        for c in range(dst.shape[0]):
            full_copy(src.at[:, pl.ds(c * 128, 128)], dst.at[c, pl.ds(0, rows), :], slot).start()
    full_copy(wg_hbm.at[:, pl.ds(f0, F - f0)], wgv_v, SEM_WGV).start()
    full_copy(wu_hbm.at[:, pl.ds(f0, F - f0)], wuv_v, SEM_WUV).start()

    zero_v = jnp.full((8, 128), zs, jnp.int32).astype(u32)

    def zrows(r0, rows, mult=8):
        return pl.ds(pl.multiple_of(zs * mult + r0, mult), rows)

    def tiles(ref, r0, rows):
        w = ref.bitcast(u32)
        return jnp.concatenate(
            [w[c, r0 // 2:(r0 + rows) // 2, :] for c in range(ref.shape[0])], axis=1)

    def token(*vals):
        return lambda: _fold_token(pltpu.bitcast(jnp.concatenate(vals, axis=0), u32), zero_v)

    def ln1_stats(xf):
        m = jnp.sum(xf, axis=-1, keepdims=True) * (1.0 / D)
        q = jnp.sum(xf * xf, axis=-1, keepdims=True) * (1.0 / D)
        inv = lax.rsqrt(jnp.maximum(q - m * m, 0.0) + EPS) * LOG2E
        return inv, m * inv

    def ln1_piece(r0, dst, p, m=None):
        fixed = isinstance(r0, int)
        if m is not None:
            x_v[zrows(S, 8) if fixed else pl.ds(S, 8), 0:128] = m[0:8, 0:128].astype(bf16)
        xa, xb = [x_v[pl.ds(_mo(r0 + hf * HT1 + p * LN_ROWS, LN_ROWS), LN_ROWS), :]
                  .astype(f32) for hf in range(2)]
        (ia, ma), (ib, mb) = ln1_stats(xa), ln1_stats(xb)
        ya, yb = xa * ia, xb * ib
        s2 = ya[:, :HD] - ma
        s5 = yb[:, HD:] - mb
        s1 = s2 + s5
        s3 = yb[:, :HD] - yb[:, HD:]
        s4 = ya[:, HD:] - ya[:, :HD]
        combos = [s1, s2, s3, s4, s5, s1 + s3, s1 + s4]
        rows = zrows(p * LN_ROWS, LN_ROWS, 16) if fixed else pl.ds(p * LN_ROWS, LN_ROWS)
        for i in range(7):
            for c in range(4):
                dst[i, c, rows, :] = combos[i][:, c * 128:(c + 1) * 128].astype(bf16)
        return token(combos[5], combos[6])

    def fold_piece(kind, c, j, pt):
        sub = lax.broadcasted_iota(jnp.int32, (8, 128), 0)
        blk = {}
        for hh in range(2):
            for kh in range(2):
                k0 = kh * HD + j * 128
                w = wqkv_v[kind * NWC + c, k0:k0 + 128, hh * 128:(hh + 1) * 128]
                f = lax.dot_general(pt[2 * c + hh], w, _NT, preferred_element_type=f32)
                refs = []
                for pp in range(2):
                    ref = jnp.where(sub >= 6, f[pp * 8:(pp + 1) * 8], 0.0)
                    ref = ref + pltpu.roll(ref, 2, 0)
                    refs.append(ref + pltpu.roll(ref, 4, 0))
                blk[hh, kh] = f - jnp.concatenate(refs + [refs[0]] * 7 + [refs[1]] * 7, axis=0)
        combos = _left_combos(blk[0, 0], blk[0, 1], blk[1, 0], blk[1, 1])
        r0 = kind * HD + c * 128
        for i in range(7):
            wt_v[i, j, r0:r0 + 128, :] = combos[i].astype(bf16)
            we_v[kind, i, j, c * 16:(c + 1) * 16, :] = combos[i][0:16].astype(bf16)

    def fold_chunk(kind, c, pt):
        for j in range(4):
            fold_piece(kind, c, j, pt)

    def vprep_piece(c, j, m):
        wqkv_v[zs + 3 * NWC, 0:8, 0:128] = m[0:8, 0:128].astype(bf16)
        blk = {}
        for hh in range(2):
            for kh in range(2):
                k0 = kh * HD + j * 128
                w = wqkv_v[V_ * NWC + c, k0:k0 + 128, hh * 128:(hh + 1) * 128]
                blk[hh, kh] = w.T.astype(f32)
        combos = _left_combos(blk[0, 0], blk[0, 1], blk[1, 0], blk[1, 1])
        r0 = V_ * HD + c * 128
        for i in range(7):
            wt_v[i, j, r0:r0 + 128, :] = combos[i].astype(bf16)
        return token(combos[1], combos[4])

    def wo_piece(w0, m):
        wo_v[D:D + 8, 0:128] = m[0:8, 0:128].astype(bf16)
        top = wo_v[pl.ds(pl.multiple_of(w0, 16), 16), :].astype(f32)
        bot = wo_v[pl.ds(pl.multiple_of(HD + w0, 16), 16), :].astype(f32)
        combos = _right_combos(top[:, :HD], top[:, HD:], bot[:, :HD], bot[:, HD:])
        for i in range(7):
            for c in range(4):
                wo7_v[i, c, pl.ds(pl.multiple_of(w0, 16), 16), :] = (
                    combos[i][:, c * 128:(c + 1) * 128].astype(bf16))
        return token(combos[5], combos[6])

    def z_piece(j, first, m):
        phik_v[0, zrows(2 * D, 16, 16), :] = m[0:16, 0:128].astype(bf16)
        ph = _unpack(tiles(phik_v, j * 128, 128)).astype(f32)
        part = (ph[:, 0:128] + ph[:, 128:256]) + (ph[:, 256:384] + ph[:, 384:512])
        z = jnp.sum(part.astype(bf16).T.astype(f32).reshape(16, 8, 128), axis=0)
        for sh in (4, 2, 1):
            z = z + pltpu.roll(z, sh, 0)
        if first:
            kv_acc[j, 64:72, :] = z
        else:
            z = kv_acc[j, 64:72, :] + z
            kv_acc[j, 64:72, :] = z
            odd = lax.broadcasted_iota(jnp.int32, (8, 128), 1) % 2
            kvt_v[j, 64:80, :] = jnp.concatenate(
                [jnp.where(odd == hl, z, 0.0) for hl in range(2)], axis=0).astype(bf16)
        return token(z)

    def run_rounds(t0, rounds, post, first):
        count = [0]
        pins = {}

        def run_jobs(m):
            for fn, span in post.get(count[0], ()):
                tok = fn(m)
                if span:
                    pins.setdefault(count[0] + span, []).append(tok())
            count[0] += 1

        for par, kind, cs in rounds:
            r0 = kind * HD + cs[0] * 128
            rows = 128 * len(cs)

            def prod(i):
                if (par, kind) == (1, V_):
                    rhs = sc7_v[i]
                else:
                    rhs = tiles(s_v[par].at[i], 0, HT1)
                if (par, kind, cs[0]) == (1, K_, 0):
                    sc7_v[i, zrows(0, HT1 // 2), :] = rhs
                if len(cs) == NWC:
                    lhs = jnp.concatenate(
                        [wl_v[kind, i]] + [tiles(wt_v.at[i], r0 + c * 128 + 16, 2 * MAIN)
                                           for c in cs], axis=0)
                else:
                    lhs = tiles(wt_v.at[i], r0, rows)
                m = lax.dot_general(_unpack(lhs),
                                    _unpack(_or_into(rhs, pins.get(count[0]))),
                                    _NT, preferred_element_type=f32)
                run_jobs(m)
                return m

            def emit(rh, ch, blk):
                tb = 2 * par + ch
                for n, c in enumerate(cs):
                    for jj in range(2):
                        pair = 4 * c + 2 * rh + jj
                        if kind == V_:
                            p = blk[n * 128 + jj * 64:n * 128 + (jj + 1) * 64]
                        elif len(cs) == NWC:
                            sub = lax.broadcasted_iota(jnp.int32, (8, HT1), 0)
                            ends = [blk[k * 16 + jj * 8:k * 16 + jj * 8 + 8] for k in range(3)]
                            if c < 3:
                                end = ends[c]
                            else:
                                end = jnp.where(
                                    sub < 2, pltpu.roll(ends[0], 2, 0),
                                    jnp.where(sub < 4, pltpu.roll(ends[1], 4, 0),
                                              pltpu.roll(ends[2], 6, 0)))
                            q0 = 48 + (2 * n + jj) * MAIN
                            p = jnp.concatenate(
                                [blk[q0:q0 + MAIN], jnp.where(sub < 6, end, 0.0)], axis=0)
                        else:
                            q0, q1 = n * 128 + 16 + jj * MAIN, n * 128 + jj * 8
                            p = jnp.concatenate([blk[q0:q0 + MAIN], blk[q1:q1 + 8]], axis=0)
                        if kind == K_:
                            phik_v[tb, zrows(pair * 128, 128, 16), :] = _dual_softmax(p)
                        elif kind == Q_:
                            phiq_v[t0 // 2, tb, pair * 128:(pair + 1) * 128, :] = (
                                _dual_softmax(p))
                        else:
                            vt_v[pair // 8][tb, zrows((pair % 8) * 64, 64, 16), :] = (
                                p.astype(bf16))

            _strassen(prod, emit)

        kr = lax.broadcasted_iota(jnp.int32, (64, 128), 0)
        kc = lax.broadcasted_iota(jnp.int32, (64, 128), 1)
        kmask = kr // 32 == kc % 2
        for j in range(NP):
            lhs = tiles(vt_v[j // 8], (j % 8) * 64, 64)
            rhs = tiles(phik_v, j * 128, 128)
            upd = lax.dot_general(_unpack(lhs), _unpack(_or_into(rhs, pins.get(count[0]))), _NT,
                                  preferred_element_type=f32)
            run_jobs(upd)
            if first:
                kv_acc[j, 0:64, :] = upd
            else:
                upd = kv_acc[j, 0:64, :] + upd
                kv_acc[j, 0:64, :] = upd
                kvt_v[j, 0:64, :] = jnp.where(kmask, upd * (1.0 / LOG2E), 0.0).astype(bf16)

    def load_best():
        return best_v[0], besti_v[...], best_v[1], best_v[2]

    def store_best(best):
        best_v[0], besti_v[...], best_v[1], best_v[2] = best

    def build_pt(g0, g1):
        def row_ids(r):
            pair = jnp.where(r < 16, r // 8, jnp.where(r < 16 + MAIN, 0, 1))
            feat = jnp.where(r < 16, MAIN + r % 8, r - 16 - pair * MAIN) // 2
            return pair, feat

        n = g1 - g0
        w2 = wphi_v[4 * g0:4 * g1].reshape(n * 128, DH)
        er = lax.broadcasted_iota(jnp.int32, (128, DH), 0)
        ec = lax.broadcasted_iota(jnp.int32, (128, DH), 1)
        e = jnp.where(ec == row_ids(er)[1], 1.0, 0.0).astype(bf16)
        ptf = lax.dot_general(e, w2, _NT, preferred_element_type=f32)
        pr = lax.broadcasted_iota(jnp.int32, (128, 128), 0)
        pc = lax.broadcasted_iota(jnp.int32, (128, 128), 1)
        keep = pc // 32 == row_ids(pr)[0] * 2 + pr % 2
        return [jnp.where(keep, ptf[:, g * 128:(g + 1) * 128], 0.0).astype(bf16)
                for g in range(n)]

    def compact(kind, i, m):
        we_v[0, 0, 0, zrows(64, 16, 16), :] = m[0:16, 0:128].astype(bf16)
        sub = lax.broadcasted_iota(jnp.int32, (8, HD), 0)
        ends = tiles(we_v.at[kind, i], 0, 64)
        for c in range(NWC - 1):
            wl_v[kind, i, zrows(c * 8, 8), :] = jnp.where(
                sub % 4 == 3, pltpu.roll(ends[24:32], 3 - c, 0), ends[c * 8:(c + 1) * 8])

    hbl_v[...] = jnp.zeros_like(hbl_v)
    hbr_v[...] = jnp.zeros_like(hbr_v)
    store_best((jnp.full((8, 128), -jnp.inf, f32), jnp.zeros((8, 128), jnp.int32),
                jnp.zeros((8, 128), f32), jnp.zeros((8, 128), f32)))
    n_ln = HT1 // LN_ROWS
    x0_copy(0).wait()
    x0_copy(1).wait()
    for p in range(n_ln // 2):
        ln1_piece(0, s_v[0], p)
    full_copy(wr_hbm, wr_v, SEM_WR).wait()
    phi_copy(0).wait()
    x0_copy(2).wait()
    x0_copy(3).wait()
    wr_row = wr_v[...].astype(f32).reshape(1, D)
    wrf_v[...] = jnp.broadcast_to(
        wr_row - jnp.sum(wr_row, axis=-1, keepdims=True) * (1.0 / D), (8, D))
    pt = build_pt(0, 4)
    for p in range(n_ln // 2, n_ln):
        ln1_piece(0, s_v[0], p)
    for part in range(2):
        k0_copy(2 * part).wait()
        k0_copy(2 * part + 1).wait()
        fold_piece(K_, 0, 2 * part, pt)
        fold_piece(K_, 0, 2 * part + 1, pt)

    def add_at(post, slot, fn, span=0):
        half = slot != int(slot)
        post.setdefault(int(slot), []).append(
            (lambda m: fn(m[m.shape[0] // 32 * 16:] if half else m), span))

    post = {}

    def at(slot, fn, span=0):
        add_at(post, slot, fn, span)

    for slot, copies in T0_WAITS:
        for cp in copies:
            if cp == 'phi':
                at(slot, lambda m: phi_copy(1).wait())
            elif cp in ('x1', 'x2', 'x3'):
                at(slot, lambda m, cp=cp: x_copy(int(cp[1])).wait())
            else:
                at(slot, lambda m, cp=cp: w_copy(cp // NWC, cp % NWC).wait())
    for n in range(1, 2 * NWC):
        if n == 2:
            at(T0_FOLD[n], lambda m: pt.extend(build_pt(4, 8)))
        at(T0_FOLD[n], lambda m, n=n: fold_chunk(n // NWC, n % NWC, pt))
    for kind in (K_, Q_):
        for i in range(7):
            at(T0_COMPACT[kind] + i, lambda m, kind=kind, i=i: compact(kind, i, m))
    for c in range(NWC):
        for j in range(4):
            at(T0_VPREP[c][j], lambda m, c=c, j=j: vprep_piece(c, j, m), T0_VSPAN[c])
    for p in range(n_ln):
        at(T0_LN[p], lambda m, p=p: ln1_piece(T1, s_v[1], p, m), T0_LNSPAN[p])
    for p in range(n_ln):
        at(T1_LN[0][p], lambda m, p=p: ln1_piece(2 * T1, s_v[0], p, m), P1_LNSPAN)
        at(T1_LN[1][p], lambda m, p=p: ln1_piece(3 * T1, s_v[1], p, m), P1_LNSPAN)
    for j in range(NP):
        at(T0_Z[j], lambda m, j=j: z_piece(j, True, m), T0_ZSPAN)
    lo, hi = [0, 1], [2, 3]
    run_rounds(0, [(0, kind, [c]) for kind in (K_, Q_) for c in range(NWC)]
               + [(1, K_, lo + hi), (1, Q_, lo + hi)] + [(0, V_, [c]) for c in range(NWC)]
               + [(1, V_, lo), (1, V_, hi)], post, True)
    full_copy(wo_hbm, wo_v.at[pl.ds(0, D), :], SEM_WO).wait()
    for i in range(4, N1):
        x_copy(i).wait()

    def phase1(i, carry):
        post = {}
        nxt = jnp.minimum(i + 1, N2 - 1) * T2
        w0 = jnp.minimum((i - 1) * WO_ROWS, HD - WO_ROWS)
        for par in range(2):
            for p in range(n_ln):
                add_at(post, P1_LN2[par][p],
                       lambda m, p=p, par=par: ln1_piece(nxt + par * T1, s_v[par], p, m),
                       P1_LNSPAN2[par])
        for p in range(WO_ROWS // 16):
            add_at(post, P1_WO[p], lambda m, p=p: wo_piece(w0 + 16 * p, m), P1_WOSPAN)
        for j in range(NP):
            add_at(post, P1_Z[j], lambda m, j=j: z_piece(j, False, m), P1_ZSPAN)
        run_rounds(2 * i, [(par, kind, lo + hi) for kind in (K_, Q_) for par in range(2)]
                   + [(par, V_, cs) for par in range(2) for cs in (lo, hi)], post, False)
        return carry

    lax.fori_loop(1, N1 // 2, phase1, 0)

    for _, dst, rows, slot in ffn_tiled:
        filled = dst.at[:, pl.ds(0, rows), :]
        full_copy(filled, filled, slot).wait()
    full_copy(wg_hbm.at[:, pl.ds(f0, F - f0)], wgv_v, SEM_WGV).wait()
    full_copy(wu_hbm.at[:, pl.ds(f0, F - f0)], wuv_v, SEM_WUV).wait()

    def o_copy(r0, rows):
        return pltpu.make_async_copy(
            out_v.at[pl.ds(r0, rows), :], out_hbm.at[0, pl.ds(r0, rows), :], sem.at[SEM_O])

    def half_stats(hh, c0):
        rows = hh.shape[0]
        parts = [hh[:, c * 128:(c + 1) * 128] for c in range(4)]
        wts = [wrf_v[:, c0 + c * 128:c0 + (c + 1) * 128] for c in range(4)]
        s1 = (parts[0] + parts[1]) + (parts[2] + parts[3])
        sq = [p * p for p in parts]
        s2 = (sq[0] + sq[1]) + (sq[2] + sq[3])
        dw = [(p.reshape(rows // 8, 8, 128) * w[None]).reshape(rows, 128)
              for p, w in zip(parts, wts)]
        s3 = (dw[0] + dw[1]) + (dw[2] + dw[3])
        return s1, s2, s3

    def first_half(hbuf, sbuf, p, c0):
        r0 = p * EP_ROWS
        hh = hbuf[c0 // HD][r0:r0 + EP_ROWS, :]
        st = jnp.concatenate(half_stats(hh, c0), axis=1)
        sbuf[zrows(r0, EP_ROWS), :] = st
        return _fold_token(pltpu.bitcast(st, u32), zero_v)

    def finish(hbuf, sbuf, base, p, valid, best, defer=None):
        r0 = p * EP_ROWS
        g0 = pl.multiple_of(base + r0, EP_ROWS)
        hl, hr = [r[r0:r0 + EP_ROWS, :] for r in hbuf]
        if sbuf is None:
            st = half_stats(hr, HD)
        else:
            st = sbuf[r0:r0 + EP_ROWS, :]
            st = [st[:, n * 128:(n + 1) * 128] for n in range(3)]
        s1, s2, s3 = [jnp.sum(v + w, axis=-1, keepdims=True)
                      for v, w in zip(half_stats(hl, 0), st)]
        m = s1 * (1.0 / D)
        var = jnp.maximum(s2 * (1.0 / D) - m * m, 0.0)
        inv = lax.rsqrt(var + EPS)
        r = s3 * inv

        def write_out(h):
            o = h * (1.0 + inv) - m * inv
            out_v[pl.ds(g0, EP_ROWS), :] = o.astype(bf16)
            return o

        if defer is None:
            o = write_out(jnp.concatenate([hl, hr], axis=1))
        else:
            defer.append(lambda: write_out(jnp.concatenate(
                [r_[r0:r0 + EP_ROWS, :] for r_ in hbuf], axis=1)))
        bv, bi, bm, bq = best
        sub = lax.broadcasted_iota(jnp.int32, (8, 128), 0)
        for g in range(EP_ROWS // 8):
            rows = slice(g * 8, (g + 1) * 8)
            rg = jnp.broadcast_to(r[rows], (8, 128))
            if valid is not None:
                rg = jnp.where(valid, rg, -jnp.inf)
            better = rg > bv
            bi = jnp.where(better, sub + (g0 + g * 8), bi)
            bv = jnp.where(better, rg, bv)
            bm = jnp.where(better, jnp.broadcast_to(m[rows], (8, 128)), bm)
            bq = jnp.where(better, jnp.broadcast_to(var[rows], (8, 128)), bq)
        best = (bv, bi, bm, bq)
        if defer is not None:
            return best, None
        tok = _fold_token(pltpu.bitcast(jnp.concatenate(
            [o[:, D - 128:], bv, bm, bq], axis=0), u32), zero_v)
        return best, tok

    n_ep = QT2 // EP_ROWS

    def phase2(i, carry):
        ot = []
        for j in range(NP):
            ph = tiles(phiq_v.at[i], j * 128, 128)
            n = jnp.dot(_unpack(kvt_v.bitcast(u32)[j]), _unpack(ph),
                        preferred_element_type=f32)
            r0h = _recip(n[64:72] + 1e-6)
            r1h = _recip(n[72:80] + 1e-6)
            ot.append((n[0:32].reshape(4, 8, T2) * r0h[None]).reshape(32, T2))
            ot.append((n[32:64].reshape(4, 8, T2) * r1h[None]).reshape(32, T2))
        lo = jnp.concatenate(ot[:H // 2], axis=0)
        hi = jnp.concatenate(ot[H // 2:], axis=0)
        quarter = lambda v, q: v[:, q * QT2:(q + 1) * QT2]
        lcs = [_left_combos(quarter(lo, 2 * u), quarter(hi, 2 * u),
                            quarter(lo, 2 * u + 1), quarter(hi, 2 * u + 1)) for u in range(2)]

        state = {'best': load_best()}
        pins = {}
        jobs = {}
        lts = {}
        ra = pl.multiple_of(i * T2, T2)
        prev = jnp.maximum(i * T2 - QT2, T2 - QT2)

        def add_job(slot, deadline, fn, gates=()):
            jobs.setdefault(slot, []).append((fn, deadline, gates))

        def finish_job(hbuf, sbuf, base, p, valid):
            def fn():
                state['best'], tok = finish(hbuf, sbuf, base, p, valid, state['best'])
                return tok
            return fn

        order = (2, 4, 6, 0, 3, 1, 5)

        def lt_job(n):
            def fn():
                lts[n] = lcs[n // 7][order[n % 7]].astype(bf16).T
                return _fold_token(pltpu.bitcast(lts[n], u32), zero_v)
            return fn

        lt_job(0)()
        for n in range(1, 14):
            add_job(LT_START[n], min(LT_START[n] + LT_SPAN[n], 4 * n), lt_job(n))
        for u in range(2):
            for p in range(n_ep):
                add_job(FB_START[u][p], FB_START[u][p] + FB_SPAN,
                        finish_job(hb_v, None, ra + QT2 if u else prev, p,
                                   None if u else i > 0), hb_v)
                add_job(SA_START[u][p], SA_START[u][p] + SA_SPAN,
                        lambda p=p: first_half(ha_v, sa_v, p, HD), ha_v[1:])
                add_job(FA_START[u][p], FA_START[u][p] + FA_SPAN[u][p],
                        finish_job(ha_v, sa_v, ra + u * HT2, p, None), ha_v)

        def xblk(q, c0):
            rows = pl.ds(pl.multiple_of(ra + q * QT2, QT2), QT2)
            return x_v[rows, c0:c0 + 128].astype(f32)

        for slot in range(56):
            u, n, c = slot // 28, (slot // 4) % 7, slot % 4
            for fn, deadline, gates in jobs.get(slot, ()):
                for ref in gates:
                    ref[zrows(QT2, 8), 0:128] = mm[0:8]
                pins.setdefault(deadline, []).append(fn())
            w = _or_into(wo7_v.bitcast(u32)[order[n], c, 0:HD // 2, :], pins.get(slot))
            mm = jnp.dot(lts[slot // 4], _unpack(w), preferred_element_type=f32)
            c0 = c * 128
            cs = slice(c0, c0 + 128)
            tmp = lambda t: tmp_v[t][:, cs]
            rows = zrows(0, QT2)
            if n == 0:
                tmp_v[0][rows, cs] = mm
            elif n == 1:
                ha_v[1][rows, cs] = (xblk(2 * u, HD + c0) + tmp(0)) + mm
                tmp_v[1][rows, cs] = xblk(2 * u, c0) - mm
            elif n == 2:
                tmp_v[2][rows, cs] = tmp(1) + mm
            elif n == 3:
                tmp_v[3][rows, cs] = tmp(2) + mm
                tmp_v[4][rows, cs] = (xblk(2 * u + 1, HD + c0) + tmp(0)) + mm
            elif n == 4:
                ha_v[0][rows, cs] = tmp(3) + mm
                tmp_v[5][rows, cs] = xblk(2 * u + 1, c0) + mm
            elif n == 5:
                hb_v[0][rows, cs] = tmp(5) + mm
                tmp_v[6][rows, cs] = tmp(4) - mm
            else:
                hb_v[1][rows, cs] = tmp(6) + mm
        store_best(state['best'])
        o_copy(ra, T2 - QT2).start()

        @pl.when(i > 0)
        def _():
            o_copy(pl.multiple_of(prev, QT2), QT2).start()

        return carry

    lax.fori_loop(0, N2, phase2, 0)
    best = load_best()
    late = []
    for p in range(n_ep):
        best, _ = finish(hb_v, None, S - QT2, p, None, best, late)

    bv, bi, bm, bq = best
    for sh in (4, 2, 1):
        ov, oi, om, oq = [pltpu.roll(t, sh, 0) for t in (bv, bi, bm, bq)]
        take = jnp.logical_or(ov > bv, jnp.logical_and(ov == bv, oi < bi))
        bv, bi, bm, bq = [jnp.where(take, o_, t)
                          for o_, t in zip((ov, oi, om, oq), (bv, bi, bm, bq))]
    idx = jnp.clip(bi[0, 0], 0, S - 1)
    for r_ in hb_v:
        r_[zrows(QT2, 8), 0:128] = bv
    for p, fn in enumerate(late):
        if LATE_AT[p] < 0:
            fn()
    b0 = pl.multiple_of((idx // 8) * 8, 8)
    t = _rb(_rb(bq) + EPS)
    inv = _recip(_rb(t * lax.rsqrt(t)))
    gate = _sigmoid(bv)
    wide = lambda v: jnp.concatenate([v] * (D // 128), axis=1)
    b1 = pl.multiple_of(jnp.minimum(b0, S - QT2 - 8), 8)
    b2 = pl.multiple_of(jnp.maximum(b0 - (S - QT2), 0), 8)
    early = wide(bi) < S - QT2
    src = jnp.where(early, out_v[pl.ds(b1, 8), :].astype(f32),
                    jnp.concatenate([r_[pl.ds(b2, 8), :] for r_ in hb_v], axis=1))
    scale = jnp.where(bi < S - QT2, inv * _recip(1.0 + lax.rsqrt(bq + EPS)), inv)
    hn = (src - wide(bm)) * wide(scale)
    xs = hn.astype(bf16)
    rows = lax.broadcasted_iota(jnp.int32, (8, D), 0) + b0

    xm = jnp.where(rows == wide(bi), hn, 0.0)
    for sh in (4, 2, 1):
        xm = xm + pltpu.roll(xm, sh, 0)
    for t in range(D // 128):
        xcol_v[t // 2][zrows((t % 2) * 128, 128), :] = jnp.concatenate(
            [xm[:, t * 128:(t + 1) * 128]] * 16, axis=0).astype(bf16).T.astype(f32)

    nblk = F // 256
    nmx = nblk - FFN_VPU_BLOCKS
    act = {}
    acc = {}

    def activate(g, u):
        return (g * _sigmoid(g) * u).astype(bf16)

    parts = D // 8 // FFN_KG

    def vpu_chunk(q):
        blk, part = nmx + q // parts, q % parts
        cur = acc.get(blk)
        for kg in range(part * FFN_KG, (part + 1) * FFN_KG):
            xc = xcol_v[kg // 32][(kg % 32) * 8:(kg % 32 + 1) * 8, :]
            w = jnp.concatenate(
                [r[kg * 8:(kg + 1) * 8, (blk - nmx) * 256:(blk - nmx + 1) * 256].astype(f32)
                 for r in (wgv_v, wuv_v)], axis=1)
            p = w * jnp.concatenate([xc] * 4, axis=1)
            cur = p if cur is None else cur + p
        acc[blk] = cur
        if part == parts - 1:
            for sh in (4, 2, 1):
                cur = cur + pltpu.roll(cur, sh, 0)
            act[blk] = activate(cur[:, :256], cur[:, 256:])
        c = q % 4
        return _fold_token(pltpu.bitcast(cur[:, c * 128:(c + 1) * 128], u32), zero_v)

    nchunk = FFN_VPU_BLOCKS * parts
    starts = [FFN_W0 + (q * (FFN_W1 - FFN_W0)) // (nchunk - 1) for q in range(nchunk)]
    pins = {}
    wave = [0]
    wgw, wuw, wdw = [r.bitcast(u32) for r in (wg_v, wu_v, wd_v)]

    def run_wave(lhs, tls):
        w = jnp.concatenate([_or_into(tls[0], pins.get(wave[0]))] + tls[1:], axis=1)
        out = jnp.dot(lhs, _unpack(w), preferred_element_type=f32)
        for p, fn in enumerate(late):
            if LATE_AT[p] == wave[0]:
                for r_ in hb_v:
                    r_[zrows(QT2, 8), 0:128] = out[:, 0:128]
                fn()
        for q, start in enumerate(starts):
            if start == wave[0]:
                pins.setdefault(wave[0] + FFN_SPAN, []).append(vpu_chunk(q))
        if wave[0] == FFN_LATE:
            o_copy(S - QT2, QT2).start()
            out_v[zrows(S, 16, 16), 0:256] = jnp.zeros((16, 256), bf16)
            pins.setdefault(wave[0] + 4, []).append(
                token(out_v[S:S + 8, 0:128].astype(f32))())
        wave[0] += 1
        return out

    for j in range(nmx):
        gu = None
        for kt in range(D // 128):
            p = run_wave(xs[:, kt * 128:(kt + 1) * 128],
                         [r[2 * j + c, kt * 64:(kt + 1) * 64, :]
                          for r in (wgw, wuw) for c in range(2)])
            gu = p if gu is None else gu + p
        act[j] = activate(gu[:, :256], gu[:, 256:])
    ys = [None, None]
    for j in range(nblk):
        for kt in range(2):
            for hf in range(2):
                r0 = (2 * j + kt) * 64
                p = run_wave(act[j][:, kt * 128:(kt + 1) * 128],
                             [wdw[4 * hf + c, r0:r0 + 64, :] for c in range(4)])
                ys[hf] = p if ys[hf] is None else ys[hf] + p
    y = jnp.concatenate(ys, axis=1)
    cur = out_v[pl.ds(b0, 8), :].astype(f32)
    fix_v[...] = jnp.where(rows == wide(bi), cur + y * wide(gate), cur).astype(bf16)
    full_copy(out_v.at[pl.ds(0, S), :], out_hbm.at[0], SEM_O).wait()
    fix = pltpu.make_async_copy(fix_v, out_hbm.at[0, pl.ds(b0, 8), :], sem.at[SEM_O])
    fix.start()
    fix.wait()


def _kernel(*refs):
    def step(i, carry):
        @pl.when(i == 0)
        def _():
            _body(i, *refs)

        return carry

    lax.fori_loop(0, 2, step, 0)


@jax.jit
def pallas_sequential_preLN__linear_kernel_hedgehog__moe_arch_mod__prompt_kernel(
    A_x: jax.Array,
    A_wqkv: jax.Array,
    A_w_phi: jax.Array,
    A_wo: jax.Array,
    B_x: jax.Array,
    B_w_r: jax.Array,
    B_w_gate: jax.Array,
    B_w_up: jax.Array,
    B_w_down: jax.Array,
):
    any_spec = pl.BlockSpec(memory_space=pl.ANY)
    return pl.pallas_call(
        _kernel,
        out_shape=jax.ShapeDtypeStruct((1, S, D), bf16),
        in_specs=[any_spec] * 8,
        out_specs=any_spec,
        scratch_shapes=[
            pltpu.VMEM((S + 16, D), bf16),
            pltpu.VMEM((3 * NWC + 1, D, WC), bf16),
            pltpu.VMEM((H, DH, DH), bf16),
            pltpu.VMEM((D + 16, D), bf16),
            pltpu.VMEM((D,), bf16),
            pltpu.VMEM((F // 128 - 2 * FFN_VPU_BLOCKS, D + PAD, 128), bf16),
            pltpu.VMEM((F // 128 - 2 * FFN_VPU_BLOCKS, D + PAD, 128), bf16),
            pltpu.VMEM((D // 128, F + PAD, 128), bf16),
            pltpu.VMEM((D, 256 * FFN_VPU_BLOCKS), bf16),
            pltpu.VMEM((D, 256 * FFN_VPU_BLOCKS), bf16),
            pltpu.VMEM((7, 4, 3 * HD + PAD, 128), bf16),
            pltpu.VMEM((2, 7, 4, 64 + PAD, 128), bf16),
            pltpu.VMEM((2, 7, 24, HD), u32),
            pltpu.VMEM((7, 4, HD + PAD, 128), bf16),
            pltpu.VMEM((7, 4, HT1 + PAD, 128), bf16),
            pltpu.VMEM((7, 4, HT1 + PAD, 128), bf16),
            pltpu.VMEM((7, HT1 // 2, HD), u32),
            pltpu.VMEM((N2, 4, 2 * D + PAD, 128), bf16),
            pltpu.VMEM((4, 2 * D + PAD, 128), bf16),
            pltpu.VMEM((4, HD + PAD, 128), bf16),
            pltpu.VMEM((4, HD + PAD, 128), bf16),
            pltpu.VMEM((NP, 72, 128), f32),
            pltpu.VMEM((NP, 80, 128), bf16),
            *[pltpu.VMEM((QT2 + 8, HD), f32) for _ in range(4)],
            pltpu.VMEM((QT2, 384), f32),
            *[pltpu.VMEM((QT2, HD), f32) for _ in range(7)],
            pltpu.VMEM((S + 16, D), bf16),
            pltpu.VMEM((8, D), f32),
            pltpu.VMEM((3, 8, 128), f32),
            pltpu.VMEM((8, 128), jnp.int32),
            pltpu.VMEM((8, D), bf16),
            *[pltpu.VMEM((256, 128), f32) for _ in range(4)],
            pltpu.SemaphoreType.DMA((NSEM,)),
        ],
        compiler_params=pltpu.CompilerParams(
            vmem_limit_bytes=110 * 1024 * 1024,
            disable_bounds_checks=True,
            disable_semaphore_checks=True),
    )(A_x, A_wqkv, A_w_phi, A_wo, B_w_r, B_w_gate, B_w_up, B_w_down)
```

```python
import jax
import jax.numpy as jnp
from jax import lax
import jax.experimental.pallas as pl
import jax.experimental.pallas.tpu as pltpu

S = 2048
D = 1024
H = 32
DH = 32
F = 3584
NP = H // 2
T1 = 256
T2 = 512
N1 = S // T1
N2 = S // T2
HT1 = T1 // 2
HT2 = T2 // 2
QT2 = T2 // 4
HD = D // 2
WC = 256
NWC = D // WC
LOG2E = 1.4426950408889634
EPS = 1e-5
PAD = 16
WO_ROWS = 176
LN_ROWS = 16
MAIN = 56
EP_ROWS = 32

T0_FOLD = (0, 5, 11, 19, 25, 33, 39, 46)
T0_WAITS = ((5, (1,)), (11, ('phi', 2)), (19, (3, 4)), (33, ('x1', 5, 6)), (46, (7,)),
            (65, (8, 9, 10, 11, 'x2', 'x3')))
T0_VPREP = ((65, 66, 66.5, 68), (68.5, 69, 70, 74), (74, 76, 78, 79), (81, 83, 84, 86))
T0_COMPACT = (22, 47)
T0_VSPAN = (2, 5, 5, 4)
T0_LN = (33, 33, 35, 35, 36, 38, 40, 45)
T0_LNSPAN = (3, 4, 0, 0, 0, 0, 0, 0)
T1_LN = ((102, 103, 104, 105, 106, 107, 108, 109), (89, 91, 93, 95, 97, 99, 100, 101))
P1_LNSPAN = 5
T0_Z = (63, 63.5, 64, 70.5, 73, 77.5, 77.5, 84, 89, 94, 95.5, 98, 98, 100.5, 105, 106)
T0_ZSPAN = 0
P1_WO = (30, 30, 32, 33, 36, 49, 51, 52, 53, 53, 55)
P1_WOSPAN = 3
P1_LN2 = ((42, 43, 44, 45, 46, 47, 49, 51), (34, 35, 35, 37, 38, 39, 41, 42))
P1_LNSPAN2 = (3, 3)
P1_Z = (28, 30, 31, 33, 36, 38, 40, 42, 43, 44, 46, 47, 50, 51, 52, 53)
P1_ZSPAN = 2
LT_START = (0, 0, 1, 5, 9, 13, 16, 19, 25, 30, 35, 38, 43, 44)
LT_SPAN = (5, 4, 7, 6, 9, 6, 6, 6, 6, 6, 4, 6, 6, 6)
FB_START = ((4, 8, 12, 16), (33, 35, 40, 44))
FB_SPAN = 4
SA_START = ((10, 10, 18, 19), (38, 41, 45, 46))
SA_SPAN = 6
FA_START = ((21, 23, 26, 29), (49, 51, 52, 55))
FA_SPAN = ((4, 4, 4, 3), (5, 5, 8, 10))
FFN_VPU_BLOCKS = 7
FFN_KG = 32
FFN_W0 = 16
FFN_W1 = 107
FFN_SPAN = 4
FFN_LATE = 16
LATE_AT = (-1, 1, 3, 5)

_NT = (((1,), (1,)), ((), ()))
f32 = jnp.float32
bf16 = jnp.bfloat16
u32 = jnp.uint32

K_, Q_, V_ = 0, 1, 2
SRC = {K_: 1, Q_: 0, V_: 2}

SEM_W = 0
SEM_X = SEM_W + 3 * NWC
SEM_X0 = SEM_X + N1
SEM_K0 = SEM_X0 + 4
SEM_PHI = SEM_K0 + 4
SEM_WO = SEM_PHI + 2
SEM_WR, SEM_WG, SEM_WU, SEM_WD, SEM_WGV, SEM_WUV, SEM_O = (SEM_WO + 1 + i for i in range(7))
NSEM = SEM_O + 1


def _rb(v):
    return v.astype(bf16).astype(f32)


def _unpack(w):
    return pltpu.bitcast(w, bf16)


def _mo(i, n):
    return i if isinstance(i, int) else pl.multiple_of(i, n)


def _recip(x):
    r = pl.reciprocal(x, approx=True)
    return r * (2.0 - x * r)


def _sigmoid(x):
    return _recip(1.0 + jnp.exp(jnp.minimum(-x, 80.0)))


def _dual_softmax(p):
    t = p.shape[-1]
    p3 = p.reshape(8, 8, t)

    def allred(v, op):
        v = op(v, pltpu.roll(v, 2, 0))
        return op(v, pltpu.roll(v, 4, 0))

    mx = allred(jnp.max(p3, axis=0), jnp.maximum)
    mn = allred(jnp.min(p3, axis=0), jnp.minimum)
    ep = jnp.exp2(p3 - mx[None])
    en = jnp.exp2(mn[None] - p3)
    sp = allred(jnp.sum(ep, axis=0), jnp.add)
    sn = allred(jnp.sum(en, axis=0), jnp.add)
    fp = (ep * _recip(sp)[None]).reshape(64, t)
    fn = (en * _recip(sn)[None]).reshape(64, t)
    return jnp.concatenate([fp, fn], axis=0).astype(bf16)


def _left_combos(a11, a12, a21, a22):
    return [a11 + a22, a21 + a22, a11, a22, a11 + a12, a21 - a11, a12 - a22]


def _right_combos(b11, b12, b21, b22):
    return [b11 + b22, b11, b12 - b22, b21 - b11, b22, b11 + b12, b21 + b22]


def _strassen(prod, emit):
    m3 = prod(2)
    m5 = prod(4)
    emit(0, 1, m3 + m5)
    m7 = prod(6)
    u = m7 - m5
    m1 = prod(0)
    u = u + m1
    w = m1 + m3
    m4 = prod(3)
    emit(0, 0, u + m4)
    m2 = prod(1)
    emit(1, 0, m2 + m4)
    w = w - m2
    m6 = prod(5)
    emit(1, 1, w + m6)


def _or_into(w, toks):
    if not toks:
        return w
    top = w[0:8, 0:128]
    for tk in toks:
        top = top | tk
    if w.shape[1] > 128:
        top = jnp.concatenate([top, w[0:8, 128:]], axis=1)
    return jnp.concatenate([top, w[8:]], axis=0)


def _fold_token(w, zero):
    r, c = w.shape
    acc = None
    for i in range(r // 8):
        for j in range(c // 128):
            blk = w[i * 8:(i + 1) * 8, j * 128:(j + 1) * 128]
            acc = blk if acc is None else acc | blk
    return acc & zero


def _body(zs, x_hbm, wqkv_hbm, wphi_hbm, wo_hbm, wr_hbm, wg_hbm, wu_hbm, wd_hbm, out_hbm,
          x_v, wqkv_v, wphi_v, wo_v, wr_v, wg_v, wu_v, wd_v, wgv_v, wuv_v,
          wt_v, we_v, wl_v, wo7_v, sa7_v, sb7_v, sc7_v, phiq_v, phik_v, vt0_v, vt1_v, kv_acc, kvt_v,
          hal_v, har_v, hbl_v, hbr_v, sa_v, t0_v, t1_v, t2_v, t3_v, t4_v, t5_v, t6_v,
          out_v, wrf_v, best_v, besti_v, fix_v, xc0_v, xc1_v, xc2_v, xc3_v, sem):
    xcol_v = (xc0_v, xc1_v, xc2_v, xc3_v)
    s_v = (sa7_v, sb7_v)
    vt_v = (vt0_v, vt1_v)
    ha_v = (hal_v, har_v)
    hb_v = (hbl_v, hbr_v)
    tmp_v = (t0_v, t1_v, t2_v, t3_v, t4_v, t5_v, t6_v)

    def x_rows(r0, rows, slot):
        return pltpu.make_async_copy(
            x_hbm.at[0, pl.ds(r0, rows), :], x_v.at[pl.ds(r0, rows), :], sem.at[slot])

    def x_copy(i):
        return x_rows(i * T1, T1, SEM_X + i)

    def x0_copy(q):
        return x_rows((q % 2) * HT1 + (q // 2) * (HT1 // 2), HT1 // 2, SEM_X0 + q)

    def w_copy(kind, c):
        return pltpu.make_async_copy(
            wqkv_hbm.at[:, pl.ds(SRC[kind] * D + c * WC, WC)],
            wqkv_v.at[kind * NWC + c], sem.at[SEM_W + kind * NWC + c])

    def k0_copy(q):
        r0 = (q % 2) * HD + (q // 2) * 256
        return pltpu.make_async_copy(
            wqkv_hbm.at[pl.ds(r0, 256), pl.ds(SRC[K_] * D, WC)],
            wqkv_v.at[K_ * NWC, pl.ds(r0, 256), :], sem.at[SEM_K0 + q])

    def phi_copy(part):
        lo, n = part * (H // 2), H // 2
        return pltpu.make_async_copy(wphi_hbm.at[pl.ds(lo, n)], wphi_v.at[pl.ds(lo, n)],
                                     sem.at[SEM_PHI + part])

    def full_copy(src, dst, slot):
        return pltpu.make_async_copy(src, dst, sem.at[slot])

    x0_copy(0).start()
    x0_copy(1).start()
    full_copy(wr_hbm, wr_v, SEM_WR).start()
    phi_copy(0).start()
    x0_copy(2).start()
    x0_copy(3).start()
    for q in range(4):
        k0_copy(q).start()
    w_copy(K_, 1).start()
    phi_copy(1).start()
    w_copy(K_, 2).start()
    w_copy(K_, 3).start()
    w_copy(Q_, 0).start()
    x_copy(1).start()
    for c in range(1, NWC):
        w_copy(Q_, c).start()
    for c in range(NWC):
        w_copy(V_, c).start()
    x_copy(2).start()
    x_copy(3).start()
    full_copy(wo_hbm, wo_v.at[pl.ds(0, D), :], SEM_WO).start()
    for i in range(4, N1):
        x_copy(i).start()
    f0 = F - 256 * FFN_VPU_BLOCKS
    ffn_tiled = ((wg_hbm, wg_v, D, SEM_WG), (wu_hbm, wu_v, D, SEM_WU), (wd_hbm, wd_v, F, SEM_WD))
    for src, dst, rows, slot in ffn_tiled:
        for c in range(dst.shape[0]):
            full_copy(src.at[:, pl.ds(c * 128, 128)], dst.at[c, pl.ds(0, rows), :], slot).start()
    full_copy(wg_hbm.at[:, pl.ds(f0, F - f0)], wgv_v, SEM_WGV).start()
    full_copy(wu_hbm.at[:, pl.ds(f0, F - f0)], wuv_v, SEM_WUV).start()

    zero_v = jnp.full((8, 128), zs, jnp.int32).astype(u32)

    def zrows(r0, rows, mult=8):
        return pl.ds(pl.multiple_of(zs * mult + r0, mult), rows)

    def tiles(ref, r0, rows):
        w = ref.bitcast(u32)
        return jnp.concatenate(
            [w[c, r0 // 2:(r0 + rows) // 2, :] for c in range(ref.shape[0])], axis=1)

    def token(*vals):
        return lambda: _fold_token(pltpu.bitcast(jnp.concatenate(vals, axis=0), u32), zero_v)

    def ln1_stats(xf):
        m = jnp.sum(xf, axis=-1, keepdims=True) * (1.0 / D)
        q = jnp.sum(xf * xf, axis=-1, keepdims=True) * (1.0 / D)
        inv = lax.rsqrt(jnp.maximum(q - m * m, 0.0) + EPS) * LOG2E
        return inv, m * inv

    def ln1_piece(r0, dst, p, m=None):
        fixed = isinstance(r0, int)
        if m is not None:
            x_v[zrows(S, 8) if fixed else pl.ds(S, 8), 0:128] = m[0:8, 0:128].astype(bf16)
        xa, xb = [x_v[pl.ds(_mo(r0 + hf * HT1 + p * LN_ROWS, LN_ROWS), LN_ROWS), :]
                  .astype(f32) for hf in range(2)]
        (ia, ma), (ib, mb) = ln1_stats(xa), ln1_stats(xb)
        ya, yb = xa * ia, xb * ib
        s2 = ya[:, :HD] - ma
        s5 = yb[:, HD:] - mb
        s1 = s2 + s5
        s3 = yb[:, :HD] - yb[:, HD:]
        s4 = ya[:, HD:] - ya[:, :HD]
        combos = [s1, s2, s3, s4, s5, s1 + s3, s1 + s4]
        rows = zrows(p * LN_ROWS, LN_ROWS, 16) if fixed else pl.ds(p * LN_ROWS, LN_ROWS)
        for i in range(7):
            for c in range(4):
                dst[i, c, rows, :] = combos[i][:, c * 128:(c + 1) * 128].astype(bf16)
        return token(combos[5], combos[6])

    def fold_piece(kind, c, j, pt):
        sub = lax.broadcasted_iota(jnp.int32, (8, 128), 0)
        blk = {}
        for hh in range(2):
            for kh in range(2):
                k0 = kh * HD + j * 128
                w = wqkv_v[kind * NWC + c, k0:k0 + 128, hh * 128:(hh + 1) * 128]
                f = lax.dot_general(pt[2 * c + hh], w, _NT, preferred_element_type=f32)
                refs = []
                for pp in range(2):
                    ref = jnp.where(sub >= 6, f[pp * 8:(pp + 1) * 8], 0.0)
                    ref = ref + pltpu.roll(ref, 2, 0)
                    refs.append(ref + pltpu.roll(ref, 4, 0))
                blk[hh, kh] = f - jnp.concatenate(refs + [refs[0]] * 7 + [refs[1]] * 7, axis=0)
        combos = _left_combos(blk[0, 0], blk[0, 1], blk[1, 0], blk[1, 1])
        r0 = kind * HD + c * 128
        for i in range(7):
            wt_v[i, j, r0:r0 + 128, :] = combos[i].astype(bf16)
            we_v[kind, i, j, c * 16:(c + 1) * 16, :] = combos[i][0:16].astype(bf16)

    def fold_chunk(kind, c, pt):
        for j in range(4):
            fold_piece(kind, c, j, pt)

    def vprep_piece(c, j, m):
        wqkv_v[zs + 3 * NWC, 0:8, 0:128] = m[0:8, 0:128].astype(bf16)
        blk = {}
        for hh in range(2):
            for kh in range(2):
                k0 = kh * HD + j * 128
                w = wqkv_v[V_ * NWC + c, k0:k0 + 128, hh * 128:(hh + 1) * 128]
                blk[hh, kh] = w.T.astype(f32)
        combos = _left_combos(blk[0, 0], blk[0, 1], blk[1, 0], blk[1, 1])
        r0 = V_ * HD + c * 128
        for i in range(7):
            wt_v[i, j, r0:r0 + 128, :] = combos[i].astype(bf16)
        return token(combos[1], combos[4])

    def wo_piece(w0, m):
        wo_v[D:D + 8, 0:128] = m[0:8, 0:128].astype(bf16)
        top = wo_v[pl.ds(pl.multiple_of(w0, 16), 16), :].astype(f32)
        bot = wo_v[pl.ds(pl.multiple_of(HD + w0, 16), 16), :].astype(f32)
        combos = _right_combos(top[:, :HD], top[:, HD:], bot[:, :HD], bot[:, HD:])
        for i in range(7):
            for c in range(4):
                wo7_v[i, c, pl.ds(pl.multiple_of(w0, 16), 16), :] = (
                    combos[i][:, c * 128:(c + 1) * 128].astype(bf16))
        return token(combos[5], combos[6])

    def z_piece(j, first, m):
        phik_v[0, zrows(2 * D, 16, 16), :] = m[0:16, 0:128].astype(bf16)
        ph = _unpack(tiles(phik_v, j * 128, 128)).astype(f32)
        part = (ph[:, 0:128] + ph[:, 128:256]) + (ph[:, 256:384] + ph[:, 384:512])
        z = jnp.sum(part.astype(bf16).T.astype(f32).reshape(16, 8, 128), axis=0)
        for sh in (4, 2, 1):
            z = z + pltpu.roll(z, sh, 0)
        if first:
            kv_acc[j, 64:72, :] = z
        else:
            z = kv_acc[j, 64:72, :] + z
            kv_acc[j, 64:72, :] = z
            odd = lax.broadcasted_iota(jnp.int32, (8, 128), 1) % 2
            kvt_v[j, 64:80, :] = jnp.concatenate(
                [jnp.where(odd == hl, z, 0.0) for hl in range(2)], axis=0).astype(bf16)
        return token(z)

    def run_rounds(t0, rounds, post, first):
        count = [0]
        pins = {}

        def run_jobs(m):
            for fn, span in post.get(count[0], ()):
                tok = fn(m)
                if span:
                    pins.setdefault(count[0] + span, []).append(tok())
            count[0] += 1

        for par, kind, cs in rounds:
            r0 = kind * HD + cs[0] * 128
            rows = 128 * len(cs)

            def prod(i):
                if (par, kind) == (1, V_):
                    rhs = sc7_v[i]
                else:
                    rhs = tiles(s_v[par].at[i], 0, HT1)
                if (par, kind, cs[0]) == (1, K_, 0):
                    sc7_v[i, zrows(0, HT1 // 2), :] = rhs
                if len(cs) == NWC:
                    lhs = jnp.concatenate(
                        [wl_v[kind, i]] + [tiles(wt_v.at[i], r0 + c * 128 + 16, 2 * MAIN)
                                           for c in cs], axis=0)
                else:
                    lhs = tiles(wt_v.at[i], r0, rows)
                m = lax.dot_general(_unpack(lhs),
                                    _unpack(_or_into(rhs, pins.get(count[0]))),
                                    _NT, preferred_element_type=f32)
                run_jobs(m)
                return m

            def emit(rh, ch, blk):
                tb = 2 * par + ch
                for n, c in enumerate(cs):
                    for jj in range(2):
                        pair = 4 * c + 2 * rh + jj
                        if kind == V_:
                            p = blk[n * 128 + jj * 64:n * 128 + (jj + 1) * 64]
                        elif len(cs) == NWC:
                            sub = lax.broadcasted_iota(jnp.int32, (8, HT1), 0)
                            ends = [blk[k * 16 + jj * 8:k * 16 + jj * 8 + 8] for k in range(3)]
                            if c < 3:
                                end = ends[c]
                            else:
                                end = jnp.where(
                                    sub < 2, pltpu.roll(ends[0], 2, 0),
                                    jnp.where(sub < 4, pltpu.roll(ends[1], 4, 0),
                                              pltpu.roll(ends[2], 6, 0)))
                            q0 = 48 + (2 * n + jj) * MAIN
                            p = jnp.concatenate(
                                [blk[q0:q0 + MAIN], jnp.where(sub < 6, end, 0.0)], axis=0)
                        else:
                            q0, q1 = n * 128 + 16 + jj * MAIN, n * 128 + jj * 8
                            p = jnp.concatenate([blk[q0:q0 + MAIN], blk[q1:q1 + 8]], axis=0)
                        if kind == K_:
                            phik_v[tb, zrows(pair * 128, 128, 16), :] = _dual_softmax(p)
                        elif kind == Q_:
                            phiq_v[t0 // 2, tb, pair * 128:(pair + 1) * 128, :] = (
                                _dual_softmax(p))
                        else:
                            vt_v[pair // 8][tb, zrows((pair % 8) * 64, 64, 16), :] = (
                                p.astype(bf16))

            _strassen(prod, emit)

        kr = lax.broadcasted_iota(jnp.int32, (64, 128), 0)
        kc = lax.broadcasted_iota(jnp.int32, (64, 128), 1)
        kmask = kr // 32 == kc % 2
        for j in range(NP):
            lhs = tiles(vt_v[j // 8], (j % 8) * 64, 64)
            rhs = tiles(phik_v, j * 128, 128)
            upd = lax.dot_general(_unpack(lhs), _unpack(_or_into(rhs, pins.get(count[0]))), _NT,
                                  preferred_element_type=f32)
            run_jobs(upd)
            if first:
                kv_acc[j, 0:64, :] = upd
            else:
                upd = kv_acc[j, 0:64, :] + upd
                kv_acc[j, 0:64, :] = upd
                kvt_v[j, 0:64, :] = jnp.where(kmask, upd * (1.0 / LOG2E), 0.0).astype(bf16)

    def load_best():
        return best_v[0], besti_v[...], best_v[1], best_v[2]

    def store_best(best):
        best_v[0], besti_v[...], best_v[1], best_v[2] = best

    def build_pt(g0, g1):
        def row_ids(r):
            pair = jnp.where(r < 16, r // 8, jnp.where(r < 16 + MAIN, 0, 1))
            feat = jnp.where(r < 16, MAIN + r % 8, r - 16 - pair * MAIN) // 2
            return pair, feat

        n = g1 - g0
        w2 = wphi_v[4 * g0:4 * g1].reshape(n * 128, DH)
        er = lax.broadcasted_iota(jnp.int32, (128, DH), 0)
        ec = lax.broadcasted_iota(jnp.int32, (128, DH), 1)
        e = jnp.where(ec == row_ids(er)[1], 1.0, 0.0).astype(bf16)
        ptf = lax.dot_general(e, w2, _NT, preferred_element_type=f32)
        pr = lax.broadcasted_iota(jnp.int32, (128, 128), 0)
        pc = lax.broadcasted_iota(jnp.int32, (128, 128), 1)
        keep = pc // 32 == row_ids(pr)[0] * 2 + pr % 2
        return [jnp.where(keep, ptf[:, g * 128:(g + 1) * 128], 0.0).astype(bf16)
                for g in range(n)]

    def compact(kind, i, m):
        we_v[0, 0, 0, zrows(64, 16, 16), :] = m[0:16, 0:128].astype(bf16)
        sub = lax.broadcasted_iota(jnp.int32, (8, HD), 0)
        ends = tiles(we_v.at[kind, i], 0, 64)
        for c in range(NWC - 1):
            wl_v[kind, i, zrows(c * 8, 8), :] = jnp.where(
                sub % 4 == 3, pltpu.roll(ends[24:32], 3 - c, 0), ends[c * 8:(c + 1) * 8])

    hbl_v[...] = jnp.zeros_like(hbl_v)
    hbr_v[...] = jnp.zeros_like(hbr_v)
    store_best((jnp.full((8, 128), -jnp.inf, f32), jnp.zeros((8, 128), jnp.int32),
                jnp.zeros((8, 128), f32), jnp.zeros((8, 128), f32)))
    n_ln = HT1 // LN_ROWS
    x0_copy(0).wait()
    x0_copy(1).wait()
    for p in range(n_ln // 2):
        ln1_piece(0, s_v[0], p)
    full_copy(wr_hbm, wr_v, SEM_WR).wait()
    phi_copy(0).wait()
    x0_copy(2).wait()
    x0_copy(3).wait()
    wr_row = wr_v[...].astype(f32).reshape(1, D)
    wrf_v[...] = jnp.broadcast_to(
        wr_row - jnp.sum(wr_row, axis=-1, keepdims=True) * (1.0 / D), (8, D))
    pt = build_pt(0, 4)
    for p in range(n_ln // 2, n_ln):
        ln1_piece(0, s_v[0], p)
    for part in range(2):
        k0_copy(2 * part).wait()
        k0_copy(2 * part + 1).wait()
        fold_piece(K_, 0, 2 * part, pt)
        fold_piece(K_, 0, 2 * part + 1, pt)

    def add_at(post, slot, fn, span=0):
        half = slot != int(slot)
        post.setdefault(int(slot), []).append(
            (lambda m: fn(m[m.shape[0] // 32 * 16:] if half else m), span))

    post = {}

    def at(slot, fn, span=0):
        add_at(post, slot, fn, span)

    for slot, copies in T0_WAITS:
        for cp in copies:
            if cp == 'phi':
                at(slot, lambda m: phi_copy(1).wait())
            elif cp in ('x1', 'x2', 'x3'):
                at(slot, lambda m, cp=cp: x_copy(int(cp[1])).wait())
            else:
                at(slot, lambda m, cp=cp: w_copy(cp // NWC, cp % NWC).wait())
    for n in range(1, 2 * NWC):
        if n == 2:
            at(T0_FOLD[n], lambda m: pt.extend(build_pt(4, 8)))
        at(T0_FOLD[n], lambda m, n=n: fold_chunk(n // NWC, n % NWC, pt))
    for kind in (K_, Q_):
        for i in range(7):
            at(T0_COMPACT[kind] + i, lambda m, kind=kind, i=i: compact(kind, i, m))
    for c in range(NWC):
        for j in range(4):
            at(T0_VPREP[c][j], lambda m, c=c, j=j: vprep_piece(c, j, m), T0_VSPAN[c])
    for p in range(n_ln):
        at(T0_LN[p], lambda m, p=p: ln1_piece(T1, s_v[1], p, m), T0_LNSPAN[p])
    for p in range(n_ln):
        at(T1_LN[0][p], lambda m, p=p: ln1_piece(2 * T1, s_v[0], p, m), P1_LNSPAN)
        at(T1_LN[1][p], lambda m, p=p: ln1_piece(3 * T1, s_v[1], p, m), P1_LNSPAN)
    for j in range(NP):
        at(T0_Z[j], lambda m, j=j: z_piece(j, True, m), T0_ZSPAN)
    lo, hi = [0, 1], [2, 3]
    run_rounds(0, [(0, kind, [c]) for kind in (K_, Q_) for c in range(NWC)]
               + [(1, K_, lo + hi), (1, Q_, lo + hi)] + [(0, V_, [c]) for c in range(NWC)]
               + [(1, V_, lo), (1, V_, hi)], post, True)
    full_copy(wo_hbm, wo_v.at[pl.ds(0, D), :], SEM_WO).wait()
    for i in range(4, N1):
        x_copy(i).wait()

    def phase1(i, carry):
        post = {}
        nxt = jnp.minimum(i + 1, N2 - 1) * T2
        w0 = jnp.minimum((i - 1) * WO_ROWS, HD - WO_ROWS)
        for par in range(2):
            for p in range(n_ln):
                add_at(post, P1_LN2[par][p],
                       lambda m, p=p, par=par: ln1_piece(nxt + par * T1, s_v[par], p, m),
                       P1_LNSPAN2[par])
        for p in range(WO_ROWS // 16):
            add_at(post, P1_WO[p], lambda m, p=p: wo_piece(w0 + 16 * p, m), P1_WOSPAN)
        for j in range(NP):
            add_at(post, P1_Z[j], lambda m, j=j: z_piece(j, False, m), P1_ZSPAN)
        run_rounds(2 * i, [(par, kind, lo + hi) for kind in (K_, Q_) for par in range(2)]
                   + [(par, V_, cs) for par in range(2) for cs in (lo, hi)], post, False)
        return carry

    lax.fori_loop(1, N1 // 2, phase1, 0)

    for _, dst, rows, slot in ffn_tiled:
        filled = dst.at[:, pl.ds(0, rows), :]
        full_copy(filled, filled, slot).wait()
    full_copy(wg_hbm.at[:, pl.ds(f0, F - f0)], wgv_v, SEM_WGV).wait()
    full_copy(wu_hbm.at[:, pl.ds(f0, F - f0)], wuv_v, SEM_WUV).wait()

    def o_copy(r0, rows):
        return pltpu.make_async_copy(
            out_v.at[pl.ds(r0, rows), :], out_hbm.at[0, pl.ds(r0, rows), :], sem.at[SEM_O])

    def half_stats(hh, c0):
        rows = hh.shape[0]
        parts = [hh[:, c * 128:(c + 1) * 128] for c in range(4)]
        wts = [wrf_v[:, c0 + c * 128:c0 + (c + 1) * 128] for c in range(4)]
        s1 = (parts[0] + parts[1]) + (parts[2] + parts[3])
        sq = [p * p for p in parts]
        s2 = (sq[0] + sq[1]) + (sq[2] + sq[3])
        dw = [(p.reshape(rows // 8, 8, 128) * w[None]).reshape(rows, 128)
              for p, w in zip(parts, wts)]
        s3 = (dw[0] + dw[1]) + (dw[2] + dw[3])
        return s1, s2, s3

    def first_half(hbuf, sbuf, p, c0):
        r0 = p * EP_ROWS
        hh = hbuf[c0 // HD][r0:r0 + EP_ROWS, :]
        st = jnp.concatenate(half_stats(hh, c0), axis=1)
        sbuf[zrows(r0, EP_ROWS), :] = st
        return _fold_token(pltpu.bitcast(st, u32), zero_v)

    def finish(hbuf, sbuf, base, p, valid, best, defer=None):
        r0 = p * EP_ROWS
        g0 = pl.multiple_of(base + r0, EP_ROWS)
        hl, hr = [r[r0:r0 + EP_ROWS, :] for r in hbuf]
        if sbuf is None:
            st = half_stats(hr, HD)
        else:
            st = sbuf[r0:r0 + EP_ROWS, :]
            st = [st[:, n * 128:(n + 1) * 128] for n in range(3)]
        s1, s2, s3 = [jnp.sum(v + w, axis=-1, keepdims=True)
                      for v, w in zip(half_stats(hl, 0), st)]
        m = s1 * (1.0 / D)
        var = jnp.maximum(s2 * (1.0 / D) - m * m, 0.0)
        inv = lax.rsqrt(var + EPS)
        r = s3 * inv

        def write_out(h):
            o = h * (1.0 + inv) - m * inv
            out_v[pl.ds(g0, EP_ROWS), :] = o.astype(bf16)
            return o

        if defer is None:
            o = write_out(jnp.concatenate([hl, hr], axis=1))
        else:
            defer.append(lambda: write_out(jnp.concatenate(
                [r_[r0:r0 + EP_ROWS, :] for r_ in hbuf], axis=1)))
        bv, bi, bm, bq = best
        sub = lax.broadcasted_iota(jnp.int32, (8, 128), 0)
        for g in range(EP_ROWS // 8):
            rows = slice(g * 8, (g + 1) * 8)
            rg = jnp.broadcast_to(r[rows], (8, 128))
            if valid is not None:
                rg = jnp.where(valid, rg, -jnp.inf)
            better = rg > bv
            bi = jnp.where(better, sub + (g0 + g * 8), bi)
            bv = jnp.where(better, rg, bv)
            bm = jnp.where(better, jnp.broadcast_to(m[rows], (8, 128)), bm)
            bq = jnp.where(better, jnp.broadcast_to(var[rows], (8, 128)), bq)
        best = (bv, bi, bm, bq)
        if defer is not None:
            return best, None
        tok = _fold_token(pltpu.bitcast(jnp.concatenate(
            [o[:, D - 128:], bv, bm, bq], axis=0), u32), zero_v)
        return best, tok

    n_ep = QT2 // EP_ROWS

    def phase2(i, carry):
        ot = []
        for j in range(NP):
            ph = tiles(phiq_v.at[i], j * 128, 128)
            n = jnp.dot(_unpack(kvt_v.bitcast(u32)[j]), _unpack(ph),
                        preferred_element_type=f32)
            r0h = _recip(n[64:72] + 1e-6)
            r1h = _recip(n[72:80] + 1e-6)
            ot.append((n[0:32].reshape(4, 8, T2) * r0h[None]).reshape(32, T2))
            ot.append((n[32:64].reshape(4, 8, T2) * r1h[None]).reshape(32, T2))
        lo = jnp.concatenate(ot[:H // 2], axis=0)
        hi = jnp.concatenate(ot[H // 2:], axis=0)
        quarter = lambda v, q: v[:, q * QT2:(q + 1) * QT2]
        lcs = [_left_combos(quarter(lo, 2 * u), quarter(hi, 2 * u),
                            quarter(lo, 2 * u + 1), quarter(hi, 2 * u + 1)) for u in range(2)]

        state = {'best': load_best()}
        pins = {}
        jobs = {}
        lts = {}
        ra = pl.multiple_of(i * T2, T2)
        prev = jnp.maximum(i * T2 - QT2, T2 - QT2)

        def add_job(slot, deadline, fn, gates=()):
            jobs.setdefault(slot, []).append((fn, deadline, gates))

        def finish_job(hbuf, sbuf, base, p, valid):
            def fn():
                state['best'], tok = finish(hbuf, sbuf, base, p, valid, state['best'])
                return tok
            return fn

        order = (2, 4, 6, 0, 3, 1, 5)

        def lt_job(n):
            def fn():
                lts[n] = lcs[n // 7][order[n % 7]].astype(bf16).T
                return _fold_token(pltpu.bitcast(lts[n], u32), zero_v)
            return fn

        lt_job(0)()
        for n in range(1, 14):
            add_job(LT_START[n], min(LT_START[n] + LT_SPAN[n], 4 * n), lt_job(n))
        for u in range(2):
            for p in range(n_ep):
                add_job(FB_START[u][p], FB_START[u][p] + FB_SPAN,
                        finish_job(hb_v, None, ra + QT2 if u else prev, p,
                                   None if u else i > 0), hb_v)
                add_job(SA_START[u][p], SA_START[u][p] + SA_SPAN,
                        lambda p=p: first_half(ha_v, sa_v, p, HD), ha_v[1:])
                add_job(FA_START[u][p], FA_START[u][p] + FA_SPAN[u][p],
                        finish_job(ha_v, sa_v, ra + u * HT2, p, None), ha_v)

        def xblk(q, c0):
            rows = pl.ds(pl.multiple_of(ra + q * QT2, QT2), QT2)
            return x_v[rows, c0:c0 + 128].astype(f32)

        for slot in range(56):
            u, n, c = slot // 28, (slot // 4) % 7, slot % 4
            for fn, deadline, gates in jobs.get(slot, ()):
                for ref in gates:
                    ref[zrows(QT2, 8), 0:128] = mm[0:8]
                pins.setdefault(deadline, []).append(fn())
            w = _or_into(wo7_v.bitcast(u32)[order[n], c, 0:HD // 2, :], pins.get(slot))
            mm = jnp.dot(lts[slot // 4], _unpack(w), preferred_element_type=f32)
            c0 = c * 128
            cs = slice(c0, c0 + 128)
            tmp = lambda t: tmp_v[t][:, cs]
            rows = zrows(0, QT2)
            if n == 0:
                tmp_v[0][rows, cs] = mm
            elif n == 1:
                ha_v[1][rows, cs] = (xblk(2 * u, HD + c0) + tmp(0)) + mm
                tmp_v[1][rows, cs] = xblk(2 * u, c0) - mm
            elif n == 2:
                tmp_v[2][rows, cs] = tmp(1) + mm
            elif n == 3:
                tmp_v[3][rows, cs] = tmp(2) + mm
                tmp_v[4][rows, cs] = (xblk(2 * u + 1, HD + c0) + tmp(0)) + mm
            elif n == 4:
                ha_v[0][rows, cs] = tmp(3) + mm
                tmp_v[5][rows, cs] = xblk(2 * u + 1, c0) + mm
            elif n == 5:
                hb_v[0][rows, cs] = tmp(5) + mm
                tmp_v[6][rows, cs] = tmp(4) - mm
            else:
                hb_v[1][rows, cs] = tmp(6) + mm
        store_best(state['best'])
        o_copy(ra, T2 - QT2).start()

        @pl.when(i > 0)
        def _():
            o_copy(pl.multiple_of(prev, QT2), QT2).start()

        return carry

    lax.fori_loop(0, N2, phase2, 0)
    best = load_best()
    late = []
    for p in range(n_ep):
        best, _ = finish(hb_v, None, S - QT2, p, None, best, late)

    bv, bi, bm, bq = best
    for sh in (4, 2, 1):
        ov, oi, om, oq = [pltpu.roll(t, sh, 0) for t in (bv, bi, bm, bq)]
        take = jnp.logical_or(ov > bv, jnp.logical_and(ov == bv, oi < bi))
        bv, bi, bm, bq = [jnp.where(take, o_, t)
                          for o_, t in zip((ov, oi, om, oq), (bv, bi, bm, bq))]
    idx = jnp.clip(bi[0, 0], 0, S - 1)
    for r_ in hb_v:
        r_[zrows(QT2, 8), 0:128] = bv
    for p, fn in enumerate(late):
        if LATE_AT[p] < 0:
            fn()
    b0 = pl.multiple_of((idx // 8) * 8, 8)
    t = _rb(_rb(bq) + EPS)
    inv = _recip(_rb(t * lax.rsqrt(t)))
    gate = _sigmoid(bv)
    wide = lambda v: jnp.concatenate([v] * (D // 128), axis=1)
    b1 = pl.multiple_of(jnp.minimum(b0, S - QT2 - 8), 8)
    b2 = pl.multiple_of(jnp.maximum(b0 - (S - QT2), 0), 8)
    early = wide(bi) < S - QT2
    src = jnp.where(early, out_v[pl.ds(b1, 8), :].astype(f32),
                    jnp.concatenate([r_[pl.ds(b2, 8), :] for r_ in hb_v], axis=1))
    scale = jnp.where(bi < S - QT2, inv * _recip(1.0 + lax.rsqrt(bq + EPS)), inv)
    hn = (src - wide(bm)) * wide(scale)
    xs = hn.astype(bf16)
    rows = lax.broadcasted_iota(jnp.int32, (8, D), 0) + b0

    xm = jnp.where(rows == wide(bi), hn, 0.0)
    for sh in (4, 2, 1):
        xm = xm + pltpu.roll(xm, sh, 0)
    for t in range(D // 128):
        xcol_v[t // 2][zrows((t % 2) * 128, 128), :] = jnp.concatenate(
            [xm[:, t * 128:(t + 1) * 128]] * 16, axis=0).astype(bf16).T.astype(f32)

    nblk = F // 256
    nmx = nblk - FFN_VPU_BLOCKS
    act = {}
    acc = {}

    def activate(g, u):
        return (g * _sigmoid(g) * u).astype(bf16)

    parts = D // 8 // FFN_KG

    def vpu_chunk(q):
        blk, part = nmx + q // parts, q % parts
        cur = acc.get(blk)
        for kg in range(part * FFN_KG, (part + 1) * FFN_KG):
            xc = xcol_v[kg // 32][(kg % 32) * 8:(kg % 32 + 1) * 8, :]
            w = jnp.concatenate(
                [r[kg * 8:(kg + 1) * 8, (blk - nmx) * 256:(blk - nmx + 1) * 256].astype(f32)
                 for r in (wgv_v, wuv_v)], axis=1)
            p = w * jnp.concatenate([xc] * 4, axis=1)
            cur = p if cur is None else cur + p
        acc[blk] = cur
        if part == parts - 1:
            for sh in (4, 2, 1):
                cur = cur + pltpu.roll(cur, sh, 0)
            act[blk] = activate(cur[:, :256], cur[:, 256:])
        c = q % 4
        return _fold_token(pltpu.bitcast(cur[:, c * 128:(c + 1) * 128], u32), zero_v)

    nchunk = FFN_VPU_BLOCKS * parts
    starts = [FFN_W0 + (q * (FFN_W1 - FFN_W0)) // (nchunk - 1) for q in range(nchunk)]
    pins = {}
    wave = [0]
    wgw, wuw, wdw = [r.bitcast(u32) for r in (wg_v, wu_v, wd_v)]

    def run_wave(lhs, tls):
        w = jnp.concatenate([_or_into(tls[0], pins.get(wave[0]))] + tls[1:], axis=1)
        out = jnp.dot(lhs, _unpack(w), preferred_element_type=f32)
        for p, fn in enumerate(late):
            if LATE_AT[p] == wave[0]:
                for r_ in hb_v:
                    r_[zrows(QT2, 8), 0:128] = out[:, 0:128]
                fn()
        for q, start in enumerate(starts):
            if start == wave[0]:
                pins.setdefault(wave[0] + FFN_SPAN, []).append(vpu_chunk(q))
        if wave[0] == FFN_LATE:
            o_copy(S - QT2, QT2).start()
            out_v[zrows(S, 16, 16), 0:256] = jnp.zeros((16, 256), bf16)
            pins.setdefault(wave[0] + 4, []).append(
                token(out_v[S:S + 8, 0:128].astype(f32))())
        wave[0] += 1
        return out

    for j in range(nmx):
        gu = None
        for kt in range(D // 128):
            p = run_wave(xs[:, kt * 128:(kt + 1) * 128],
                         [r[2 * j + c, kt * 64:(kt + 1) * 64, :]
                          for r in (wgw, wuw) for c in range(2)])
            gu = p if gu is None else gu + p
        act[j] = activate(gu[:, :256], gu[:, 256:])
    ys = [None, None]
    for j in range(nblk):
        for kt in range(2):
            for hf in range(2):
                r0 = (2 * j + kt) * 64
                p = run_wave(act[j][:, kt * 128:(kt + 1) * 128],
                             [wdw[4 * hf + c, r0:r0 + 64, :] for c in range(4)])
                ys[hf] = p if ys[hf] is None else ys[hf] + p
    y = jnp.concatenate(ys, axis=1)
    cur = out_v[pl.ds(b0, 8), :].astype(f32)
    fix_v[...] = jnp.where(rows == wide(bi), cur + y * wide(gate), cur).astype(bf16)
    full_copy(out_v.at[pl.ds(0, S), :], out_hbm.at[0], SEM_O).wait()
    fix = pltpu.make_async_copy(fix_v, out_hbm.at[0, pl.ds(b0, 8), :], sem.at[SEM_O])
    fix.start()
    fix.wait()


def _kernel(*refs):
    def step(i, carry):
        @pl.when(i == 0)
        def _():
            _body(i, *refs)

        return carry

    lax.fori_loop(0, 2, step, 0)


@jax.jit
def pallas_sequential_preLN__linear_kernel_hedgehog__moe_arch_mod__prompt_kernel(
    A_x: jax.Array,
    A_wqkv: jax.Array,
    A_w_phi: jax.Array,
    A_wo: jax.Array,
    B_x: jax.Array,
    B_w_r: jax.Array,
    B_w_gate: jax.Array,
    B_w_up: jax.Array,
    B_w_down: jax.Array,
):
    any_spec = pl.BlockSpec(memory_space=pl.ANY)
    return pl.pallas_call(
        _kernel,
        out_shape=jax.ShapeDtypeStruct((1, S, D), bf16),
        in_specs=[any_spec] * 8,
        out_specs=any_spec,
        scratch_shapes=[
            pltpu.VMEM((S + 16, D), bf16),
            pltpu.VMEM((3 * NWC + 1, D, WC), bf16),
            pltpu.VMEM((H, DH, DH), bf16),
            pltpu.VMEM((D + 16, D), bf16),
            pltpu.VMEM((D,), bf16),
            pltpu.VMEM((F // 128 - 2 * FFN_VPU_BLOCKS, D + PAD, 128), bf16),
            pltpu.VMEM((F // 128 - 2 * FFN_VPU_BLOCKS, D + PAD, 128), bf16),
            pltpu.VMEM((D // 128, F + PAD, 128), bf16),
            pltpu.VMEM((D, 256 * FFN_VPU_BLOCKS), bf16),
            pltpu.VMEM((D, 256 * FFN_VPU_BLOCKS), bf16),
            pltpu.VMEM((7, 4, 3 * HD + PAD, 128), bf16),
            pltpu.VMEM((2, 7, 4, 64 + PAD, 128), bf16),
            pltpu.VMEM((2, 7, 24, HD), u32),
            pltpu.VMEM((7, 4, HD + PAD, 128), bf16),
            pltpu.VMEM((7, 4, HT1 + PAD, 128), bf16),
            pltpu.VMEM((7, 4, HT1 + PAD, 128), bf16),
            pltpu.VMEM((7, HT1 // 2, HD), u32),
            pltpu.VMEM((N2, 4, 2 * D + PAD, 128), bf16),
            pltpu.VMEM((4, 2 * D + PAD, 128), bf16),
            pltpu.VMEM((4, HD + PAD, 128), bf16),
            pltpu.VMEM((4, HD + PAD, 128), bf16),
            pltpu.VMEM((NP, 72, 128), f32),
            pltpu.VMEM((NP, 80, 128), bf16),
            *[pltpu.VMEM((QT2 + 8, HD), f32) for _ in range(4)],
            pltpu.VMEM((QT2, 384), f32),
            *[pltpu.VMEM((QT2, HD), f32) for _ in range(7)],
            pltpu.VMEM((S + 16, D), bf16),
            pltpu.VMEM((8, D), f32),
            pltpu.VMEM((3, 8, 128), f32),
            pltpu.VMEM((8, 128), jnp.int32),
            pltpu.VMEM((8, D), bf16),
            *[pltpu.VMEM((256, 128), f32) for _ in range(4)],
            pltpu.SemaphoreType.DMA((NSEM,)),
        ],
        compiler_params=pltpu.CompilerParams(
            vmem_limit_bytes=110 * 1024 * 1024,
            disable_bounds_checks=True,
            disable_semaphore_checks=True),
    )(A_x, A_wqkv, A_w_phi, A_wo, B_w_r, B_w_gate, B_w_up, B_w_down)
```
